```python
import jax
import jax.numpy as jnp

def _softmax(x, axis=-1):
    return jax.nn.softmax(x, axis=axis)
def _gelu(x):
    return jax.nn.gelu(x, approximate=True)
def _silu(x):
    return jax.nn.silu(x)
def _sigmoid(x):
    return jax.nn.sigmoid(x)
def _layernorm(x, axis=-1, eps=1e-5):
    m = jnp.mean(x, axis=axis, keepdims=True)
    v = jnp.var(x, axis=axis, keepdims=True)
    return (x - m) / jnp.sqrt(v + eps)
def _scatter_add(tgt, idx, src, axis=0):
    return tgt.at[idx].add(src)
def _segment_sum(src, seg, n):
    return jax.ops.segment_sum(src, seg, n)
class _Rng:
    def __init__(self, key):
        self._k = key
    def _next(self):
        self._k, sub = jax.random.split(self._k)
        return sub
    def normal(self, shape):
        return jax.random.normal(self._next(), shape, dtype=jnp.bfloat16)
    def randint(self, lo, hi, shape):
        return jax.random.randint(self._next(), shape, lo, hi, dtype=jnp.int32)
    def uniform(self, shape, lo=0.0, hi=1.0):
        return jax.random.uniform(self._next(), shape, jnp.bfloat16, lo, hi)
    def permutation(self, n):
        return jax.random.permutation(self._next(), n)


kernel_name = 'interleave_layers__sliding_block_cached__mixer_s_mlp__decode'

def setup_inputs():
    _rng = _Rng(jax.random.key(int.from_bytes(__import__("os").urandom(4), "little")))
    _w = (lambda a: (lambda t: t.astype(jnp.bfloat16) if jnp.issubdtype(t.dtype, jnp.floating) else t)(jnp.asarray(a)))
    def _A_setup():
        B, Sq, D = 1, 1, 640
        Hq, Hkv, Sk, Dh = 32, 32, 32768, 192
        assert Hq % Hkv == 0, (Hq, Hkv)
        return {
            "x": _w((lambda *s: _rng.normal(s) * 0.05)(B, Sq, D)),
            "k_cache": _w((lambda *s: _rng.normal(s) * 0.05)(B, Hkv, Sk, Dh)),
            "v_cache": _w((lambda *s: _rng.normal(s) * 0.05)(B, Hkv, Sk, Dh)),
            "wq": _w((lambda *s: _rng.normal(s) * 0.05)(D, Hq * Dh) * (D ** -0.5)),
            "wo": _w((lambda *s: _rng.normal(s) * 0.05)(Hq * Dh, D) * ((Hq * Dh) ** -0.5)),
        }
    _A_in = _A_setup()

    def _B_setup():
        B, S, D, F = 1, 1, 640, 1536
        return {
            "x":  _w((lambda *s: _rng.normal(s) * 0.05)(B, S, D)),
            "w1": _w((lambda *s: _rng.normal(s) * 0.05)(D, D) * (D ** -0.5)),
            "w2": _w((lambda *s: _rng.normal(s) * 0.05)(D, D) * (D ** -0.5)),
            "w3": _w((lambda *s: _rng.normal(s) * 0.05)(D, F) * (D ** -0.5)),
            "w4": _w((lambda *s: _rng.normal(s) * 0.05)(F, D) * (F ** -0.5)),
        }
    _B_in = _B_setup()

    return {
        "A_x": _A_in["x"],
        "A_k_cache": _A_in["k_cache"],
        "A_v_cache": _A_in["v_cache"],
        "A_wq": _A_in["wq"],
        "A_wo": _A_in["wo"],
        "B_x": _B_in["x"],
        "B_w1": _B_in["w1"],
        "B_w2": _B_in["w2"],
        "B_w3": _B_in["w3"],
        "B_w4": _B_in["w4"],
    }

def reference(A_x, A_k_cache, A_v_cache, A_wq, A_wo, B_x, B_w1, B_w2, B_w3, B_w4):
    def _A_ref(x, k_cache, v_cache, wq, wo):
        B, Sq, D = x.shape
        Hq, Dh = 32, 192
        Hkv, Sk = k_cache.shape[1], k_cache.shape[2]
        W = min(4096, max(256, Sk // 4))
        rep = Hq // Hkv
        q = (lambda x, *d: x.transpose(*d))((x @ wq).reshape(B, Sq, Hq, Dh), 0, 2, 1, 3)
        k = jnp.repeat(k_cache[:, :, Sk - W:, :], rep, axis=1)
        v = jnp.repeat(v_cache[:, :, Sk - W:, :], rep, axis=1)
        scores = jnp.einsum("bhqd,bhkd->bhqk", q, k) * (Dh ** -0.5)
        p = _softmax(scores, axis=-1)
        o = jnp.einsum("bhqk,bhkd->bhqd", p, v)
        return (lambda x, *d: x.transpose(*d))(o, 0, 2, 1, 3).reshape(B, Sq, Hq * Dh) @ wo

    def _B_ref(x, w1, w2, w3, w4):
        B, S, D = x.shape
        h = _gelu(_layernorm(x, axis=-1) @ w1)
        c = D // 4
        g0 = jnp.pad(h[:, :, 0*c:1*c], ((0, 0), (1, 0), (0, 0)))[:, :S, :]
        g1 = jnp.pad(h[:, :, 1*c:2*c], ((0, 0), (0, 1), (0, 0)))[:, 1:, :]
        g2 = jnp.pad(h[:, :, 2*c:3*c], ((0, 0), (2, 0), (0, 0)))[:, :S, :]
        g3 = jnp.pad(h[:, :, 3*c:   ], ((0, 0), (0, 2), (0, 0)))[:, 2:, :]
        hs = jnp.concatenate([g0, g1, g2, g3], axis=-1) @ w2
        x1 = x + hs
        h2 = _gelu(_layernorm(x1, axis=-1) @ w3) @ w4
        return x1 + h2

    x = A_x
    x = x + _A_ref(_layernorm(x, axis=-1), A_k_cache, A_v_cache, A_wq, A_wo)
    x = x + _B_ref(_layernorm(x, axis=-1), B_w1, B_w2, B_w3, B_w4)
    x = x + _A_ref(_layernorm(x, axis=-1), A_k_cache, A_v_cache, A_wq, A_wo)
    x = x + _B_ref(_layernorm(x, axis=-1), B_w1, B_w2, B_w3, B_w4)
    return x
```

```python
import jax
import jax.numpy as jnp
from jax import lax
import jax.experimental.pallas as pl
import jax.experimental.pallas.tpu as pltpu

F32 = jnp.float32
BF16 = jnp.bfloat16
U32 = jnp.uint32

D = 640
H = 32
DH = 192
FF = 1536
NU = H // 2
UT = 2 * DH // 16
EPS = 1e-5
PV_NH = 3
TOK_LAG = 260
TOK_OFF = 15


def _tile_view(a):
    r, c = a.shape
    a = a.reshape(r // 16, 2, 8, c // 128, 128)
    return jnp.swapaxes(a, 2, 3)


def _as_bf16(w32):
    n = w32.shape[0]
    return pltpu.bitcast(w32.reshape(n * 8, 128), BF16)


def _bf16_bits(x):
    return pltpu.bitcast(x.astype(BF16).astype(F32), U32)


def _dup_lhs(x):
    r = _bf16_bits(x)
    return r | (r >> 16)


def _layernorm(x):
    m = jnp.mean(x, axis=-1, keepdims=True)
    xc = x - m
    v = jnp.mean(xc * xc, axis=-1, keepdims=True)
    return xc * lax.rsqrt(v + EPS)


def _dot(a, b):
    return jnp.dot(a, b, preferred_element_type=F32)


def _make_kernel(sk, win):
    nj = win // 128
    j0 = (sk - win) // 128
    jq = nj // 4
    scale = DH ** -0.5

    def kernel(x_hbm, k_hbm, v_hbm, wq_hbm, wo_hbm, w3_hbm, w4_hbm, o_ref,
               kbuf, vbuf, wqbuf, wobuf, w3buf, w4buf, xin,
               xs, ulhs, qp, qlhs, sx, sy, pbuf, abuf, olhs, gp, gacc, sems):

        def cp_x():
            return pltpu.make_async_copy(x_hbm, xin, sems.at[0])

        def cp_w(hbm, buf, base, e, lo=0, n=None):
            n = buf.shape[0] if n is None else n
            return pltpu.make_async_copy(
                hbm.at[pl.ds(lo, n), e],
                buf.at[pl.ds(lo, n), :, pl.ds(e * 8, 8), :],
                sems.at[base + e])

        def cp_kv(hbm, buf, base, u, e):
            return pltpu.make_async_copy(
                hbm.at[pl.ds(u * UT, UT), e, pl.ds(j0, nj)],
                buf.at[pl.ds(u * UT, UT), :, pl.ds(e * 8, 8), :],
                sems.at[base + 2 * u + e])

        S_WQ, S_WO, S_W3, S_W4, S_K = 1, 3, 5, 7, 11
        S_V = S_K + 2 * NU
        w4_split = ((0, 64), (64, 32))

        cp_x().start()
        for e in range(2):
            cp_w(wq_hbm, wqbuf, S_WQ, e).start()
        for u in range(NU):
            for e in range(2):
                cp_kv(k_hbm, kbuf, S_K, u, e).start()
            for e in range(2):
                cp_kv(v_hbm, vbuf, S_V, u, e).start()
            if u == 0:
                for e in range(2):
                    cp_w(wo_hbm, wobuf, S_WO, e).start()
        for e in range(2):
            cp_w(w3_hbm, w3buf, S_W3, e).start()
        for i, (lo, n) in enumerate(w4_split):
            for e in range(2):
                cp_w(w4_hbm, w4buf, S_W4 + 2 * i, e, lo, n).start()

        k32 = kbuf.bitcast(U32)
        v32 = vbuf.bitcast(U32)
        wq32 = wqbuf.bitcast(U32)
        wo32 = wobuf.bitcast(U32)
        w332 = w3buf.bitcast(U32)
        w432 = w4buf.bitcast(U32)

        def st_qproj(u, sl):
            lhs = pltpu.bitcast(ulhs[...], BF16)
            for kt in range(D // 128):
                for nt in range(3):
                    w = _as_bf16(wq32[pl.ds(kt * 8, 8), u * 3 + nt])
                    r = _dot(lhs[:, kt * 128:(kt + 1) * 128], w)
                    qp[sl, kt, :, nt * 128:(nt + 1) * 128] = r[0:8]

        def st_qpack(sl):
            q = qp[sl, 0]
            for kt in range(1, D // 128):
                q = q + qp[sl, kt]
            r = _bf16_bits(q)
            lane = lax.broadcasted_iota(jnp.int32, r.shape, 1)
            lo = jnp.where((lane < DH) | (lane >= 256), r >> 16, jnp.uint32(0))
            hi = jnp.where((lane < 128) | (lane >= DH), r, jnp.uint32(0))
            sub = lax.broadcasted_iota(jnp.int32, r.shape, 0)
            qlhs[sl] = jnp.where(sub < 4, lo | hi, jnp.uint32(0))

        def st_qk(u, sl):
            lhs = pltpu.bitcast(qlhs[sl], BF16)
            toks = []
            for j in range(nj):
                ra = 2 * (j // jq)
                cs = slice((j % jq) * 128, (j % jq + 1) * 128)
                for t in range(3):
                    w = _as_bf16(k32[pl.ds(u * UT + t * 8, 8), j])
                    r = _dot(lhs[:, t * 128:(t + 1) * 128], w)
                    toks.append(r[8:16])
                    if t == 0:
                        sx[sl, ra:ra + 1, cs] = r[0:1]
                    elif t == 1:
                        sy[sl, ra:ra + 2, cs] = r[ra:ra + 2]
                    else:
                        sx[sl, ra + 1:ra + 2, cs] = r[0:1]
            return toks

        def st_softmax(slot):
            s = (sx[slot] + sy[slot]) * scale
            m = s[:, 0:128]
            for c in range(1, jq):
                m = jnp.maximum(m, s[:, c * 128:(c + 1) * 128])
            m = jnp.maximum(m, pltpu.roll(m, 2, 0))
            m = jnp.maximum(m, pltpu.roll(m, 4, 0))
            m = jnp.max(m, axis=1, keepdims=True)
            p = jnp.exp(s - m)
            l = p[:, 0:128]
            for c in range(1, jq):
                l = l + p[:, c * 128:(c + 1) * 128]
            l = l + pltpu.roll(l, 2, 0)
            l = l + pltpu.roll(l, 4, 0)
            l = jnp.sum(l, axis=1, keepdims=True)
            pbuf[slot] = p * (1.0 / l)

        def st_pv(u, slot, toks):
            nhalf = PV_NH
            for hd in range(2):
                for half in range(12 // nhalf):
                    piece = hd * (12 // nhalf) + half
                    tok = None
                    if toks is not None:
                        ti = (piece * nhalf * 49 - TOK_LAG) // 8 - TOK_OFF
                        if ti >= 0:
                            tok = toks[min(ti, len(toks) - 1)]
                    lo = [None] * nhalf
                    hi = [None] * nhalf
                    for j in range(nj):
                        row = 2 * (j // jq) + hd
                        cs = slice((j % jq) * 128, (j % jq + 1) * 128)
                        pb = jnp.broadcast_to(pbuf[slot, row:row + 1, cs], (8, 128))
                        if j == 0 and tok is not None:
                            pb = pb + tok
                        for i in range(nhalf):
                            w = v32[u * UT + hd * 12 + half * nhalf + i, j]
                            a = pltpu.bitcast(w << 16, F32) * pb
                            b = pltpu.bitcast(w & jnp.uint32(0xFFFF0000), F32) * pb
                            lo[i] = a if lo[i] is None else lo[i] + a
                            hi[i] = b if hi[i] is None else hi[i] + b
                    for i in range(nhalf):
                        base = (hd * 12 + half * nhalf + i) * 16
                        abuf[slot, pl.ds(base, 8, stride=2), :] = lo[i]
                        abuf[slot, pl.ds(base + 1, 8, stride=2), :] = hi[i]

        def st_ored(sl):
            at = abuf[sl].T
            o = at[0:8]
            for i in range(1, 16):
                o = o + at[i * 8:(i + 1) * 8]
            o = o + pltpu.roll(o, 4, 0)
            o = o + pltpu.roll(o, 2, 0)
            o = o + pltpu.roll(o, 1, 0)
            olhs[sl] = _dup_lhs(o)

        def st_oproj(u, sl):
            lhs = pltpu.bitcast(olhs[sl], BF16)
            for t in range(3):
                for n in range(D // 128):
                    w = _as_bf16(wo32[pl.ds(u * UT + t * 8, 8), n])
                    r = _dot(lhs[:, t * 128:(t + 1) * 128], w)
                    gp[sl, t, :, n * 128:(n + 1) * 128] = r[0:8]

        def st_oacc(sl):
            gacc[...] = gacc[...] + (gp[sl, 0] + gp[sl, 1] + gp[sl, 2])

        cp_x().wait()
        xs[...] = jnp.broadcast_to(xin[...].astype(F32), (8, D))

        def layer(li, carry):
            first = li == 0

            def wait_w(hbm, buf, base, lo=0, n=None):
                @pl.when(first)
                def _():
                    for e in range(2):
                        cp_w(hbm, buf, base, e, lo, n).wait()

            def wait_kv(hbm, buf, base, u):
                @pl.when(first)
                def _():
                    for e in range(2):
                        cp_kv(hbm, buf, base, u, e).wait()

            def step(t, static, par):
                def on(k):
                    return (not static) or (0 <= t + k < NU)
                if on(2):
                    wait_kv(k_hbm, kbuf, S_K, t + 2)
                if on(0):
                    wait_kv(v_hbm, vbuf, S_V, t)
                if on(-3):
                    st_oacc(1 - par)
                if on(-2):
                    st_oproj(t - 2, par)
                if on(-1):
                    st_ored(1 - par)
                toks = None
                if on(2):
                    toks = st_qk(t + 2, par)
                if on(0):
                    st_pv(t, par, toks)
                if on(1):
                    st_softmax(1 - par)
                if on(3):
                    st_qpack(1 - par)
                if on(4):
                    st_qproj(t + 4, par)

            ulhs[...] = _dup_lhs(_layernorm(xs[...]))
            gacc[...] = jnp.zeros_like(gacc)
            wait_w(wq_hbm, wqbuf, S_WQ)
            for t in range(-4, 4):
                if t == 2:
                    wait_w(wo_hbm, wobuf, S_WO)
                step(t, True, t % 2)

            def body(i, c):
                step(2 * i, False, 0)
                step(2 * i + 1, False, 1)
                return c
            lax.fori_loop(2, (NU - 4) // 2, body, 0)

            for t in range(NU - 4, NU + 3):
                step(t, True, t % 2)

            x1 = xs[...] + gacc[...]
            y = _layernorm(x1)
            z = pltpu.bitcast(_dup_lhs(_layernorm(y)), BF16)
            wait_w(w3_hbm, w3buf, S_W3)
            hs = []
            for n in range(FF // 128):
                hs.append(_dot(z, _as_bf16(w332[:, n]))[0:8])
            hmid = jax.nn.gelu(jnp.concatenate(hs, axis=1), approximate=True)
            hl = pltpu.bitcast(_dup_lhs(hmid), BF16)
            xs[...] = x1 + y
            for i, (lo, n) in enumerate(w4_split):
                wait_w(w4_hbm, w4buf, S_W4 + 2 * i, lo, n)
                outs = []
                for c in range(D // 128):
                    outs.append(_dot(hl[:, lo * 16:(lo + n) * 16],
                                     _as_bf16(w432[pl.ds(lo, n), c]))[0:8])
                xs[...] = xs[...] + jnp.concatenate(outs, axis=1)
            return carry

        lax.fori_loop(0, 2, layer, 0)
        o_ref[...] = xs[0:1, :].astype(o_ref.dtype)

    return kernel


@jax.jit
def pallas_interleave_layers__sliding_block_cached__mixer_s_mlp__decode_kernel(
    A_x: jax.Array,
    A_k_cache: jax.Array,
    A_v_cache: jax.Array,
    A_wq: jax.Array,
    A_wo: jax.Array,
    B_x: jax.Array,
    B_w1: jax.Array,
    B_w2: jax.Array,
    B_w3: jax.Array,
    B_w4: jax.Array,
):
    b, sq, d = A_x.shape
    _, hkv, sk, dh = A_k_cache.shape
    assert (b, sq, d, hkv, dh) == (1, 1, D, H, DH)
    win = min(4096, max(256, sk // 4))
    assert win % 512 == 0 and sk % 128 == 0
    nj = win // 128

    kt = _tile_view(jnp.swapaxes(A_k_cache, 2, 3).reshape(H * DH, sk))
    vt = _tile_view(jnp.swapaxes(A_v_cache, 2, 3).reshape(H * DH, sk))

    def buf(r, c):
        return pltpu.VMEM((r // 16, c // 128, 16, 128), BF16)

    any_spec = pl.BlockSpec(memory_space=pl.ANY)
    out = pl.pallas_call(
        _make_kernel(sk, win),
        out_shape=jax.ShapeDtypeStruct((1, D), A_x.dtype),
        in_specs=[any_spec] * 7,
        out_specs=pl.BlockSpec(memory_space=pltpu.VMEM),
        scratch_shapes=[
            buf(H * DH, win), buf(H * DH, win),
            buf(D, H * DH), buf(H * DH, D), buf(D, FF), buf(FF, D),
            pltpu.VMEM((1, D), BF16),
            pltpu.VMEM((8, D), F32),
            pltpu.VMEM((8, D), U32),
            pltpu.VMEM((2, D // 128, 8, 384), F32),
            pltpu.VMEM((2, 8, 384), U32),
            pltpu.VMEM((2, 8, win // 4), F32),
            pltpu.VMEM((2, 8, win // 4), F32),
            pltpu.VMEM((2, 8, win // 4), F32),
            pltpu.VMEM((2, 384, 128), F32),
            pltpu.VMEM((2, 8, 384), U32),
            pltpu.VMEM((2, 3, 8, D), F32),
            pltpu.VMEM((8, D), F32),
            pltpu.SemaphoreType.DMA((11 + 4 * NU,)),
        ],
        compiler_params=pltpu.CompilerParams(vmem_limit_bytes=124 * 1024 * 1024),
        name="interleave_decode",
    )(A_x.reshape(1, D), kt, vt, _tile_view(A_wq), _tile_view(A_wo),
      _tile_view(B_w3), _tile_view(B_w4))
    return out.reshape(b, sq, d)
```

```python
import jax
import jax.numpy as jnp
from jax import lax
import jax.experimental.pallas as pl
import jax.experimental.pallas.tpu as pltpu

F32 = jnp.float32
BF16 = jnp.bfloat16
U32 = jnp.uint32

D = 640
H = 32
DH = 192
FF = 1536
NU = H // 2
UT = 2 * DH // 16
EPS = 1e-5
CFG = dict(pv_nh=2, tok_lag=230, tok_rate=9.0,
           oproj_at={12: (0,), 13: (1,), 14: (2, 3, 4, 5, 6, 7, 8), 15: (9, 10, 11, 12, 13),
                     16: (14,), 17: (15,)},
           tok_mem=0, w4_a=88, bench=0)


def _tile_view(a):
    r, c = a.shape
    a = a.reshape(r // 16, 2, 8, c // 128, 128)
    return jnp.swapaxes(a, 2, 3)


def _as_bf16(w32):
    n = w32.shape[0]
    return pltpu.bitcast(w32.reshape(n * 8, 128), BF16)


def _bf16_bits(x):
    return pltpu.bitcast(x.astype(BF16).astype(F32), U32)


def _dup_lhs(x):
    r = _bf16_bits(x)
    return r | (r >> 16)


def _layernorm(x):
    m = jnp.mean(x, axis=-1, keepdims=True)
    m2 = jnp.mean(x * x, axis=-1, keepdims=True)
    v = jnp.maximum(m2 - m * m, 0.0)
    return (x - m) * lax.rsqrt(v + EPS)


def _dot(a, b):
    return jnp.dot(a, b, preferred_element_type=F32)


def _make_kernel(sk, win, cfg):
    nj = win // 128
    j0 = (sk - win) // 128
    jq = nj // 4
    scale = DH ** -0.5

    def kernel(x_hbm, k_hbm, v_hbm, wq_hbm, wo_hbm, w3_hbm, w4_hbm, o_ref,
               kbuf, vbuf, wqbuf, wobuf, w3buf, w4buf, xin,
               xs, ulhs, qp, qlhs, sx, sy, pbuf, abuf, olhs, gp, sems, *tokb):

        bench = cfg["bench"]

        def cps_w(hbm, buf, sem, lo=0, n=None):
            n = buf.shape[0] if n is None else n
            return [pltpu.make_async_copy(
                hbm.at[pl.ds(lo, n), e],
                buf.at[pl.ds(lo, n), :, pl.ds(e * 8, 8), :],
                sems.at[sem]) for e in range(2)]

        def cps_kv(hbm, buf, sem, u):
            return [pltpu.make_async_copy(
                hbm.at[pl.ds(u * UT, UT), e, pl.ds(j0, nj)],
                buf.at[pl.ds(u * UT, UT), :, pl.ds(e * 8, 8), :],
                sems.at[sem]) for e in range(2)]

        w4_a = cfg["w4_a"]
        cps_k = lambda u, par: cps_kv(k_hbm, kbuf, par, u)
        cps_v = lambda u, par: cps_kv(v_hbm, vbuf, 2 + par, u)
        cps_x_wq = lambda: [pltpu.make_async_copy(x_hbm, xin, sems.at[4])] + cps_w(wq_hbm, wqbuf, 4)
        cps_wo = lambda: cps_w(wo_hbm, wobuf, 4)
        cps_w3 = lambda: cps_w(w3_hbm, w3buf, 0)
        cps_w4a = lambda: cps_w(w4_hbm, w4buf, 1, 0, w4_a)
        cps_w4b = lambda: cps_w(w4_hbm, w4buf, 4, w4_a, FF // 16 - w4_a)

        def start(cps):
            for c in cps:
                c.start()

        def wait(cps):
            for c in cps:
                c.wait()

        if not bench:
            start(cps_x_wq())
            start(cps_k(0, 0))
            start(cps_k(1, 1))
            start(cps_v(0, 0))

        k32 = kbuf.bitcast(U32)
        v32 = vbuf.bitcast(U32)
        wq32 = wqbuf.bitcast(U32)
        wo32 = wobuf.bitcast(U32)
        w332 = w3buf.bitcast(U32)
        w432 = w4buf.bitcast(U32)

        def st_qproj(u, sl):
            lhs = pltpu.bitcast(ulhs[...], BF16)
            for kt in range(D // 128):
                for nt in range(3):
                    w = _as_bf16(wq32[pl.ds(kt * 8, 8), u * 3 + nt])
                    r = _dot(lhs[:, kt * 128:(kt + 1) * 128], w)
                    qp[sl, kt, :, nt * 128:(nt + 1) * 128] = r[0:8]

        def st_qpack(sl):
            q = qp[sl, 0]
            for kt in range(1, D // 128):
                q = q + qp[sl, kt]
            r = _bf16_bits(q)
            lane = lax.broadcasted_iota(jnp.int32, r.shape, 1)
            lo = jnp.where((lane < DH) | (lane >= 256), r >> 16, jnp.uint32(0))
            hi = jnp.where((lane < 128) | (lane >= DH), r, jnp.uint32(0))
            sub = lax.broadcasted_iota(jnp.int32, r.shape, 0)
            qlhs[sl] = jnp.where(sub < 4, lo | hi, jnp.uint32(0))

        def st_qk(u, sl):
            lhs = pltpu.bitcast(qlhs[sl], BF16)
            toks = []
            for j in range(nj):
                ra = 2 * (j // jq)
                cs = slice((j % jq) * 128, (j % jq + 1) * 128)
                for t in range(3):
                    w = _as_bf16(k32[pl.ds(u * UT + t * 8, 8), j])
                    r = _dot(lhs[:, t * 128:(t + 1) * 128], w)
                    toks.append(r[8:16])
                    if t == 0:
                        sx[sl, ra:ra + 1, cs] = r[0:1]
                    elif t == 1:
                        sy[sl, ra:ra + 2, cs] = r[ra:ra + 2]
                    else:
                        sx[sl, ra + 1:ra + 2, cs] = r[0:1]
            return toks

        def st_softmax(slot):
            s = (sx[slot] + sy[slot]) * scale
            m = s[:, 0:128]
            for c in range(1, jq):
                m = jnp.maximum(m, s[:, c * 128:(c + 1) * 128])
            m = jnp.maximum(m, pltpu.roll(m, 2, 0))
            m = jnp.maximum(m, pltpu.roll(m, 4, 0))
            m = jnp.max(m, axis=1, keepdims=True)
            p = jnp.exp(s - m)
            l = p[:, 0:128]
            for c in range(1, jq):
                l = l + p[:, c * 128:(c + 1) * 128]
            l = l + pltpu.roll(l, 2, 0)
            l = l + pltpu.roll(l, 4, 0)
            l = jnp.sum(l, axis=1, keepdims=True)
            pbuf[slot] = p * (1.0 / l)

        def st_pv(u, slot, toks, zdyn):
            nh = cfg["pv_nh"]
            npc = 12 // nh
            for hd in range(2):
                for half in range(npc):
                    piece = hd * npc + half
                    tok = None
                    if toks:
                        ti = int((piece * nh * 49 - cfg["tok_lag"]) / cfg["tok_rate"])
                        if ti >= 0:
                            tok = toks[min(ti, len(toks) - 1)]
                            if cfg["tok_mem"]:
                                tokb[piece][zdyn] = tok
                                tok = tokb[piece][0]
                    lo = hi = None
                    t0 = hd * 12 + half * nh
                    for j in range(nj):
                        row = 2 * (j // jq) + hd
                        cs = slice((j % jq) * 128, (j % jq + 1) * 128)
                        pb = jnp.broadcast_to(pbuf[slot, row:row + 1, cs], (8, 128))
                        if j == 0 and tok is not None:
                            pb = pb + tok
                        w = v32[pl.ds(u * UT + t0, nh), j]
                        a = pltpu.bitcast(w << 16, F32) * pb
                        b = pltpu.bitcast(w & jnp.uint32(0xFFFF0000), F32) * pb
                        lo = a if lo is None else lo + a
                        hi = b if hi is None else hi + b
                    for i in range(nh):
                        base = (t0 + i) * 16
                        abuf[slot, pl.ds(base, 8, stride=2), :] = lo[i]
                        abuf[slot, pl.ds(base + 1, 8, stride=2), :] = hi[i]

        def st_ored(u, sl):
            at = abuf[sl].T
            o = at[0:8]
            for i in range(1, 16):
                o = o + at[i * 8:(i + 1) * 8]
            o = o + pltpu.roll(o, 4, 0)
            o = o + pltpu.roll(o, 2, 0)
            o = o + pltpu.roll(o, 1, 0)
            sub = lax.broadcasted_iota(jnp.int32, o.shape, 0)
            olhs[u] = jnp.where(sub < 4, _bf16_bits(o) >> 16, jnp.uint32(0))

        def st_oproj(u):
            lhs = pltpu.bitcast(olhs[u], BF16)
            toks = []
            for t in range(3):
                g, row = divmod(u * 3 + t, 8)
                for n in range(D // 128):
                    w = _as_bf16(wo32[pl.ds(u * UT + t * 8, 8), n])
                    r = _dot(lhs[:, t * 128:(t + 1) * 128], w)
                    toks.append(r[8:16])
                    gp[g, row:row + 1, n * 128:(n + 1) * 128] = r[0:1]
            return toks

        def mlp(first):
            g = gp[0]
            for i in range(1, 3 * NU // 8):
                g = g + gp[i]
            g = g + pltpu.roll(g, 4, 0)
            g = g + pltpu.roll(g, 2, 0)
            g = g + pltpu.roll(g, 1, 0)
            x1 = xs[...] + g
            y = _layernorm(x1)
            z = pltpu.bitcast(_dup_lhs(_layernorm(y)), BF16)
            hs = []
            for n in range(FF // 128):
                hs.append(_dot(z, _as_bf16(w332[:, n]))[0:8])
            hmid = jax.nn.gelu(jnp.concatenate(hs, axis=1), approximate=True)
            hl = pltpu.bitcast(_dup_lhs(hmid), BF16)
            acc = x1 + y
            parts = ((0, w4_a, cps_w4a), (w4_a, FF // 16 - w4_a, cps_w4b))
            if not first:
                parts = ((0, FF // 16, None),)
            for lo, n, cps in parts:
                if cps is not None:
                    wait(cps())
                outs = []
                for c in range(D // 128):
                    outs.append(_dot(hl[:, lo * 16:(lo + n) * 16],
                                     _as_bf16(w432[pl.ds(lo, n), c]))[0:8])
                acc = acc + jnp.concatenate(outs, axis=1)
            xs[...] = acc

        if not bench:
            wait(cps_x_wq())
            start(cps_wo())
            wait(cps_k(0, 0))
            start(cps_k(2, 0))
            wait(cps_k(1, 1))
        xs[...] = jnp.broadcast_to(xin[...].astype(F32), (8, D))

        def layer(li, carry):
            first = li == 0
            n_first = 1 - li
            if bench:
                first = li == -1
                n_first = li >> 4

            def step_dma(t, static, par):
                def ok(k):
                    return (not static) or t + k < NU

                def dma_ops(_, c):
                    if ok(3):
                        start(cps_k(t + 3, 1 - par))
                    if ok(1):
                        start(cps_v(t + 1, 1 - par))
                    if static and t == NU - 2:
                        start(cps_w3())
                        start(cps_w4a())
                        start(cps_w4b())
                    if static and t == NU - 4:
                        wait(cps_wo())
                    if ok(2):
                        wait(cps_k(t + 2, par))
                    return c

                if ok(1):
                    lax.fori_loop(0, n_first, dma_ops, 0)
                pl.when(first)(lambda: wait(cps_v(t, par)))

            def step(t, static, par):
                def on(k):
                    return (not static) or (0 <= t + k < NU)
                if on(0):
                    step_dma(t, static, par)
                if on(-1):
                    st_ored(t - 1, 1 - par)
                toks = []
                if on(2):
                    toks = st_qk(t + 2, par)
                if static:
                    for u in cfg["oproj_at"].get(t, ()):
                        toks = toks + st_oproj(u)
                if on(0):
                    st_pv(t, par, toks, li >> 4)
                if on(1):
                    st_softmax(1 - par)
                if on(3):
                    st_qpack(1 - par)
                if on(4):
                    st_qproj(t + 4, par)

            def body(i, c):
                step(2 * i, False, 0)
                step(2 * i + 1, False, 1)
                return c

            if bench:
                lax.fori_loop(0, bench, lambda i, c: body(i % 4 + 1, c), 0)
                return carry

            ulhs[...] = _dup_lhs(_layernorm(xs[...]))
            for t in range(-4, 2):
                step(t, True, t % 2)
            lax.fori_loop(1, (NU - 4) // 2, body, 0)
            for t in range(NU - 4, NU):
                step(t, True, t % 2)

            def tail(first_static):
                if first_static:
                    wait(cps_w3())
                for t in range(NU, NU + 2):
                    step(t, True, t % 2)
                mlp(first_static)

            pl.when(first)(lambda: tail(True))
            pl.when(jnp.logical_not(first))(lambda: tail(False))
            return carry

        lax.fori_loop(0, 2, layer, 0)
        o_ref[...] = xs[0:1, :].astype(o_ref.dtype)

    return kernel


@jax.jit
def pallas_interleave_layers__sliding_block_cached__mixer_s_mlp__decode_kernel(
    A_x: jax.Array,
    A_k_cache: jax.Array,
    A_v_cache: jax.Array,
    A_wq: jax.Array,
    A_wo: jax.Array,
    B_x: jax.Array,
    B_w1: jax.Array,
    B_w2: jax.Array,
    B_w3: jax.Array,
    B_w4: jax.Array,
):
    b, sq, d = A_x.shape
    _, hkv, sk, dh = A_k_cache.shape
    assert (b, sq, d, hkv, dh) == (1, 1, D, H, DH)
    win = min(4096, max(256, sk // 4))
    assert win % 512 == 0 and sk % 128 == 0
    nj = win // 128

    kt = _tile_view(jnp.swapaxes(A_k_cache, 2, 3).reshape(H * DH, sk))
    vt = _tile_view(jnp.swapaxes(A_v_cache, 2, 3).reshape(H * DH, sk))

    def buf(r, c):
        return pltpu.VMEM((r // 16, c // 128, 16, 128), BF16)

    any_spec = pl.BlockSpec(memory_space=pl.ANY)
    out = pl.pallas_call(
        _make_kernel(sk, win, CFG),
        out_shape=jax.ShapeDtypeStruct((1, D), A_x.dtype),
        in_specs=[any_spec] * 7,
        out_specs=pl.BlockSpec(memory_space=pltpu.VMEM),
        scratch_shapes=[
            buf(H * DH, win), buf(H * DH, win),
            buf(D, H * DH), buf(H * DH, D), buf(D, FF), buf(FF, D),
            pltpu.VMEM((1, D), BF16),
            pltpu.VMEM((8, D), F32),
            pltpu.VMEM((8, D), U32),
            pltpu.VMEM((2, D // 128, 8, 384), F32),
            pltpu.VMEM((2, 8, 384), U32),
            pltpu.VMEM((2, 8, win // 4), F32),
            pltpu.VMEM((2, 8, win // 4), F32),
            pltpu.VMEM((2, 8, win // 4), F32),
            pltpu.VMEM((2, 384, 128), F32),
            pltpu.VMEM((NU, 8, 384), U32),
            pltpu.VMEM((3 * NU // 8, 8, D), F32),
            pltpu.SemaphoreType.DMA((5,)),
        ] + [pltpu.VMEM((2, 8, 128), F32)] * 24,
        compiler_params=pltpu.CompilerParams(vmem_limit_bytes=124 * 1024 * 1024),
        name="interleave_decode",
    )(A_x.reshape(1, D), kt, vt, _tile_view(A_wq), _tile_view(A_wo),
      _tile_view(B_w3), _tile_view(B_w4))
    return out.reshape(b, sq, d)
```

```python
import jax
import jax.numpy as jnp
from jax import lax
import jax.experimental.pallas as pl
import jax.experimental.pallas.tpu as pltpu

F32 = jnp.float32
BF16 = jnp.bfloat16
U32 = jnp.uint32

D = 640
H = 32
DH = 192
FF = 1536
NU = H // 2
UT = 2 * DH // 16
EPS = 1e-5
CFG = dict(pv_nh=2, tok_lag=230, tok_rate=9.0,
           jsplit=6,
           oproj_at={12: (0,), 13: (1, 2), 14: (3, 4, 5), 15: (6, 7, 8, 9, 10, 11, 12, 13),
                     16: (14,), 17: (15,)},
           tok_mem=0, w4_a=80, layers=2, bench=0,
           tok_map=[-1, -1, -1, 10, 21, 33, 45, 60, 68, 79, 88, 99])


def _tile_view(a):
    r, c = a.shape
    a = a.reshape(r // 16, 2, 8, c // 128, 128)
    return jnp.swapaxes(a, 2, 3)


def _head_view(a):
    c = a.shape[1]
    a = a.reshape(H, 2, DH // 16, 8, c // 128, 128)
    return jnp.swapaxes(a, 3, 4)


def _as_bf16(w32):
    n = w32.shape[0]
    return pltpu.bitcast(w32.reshape(n * 8, 128), BF16)


def _bf16_bits(x):
    return pltpu.bitcast(x.astype(BF16).astype(F32), U32)


def _dup_lhs(x):
    r = _bf16_bits(x)
    return r | (r >> 16)


def _layernorm(x):
    m = jnp.mean(x, axis=-1, keepdims=True)
    m2 = jnp.mean(x * x, axis=-1, keepdims=True)
    v = jnp.maximum(m2 - m * m, 0.0)
    return (x - m) * lax.rsqrt(v + EPS)


def _dot(a, b):
    return jnp.dot(a, b, preferred_element_type=F32)


def _make_kernel(sk, win, cfg):
    nj = win // 128
    j0 = (sk - win) // 128
    jq = nj // 4
    scale = DH ** -0.5

    def kernel(x_hbm, k_hbm, v_hbm, wq_hbm, wo_hbm, w3_hbm, w4_hbm, o_ref,
               kbuf, vbuf, wqbuf, wobuf, w3buf, w4buf, xin,
               xs, ulhs, qp, qlhs, sx, sy, pbuf, linv, abuf, olhs, gp, sems, *tokb):

        bench = cfg["bench"]

        def cps_w(hbm, buf, sem, lo=0, n=None):
            n = buf.shape[0] if n is None else n
            return [pltpu.make_async_copy(
                hbm.at[pl.ds(lo, n), e],
                buf.at[pl.ds(lo, n), :, pl.ds(e * 8, 8), :],
                sems.at[sem]) for e in range(2)]

        def cps_kv(hbm, buf, sem, u):
            return [pltpu.make_async_copy(
                hbm.at[pl.ds(u * UT, UT), e, pl.ds(j0, nj)],
                buf.at[pl.ds(u * UT, UT), :, pl.ds(e * 8, 8), :],
                sems.at[sem]) for e in range(2)]

        def cps_v(u, par):
            return [pltpu.make_async_copy(
                v_hbm.at[pl.ds(2 * u, 2), e, :, pl.ds(j0, nj)],
                vbuf.at[pl.ds(2 * u, 2), :, :, pl.ds(e * 8, 8), :],
                sems.at[2 + par]) for e in range(2)]

        def cps_wo():
            return [pltpu.make_async_copy(
                wo_hbm.at[:, e], wobuf.at[:, :, :, pl.ds(e * 8, 8), :],
                sems.at[4]) for e in range(2)]

        w4_a = cfg["w4_a"]
        cps_k = lambda u, par: cps_kv(k_hbm, kbuf, par, u)
        cps_x_wq = lambda: [pltpu.make_async_copy(x_hbm, xin, sems.at[4])] + cps_w(wq_hbm, wqbuf, 4)
        cps_w3 = lambda: cps_w(w3_hbm, w3buf, 0)
        cps_w4a = lambda: cps_w(w4_hbm, w4buf, 1, 0, w4_a)
        cps_w4b = lambda: cps_w(w4_hbm, w4buf, 4, w4_a, FF // 16 - w4_a)

        def start(cps):
            for c in cps:
                c.start()

        def wait(cps):
            for c in cps:
                c.wait()

        if not bench:
            start(cps_x_wq())
            start(cps_k(0, 0))
            start(cps_k(1, 1))
            start(cps_v(0, 0))

        k32 = kbuf.bitcast(U32)
        v32 = vbuf.bitcast(U32)
        wq32 = wqbuf.bitcast(U32)
        wo32 = wobuf.bitcast(U32)
        w332 = w3buf.bitcast(U32)
        w432 = w4buf.bitcast(U32)

        def st_qproj(u, sl):
            lhs = pltpu.bitcast(ulhs[...], BF16)
            toks = []
            for kt in range(D // 128):
                for nt in range(3):
                    w = _as_bf16(wq32[pl.ds(kt * 8, 8), u * 3 + nt])
                    r = _dot(lhs[:, kt * 128:(kt + 1) * 128], w)
                    toks.append(r[8:16])
                    qp[sl, kt, :, nt * 128:(nt + 1) * 128] = r[0:8]
            return toks

        def st_qpack(sl):
            q = qp[sl, 0]
            for kt in range(1, D // 128):
                q = q + qp[sl, kt]
            r = _bf16_bits(q)
            lane = lax.broadcasted_iota(jnp.int32, r.shape, 1)
            lo = jnp.where((lane < DH) | (lane >= 256), r >> 16, jnp.uint32(0))
            hi = jnp.where((lane < 128) | (lane >= DH), r, jnp.uint32(0))
            sub = lax.broadcasted_iota(jnp.int32, r.shape, 0)
            qlhs[sl] = jnp.where(sub < 4, lo | hi, jnp.uint32(0))

        def st_qk(u, sl, js):
            lhs = pltpu.bitcast(qlhs[sl], BF16)
            toks = []
            for j in js:
                ra = 2 * (j // jq)
                cs = slice((j % jq) * 128, (j % jq + 1) * 128)
                for t in range(3):
                    w = _as_bf16(k32[pl.ds(u * UT + t * 8, 8), j])
                    r = _dot(lhs[:, t * 128:(t + 1) * 128], w)
                    toks.append(r[8:16])
                    if t == 0:
                        sx[sl, ra:ra + 1, cs] = r[0:1]
                    elif t == 1:
                        sy[sl, ra:ra + 2, cs] = r[ra:ra + 2]
                    else:
                        sx[sl, ra + 1:ra + 2, cs] = r[0:1]
            return toks

        def st_softmax(slot):
            s = (sx[slot] + sy[slot]) * scale
            m = s[:, 0:128]
            for c in range(1, jq):
                m = jnp.maximum(m, s[:, c * 128:(c + 1) * 128])
            m = jnp.maximum(m, pltpu.roll(m, 2, 0))
            m = jnp.maximum(m, pltpu.roll(m, 4, 0))
            m = jnp.max(m, axis=1, keepdims=True)
            pbuf[slot] = jnp.exp(s - m)

        def st_lsum(slot):
            l = pbuf[slot, :, 0:128]
            for c in range(1, jq):
                l = l + pbuf[slot, :, c * 128:(c + 1) * 128]
            l = l + pltpu.roll(l, 2, 0)
            l = l + pltpu.roll(l, 4, 0)
            l = jnp.sum(l, axis=1, keepdims=True)
            linv[slot] = jnp.broadcast_to(1.0 / l, (8, 128))

        def st_pv(u, slot, toks, zdyn):
            nh = cfg["pv_nh"]
            npc = 12 // nh
            for hd in range(2):
                for half in range(npc):
                    piece = hd * npc + half
                    tok = None
                    if toks:
                        ti = int((piece * nh * 49 - cfg["tok_lag"]) / cfg["tok_rate"])
                        if cfg.get("tok_map") is not None:
                            ti = cfg["tok_map"][piece]
                        if ti >= 0:
                            tok = toks[min(ti, len(toks) - 1)]
                            if cfg["tok_mem"]:
                                tokb[piece][zdyn] = tok
                                tok = tokb[piece][0]
                    lo = hi = None
                    t0 = hd * 12 + half * nh
                    for j in range(nj):
                        row = 2 * (j // jq) + hd
                        cs = slice((j % jq) * 128, (j % jq + 1) * 128)
                        pb = jnp.broadcast_to(pbuf[slot, row:row + 1, cs], (8, 128))
                        if j == 0 and tok is not None:
                            pb = pb + tok
                        w = v32[2 * u + hd, pl.ds(half * nh, nh), j]
                        a = pltpu.bitcast(w << 16, F32) * pb
                        b = pltpu.bitcast(w & jnp.uint32(0xFFFF0000), F32) * pb
                        lo = a if lo is None else lo + a
                        hi = b if hi is None else hi + b
                    for i in range(nh):
                        base = (t0 + i) * 16
                        abuf[slot, pl.ds(base, 8, stride=2), :] = lo[i]
                        abuf[slot, pl.ds(base + 1, 8, stride=2), :] = hi[i]

        def st_ored(u, sl):
            at = abuf[sl].T
            o = at[0:8]
            for i in range(1, 16):
                o = o + at[i * 8:(i + 1) * 8]
            o = o + pltpu.roll(o, 4, 0)
            o = o + pltpu.roll(o, 2, 0)
            o = o + pltpu.roll(o, 1, 0)
            ia = linv[sl]
            ib = pltpu.roll(ia, 1, 0)
            lane = lax.broadcasted_iota(jnp.int32, (8, 128), 1)
            o = o * jnp.concatenate([ia, jnp.where(lane < DH - 128, ia, ib), ib], axis=1)
            sub = lax.broadcasted_iota(jnp.int32, o.shape, 0)
            olhs[u] = jnp.where(sub < 4, _bf16_bits(o) >> 16, jnp.uint32(0))

        def st_oproj(u):
            lhs = pltpu.bitcast(olhs[u], BF16)
            toks = []
            for t in range(3):
                g, row = divmod(u * 3 + t, 8)
                for n in range(D // 128):
                    if t == 1:
                        w32 = jnp.concatenate([wo32[2 * u, 8:12, n], wo32[2 * u + 1, 0:4, n]], axis=0)
                    else:
                        w32 = wo32[2 * u + t // 2, 2 * t:2 * t + 8, n]
                    w = _as_bf16(w32)
                    r = _dot(lhs[:, t * 128:(t + 1) * 128], w)
                    toks.append(r[8:16])
                    gp[g, row:row + 1, n * 128:(n + 1) * 128] = r[0:1]
            return toks

        def mlp(first):
            g = gp[0]
            for i in range(1, 3 * NU // 8):
                g = g + gp[i]
            g = g + pltpu.roll(g, 4, 0)
            g = g + pltpu.roll(g, 2, 0)
            g = g + pltpu.roll(g, 1, 0)
            x1 = xs[...] + g
            y = _layernorm(x1)
            z = pltpu.bitcast(_dup_lhs(_layernorm(y)), BF16)
            hs = []
            for n in range(FF // 128):
                hs.append(_dot(z, _as_bf16(w332[:, n]))[0:8])
            hmid = jax.nn.gelu(jnp.concatenate(hs, axis=1), approximate=True)
            hl = pltpu.bitcast(_dup_lhs(hmid), BF16)
            acc = x1 + y
            parts = ((0, w4_a, cps_w4a), (w4_a, FF // 16 - w4_a, cps_w4b))
            if not first:
                parts = ((0, FF // 16, None),)
            for lo, n, cps in parts:
                if cps is not None:
                    wait(cps())
                outs = []
                for c in range(D // 128):
                    outs.append(_dot(hl[:, lo * 16:(lo + n) * 16],
                                     _as_bf16(w432[pl.ds(lo, n), c]))[0:8])
                acc = acc + jnp.concatenate(outs, axis=1)
            xs[...] = acc

        if not bench:
            wait(cps_x_wq())
            start(cps_wo())
            wait(cps_k(0, 0))
            start(cps_k(2, 0))
            wait(cps_k(1, 1))
        xs[...] = jnp.broadcast_to(xin[...].astype(F32), (8, D))

        def layer(li, carry):
            first = li == 0
            n_first = 1 - li
            if bench:
                first = li == -1
                n_first = li >> 4

            def step_dma(t, static, par):
                def ok(k):
                    return (not static) or t + k < NU

                def dma_ops(_, c):
                    if ok(3):
                        start(cps_k(t + 3, 1 - par))
                    if ok(1):
                        start(cps_v(t + 1, 1 - par))
                    if static and t == NU - 2:
                        start(cps_w3())
                        start(cps_w4a())
                        start(cps_w4b())
                    if static and t == NU - 4:
                        wait(cps_wo())
                    if ok(2):
                        wait(cps_k(t + 2, par))
                    return c

                if ok(1):
                    lax.fori_loop(0, n_first, dma_ops, 0)
                pl.when(first)(lambda: wait(cps_v(t, par)))

            def step(t, static, par):
                def on(k):
                    return (not static) or (0 <= t + k < NU)
                if on(0):
                    step_dma(t, static, par)
                if on(-1):
                    st_ored(t - 1, 1 - par)
                toks = []
                if on(1):
                    toks = toks + st_qk(t + 1, 1 - par, range(cfg["jsplit"], nj))
                if on(2):
                    toks = toks + st_qk(t + 2, par, range(cfg["jsplit"]))
                if on(4):
                    toks = toks + st_qproj(t + 4, par)
                if static:
                    for u in cfg["oproj_at"].get(t, ()):
                        toks = toks + st_oproj(u)
                if on(0):
                    st_pv(t, par, toks, li >> 4)
                if on(1):
                    st_softmax(1 - par)
                if on(0):
                    st_lsum(par)
                if on(3):
                    st_qpack(1 - par)

            def body(i, c):
                step(2 * i, False, 0)
                step(2 * i + 1, False, 1)
                return c

            if bench:
                lax.fori_loop(0, bench, lambda i, c: body(i % 4 + 1, c), 0)
                return carry

            sub = lax.broadcasted_iota(jnp.int32, (8, D), 0)
            ulhs[...] = jnp.where(sub < 4, _dup_lhs(_layernorm(xs[...])), jnp.uint32(0))
            for t in range(-4, 2):
                step(t, True, t % 2)
            lax.fori_loop(1, (NU - 4) // 2, body, 0)
            for t in range(NU - 4, NU):
                step(t, True, t % 2)

            def tail(first_static):
                if first_static:
                    wait(cps_w3())
                for t in range(NU, NU + 2):
                    step(t, True, t % 2)
                mlp(first_static)

            pl.when(first)(lambda: tail(True))
            pl.when(jnp.logical_not(first))(lambda: tail(False))
            return carry

        lax.fori_loop(0, cfg["layers"], layer, 0)
        o_ref[...] = xs[0:1, :].astype(o_ref.dtype)

    return kernel


@jax.jit
def pallas_interleave_layers__sliding_block_cached__mixer_s_mlp__decode_kernel(
    A_x: jax.Array,
    A_k_cache: jax.Array,
    A_v_cache: jax.Array,
    A_wq: jax.Array,
    A_wo: jax.Array,
    B_x: jax.Array,
    B_w1: jax.Array,
    B_w2: jax.Array,
    B_w3: jax.Array,
    B_w4: jax.Array,
):
    b, sq, d = A_x.shape
    _, hkv, sk, dh = A_k_cache.shape
    assert (b, sq, d, hkv, dh) == (1, 1, D, H, DH)
    win = min(4096, max(256, sk // 4))
    assert win % 512 == 0 and sk % 128 == 0
    nj = win // 128

    kt = _tile_view(jnp.swapaxes(A_k_cache, 2, 3).reshape(H * DH, sk))
    vt = _head_view(jnp.swapaxes(A_v_cache, 2, 3).reshape(H * DH, sk))

    def buf(r, c):
        return pltpu.VMEM((r // 16, c // 128, 16, 128), BF16)

    def hbuf(c):
        return pltpu.VMEM((H, DH // 16, c // 128, 16, 128), BF16)

    any_spec = pl.BlockSpec(memory_space=pl.ANY)
    out = pl.pallas_call(
        _make_kernel(sk, win, CFG),
        out_shape=jax.ShapeDtypeStruct((1, D), A_x.dtype),
        in_specs=[any_spec] * 7,
        out_specs=pl.BlockSpec(memory_space=pltpu.VMEM),
        scratch_shapes=[
            buf(H * DH, win), hbuf(win),
            buf(D, H * DH), hbuf(D), buf(D, FF), buf(FF, D),
            pltpu.VMEM((1, D), BF16),
            pltpu.VMEM((8, D), F32),
            pltpu.VMEM((8, D), U32),
            pltpu.VMEM((2, D // 128, 8, 384), F32),
            pltpu.VMEM((2, 8, 384), U32),
            pltpu.VMEM((2, 8, win // 4), F32),
            pltpu.VMEM((2, 8, win // 4), F32),
            pltpu.VMEM((2, 8, win // 4), F32),
            pltpu.VMEM((2, 8, 128), F32),
            pltpu.VMEM((2, 384, 128), F32),
            pltpu.VMEM((NU, 8, 384), U32),
            pltpu.VMEM((3 * NU // 8, 8, D), F32),
            pltpu.SemaphoreType.DMA((5,)),
        ] + [pltpu.VMEM((2, 8, 128), F32)] * 24,
        compiler_params=pltpu.CompilerParams(vmem_limit_bytes=124 * 1024 * 1024),
        name="interleave_decode",
    )(A_x.reshape(1, D), kt, vt, _tile_view(A_wq), _head_view(A_wo),
      _tile_view(B_w3), _tile_view(B_w4))
    return out.reshape(b, sq, d)
```

```python
import jax
import jax.numpy as jnp
from jax import lax
import jax.experimental.pallas as pl
import jax.experimental.pallas.tpu as pltpu

F32 = jnp.float32
BF16 = jnp.bfloat16
U32 = jnp.uint32

D = 640
H = 32
DH = 192
FF = 1536
NU = H // 2
UT = 2 * DH // 16
EPS = 1e-5
CFG = dict(pv_nh=2, tok_lag=230, tok_rate=9.0,
           jsplit=6,
           oproj_at={12: (0,), 13: (1, 2), 14: (3, 4, 5), 15: (6, 7, 8, 9, 10, 11, 12, 13),
                     16: (14,), 17: (15,)},
           tok_mem=0, w4_a=80, layers=2, bench=0,
           tok_map=[-1, -1, -1, 10, 21, 33, 45, 60, 68, 79, 88, 99])


def _tile_view(a):
    r, c = a.shape
    a = a.reshape(r // 16, 2, 8, c // 128, 128)
    return jnp.swapaxes(a, 2, 3)


def _head_view(a):
    c = a.shape[1]
    a = a.reshape(H, 2, DH // 16, 8, c // 128, 128)
    return jnp.swapaxes(a, 3, 4)


def _as_bf16(w32):
    n = w32.shape[0]
    return pltpu.bitcast(w32.reshape(n * 8, 128), BF16)


def _bf16_bits(x):
    return pltpu.bitcast(x.astype(BF16).astype(F32), U32)


def _dup_lhs(x):
    r = _bf16_bits(x)
    return r | (r >> 16)


def _ln_stats(x):
    m = jnp.mean(x, axis=-1, keepdims=True)
    m2 = jnp.mean(x * x, axis=-1, keepdims=True)
    v = jnp.maximum(m2 - m * m, 0.0)
    return m, lax.rsqrt(v + EPS)


def _round_bf16(x):
    return x.astype(BF16).astype(F32)


def _lhs_with_ones(x):
    r = pltpu.bitcast(x, U32)
    sub = lax.broadcasted_iota(jnp.int32, r.shape, 0)
    return pltpu.bitcast(jnp.where(sub < 4, r | (r >> 16), jnp.uint32(0x3F803F80)), BF16)


def _dot(a, b):
    return jnp.dot(a, b, preferred_element_type=F32)


def _make_kernel(sk, win, cfg):
    nj = win // 128
    j0 = (sk - win) // 128
    jq = nj // 4
    scale = DH ** -0.5

    def kernel(x_hbm, k_hbm, v_hbm, wq_hbm, wo_hbm, w3_hbm, w4_hbm, o_ref,
               kbuf, vbuf, wqbuf, wobuf, w3buf, w4buf, xin,
               xs, ulhs, qp, qlhs, sx, sy, pbuf, linv, abuf, olhs, gp, sems, *tokb):

        bench = cfg["bench"]

        def cps_w(hbm, buf, sem, lo=0, n=None):
            n = buf.shape[0] if n is None else n
            return [pltpu.make_async_copy(
                hbm.at[pl.ds(lo, n), e],
                buf.at[pl.ds(lo, n), :, pl.ds(e * 8, 8), :],
                sems.at[sem]) for e in range(2)]

        def cps_kv(hbm, buf, sem, u):
            return [pltpu.make_async_copy(
                hbm.at[pl.ds(u * UT, UT), e, pl.ds(j0, nj)],
                buf.at[pl.ds(u * UT, UT), :, pl.ds(e * 8, 8), :],
                sems.at[sem]) for e in range(2)]

        def cps_v(u, par):
            return [pltpu.make_async_copy(
                v_hbm.at[pl.ds(2 * u, 2), e, :, pl.ds(j0, nj)],
                vbuf.at[pl.ds(2 * u, 2), :, :, pl.ds(e * 8, 8), :],
                sems.at[2 + par]) for e in range(2)]

        def cps_wo():
            return [pltpu.make_async_copy(
                wo_hbm.at[:, e], wobuf.at[:, :, :, pl.ds(e * 8, 8), :],
                sems.at[4]) for e in range(2)]

        w4_a = cfg["w4_a"]
        cps_k = lambda u, par: cps_kv(k_hbm, kbuf, par, u)
        cps_x_wq = lambda: [pltpu.make_async_copy(x_hbm, xin, sems.at[4])] + cps_w(wq_hbm, wqbuf, 4)
        cps_w3 = lambda: cps_w(w3_hbm, w3buf, 0)
        cps_w4a = lambda: cps_w(w4_hbm, w4buf, 1, 0, w4_a)
        cps_w4b = lambda: cps_w(w4_hbm, w4buf, 4, w4_a, FF // 16 - w4_a)

        def start(cps):
            for c in cps:
                c.start()

        def wait(cps):
            for c in cps:
                c.wait()

        if not bench:
            start(cps_x_wq())
            start(cps_k(0, 0))
            start(cps_k(1, 1))
            start(cps_v(0, 0))

        k32 = kbuf.bitcast(U32)
        v32 = vbuf.bitcast(U32)
        wq32 = wqbuf.bitcast(U32)
        wo32 = wobuf.bitcast(U32)
        w332 = w3buf.bitcast(U32)
        w432 = w4buf.bitcast(U32)

        def st_qproj(u, sl):
            lhs = pltpu.bitcast(ulhs[...], BF16)
            toks = []
            for kt in range(D // 128):
                for nt in range(3):
                    w = _as_bf16(wq32[pl.ds(kt * 8, 8), u * 3 + nt])
                    r = _dot(lhs[:, kt * 128:(kt + 1) * 128], w)
                    toks.append(r[8:16])
                    qp[sl, kt, :, nt * 128:(nt + 1) * 128] = r[0:8]
            return toks

        def st_qpack(sl):
            q = qp[sl, 0]
            for kt in range(1, D // 128):
                q = q + qp[sl, kt]
            pack_q(q, sl)

        def pack_q(q, sl):
            r = _bf16_bits(q)
            lane = lax.broadcasted_iota(jnp.int32, r.shape, 1)
            lo = jnp.where((lane < DH) | (lane >= 256), r >> 16, jnp.uint32(0))
            hi = jnp.where((lane < 128) | (lane >= DH), r, jnp.uint32(0))
            sub = lax.broadcasted_iota(jnp.int32, r.shape, 0)
            qlhs[sl] = jnp.where(sub < 4, lo | hi, jnp.uint32(0))

        def st_qk(u, sl, js):
            lhs = pltpu.bitcast(qlhs[sl], BF16)
            toks = []
            for j in js:
                ra = 2 * (j // jq)
                cs = slice((j % jq) * 128, (j % jq + 1) * 128)
                for t in range(3):
                    w = _as_bf16(k32[pl.ds(u * UT + t * 8, 8), j])
                    r = _dot(lhs[:, t * 128:(t + 1) * 128], w)
                    toks.append(r[8:16])
                    if t == 0:
                        sx[sl, ra:ra + 1, cs] = r[0:1]
                    elif t == 1:
                        sy[sl, ra:ra + 2, cs] = r[ra:ra + 2]
                    else:
                        sx[sl, ra + 1:ra + 2, cs] = r[0:1]
            return toks

        def st_softmax(slot):
            s = (sx[slot] + sy[slot]) * scale
            m = s[:, 0:128]
            for c in range(1, jq):
                m = jnp.maximum(m, s[:, c * 128:(c + 1) * 128])
            m = jnp.maximum(m, pltpu.roll(m, 2, 0))
            m = jnp.maximum(m, pltpu.roll(m, 4, 0))
            m = jnp.max(m, axis=1, keepdims=True)
            pbuf[slot] = jnp.exp(s - m)

        def st_lsum(slot):
            l = pbuf[slot, :, 0:128]
            for c in range(1, jq):
                l = l + pbuf[slot, :, c * 128:(c + 1) * 128]
            l = l + pltpu.roll(l, 2, 0)
            l = l + pltpu.roll(l, 4, 0)
            l = jnp.sum(l, axis=1, keepdims=True)
            linv[slot] = jnp.broadcast_to(1.0 / l, (8, 128))

        def st_pv(u, slot, toks, zdyn):
            nh = cfg["pv_nh"]
            npc = 12 // nh
            for hd in range(2):
                for half in range(npc):
                    piece = hd * npc + half
                    tok = None
                    if toks:
                        ti = int((piece * nh * 49 - cfg["tok_lag"]) / cfg["tok_rate"])
                        if cfg.get("tok_map") is not None:
                            ti = cfg["tok_map"][piece]
                        if ti >= 0:
                            tok = toks[min(ti, len(toks) - 1)]
                            if cfg["tok_mem"]:
                                tokb[piece][zdyn] = tok
                                tok = tokb[piece][0]
                    lo = hi = None
                    t0 = hd * 12 + half * nh
                    for j in range(nj):
                        row = 2 * (j // jq) + hd
                        cs = slice((j % jq) * 128, (j % jq + 1) * 128)
                        pb = jnp.broadcast_to(pbuf[slot, row:row + 1, cs], (8, 128))
                        if j == 0 and tok is not None:
                            pb = pb + tok
                        w = v32[2 * u + hd, pl.ds(half * nh, nh), j]
                        a = pltpu.bitcast(w << 16, F32) * pb
                        b = pltpu.bitcast(w & jnp.uint32(0xFFFF0000), F32) * pb
                        lo = a if lo is None else lo + a
                        hi = b if hi is None else hi + b
                    for i in range(nh):
                        base = (t0 + i) * 16
                        abuf[slot, pl.ds(base, 8, stride=2), :] = lo[i]
                        abuf[slot, pl.ds(base + 1, 8, stride=2), :] = hi[i]

        def st_ored(u, sl):
            at = abuf[sl].T
            o = at[0:8]
            for i in range(1, 16):
                o = o + at[i * 8:(i + 1) * 8]
            o = o + pltpu.roll(o, 4, 0)
            o = o + pltpu.roll(o, 2, 0)
            o = o + pltpu.roll(o, 1, 0)
            ia = linv[sl]
            ib = pltpu.roll(ia, 1, 0)
            lane = lax.broadcasted_iota(jnp.int32, (8, 128), 1)
            o = o * jnp.concatenate([ia, jnp.where(lane < DH - 128, ia, ib), ib], axis=1)
            sub = lax.broadcasted_iota(jnp.int32, o.shape, 0)
            olhs[u] = jnp.where(sub < 4, _bf16_bits(o) >> 16, jnp.uint32(0))

        def st_oproj(u):
            lhs = pltpu.bitcast(olhs[u], BF16)
            toks = []
            for t in range(3):
                g, row = divmod(u * 3 + t, 8)
                for n in range(D // 128):
                    if t == 1:
                        w32 = jnp.concatenate([wo32[2 * u, 8:12, n], wo32[2 * u + 1, 0:4, n]], axis=0)
                    else:
                        w32 = wo32[2 * u + t // 2, 2 * t:2 * t + 8, n]
                    w = _as_bf16(w32)
                    r = _dot(lhs[:, t * 128:(t + 1) * 128], w)
                    toks.append(r[8:16])
                    gp[g, row:row + 1, n * 128:(n + 1) * 128] = r[0:1]
            return toks

        def mlp(first):
            g = gp[0]
            for i in range(1, 3 * NU // 8):
                g = g + gp[i]
            g = g + pltpu.roll(g, 4, 0)
            g = g + pltpu.roll(g, 2, 0)
            g = g + pltpu.roll(g, 1, 0)
            x1 = _round_bf16(xs[...] + g)
            lhs = _lhs_with_ones(x1)
            m1, r1 = _ln_stats(x1)
            y = (x1 - m1) * r1
            m2, r2 = _ln_stats(y)
            a = r1 * r2
            b = (m1 * r1 + m2) * r2
            hs = []
            for n in range(FF // 128):
                r = _dot(lhs, _as_bf16(w332[:, n]))
                hs.append(r[0:8] * a - r[8:16] * b)
            hmid = jax.nn.gelu(jnp.concatenate(hs, axis=1), approximate=True)
            hl = pltpu.bitcast(_dup_lhs(hmid), BF16)
            acc = x1 + y
            parts = ((0, w4_a, cps_w4a), (w4_a, FF // 16 - w4_a, cps_w4b))
            if not first:
                parts = ((0, FF // 16, None),)
            for lo, n, cps in parts:
                if cps is not None:
                    wait(cps())
                outs = []
                for c in range(D // 128):
                    outs.append(_dot(hl[:, lo * 16:(lo + n) * 16],
                                     _as_bf16(w432[pl.ds(lo, n), c]))[0:8])
                acc = acc + jnp.concatenate(outs, axis=1)
            xs[...] = _round_bf16(acc)

        if not bench:
            wait(cps_x_wq())
            start(cps_wo())
            wait(cps_k(0, 0))
            start(cps_k(2, 0))
            wait(cps_k(1, 1))
        xs[...] = jnp.broadcast_to(xin[...].astype(F32), (8, D))

        def layer(li, carry):
            first = li == 0
            n_first = 1 - li
            if bench:
                first = li == -1
                n_first = li >> 4

            def step_dma(t, static, par):
                def ok(k):
                    return (not static) or t + k < NU

                def dma_ops(_, c):
                    if ok(3):
                        start(cps_k(t + 3, 1 - par))
                    if ok(1):
                        start(cps_v(t + 1, 1 - par))
                    if static and t == NU - 2:
                        start(cps_w3())
                        start(cps_w4a())
                        start(cps_w4b())
                    if static and t == NU - 4:
                        wait(cps_wo())
                    if ok(2):
                        wait(cps_k(t + 2, par))
                    return c

                if ok(1):
                    lax.fori_loop(0, n_first, dma_ops, 0)
                pl.when(first)(lambda: wait(cps_v(t, par)))

            def step(t, static, par):
                def on(k):
                    return (not static) or (0 <= t + k < NU)
                if on(0):
                    step_dma(t, static, par)
                if on(-1):
                    st_ored(t - 1, 1 - par)
                toks = []
                if on(1):
                    toks = toks + st_qk(t + 1, 1 - par, range(cfg["jsplit"], nj))
                if on(2):
                    toks = toks + st_qk(t + 2, par, range(cfg["jsplit"]))
                if on(4):
                    toks = toks + st_qproj(t + 4, par)
                if static:
                    for u in cfg["oproj_at"].get(t, ()):
                        toks = toks + st_oproj(u)
                if on(0):
                    st_pv(t, par, toks, li >> 4)
                if on(1):
                    st_softmax(1 - par)
                if on(0):
                    st_lsum(par)
                if on(3):
                    st_qpack(1 - par)

            def body(i, c):
                step(2 * i, False, 0)
                step(2 * i + 1, False, 1)
                return c

            if bench:
                lax.fori_loop(0, bench, lambda i, c: body(i % 4 + 1, c), 0)
                return carry

            x = xs[...]
            m, r = _ln_stats(x)
            lhs = _lhs_with_ones(x)
            for u in range(2):
                qs = []
                for nt in range(3):
                    qq = _dot(lhs, _as_bf16(wq32[:, u * 3 + nt]))
                    qs.append((qq[0:8] - qq[8:16] * m) * r)
                pack_q(jnp.concatenate(qs, axis=1), u)
            sub = lax.broadcasted_iota(jnp.int32, (8, D), 0)
            ulhs[...] = jnp.where(sub < 4, _dup_lhs((x - m) * r), jnp.uint32(0))
            st_qk(0, 0, range(nj))
            st_qproj(2, 0)
            st_qk(1, 1, range(cfg["jsplit"]))
            st_qproj(3, 1)
            st_softmax(0)
            st_qpack(0)
            for t in range(2):
                step(t, True, t % 2)
            lax.fori_loop(1, (NU - 4) // 2, body, 0)
            for t in range(NU - 4, NU):
                step(t, True, t % 2)

            def tail(first_static):
                if first_static:
                    wait(cps_w3())
                for t in range(NU, NU + 2):
                    step(t, True, t % 2)
                mlp(first_static)

            pl.when(first)(lambda: tail(True))
            pl.when(jnp.logical_not(first))(lambda: tail(False))
            return carry

        lax.fori_loop(0, cfg["layers"], layer, 0)
        o_ref[...] = xs[0:1, :].astype(o_ref.dtype)

    return kernel


@jax.jit
def pallas_interleave_layers__sliding_block_cached__mixer_s_mlp__decode_kernel(
    A_x: jax.Array,
    A_k_cache: jax.Array,
    A_v_cache: jax.Array,
    A_wq: jax.Array,
    A_wo: jax.Array,
    B_x: jax.Array,
    B_w1: jax.Array,
    B_w2: jax.Array,
    B_w3: jax.Array,
    B_w4: jax.Array,
):
    b, sq, d = A_x.shape
    _, hkv, sk, dh = A_k_cache.shape
    assert (b, sq, d, hkv, dh) == (1, 1, D, H, DH)
    win = min(4096, max(256, sk // 4))
    assert win % 512 == 0 and sk % 128 == 0
    nj = win // 128

    kt = _tile_view(jnp.swapaxes(A_k_cache, 2, 3).reshape(H * DH, sk))
    vt = _head_view(jnp.swapaxes(A_v_cache, 2, 3).reshape(H * DH, sk))

    def buf(r, c):
        return pltpu.VMEM((r // 16, c // 128, 16, 128), BF16)

    def hbuf(c):
        return pltpu.VMEM((H, DH // 16, c // 128, 16, 128), BF16)

    any_spec = pl.BlockSpec(memory_space=pl.ANY)
    out = pl.pallas_call(
        _make_kernel(sk, win, CFG),
        out_shape=jax.ShapeDtypeStruct((1, D), A_x.dtype),
        in_specs=[any_spec] * 7,
        out_specs=pl.BlockSpec(memory_space=pltpu.VMEM),
        scratch_shapes=[
            buf(H * DH, win), hbuf(win),
            buf(D, H * DH), hbuf(D), buf(D, FF), buf(FF, D),
            pltpu.VMEM((1, D), BF16),
            pltpu.VMEM((8, D), F32),
            pltpu.VMEM((8, D), U32),
            pltpu.VMEM((2, D // 128, 8, 384), F32),
            pltpu.VMEM((2, 8, 384), U32),
            pltpu.VMEM((2, 8, win // 4), F32),
            pltpu.VMEM((2, 8, win // 4), F32),
            pltpu.VMEM((2, 8, win // 4), F32),
            pltpu.VMEM((2, 8, 128), F32),
            pltpu.VMEM((2, 384, 128), F32),
            pltpu.VMEM((NU, 8, 384), U32),
            pltpu.VMEM((3 * NU // 8, 8, D), F32),
            pltpu.SemaphoreType.DMA((5,)),
        ] + [pltpu.VMEM((2, 8, 128), F32)] * 24,
        compiler_params=pltpu.CompilerParams(vmem_limit_bytes=124 * 1024 * 1024),
        name="interleave_decode",
    )(A_x.reshape(1, D), kt, vt, _tile_view(A_wq), _head_view(A_wo),
      _tile_view(B_w3), _tile_view(B_w4))
    return out.reshape(b, sq, d)
```

```python
import jax
import jax.numpy as jnp
from jax import lax
import jax.experimental.pallas as pl
import jax.experimental.pallas.tpu as pltpu

F32 = jnp.float32
BF16 = jnp.bfloat16
U32 = jnp.uint32

D = 640
H = 32
DH = 192
FF = 1536
NU = H // 2
UT = 2 * DH // 16
EPS = 1e-5
NPIECE = 12

CFG = dict(
    jsplit=6,
    jsplit0=2,
    oproj_now=(0,),
    oproj_at={13: (0,), 14: (1, 2, 3), 15: (4, 5, 6, 7, 8, 9, 10), 16: (11, 12)},
    last_split=8,
    tok={
        0: [-1,-1,-1,-1,-1,2,8,14,20,26,32,38,44,50,56,63,69,75,81,87,93,99,105,112],
        1: [-1,-1,-1,-1,-1,-1,4,10,16,21,27,33,39,44,50,56,60,67,73,79,84,90,96,99],
        "loop0": [-1,-1,-1,-1,-1,3,6,12,18,24,30,36,41,47,53,59,65,71,77,82,88,94,100,106],
        "loop1": [-1,-1,-1,-1,-1,-1,8,10,16,22,28,34,40,46,52,58,64,70,76,82,88,94,102,109],
        12: [-1,-1,-1,-1,-1,1,7,13,19,25,31,37,43,48,54,60,66,72,78,84,90,96,101,110],
        13: [-1,-1,-1,-1,-1,2,8,14,18,24,29,35,41,50,52,58,63,69,74,80,83,91,97,102],
        14: [-1,-1,-1,-1,-1,-1,6,12,17,23,29,35,40,42,52,57,63,69,74,78,91,92,97,103],
        15: [-1,-1,-1,-1,-1,-1,5,11,19,27,29,41,47,53,59,65,71,77,84,90,96,102,108,114],
        16: [-1,-1,-1,-1,-1,-1,-1,-1,-1,-1,-1,-1,-1,-1,-1,-1,-1,-1,-1,-1,0,6,14,20],
    },
    w4_a=80, layers=2, bench=0)


def _tile_view(a):
    r, c = a.shape
    a = a.reshape(r // 16, 2, 8, c // 128, 128)
    return jnp.swapaxes(a, 2, 3)


def _head_view(a):
    c = a.shape[1]
    a = a.reshape(H, 2, DH // 16, 8, c // 128, 128)
    return jnp.swapaxes(a, 3, 4)


def _as_bf16(w32):
    n = w32.shape[0]
    return pltpu.bitcast(w32.reshape(n * 8, 128), BF16)


def _lhs(top, fill=0.0):
    return jnp.concatenate([top, jnp.full(top.shape, fill, F32)], axis=0).astype(BF16)


def _ln_stats(x):
    m = jnp.mean(x, axis=-1, keepdims=True)
    m2 = jnp.mean(x * x, axis=-1, keepdims=True)
    v = jnp.maximum(m2 - m * m, 0.0)
    return m, lax.rsqrt(v + EPS)


def _round_bf16(x):
    return x.astype(BF16).astype(F32)


def _dot(a, b):
    return jnp.dot(a, b, preferred_element_type=F32)


def _make_kernel(sk, win, cfg):
    nj = win // 128
    j0 = (sk - win) // 128
    jq = nj // 4
    qscale = DH ** -0.5 * 1.4426950408889634

    def kernel(x_hbm, k_hbm, v_hbm, wq_hbm, wo_hbm, w3_hbm, w4_hbm, o_ref,
               kbuf, vbuf, wqbuf, wobuf, w3buf, w4buf, xin,
               xs, ulhs, qp, qlhs, sx, sy, pbuf, lpart, abuf, olhs, gp, sems):

        bench = cfg["bench"]

        def cps_w(hbm, buf, sem, lo=0, n=None):
            n = buf.shape[0] if n is None else n
            return [pltpu.make_async_copy(
                hbm.at[pl.ds(lo, n), e],
                buf.at[pl.ds(lo, n), :, pl.ds(e * 8, 8), :],
                sems.at[sem]) for e in range(2)]

        def cps_kv(hbm, buf, sem, u):
            return [pltpu.make_async_copy(
                hbm.at[pl.ds(u * UT, UT), e, pl.ds(j0, nj)],
                buf.at[pl.ds(u * UT, UT), :, pl.ds(e * 8, 8), :],
                sems.at[sem]) for e in range(2)]

        def cps_v(u, par):
            return [pltpu.make_async_copy(
                v_hbm.at[pl.ds(2 * u, 2), e, :, pl.ds(j0, nj)],
                vbuf.at[pl.ds(2 * u, 2), :, :, pl.ds(e * 8, 8), :],
                sems.at[2 + par]) for e in range(2)]

        def cps_wo():
            return [pltpu.make_async_copy(
                wo_hbm.at[:, e], wobuf.at[:, :, :, pl.ds(e * 8, 8), :],
                sems.at[4]) for e in range(2)]

        w4_a = cfg["w4_a"]
        cps_k = lambda u, par: cps_kv(k_hbm, kbuf, par, u)
        cps_x_wq = lambda: [pltpu.make_async_copy(x_hbm, xin, sems.at[4])] + cps_w(wq_hbm, wqbuf, 4)
        cps_w3 = lambda: cps_w(w3_hbm, w3buf, 0)
        cps_w4a = lambda: cps_w(w4_hbm, w4buf, 1, 0, w4_a)
        cps_w4b = lambda: cps_w(w4_hbm, w4buf, 4, w4_a, FF // 16 - w4_a)

        def start(cps):
            for c in cps:
                c.start()

        def wait(cps):
            for c in cps:
                c.wait()

        if not bench:
            start(cps_x_wq())
            start(cps_k(0, 0))
            start(cps_k(1, 1))
            start(cps_v(0, 0))

        k32 = kbuf.bitcast(U32)
        v32 = vbuf.bitcast(U32)
        wq32 = wqbuf.bitcast(U32)
        wo32 = wobuf.bitcast(U32)
        w332 = w3buf.bitcast(U32)
        w432 = w4buf.bitcast(U32)

        def st_qproj(u, zdyn):
            lhs = pltpu.bitcast(ulhs[...], BF16)
            toks = []
            for kt in range(D // 128):
                for nt in range(3):
                    w = _as_bf16(wq32[pl.ds(kt * 8, 8), u * 3 + nt])
                    r = _dot(lhs[:, kt * 128:(kt + 1) * 128], w)
                    toks.append(r[8:16])
                    qp[zdyn, kt, :, nt * 128:(nt + 1) * 128] = r[0:8]
            return toks

        def pack_q(q, sl):
            q = q * qscale
            lane = lax.broadcasted_iota(jnp.int32, (8, 128), 1)
            sub = lax.broadcasted_iota(jnp.int32, (8, 128), 0)
            keep = (lane < DH - 128) == (sub % 2 == 0)
            q = jnp.concatenate(
                [q[:, 0:128], jnp.where(keep, q[:, 128:256], 0.0), q[:, 256:384]], axis=1)
            qlhs[sl] = pltpu.bitcast(_lhs(q), U32)

        def st_qpack(sl):
            q = qp[0, 0]
            for kt in range(1, D // 128):
                q = q + qp[0, kt]
            pack_q(q, sl)

        def st_qk(u, sl, js):
            lhs = pltpu.bitcast(qlhs[sl], BF16)
            toks = []
            for j in js:
                ra = 2 * (j // jq)
                cs = slice((j % jq) * 128, (j % jq + 1) * 128)
                for t in range(3):
                    w = _as_bf16(k32[pl.ds(u * UT + t * 8, 8), j])
                    r = _dot(lhs[:, t * 128:(t + 1) * 128], w)
                    toks.append(r[8:16])
                    if t == 0:
                        sx[sl, ra:ra + 1, cs] = r[0:1]
                    elif t == 1:
                        sy[sl, ra:ra + 2, cs] = r[ra:ra + 2]
                    else:
                        sx[sl, ra + 1:ra + 2, cs] = r[0:1]
            return toks

        def st_softmax(sl):
            s = sx[sl] + sy[sl]
            m = s[:, 0:128]
            for c in range(1, jq):
                m = jnp.maximum(m, s[:, c * 128:(c + 1) * 128])
            m = jnp.maximum(m, pltpu.roll(m, 2, 0))
            m = jnp.maximum(m, pltpu.roll(m, 4, 0))
            m = jnp.max(m, axis=1, keepdims=True)
            pbuf[sl] = jnp.exp2(s - m)

        def st_lsum(sl):
            l = pbuf[sl, :, 0:128]
            for c in range(1, jq):
                l = l + pbuf[sl, :, c * 128:(c + 1) * 128]
            l = l + pltpu.roll(l, 2, 0)
            lpart[sl] = l + pltpu.roll(l, 4, 0)

        def st_pv(u, sl, pieces, toks, tok_map):
            for piece in pieces:
                hd, half = divmod(piece, NPIECE // 2)
                sub = len(tok_map) // NPIECE
                lo = hi = None
                for j in range(nj):
                    row = 2 * (j // jq) + hd
                    cs = slice((j % jq) * 128, (j % jq + 1) * 128)
                    pb = jnp.broadcast_to(pbuf[sl, row:row + 1, cs], (8, 128))
                    ti = tok_map[piece * sub + j * sub // nj] if j % (nj // sub) == 0 else -1
                    if toks and ti >= 0:
                        pb = pb + toks[min(ti, len(toks) - 1)]
                    w = v32[2 * u + hd, pl.ds(half * 2, 2), j]
                    a = pltpu.bitcast(w << 16, F32) * pb
                    b = pltpu.bitcast(w & jnp.uint32(0xFFFF0000), F32) * pb
                    lo = a if lo is None else lo + a
                    hi = b if hi is None else hi + b
                for i in range(2):
                    base = (piece * 2 + i) * 16
                    abuf[sl, pl.ds(base, 8, stride=2), :] = lo[i]
                    abuf[sl, pl.ds(base + 1, 8, stride=2), :] = hi[i]

        def st_ored(u, sl, ts=(0, 1, 2)):
            l = jnp.sum(lpart[sl], axis=1, keepdims=True)
            ia = jnp.broadcast_to(1.0 / l, (8, 128))
            ib = pltpu.roll(ia, 1, 0)
            lane = lax.broadcasted_iota(jnp.int32, (8, 128), 1)
            for t in ts:
                at = abuf[sl, t * 128:(t + 1) * 128, :].T
                o = at[0:8]
                for i in range(1, 16):
                    o = o + at[i * 8:(i + 1) * 8]
                o = o + pltpu.roll(o, 4, 0)
                o = o + pltpu.roll(o, 2, 0)
                o = o + pltpu.roll(o, 1, 0)
                o = o * (ia, jnp.where(lane < DH - 128, ia, ib), ib)[t]
                olhs[u, :, t * 128:(t + 1) * 128] = pltpu.bitcast(_lhs(o), U32)

        def st_oproj(u, ts=(0, 1, 2)):
            lhs = pltpu.bitcast(olhs[u], BF16)
            toks = []
            for t in ts:
                for n in range(D // 128):
                    if t == 1:
                        w32 = jnp.concatenate(
                            [wo32[2 * u, 8:12, n], wo32[2 * u + 1, 0:4, n]], axis=0)
                    else:
                        w32 = wo32[2 * u + t // 2, 2 * t:2 * t + 8, n]
                    r = _dot(lhs[:, t * 128:(t + 1) * 128], _as_bf16(w32))
                    toks.append(r[8:16])
                    gp[t, n, pl.ds(u, 1), :] = r[0:1]
            return toks

        def mlp(first):
            g = gp[0] + gp[1] + gp[2]
            g = g[:, 0:8] + g[:, 8:16]
            g = jnp.concatenate([g[n] for n in range(D // 128)], axis=1)
            g = g + pltpu.roll(g, 4, 0)
            g = g + pltpu.roll(g, 2, 0)
            g = g + pltpu.roll(g, 1, 0)
            x1 = _round_bf16(xs[...] + g)
            lhs = _lhs(x1, 1.0)
            m1, r1 = _ln_stats(x1)
            y = (x1 - m1) * r1
            m2, r2 = _ln_stats(y)
            a = r1 * r2
            b = (m1 * r1 + m2) * r2
            hl = []
            for n in range(FF // 128):
                r = _dot(lhs, _as_bf16(w332[:, n]))
                hl.append(_lhs(jax.nn.gelu(r[0:8] * a - r[8:16] * b, approximate=True)))
            acc = x1 + y
            acc = [acc[:, c * 128:(c + 1) * 128] for c in range(D // 128)]
            for kt in range(FF // 128):
                if first and kt == 0:
                    wait(cps_w4a())
                if first and kt * 8 == w4_a:
                    wait(cps_w4b())
                for c in range(D // 128):
                    w = _as_bf16(w432[pl.ds(kt * 8, 8), c])
                    acc[c] = acc[c] + _dot(hl[kt], w)[0:8]
            xs[...] = _round_bf16(jnp.concatenate(acc, axis=1))

        if not bench:
            wait(cps_x_wq())
            start(cps_wo())
            wait(cps_k(0, 0))
            start(cps_k(2, 0))
            wait(cps_k(1, 1))
        xs[...] = jnp.broadcast_to(xin[...].astype(F32), (8, D))

        def layer(li, carry):
            first = li == 0
            n_first = jnp.maximum(1 - li, 0)
            zdyn = li >> 4
            if bench:
                first = li == -1
                n_first = li >> 4

            late_ts = tuple(t for t in range(3) if t not in cfg["oproj_now"])

            def step_dma(t, static, par):
                def ok(k):
                    return (not static) or t + k < NU

                def dma_ops(_, c):
                    if ok(3):
                        start(cps_k(t + 3, 1 - par))
                    if ok(1):
                        start(cps_v(t + 1, 1 - par))
                    if static and t == NU - 2:
                        start(cps_w3())
                        start(cps_w4a())
                        start(cps_w4b())
                    if static and t == 1:
                        wait(cps_wo())
                    if ok(2):
                        wait(cps_k(t + 2, par))
                    return c

                if ok(1):
                    lax.fori_loop(0, n_first, dma_ops, 0)
                pl.when(first)(lambda: wait(cps_v(t, par)))

            def step(t, static, par):
                def on(k):
                    return (not static) or (0 <= t + k < NU)
                js_in = cfg["jsplit0"] if (static and t == 0) else cfg["jsplit"]
                step_dma(t, static, par)
                toks = []
                if on(1):
                    toks += st_qk(t + 1, 1 - par, range(js_in, nj))
                if on(3):
                    toks += st_qproj(t + 3, zdyn)
                if on(2):
                    toks += st_qk(t + 2, par, range(cfg["jsplit"]))
                if on(-2):
                    toks += st_oproj(t - 2, cfg["oproj_now"])
                if static:
                    for u in cfg["oproj_at"].get(t, ()):
                        toks += st_oproj(u, late_ts)
                if on(-1):
                    st_ored(t - 1, 1 - par)
                npc = cfg["last_split"] if (static and t == NU - 1) else NPIECE
                st_pv(t, par, range(npc), toks, cfg["tok"][t if static else "loop%d" % par])
                if on(1):
                    st_softmax(1 - par)
                st_lsum(par)
                if on(3):
                    st_qpack(1 - par)

            def body(i, c):
                step(2 * i, False, 0)
                step(2 * i + 1, False, 1)
                return c

            if bench:
                lax.fori_loop(0, bench, lambda i, c: body(i % 4 + 1, c), 0)
                return carry

            x = xs[...]
            m, r = _ln_stats(x)
            lhs = _lhs(x, 1.0)

            def q_direct(u):
                qs = []
                for nt in range(3):
                    qq = _dot(lhs, _as_bf16(wq32[:, u * 3 + nt]))
                    qs.append((qq[0:8] - qq[8:16] * m) * r)
                pack_q(jnp.concatenate(qs, axis=1), u % 2)

            q_direct(0)
            q_direct(1)
            ulhs[...] = pltpu.bitcast(_lhs((x - m) * r), U32)
            st_qk(0, 0, range(nj))
            q_direct(2)
            st_qk(1, 1, range(cfg["jsplit0"]))
            st_softmax(0)

            for t in range(2):
                step(t, True, t % 2)
            lax.fori_loop(1, (NU - 4) // 2, body, 0)
            for t in range(NU - 4, NU):
                step(t, True, t % 2)

            last, lpar = NU - 1, (NU - 1) % 2
            done_t = cfg["last_split"] // 4
            if cfg["last_split"] < NPIECE:
                pl.when(first)(lambda: wait(cps_w3()))
                st_ored(last, lpar, range(done_t))
                toks = []
                toks += st_oproj(NU - 2, cfg["oproj_now"])
                for u in cfg["oproj_at"].get(NU, ()):
                    toks += st_oproj(u, late_ts)
                st_pv(last, lpar, range(cfg["last_split"], NPIECE), toks, cfg["tok"][NU])
            else:
                done_t = 0

            def tail(first_static):
                if first_static and cfg["last_split"] == NPIECE:
                    wait(cps_w3())
                st_ored(last, lpar, range(done_t, 3))
                seen = [u for us in cfg["oproj_at"].values() for u in us]
                if cfg["last_split"] == NPIECE:
                    st_oproj(NU - 2, cfg["oproj_now"])
                for u in range(NU - 1):
                    if u not in seen:
                        st_oproj(u, late_ts)
                st_oproj(NU - 1)
                mlp(first_static)

            pl.when(first)(lambda: tail(True))
            pl.when(jnp.logical_not(first))(lambda: tail(False))
            return carry

        lax.fori_loop(0, cfg["layers"], layer, 0)
        o_ref[...] = xs[0:1, :].astype(o_ref.dtype)

    return kernel


@jax.jit
def pallas_interleave_layers__sliding_block_cached__mixer_s_mlp__decode_kernel(
    A_x: jax.Array,
    A_k_cache: jax.Array,
    A_v_cache: jax.Array,
    A_wq: jax.Array,
    A_wo: jax.Array,
    B_x: jax.Array,
    B_w1: jax.Array,
    B_w2: jax.Array,
    B_w3: jax.Array,
    B_w4: jax.Array,
):
    b, sq, d = A_x.shape
    _, hkv, sk, dh = A_k_cache.shape
    assert (b, sq, d, hkv, dh) == (1, 1, D, H, DH)
    win = min(4096, max(256, sk // 4))
    assert win % 512 == 0 and sk % 128 == 0
    nj = win // 128

    kt = _tile_view(jnp.swapaxes(A_k_cache, 2, 3).reshape(H * DH, sk))
    vt = _head_view(jnp.swapaxes(A_v_cache, 2, 3).reshape(H * DH, sk))

    def buf(r, c):
        return pltpu.VMEM((r // 16, c // 128, 16, 128), BF16)

    def hbuf(c):
        return pltpu.VMEM((H, DH // 16, c // 128, 16, 128), BF16)

    any_spec = pl.BlockSpec(memory_space=pl.ANY)
    out = pl.pallas_call(
        _make_kernel(sk, win, CFG),
        out_shape=jax.ShapeDtypeStruct((1, D), A_x.dtype),
        in_specs=[any_spec] * 7,
        out_specs=pl.BlockSpec(memory_space=pltpu.VMEM),
        scratch_shapes=[
            buf(H * DH, win), hbuf(win),
            buf(D, H * DH), hbuf(D), buf(D, FF), buf(FF, D),
            pltpu.VMEM((1, D), BF16),
            pltpu.VMEM((8, D), F32),
            pltpu.VMEM((8, D), U32),
            pltpu.VMEM((2, D // 128, 8, 384), F32),
            pltpu.VMEM((2, 8, 384), U32),
            pltpu.VMEM((2, 8, win // 4), F32),
            pltpu.VMEM((2, 8, win // 4), F32),
            pltpu.VMEM((2, 8, win // 4), F32),
            pltpu.VMEM((2, 8, 128), F32),
            pltpu.VMEM((2, 384, 128), F32),
            pltpu.VMEM((NU, 8, 384), U32),
            pltpu.VMEM((3, D // 128, NU, 128), F32),
            pltpu.SemaphoreType.DMA((5,)),
        ],
        compiler_params=pltpu.CompilerParams(vmem_limit_bytes=124 * 1024 * 1024),
        name="interleave_decode",
    )(A_x.reshape(1, D), kt, vt, _tile_view(A_wq), _head_view(A_wo),
      _tile_view(B_w3), _tile_view(B_w4))
    return out.reshape(b, sq, d)
```

```python
import jax
import jax.numpy as jnp
from jax import lax
import jax.experimental.pallas as pl
import jax.experimental.pallas.tpu as pltpu

F32 = jnp.float32
BF16 = jnp.bfloat16
U32 = jnp.uint32

D = 640
H = 32
DH = 192
FF = 1536
NU = H // 2
UT = 2 * DH // 16
EPS = 1e-5
NPIECE = 12

CFG = dict(
    jsplit=6,
    jsplit0=2,
    oproj_now=(0,),
    oproj_at={13: (0,), 14: (1, 2, 3), 15: (4, 5, 6, 7, 8, 9, 10, 11, 12)},
    nm=1, nm_at={0: 0, 15: 3},
    last_split=12,
    tok={
        0: [-1,-1,-1,-1,2,5,7,18,20,25,34,36,45,50,58,63,71,73,85,89,98,103,104,118],
        1: [-1,-1,-1,-1,-1,1,5,12,18,26,33,33,39,45,55,61,63,70,79,85,91,96,108,110],
        "loop0": [-1,-1,-1,-1,1,2,7,14,22,24,27,40,47,49,53,62,70,76,82,87,99,100,109,114],
        "loop1": [-1,-1,-1,-1,-1,-1,6,14,18,23,27,38,44,51,55,63,64,71,75,89,96,103,109,114],
        12: [-1,-1,-1,-1,-1,3,6,10,20,26,34,39,45,48,58,63,65,80,83,89,95,101,108,114],
        13: [-1,-1,-1,-1,-1,-1,8,13,16,26,32,37,42,48,55,56,65,71,78,82,89,96,106,107],
        14: [-1,-1,-1,-1,-1,1,5,19,22,27,29,40,42,44,53,59,64,70,78,79,86,97,104,107],
        15: [-1,-1,-1,-1,-1,-1,1,10,13,18,19,30,38,38,44,45,49,63,66,70,78,81,92,96],
        16: [-1,-1,-1,-1,-1,-1,-1,-1,-1,-1,-1,-1,-1,-1,-1,-1,-1,-1,-1,-1,-1,9,10,22],
    },
    w4_a=80, layers=2, bench=0)


def _tile_view(a):
    r, c = a.shape
    a = a.reshape(r // 16, 2, 8, c // 128, 128)
    return jnp.swapaxes(a, 2, 3)


def _head_view(a):
    c = a.shape[1]
    a = a.reshape(H, 2, DH // 16, 8, c // 128, 128)
    return jnp.swapaxes(a, 3, 4)


def _as_bf16(w32):
    n = w32.shape[0]
    return pltpu.bitcast(w32.reshape(n * 8, 128), BF16)


def _lhs(top, fill=0.0):
    return jnp.concatenate([top, jnp.full(top.shape, fill, F32)], axis=0).astype(BF16)


def _ln_stats(x):
    m = jnp.mean(x, axis=-1, keepdims=True)
    m2 = jnp.mean(x * x, axis=-1, keepdims=True)
    v = jnp.maximum(m2 - m * m, 0.0)
    return m, lax.rsqrt(v + EPS)


def _round_bf16(x):
    return x.astype(BF16).astype(F32)


def _dot(a, b):
    return jnp.dot(a, b, preferred_element_type=F32)


def _make_kernel(sk, win, cfg):
    nj = win // 128
    j0 = (sk - win) // 128
    jq = nj // 4
    qscale = DH ** -0.5 * 1.4426950408889634

    def kernel(x_hbm, k_hbm, v_hbm, wq_hbm, wo_hbm, w3_hbm, w4_hbm, o_ref,
               kbuf, vbuf, wqbuf, wobuf, w3buf, w4buf, xin,
               xs, ulhs, qp, qlhs, sx, sy, pbuf, plhs, mbuf, lpart, abuf, olhs, gp, sems):

        bench = cfg["bench"]

        def cps_w(hbm, buf, sem, lo=0, n=None):
            n = buf.shape[0] if n is None else n
            return [pltpu.make_async_copy(
                hbm.at[pl.ds(lo, n), e],
                buf.at[pl.ds(lo, n), :, pl.ds(e * 8, 8), :],
                sems.at[sem]) for e in range(2)]

        def cps_kv(hbm, buf, sem, u):
            return [pltpu.make_async_copy(
                hbm.at[pl.ds(u * UT, UT), e, pl.ds(j0, nj)],
                buf.at[pl.ds(u * UT, UT), :, pl.ds(e * 8, 8), :],
                sems.at[sem]) for e in range(2)]

        def cps_v(u, par):
            return [pltpu.make_async_copy(
                v_hbm.at[pl.ds(2 * u, 2), e, :, pl.ds(j0, nj)],
                vbuf.at[pl.ds(2 * u, 2), :, :, pl.ds(e * 8, 8), :],
                sems.at[2 + par]) for e in range(2)]

        def cps_wo():
            return [pltpu.make_async_copy(
                wo_hbm.at[:, e], wobuf.at[:, :, :, pl.ds(e * 8, 8), :],
                sems.at[4]) for e in range(2)]

        w4_a = cfg["w4_a"]
        cps_k = lambda u, par: cps_kv(k_hbm, kbuf, par, u)
        cps_x_wq = lambda: [pltpu.make_async_copy(x_hbm, xin, sems.at[4])] + cps_w(wq_hbm, wqbuf, 4)
        cps_w3 = lambda: cps_w(w3_hbm, w3buf, 0)
        cps_w4a = lambda: cps_w(w4_hbm, w4buf, 1, 0, w4_a)
        cps_w4b = lambda: cps_w(w4_hbm, w4buf, 4, w4_a, FF // 16 - w4_a)

        def start(cps):
            for c in cps:
                c.start()

        def wait(cps):
            for c in cps:
                c.wait()

        if not bench:
            start(cps_x_wq())
            start(cps_k(0, 0))
            start(cps_k(1, 1))
            start(cps_v(0, 0))

        k32 = kbuf.bitcast(U32)
        v32 = vbuf.bitcast(U32)
        wq32 = wqbuf.bitcast(U32)
        wo32 = wobuf.bitcast(U32)
        w332 = w3buf.bitcast(U32)
        w432 = w4buf.bitcast(U32)

        def st_qproj(u, zdyn):
            lhs = pltpu.bitcast(ulhs[...], BF16)
            toks = []
            for kt in range(D // 128):
                for nt in range(3):
                    w = _as_bf16(wq32[pl.ds(kt * 8, 8), u * 3 + nt])
                    r = _dot(lhs[:, kt * 128:(kt + 1) * 128], w)
                    toks.append(r[8:16])
                    qp[zdyn, kt, :, nt * 128:(nt + 1) * 128] = r[0:8]
            return toks

        def pack_q(q, sl):
            q = q * qscale
            lane = lax.broadcasted_iota(jnp.int32, (8, 128), 1)
            sub = lax.broadcasted_iota(jnp.int32, (8, 128), 0)
            keep = (lane < DH - 128) == (sub % 2 == 0)
            q = jnp.concatenate(
                [q[:, 0:128], jnp.where(keep, q[:, 128:256], 0.0), q[:, 256:384]], axis=1)
            qlhs[sl] = pltpu.bitcast(_lhs(q), U32)

        def st_qpack(sl):
            q = qp[0, 0]
            for kt in range(1, D // 128):
                q = q + qp[0, kt]
            pack_q(q, sl)

        def st_qk(u, sl, js):
            lhs = pltpu.bitcast(qlhs[sl], BF16)
            toks = []
            for j in js:
                ra = 2 * (j // jq)
                cs = slice((j % jq) * 128, (j % jq + 1) * 128)
                for t in range(3):
                    w = _as_bf16(k32[pl.ds(u * UT + t * 8, 8), j])
                    r = _dot(lhs[:, t * 128:(t + 1) * 128], w)
                    toks.append(r[8:16])
                    if t == 0:
                        sx[sl, ra:ra + 1, cs] = r[0:1]
                    elif t == 1:
                        sy[sl, ra:ra + 2, cs] = r[ra:ra + 2]
                    else:
                        sx[sl, ra + 1:ra + 2, cs] = r[0:1]
            return toks

        def st_softmax(sl, nm):
            s = sx[sl] + sy[sl]
            m = s[:, 0:128]
            for c in range(1, jq):
                m = jnp.maximum(m, s[:, c * 128:(c + 1) * 128])
            m = jnp.maximum(m, pltpu.roll(m, 2, 0))
            m = jnp.maximum(m, pltpu.roll(m, 4, 0))
            m = jnp.max(m, axis=1, keepdims=True)
            p = jnp.exp2(s - m)
            pbuf[sl] = p
            for i in range(nm):
                c = jq - 1 - i
                plhs[sl, i] = pltpu.bitcast(_lhs(p[:, c * 128:(c + 1) * 128]), U32)

        def st_lsum(sl):
            l = pbuf[sl, :, 0:128]
            for c in range(1, jq):
                l = l + pbuf[sl, :, c * 128:(c + 1) * 128]
            l = l + pltpu.roll(l, 2, 0)
            lpart[sl] = l + pltpu.roll(l, 4, 0)

        def st_pvm(u, sl, nm):
            toks = []
            for i in range(nm):
                lhs = pltpu.bitcast(plhs[sl, i], BF16)
                j = nj - 1 - i
                for t in range(3):
                    if t == 1:
                        w32 = jnp.concatenate(
                            [v32[2 * u, 8:12, j], v32[2 * u + 1, 0:4, j]], axis=0)
                    else:
                        w32 = v32[2 * u + t // 2, 2 * t:2 * t + 8, j]
                    r = lax.dot_general(lhs, _as_bf16(w32), (((1,), (1,)), ((), ())),
                                        preferred_element_type=F32)
                    toks.append(r[8:16])
                    mbuf[sl, i, t] = r[0:8]
            return toks

        def st_pv(u, sl, nm, pieces, toks, tok_map):
            for piece in pieces:
                hd, half = divmod(piece, NPIECE // 2)
                sub = len(tok_map) // NPIECE
                lo = hi = None
                for j in range(nj - nm):
                    row = 2 * (j // jq) + hd
                    cs = slice((j % jq) * 128, (j % jq + 1) * 128)
                    pb = jnp.broadcast_to(pbuf[sl, row:row + 1, cs], (8, 128))
                    ti = tok_map[piece * sub + j * sub // nj] if j % (nj // sub) == 0 else -1
                    if toks and ti >= 0:
                        pb = pb + toks[min(ti, len(toks) - 1)]
                    w = v32[2 * u + hd, pl.ds(half * 2, 2), j]
                    a = pltpu.bitcast(w << 16, F32) * pb
                    b = pltpu.bitcast(w & jnp.uint32(0xFFFF0000), F32) * pb
                    lo = a if lo is None else lo + a
                    hi = b if hi is None else hi + b
                for i in range(2):
                    base = (piece * 2 + i) * 16
                    abuf[sl, pl.ds(base, 8, stride=2), :] = lo[i]
                    abuf[sl, pl.ds(base + 1, 8, stride=2), :] = hi[i]

        def st_ored(u, sl, nm, ts=(0, 1, 2)):
            l = jnp.sum(lpart[sl], axis=1, keepdims=True)
            ia = jnp.broadcast_to(1.0 / l, (8, 128))
            ib = pltpu.roll(ia, 1, 0)
            lane = lax.broadcasted_iota(jnp.int32, (8, 128), 1)
            for t in ts:
                at = abuf[sl, t * 128:(t + 1) * 128, :].T
                o = at[0:8]
                for i in range(1, 16):
                    o = o + at[i * 8:(i + 1) * 8]
                if nm:
                    om = mbuf[sl, 0, t]
                    for i in range(1, nm):
                        om = om + mbuf[sl, i, t]
                    sub = lax.broadcasted_iota(jnp.int32, (8, 128), 0)
                    row = (6, jnp.where(lane < DH - 128, 6, 7), 7)[t]
                    o = o + jnp.where(sub == row, om, 0.0)
                o = o + pltpu.roll(o, 4, 0)
                o = o + pltpu.roll(o, 2, 0)
                o = o + pltpu.roll(o, 1, 0)
                o = o * (ia, jnp.where(lane < DH - 128, ia, ib), ib)[t]
                olhs[u, :, t * 128:(t + 1) * 128] = pltpu.bitcast(_lhs(o), U32)

        def st_oproj(u, ts=(0, 1, 2)):
            lhs = pltpu.bitcast(olhs[u], BF16)
            toks = []
            for t in ts:
                for n in range(D // 128):
                    if t == 1:
                        w32 = jnp.concatenate(
                            [wo32[2 * u, 8:12, n], wo32[2 * u + 1, 0:4, n]], axis=0)
                    else:
                        w32 = wo32[2 * u + t // 2, 2 * t:2 * t + 8, n]
                    r = _dot(lhs[:, t * 128:(t + 1) * 128], _as_bf16(w32))
                    toks.append(r[8:16])
                    gp[t, n, pl.ds(u, 1), :] = r[0:1]
            return toks

        def mlp(first):
            g = gp[0] + gp[1] + gp[2]
            g = g[:, 0:8] + g[:, 8:16]
            g = jnp.concatenate([g[n] for n in range(D // 128)], axis=1)
            g = g + pltpu.roll(g, 4, 0)
            g = g + pltpu.roll(g, 2, 0)
            g = g + pltpu.roll(g, 1, 0)
            x1 = _round_bf16(xs[...] + g)
            lhs = _lhs(x1, 1.0)
            m1, r1 = _ln_stats(x1)
            y = (x1 - m1) * r1
            m2, r2 = _ln_stats(y)
            a = r1 * r2
            b = (m1 * r1 + m2) * r2
            hl = []
            for n in range(FF // 128):
                r = _dot(lhs, _as_bf16(w332[:, n]))
                hl.append(_lhs(jax.nn.gelu(r[0:8] * a - r[8:16] * b, approximate=True)))
            acc = x1 + y
            acc = [acc[:, c * 128:(c + 1) * 128] for c in range(D // 128)]
            for kt in range(FF // 128):
                if first and kt == 0:
                    wait(cps_w4a())
                if first and kt * 8 == w4_a:
                    wait(cps_w4b())
                for c in range(D // 128):
                    w = _as_bf16(w432[pl.ds(kt * 8, 8), c])
                    acc[c] = acc[c] + _dot(hl[kt], w)[0:8]
            xs[...] = _round_bf16(jnp.concatenate(acc, axis=1))

        if not bench:
            wait(cps_x_wq())
            start(cps_wo())
            wait(cps_k(0, 0))
            start(cps_k(2, 0))
            wait(cps_k(1, 1))
        xs[...] = jnp.broadcast_to(xin[...].astype(F32), (8, D))

        def layer(li, carry):
            first = li == 0
            n_first = jnp.maximum(1 - li, 0)
            zdyn = li >> 4
            if bench:
                first = li == -1
                n_first = li >> 4

            late_ts = tuple(t for t in range(3) if t not in cfg["oproj_now"])

            def nmx(t, static):
                return cfg["nm_at"].get(t, cfg["nm"]) if static else cfg["nm"]

            def step_dma(t, static, par):
                def ok(k):
                    return (not static) or t + k < NU

                def dma_ops(_, c):
                    if ok(3):
                        start(cps_k(t + 3, 1 - par))
                    if ok(1):
                        start(cps_v(t + 1, 1 - par))
                    if static and t == NU - 2:
                        start(cps_w3())
                        start(cps_w4a())
                        start(cps_w4b())
                    if static and t == 1:
                        wait(cps_wo())
                    if ok(2):
                        wait(cps_k(t + 2, par))
                    return c

                if ok(1):
                    lax.fori_loop(0, n_first, dma_ops, 0)
                pl.when(first)(lambda: wait(cps_v(t, par)))

            def step(t, static, par):
                def on(k):
                    return (not static) or (0 <= t + k < NU)
                js_in = cfg["jsplit0"] if (static and t == 0) else cfg["jsplit"]
                step_dma(t, static, par)
                toks = []
                if on(1):
                    toks += st_qk(t + 1, 1 - par, range(js_in, nj))
                if on(3):
                    toks += st_qproj(t + 3, zdyn)
                if on(2):
                    toks += st_qk(t + 2, par, range(cfg["jsplit"]))
                toks += st_pvm(t, par, nmx(t, static))
                if on(-2):
                    toks += st_oproj(t - 2, cfg["oproj_now"])
                if static:
                    for u in cfg["oproj_at"].get(t, ()):
                        toks += st_oproj(u, late_ts)
                if on(-1):
                    st_ored(t - 1, 1 - par, nmx(t - 1, static))
                npc = cfg["last_split"] if (static and t == NU - 1) else NPIECE
                st_pv(t, par, nmx(t, static), range(npc), toks,
                      cfg["tok"][t if static else "loop%d" % par])
                if on(1):
                    st_softmax(1 - par, nmx(t + 1, static))
                st_lsum(par)
                if on(3):
                    st_qpack(1 - par)

            def body(i, c):
                step(2 * i, False, 0)
                step(2 * i + 1, False, 1)
                return c

            if bench:
                lax.fori_loop(0, bench, lambda i, c: body(i % 4 + 1, c), 0)
                return carry
            if cfg.get("only") is not None:
                for t in cfg["only"]:
                    if t == "loop":
                        lax.fori_loop(1, (NU - 4) // 2, body, 0)
                    else:
                        step(t, True, t % 2)
                lax.fori_loop(0, n_first, lambda i, c: c + 1, 0)
                pl.when(first)(lambda: wait(cps_w3()))
                return carry

            x = xs[...]
            m, r = _ln_stats(x)
            lhs = _lhs(x, 1.0)

            def q_direct(u):
                qs = []
                for nt in range(3):
                    qq = _dot(lhs, _as_bf16(wq32[:, u * 3 + nt]))
                    qs.append((qq[0:8] - qq[8:16] * m) * r)
                pack_q(jnp.concatenate(qs, axis=1), u % 2)

            q_direct(0)
            q_direct(1)
            ulhs[...] = pltpu.bitcast(_lhs((x - m) * r), U32)
            st_qk(0, 0, range(nj))
            q_direct(2)
            st_qk(1, 1, range(cfg["jsplit0"]))
            st_softmax(0, nmx(0, True))

            for t in range(2):
                step(t, True, t % 2)
            lax.fori_loop(1, (NU - 4) // 2, body, 0)
            for t in range(NU - 4, NU):
                step(t, True, t % 2)

            last, lpar = NU - 1, (NU - 1) % 2
            done_t = cfg["last_split"] // 4
            if cfg["last_split"] < NPIECE:
                pl.when(first)(lambda: wait(cps_w3()))
                st_ored(last, lpar, nmx(last, True), range(done_t))
                toks = []
                toks += st_oproj(NU - 2, cfg["oproj_now"])
                for u in cfg["oproj_at"].get(NU, ()):
                    toks += st_oproj(u, late_ts)
                st_pv(last, lpar, nmx(last, True), range(cfg["last_split"], NPIECE),
                      toks, cfg["tok"][NU])
            else:
                done_t = 0

            def tail(first_static):
                if first_static and cfg["last_split"] == NPIECE:
                    wait(cps_w3())
                st_ored(last, lpar, nmx(last, True), range(done_t, 3))
                seen = [u for us in cfg["oproj_at"].values() for u in us]
                if cfg["last_split"] == NPIECE:
                    st_oproj(NU - 2, cfg["oproj_now"])
                for u in range(NU - 1):
                    if u not in seen:
                        st_oproj(u, late_ts)
                st_oproj(NU - 1)
                mlp(first_static)

            pl.when(first)(lambda: tail(True))
            pl.when(jnp.logical_not(first))(lambda: tail(False))
            return carry

        lax.fori_loop(0, cfg["layers"], layer, 0)
        o_ref[...] = xs[0:1, :].astype(o_ref.dtype)

    return kernel


@jax.jit
def pallas_interleave_layers__sliding_block_cached__mixer_s_mlp__decode_kernel(
    A_x: jax.Array,
    A_k_cache: jax.Array,
    A_v_cache: jax.Array,
    A_wq: jax.Array,
    A_wo: jax.Array,
    B_x: jax.Array,
    B_w1: jax.Array,
    B_w2: jax.Array,
    B_w3: jax.Array,
    B_w4: jax.Array,
):
    b, sq, d = A_x.shape
    _, hkv, sk, dh = A_k_cache.shape
    assert (b, sq, d, hkv, dh) == (1, 1, D, H, DH)
    win = min(4096, max(256, sk // 4))
    assert win % 512 == 0 and sk % 128 == 0
    nj = win // 128

    kt = _tile_view(jnp.swapaxes(A_k_cache, 2, 3).reshape(H * DH, sk))
    vt = _head_view(jnp.swapaxes(A_v_cache, 2, 3).reshape(H * DH, sk))

    def buf(r, c):
        return pltpu.VMEM((r // 16, c // 128, 16, 128), BF16)

    def hbuf(c):
        return pltpu.VMEM((H, DH // 16, c // 128, 16, 128), BF16)

    any_spec = pl.BlockSpec(memory_space=pl.ANY)
    out = pl.pallas_call(
        _make_kernel(sk, win, CFG),
        out_shape=jax.ShapeDtypeStruct((1, D), A_x.dtype),
        in_specs=[any_spec] * 7,
        out_specs=pl.BlockSpec(memory_space=pltpu.VMEM),
        scratch_shapes=[
            buf(H * DH, win), hbuf(win),
            buf(D, H * DH), hbuf(D), buf(D, FF), buf(FF, D),
            pltpu.VMEM((1, D), BF16),
            pltpu.VMEM((8, D), F32),
            pltpu.VMEM((8, D), U32),
            pltpu.VMEM((2, D // 128, 8, 384), F32),
            pltpu.VMEM((2, 8, 384), U32),
            pltpu.VMEM((2, 8, win // 4), F32),
            pltpu.VMEM((2, 8, win // 4), F32),
            pltpu.VMEM((2, 8, win // 4), F32),
            pltpu.VMEM((2, 8, 8, 128), U32),
            pltpu.VMEM((2, 8, 3, 8, 128), F32),
            pltpu.VMEM((2, 8, 128), F32),
            pltpu.VMEM((2, 384, 128), F32),
            pltpu.VMEM((NU, 8, 384), U32),
            pltpu.VMEM((3, D // 128, NU, 128), F32),
            pltpu.SemaphoreType.DMA((5,)),
        ],
        compiler_params=pltpu.CompilerParams(vmem_limit_bytes=124 * 1024 * 1024),
        name="interleave_decode",
    )(A_x.reshape(1, D), kt, vt, _tile_view(A_wq), _head_view(A_wo),
      _tile_view(B_w3), _tile_view(B_w4))
    return out.reshape(b, sq, d)
```

```python
import jax
import jax.numpy as jnp
from jax import lax
import jax.experimental.pallas as pl
import jax.experimental.pallas.tpu as pltpu

F32 = jnp.float32
BF16 = jnp.bfloat16
U32 = jnp.uint32

D = 640
H = 32
DH = 192
FF = 1536
NU = H // 2
UT = 2 * DH // 16
EPS = 1e-5
NPIECE = 12

CFG = dict(
    jsplit=6,
    jsplit0=2,
    oproj_now=((0,), (0,)),
    oproj_at={13: (0,), 14: (1, 2, 3), 15: (4, 5, 6, 7, 8, 9, 10, 11, 12)},
    nm=0, nm_at={15: 1},
    jx=(1, 5, 9, 13, 17, 21, 25), vmem_mb=127,
    tok={
        "loop0": [-1,-1,-1,-1,-1,0,5,8,18,22,26,36,39,47,51,61,62,67,77,83,87,97,102,107],
        "loop1": [-1,-1,-1,-1,-1,0,6,10,15,23,27,37,41,41,51,53,65,66,69,84,90,96,101,107],
        0: [-1,-1,-1,-1,-1,1,4,12,20,26,26,36,43,46,50,58,69,70,74,78,90,94,96,102],
        1: [-1,-1,-1,-1,-1,-1,6,11,13,20,29,31,41,43,50,52,61,63,67,82,83,93,97,102],
        12: [-1,-1,-1,-1,-1,-1,8,10,15,24,27,32,39,43,48,60,63,71,79,81,86,99,100,106],
        13: [-1,-1,-1,-1,-1,1,4,9,15,23,27,34,37,44,50,55,59,71,73,81,84,90,96,103],
        14: [-1,-1,-1,-1,-1,0,7,7,16,19,28,32,42,42,49,52,63,70,75,81,88,98,102,106],
        15: [-1,-1,-1,-1,-1,-1,1,5,11,12,23,25,27,38,39,46,46,60,61,67,71,75,89,93],
    },
    w4_a=80, layers=2, bench=0)


def _tile_view(a):
    r, c = a.shape
    a = a.reshape(r // 16, 2, 8, c // 128, 128)
    return jnp.swapaxes(a, 2, 3)


def _head_view(a):
    c = a.shape[1]
    a = a.reshape(H, 2, DH // 16, 8, c // 128, 128)
    return jnp.swapaxes(a, 3, 4)


def _as_bf16(w32):
    n = w32.shape[0]
    return pltpu.bitcast(w32.reshape(n * 8, 128), BF16)


def _lhs(top, fill=0.0):
    return jnp.concatenate([top, jnp.full(top.shape, fill, F32)], axis=0).astype(BF16)


def _ln_stats(x):
    m = jnp.mean(x, axis=-1, keepdims=True)
    m2 = jnp.mean(x * x, axis=-1, keepdims=True)
    v = jnp.maximum(m2 - m * m, 0.0)
    return m, lax.rsqrt(v + EPS)


def _round_bf16(x):
    return x.astype(BF16).astype(F32)


def _dot(a, b):
    return jnp.dot(a, b, preferred_element_type=F32)


def _make_kernel(sk, win, cfg):
    nj = win // 128
    j0 = (sk - win) // 128
    jq = nj // 4
    jx = list(cfg["jx"])
    qscale = DH ** -0.5 * 1.4426950408889634

    def kernel(x_hbm, k_hbm, v_hbm, wq_hbm, wo_hbm, w3_hbm, w4_hbm, o_ref,
               kbuf, vbuf, vx, wqbuf, wobuf, w3buf, w4buf, xin,
               xs, ulhs, qp, qlhs, sx, sy, pbuf, plhs, mbuf, lpart, abuf, olhs, gp, sems):

        bench = cfg["bench"]

        def cps_w(hbm, buf, sem, lo=0, n=None):
            n = buf.shape[0] if n is None else n
            return [pltpu.make_async_copy(
                hbm.at[pl.ds(lo, n), e],
                buf.at[pl.ds(lo, n), :, pl.ds(e * 8, 8), :],
                sems.at[sem]) for e in range(2)]

        def cps_kv(hbm, buf, sem, u):
            return [pltpu.make_async_copy(
                hbm.at[pl.ds(u * UT, UT), e, pl.ds(j0, nj)],
                buf.at[pl.ds(u * UT, UT), :, pl.ds(e * 8, 8), :],
                sems.at[sem]) for e in range(2)]

        def cps_v(u, par):
            return [pltpu.make_async_copy(
                v_hbm.at[pl.ds(2 * u, 2), e, :, pl.ds(j0, nj)],
                vbuf.at[pl.ds(2 * u, 2), :, :, pl.ds(e * 8, 8), :],
                sems.at[2 + par]) for e in range(2)]

        def cps_wo():
            return [pltpu.make_async_copy(
                wo_hbm.at[:, e], wobuf.at[:, :, :, pl.ds(e * 8, 8), :],
                sems.at[4]) for e in range(2)]

        w4_a = cfg["w4_a"]
        cps_k = lambda u, par: cps_kv(k_hbm, kbuf, par, u)
        cps_x_wq = lambda: [pltpu.make_async_copy(x_hbm, xin, sems.at[4])] + cps_w(wq_hbm, wqbuf, 4)
        cps_w3 = lambda: cps_w(w3_hbm, w3buf, 0)
        cps_w4a = lambda: cps_w(w4_hbm, w4buf, 1, 0, w4_a)
        cps_w4b = lambda: cps_w(w4_hbm, w4buf, 4, w4_a, FF // 16 - w4_a)

        def start(cps):
            for c in cps:
                c.start()

        def wait(cps):
            for c in cps:
                c.wait()

        if not bench:
            start(cps_x_wq())
            start(cps_k(0, 0))
            start(cps_k(1, 1))
            start(cps_v(0, 0))
            start(cps_v(1, 1))

        k32 = kbuf.bitcast(U32)
        v32 = vbuf.bitcast(U32)
        wq32 = wqbuf.bitcast(U32)
        wo32 = wobuf.bitcast(U32)
        w332 = w3buf.bitcast(U32)
        w432 = w4buf.bitcast(U32)

        def st_qproj(u, zdyn):
            lhs = pltpu.bitcast(ulhs[...], BF16)
            toks = []
            for kt in range(D // 128):
                for nt in range(3):
                    w = _as_bf16(wq32[pl.ds(kt * 8, 8), u * 3 + nt])
                    r = _dot(lhs[:, kt * 128:(kt + 1) * 128], w)
                    toks.append(r[8:16])
                    qp[zdyn, kt, :, nt * 128:(nt + 1) * 128] = r[0:8]
            return toks

        def pack_q(q, sl):
            q = q * qscale
            lane = lax.broadcasted_iota(jnp.int32, (8, 128), 1)
            sub = lax.broadcasted_iota(jnp.int32, (8, 128), 0)
            keep = (lane < DH - 128) == (sub % 2 == 0)
            q = jnp.concatenate(
                [q[:, 0:128], jnp.where(keep, q[:, 128:256], 0.0), q[:, 256:384]], axis=1)
            qlhs[sl] = pltpu.bitcast(_lhs(q), U32)

        def st_qpack(sl):
            q = qp[0, 0]
            for kt in range(1, D // 128):
                q = q + qp[0, kt]
            pack_q(q, sl)

        def st_qk(u, sl, js):
            lhs = pltpu.bitcast(qlhs[sl], BF16)
            toks = []
            for j in js:
                ra = 2 * (j // jq)
                cs = slice((j % jq) * 128, (j % jq + 1) * 128)
                for t in range(3):
                    w = _as_bf16(k32[pl.ds(u * UT + t * 8, 8), j])
                    r = _dot(lhs[:, t * 128:(t + 1) * 128], w)
                    toks.append(r[8:16])
                    if t == 0:
                        sx[sl, ra:ra + 1, cs] = r[0:1]
                    elif t == 1:
                        sy[sl, ra:ra + 2, cs] = r[ra:ra + 2]
                    else:
                        sx[sl, ra + 1:ra + 2, cs] = r[0:1]
            return toks

        def st_softmax(sl, nm):
            s = sx[sl] + sy[sl]
            m = s[:, 0:128]
            for c in range(1, jq):
                m = jnp.maximum(m, s[:, c * 128:(c + 1) * 128])
            m = jnp.maximum(m, pltpu.roll(m, 2, 0))
            m = jnp.maximum(m, pltpu.roll(m, 4, 0))
            m = jnp.max(m, axis=1, keepdims=True)
            p = jnp.exp2(s - m)
            pbuf[sl] = p
            for i in range(nm):
                c = jq - 1 - i
                plhs[sl, i] = pltpu.bitcast(_lhs(p[:, c * 128:(c + 1) * 128]), U32)

        def st_lsum(sl):
            l = pbuf[sl, :, 0:128]
            for c in range(1, jq):
                l = l + pbuf[sl, :, c * 128:(c + 1) * 128]
            l = l + pltpu.roll(l, 2, 0)
            lpart[sl] = l + pltpu.roll(l, 4, 0)

        def st_pvm(u, sl, nm):
            toks = []
            for i in range(nm):
                lhs = pltpu.bitcast(plhs[sl, i], BF16)
                j = nj - 1 - i
                for t in range(3):
                    if t == 1:
                        w32 = jnp.concatenate(
                            [v32[2 * u, 8:12, j], v32[2 * u + 1, 0:4, j]], axis=0)
                    else:
                        w32 = v32[2 * u + t // 2, 2 * t:2 * t + 8, j]
                    r = lax.dot_general(lhs, _as_bf16(w32), (((1,), (1,)), ((), ())),
                                        preferred_element_type=F32)
                    toks.append(r[8:16])
                    mbuf[sl, i, t] = r[0:8]
            return toks

        def st_expand(u):
            def body(i, c):
                hd, dt = i // 12, i % 12
                for ix, j in enumerate(jx):
                    w = v32[2 * u + hd, dt, j]
                    vx[2 * u + hd, dt, ix] = pltpu.bitcast(w << 16, F32)
                    vbuf[2 * u + hd, dt, j] = pltpu.bitcast(w & jnp.uint32(0xFFFF0000), BF16)
                return c
            if jx:
                lax.fori_loop(0, UT, body, 0)

        def st_pv(u, sl, nm, pieces, toks, tok_map):
            for piece in pieces:
                hd, half = divmod(piece, NPIECE // 2)
                sub = len(tok_map) // NPIECE
                lo = hi = None
                for j in range(nj - nm):
                    row = 2 * (j // jq) + hd
                    cs = slice((j % jq) * 128, (j % jq + 1) * 128)
                    pb = jnp.broadcast_to(pbuf[sl, row:row + 1, cs], (8, 128))
                    ti = tok_map[piece * sub + j * sub // nj] if j % (nj // sub) == 0 else -1
                    if toks and ti >= 0:
                        pb = pb + toks[min(ti, len(toks) - 1)]
                    w = v32[2 * u + hd, pl.ds(half * 2, 2), j]
                    if j in jx:
                        a = vx[2 * u + hd, pl.ds(half * 2, 2), jx.index(j)] * pb
                        b = pltpu.bitcast(w, F32) * pb
                    else:
                        a = pltpu.bitcast(w << 16, F32) * pb
                        b = pltpu.bitcast(w & jnp.uint32(0xFFFF0000), F32) * pb
                    lo = a if lo is None else lo + a
                    hi = b if hi is None else hi + b
                for i in range(2):
                    base = (piece * 2 + i) * 16
                    abuf[sl, pl.ds(base, 8, stride=2), :] = lo[i]
                    abuf[sl, pl.ds(base + 1, 8, stride=2), :] = hi[i]

        def st_ored(u, sl, nm, ts=(0, 1, 2)):
            l = jnp.sum(lpart[sl], axis=1, keepdims=True)
            ia = jnp.broadcast_to(1.0 / l, (8, 128))
            ib = pltpu.roll(ia, 1, 0)
            lane = lax.broadcasted_iota(jnp.int32, (8, 128), 1)
            for t in ts:
                at = abuf[sl, t * 128:(t + 1) * 128, :].T
                o = at[0:8]
                for i in range(1, 16):
                    o = o + at[i * 8:(i + 1) * 8]
                if nm:
                    om = mbuf[sl, 0, t]
                    for i in range(1, nm):
                        om = om + mbuf[sl, i, t]
                    sub = lax.broadcasted_iota(jnp.int32, (8, 128), 0)
                    row = (6, jnp.where(lane < DH - 128, 6, 7), 7)[t]
                    o = o + jnp.where(sub == row, om, 0.0)
                o = o + pltpu.roll(o, 4, 0)
                o = o + pltpu.roll(o, 2, 0)
                o = o + pltpu.roll(o, 1, 0)
                o = o * (ia, jnp.where(lane < DH - 128, ia, ib), ib)[t]
                olhs[u, :, t * 128:(t + 1) * 128] = pltpu.bitcast(_lhs(o), U32)

        def st_oproj(u, ts=(0, 1, 2)):
            lhs = pltpu.bitcast(olhs[u], BF16)
            toks = []
            for t in ts:
                for n in range(D // 128):
                    if t == 1:
                        w32 = jnp.concatenate(
                            [wo32[2 * u, 8:12, n], wo32[2 * u + 1, 0:4, n]], axis=0)
                    else:
                        w32 = wo32[2 * u + t // 2, 2 * t:2 * t + 8, n]
                    r = _dot(lhs[:, t * 128:(t + 1) * 128], _as_bf16(w32))
                    toks.append(r[8:16])
                    gp[t, n, pl.ds(u, 1), :] = r[0:1]
            return toks

        def mlp(first):
            g = gp[0] + gp[1] + gp[2]
            g = g[:, 0:8] + g[:, 8:16]
            g = jnp.concatenate([g[n] for n in range(D // 128)], axis=1)
            g = g + pltpu.roll(g, 4, 0)
            g = g + pltpu.roll(g, 2, 0)
            g = g + pltpu.roll(g, 1, 0)
            x1 = _round_bf16(xs[...] + g)
            lhs = _lhs(x1, 1.0)
            m1, r1 = _ln_stats(x1)
            y = (x1 - m1) * r1
            m2, r2 = _ln_stats(y)
            a = r1 * r2
            b = (m1 * r1 + m2) * r2
            hl = []
            for n in range(FF // 128):
                r = _dot(lhs, _as_bf16(w332[:, n]))
                hl.append(_lhs(jax.nn.gelu(r[0:8] * a - r[8:16] * b, approximate=True)))
            acc = x1 + y
            acc = [acc[:, c * 128:(c + 1) * 128] for c in range(D // 128)]
            for kt in range(FF // 128):
                if first and kt == 0:
                    wait(cps_w4a())
                if first and kt * 8 == w4_a:
                    wait(cps_w4b())
                for c in range(D // 128):
                    w = _as_bf16(w432[pl.ds(kt * 8, 8), c])
                    acc[c] = acc[c] + _dot(hl[kt], w)[0:8]
            xs[...] = _round_bf16(jnp.concatenate(acc, axis=1))

        if not bench:
            wait(cps_x_wq())
            start(cps_wo())
            wait(cps_k(0, 0))
            start(cps_k(2, 0))
            wait(cps_k(1, 1))
            wait(cps_v(0, 0))
        xs[...] = jnp.broadcast_to(xin[...].astype(F32), (8, D))

        def layer(li, carry):
            first = li == 0
            n_first = jnp.maximum(1 - li, 0)
            zdyn = li >> 4
            if bench:
                first = li == -1
                n_first = li >> 4

            def now_ts(par):
                return cfg["oproj_now"][par]

            def late_ts(u):
                return tuple(t for t in range(3) if t not in now_ts(u % 2))

            def nmx(t, static):
                return cfg["nm_at"].get(t, cfg["nm"]) if static else cfg["nm"]

            def step_dma(t, static, par):
                def ok(k):
                    return (not static) or t + k < NU

                def dma_ops(_, c):
                    if ok(3):
                        start(cps_k(t + 3, 1 - par))
                    if ok(2):
                        start(cps_v(t + 2, par))
                    if static and t == NU - 2:
                        start(cps_w3())
                        start(cps_w4a())
                        start(cps_w4b())
                    if static and t == 1:
                        wait(cps_wo())
                    st_expand(t)
                    if ok(2):
                        wait(cps_k(t + 2, par))
                    return c

                lax.fori_loop(0, n_first, dma_ops, 0)
                pl.when(first)(lambda: wait(cps_v(t + 1, 1 - par) if ok(1) else cps_w3()))

            def step(t, static, par):
                def on(k):
                    return (not static) or (0 <= t + k < NU)
                js_in = cfg["jsplit0"] if (static and t == 0) else cfg["jsplit"]
                step_dma(t, static, par)
                toks = []
                if on(1):
                    toks += st_qk(t + 1, 1 - par, range(js_in, nj))
                if on(3):
                    toks += st_qproj(t + 3, zdyn)
                if on(2):
                    toks += st_qk(t + 2, par, range(cfg["jsplit"]))
                toks += st_pvm(t, par, nmx(t, static))
                if on(-2):
                    toks += st_oproj(t - 2, now_ts(par))
                if static:
                    for u in cfg["oproj_at"].get(t, ()):
                        toks += st_oproj(u, late_ts(u))
                if on(-1):
                    st_ored(t - 1, 1 - par, nmx(t - 1, static))
                st_pv(t, par, nmx(t, static), range(NPIECE), toks,
                      cfg["tok"][t if static else "loop%d" % par])
                if on(1):
                    st_softmax(1 - par, nmx(t + 1, static))
                st_lsum(par)
                if on(3):
                    st_qpack(1 - par)

            def body(i, c):
                step(2 * i, False, 0)
                step(2 * i + 1, False, 1)
                return c

            if bench:
                lax.fori_loop(0, bench, lambda i, c: body(i % 4 + 1, c), 0)
                return carry
            if cfg.get("only") is not None:
                for t in cfg["only"]:
                    if t == "loop":
                        lax.fori_loop(1, (NU - 4) // 2, body, 0)
                    else:
                        step(t, True, t % 2)
                lax.fori_loop(0, n_first, lambda i, c: c + 1, 0)
                pl.when(first)(lambda: wait(cps_w3()))
                return carry

            x = xs[...]
            m, r = _ln_stats(x)
            lhs = _lhs(x, 1.0)

            def q_direct(u):
                qs = []
                for nt in range(3):
                    qq = _dot(lhs, _as_bf16(wq32[:, u * 3 + nt]))
                    qs.append((qq[0:8] - qq[8:16] * m) * r)
                pack_q(jnp.concatenate(qs, axis=1), u % 2)

            q_direct(0)
            q_direct(1)
            ulhs[...] = pltpu.bitcast(_lhs((x - m) * r), U32)
            st_qk(0, 0, range(nj))
            q_direct(2)
            st_qk(1, 1, range(cfg["jsplit0"]))
            st_softmax(0, nmx(0, True))

            for t in range(2):
                step(t, True, t % 2)
            lax.fori_loop(1, (NU - 4) // 2, body, 0)
            for t in range(NU - 4, NU):
                step(t, True, t % 2)

            last, lpar = NU - 1, (NU - 1) % 2

            def tail(first_static):
                st_ored(last, lpar, nmx(last, True))
                seen = [u for us in cfg["oproj_at"].values() for u in us]
                st_oproj(NU - 2, now_ts(NU % 2))
                for u in range(NU - 1):
                    if u not in seen:
                        st_oproj(u, late_ts(u))
                st_oproj(NU - 1)
                mlp(first_static)

            pl.when(first)(lambda: tail(True))
            pl.when(jnp.logical_not(first))(lambda: tail(False))
            return carry

        lax.fori_loop(0, cfg["layers"], layer, 0)
        o_ref[...] = xs[0:1, :].astype(o_ref.dtype)

    return kernel


@jax.jit
def pallas_interleave_layers__sliding_block_cached__mixer_s_mlp__decode_kernel(
    A_x: jax.Array,
    A_k_cache: jax.Array,
    A_v_cache: jax.Array,
    A_wq: jax.Array,
    A_wo: jax.Array,
    B_x: jax.Array,
    B_w1: jax.Array,
    B_w2: jax.Array,
    B_w3: jax.Array,
    B_w4: jax.Array,
):
    b, sq, d = A_x.shape
    _, hkv, sk, dh = A_k_cache.shape
    assert (b, sq, d, hkv, dh) == (1, 1, D, H, DH)
    win = min(4096, max(256, sk // 4))
    assert win % 512 == 0 and sk % 128 == 0
    nj = win // 128

    kt = _tile_view(jnp.swapaxes(A_k_cache, 2, 3).reshape(H * DH, sk))
    vt = _head_view(jnp.swapaxes(A_v_cache, 2, 3).reshape(H * DH, sk))

    def buf(r, c):
        return pltpu.VMEM((r // 16, c // 128, 16, 128), BF16)

    def hbuf(c):
        return pltpu.VMEM((H, DH // 16, c // 128, 16, 128), BF16)

    nm_max = max([1, CFG["nm"]] + list(CFG["nm_at"].values()))
    any_spec = pl.BlockSpec(memory_space=pl.ANY)
    out = pl.pallas_call(
        _make_kernel(sk, win, CFG),
        out_shape=jax.ShapeDtypeStruct((1, D), A_x.dtype),
        in_specs=[any_spec] * 7,
        out_specs=pl.BlockSpec(memory_space=pltpu.VMEM),
        scratch_shapes=[
            buf(H * DH, win), hbuf(win),
            pltpu.VMEM((H, DH // 16, max(len(CFG["jx"]), 1), 8, 128), F32),
            buf(D, H * DH), hbuf(D), buf(D, FF), buf(FF, D),
            pltpu.VMEM((1, D), BF16),
            pltpu.VMEM((8, D), F32),
            pltpu.VMEM((8, D), U32),
            pltpu.VMEM((2, D // 128, 8, 384), F32),
            pltpu.VMEM((2, 8, 384), U32),
            pltpu.VMEM((2, 8, win // 4), F32),
            pltpu.VMEM((2, 8, win // 4), F32),
            pltpu.VMEM((2, 8, win // 4), F32),
            pltpu.VMEM((2, nm_max, 8, 128), U32),
            pltpu.VMEM((2, nm_max, 3, 8, 128), F32),
            pltpu.VMEM((2, 8, 128), F32),
            pltpu.VMEM((2, 384, 128), F32),
            pltpu.VMEM((NU, 8, 384), U32),
            pltpu.VMEM((3, D // 128, NU, 128), F32),
            pltpu.SemaphoreType.DMA((5,)),
        ],
        compiler_params=pltpu.CompilerParams(vmem_limit_bytes=int(CFG["vmem_mb"] * 1024 * 1024)),
        name="interleave_decode",
    )(A_x.reshape(1, D), kt, vt, _tile_view(A_wq), _head_view(A_wo),
      _tile_view(B_w3), _tile_view(B_w4))
    return out.reshape(b, sq, d)
```

```python
import jax
import jax.numpy as jnp
from jax import lax
import jax.experimental.pallas as pl
import jax.experimental.pallas.tpu as pltpu

F32 = jnp.float32
BF16 = jnp.bfloat16
U32 = jnp.uint32

D = 640
H = 32
DH = 192
FF = 1536
NU = H // 2
UT = 2 * DH // 16
EPS = 1e-5
NPIECE = 12

NTOK = {}
CFG = dict(
    blocks=((0, 4), (4, 8), (8, 12), (12, 15), (15, 16)), ns=7,
    jsplit=8, js_at={},
    pvm_back=2, pvm_back0=0, pretr=1,
    nm=2, nm_at={0: 3, 1: 3, 2: 3, 3: 3},
    qproj_at={t: (t + 3,) for t in range(13)},
    oproj_at={4: ((0, (2,)),), 5: ((1, (2,)),), 6: ((2, (2,)),), 7: ((3, (2,)),),
              8: ((4, (2,)),), 9: ((5, (2,)),), 10: ((6, (2,)),), 11: ((7, (2,)),),
              12: ((8, (2,)),), 13: ((9, (2,)), (10, (2,)), (0, (0, 1))),
              14: ((11, (2,)), (1, (0, 1)), (2, (0, 1)), (3, (0, 1))),
              15: ((4, (0, 1)), (5, (0, 1)), (6, (0, 1)), (7, (0, 1)), (8, (0, 1)), (9, (0, 1)),
                   (10, (0, 1)), (11, (0, 1)), 12)},
    jx=(1, 5, 9, 13, 17, 21, 25), vmem_mb=128,
    tok={
        0: [-27,-24,-22,-20,-17,-15,-13,-11,-8,-6,-4,-1,1,3,6,8,10,13,16,19,21,24,27,30,33,35,38,41,44,47,49,52,55,58,60,63,65,68,70,73,76,78,81,83,86,88,91,93],
        1: [-24,-21,-19,-16,-14,-11,-9,-6,-4,-1,2,4,7,9,12,14,17,19,22,25,27,30,32,35,37,40,42,45,48,50,53,55,58,60,63,65,68,71,73,76,78,81,83,86,88,91,94,96],
        2: [-21,-19,-16,-14,-11,-9,-6,-3,-1,2,4,7,9,12,14,17,20,22,25,27,30,32,35,37,40,43,45,48,50,53,55,58,60,63,66,68,71,73,76,78,81,83,86,89,91,94,96,99],
        3: [-19,-16,-14,-11,-8,-6,-3,-1,2,4,7,9,12,15,17,20,22,25,27,30,32,35,38,40,43,45,48,50,53,55,58,61,63,66,68,71,73,76,78,81,84,86,89,91,94,96,99,101],
        4: [-27,-24,-22,-19,-17,-14,-12,-9,-7,-5,-2,0,3,5,8,10,13,16,18,21,24,26,29,32,34,37,40,42,45,48,50,53,56,59,61,64,67,69,72,75,77,80,83,85,88,91,93,96],
        5: [-29,-27,-24,-21,-19,-16,-14,-11,-8,-6,-3,-1,2,5,7,10,13,15,18,20,23,26,28,31,34,36,39,41,44,47,49,52,54,57,60,62,65,68,70,73,75,78,81,83,86,89,91,94],
        6: [-26,-23,-20,-18,-15,-13,-10,-7,-5,-2,1,3,6,8,11,14,16,19,21,24,27,29,32,35,37,40,42,45,48,50,53,56,58,61,63,66,69,71,74,76,79,82,84,87,90,92,95,97],
        7: [-22,-19,-17,-14,-12,-9,-6,-4,-1,2,4,7,9,12,15,17,20,23,26,28,31,34,37,40,43,46,49,51,54,57,60,63,66,68,71,73,76,78,81,83,85,88,90,93,95,98,100,103],
        8: [-21,-19,-16,-14,-12,-9,-7,-5,-2,0,2,4,7,9,11,14,16,19,21,24,27,29,32,34,37,40,42,45,48,50,53,56,58,61,64,67,70,73,76,79,81,84,87,90,93,96,99,102],
        9: [-23,-21,-18,-16,-13,-11,-8,-6,-3,0,2,5,7,10,12,15,17,20,23,25,28,30,33,36,38,41,44,46,49,51,54,57,59,62,65,67,70,73,76,79,81,84,87,90,92,95,98,101],
        10: [-19,-16,-13,-11,-8,-5,-3,0,3,5,8,11,13,16,19,21,24,26,29,32,34,37,40,42,45,48,50,53,56,58,61,63,66,69,71,74,77,79,82,85,87,90,93,95,98,100,103,106],
        11: [-14,-11,-8,-6,-3,0,2,5,8,10,13,15,18,21,23,26,29,31,34,37,39,42,45,47,50,52,55,58,60,63,66,68,71,74,76,79,82,84,87,90,92,95,97,100,103,105,108,111],
        12: [-28,-26,-23,-21,-18,-16,-13,-10,-8,-5,-3,0,2,5,7,10,13,15,18,20,23,26,28,31,33,36,39,41,44,47,49,52,54,57,60,63,66,69,72,75,78,81,84,87,90,93,96,99],
        13: [-26,-24,-21,-18,-16,-13,-11,-8,-5,-3,0,3,5,8,10,13,16,18,21,24,26,29,32,35,37,40,43,45,48,51,54,56,59,62,64,67,69,72,75,77,80,82,85,88,90,93,96,98],
        14: [-21,-19,-16,-14,-11,-9,-6,-4,-1,1,4,7,9,12,14,17,19,22,25,27,30,33,35,38,41,43,46,49,52,54,57,60,62,65,67,70,73,75,78,80,83,85,88,90,93,95,98,100],
        15: [-22,-21,-19,-17,-15,-14,-12,-10,-8,-6,-5,-3,-1,1,2,4,6,9,12,14,17,20,23,26,29,31,34,37,40,43,46,48,51,54,56,59,62,64,67,70,72,75,77,80,83,85,88,90],
    },
    tok_lin=(24, 18),
    w4_a=80, layers=2)


def _tile_view(a):
    r, c = a.shape
    a = a.reshape(r // 16, 2, 8, c // 128, 128)
    return jnp.swapaxes(a, 2, 3)


def _head_view(a):
    c = a.shape[1]
    a = a.reshape(H, 2, DH // 16, 8, c // 128, 128)
    return jnp.swapaxes(a, 3, 4)


def _as_bf16(w32):
    n = w32.shape[0]
    return pltpu.bitcast(w32.reshape(n * 8, 128), BF16)


def _lhs(top, fill=0.0):
    return jnp.concatenate([top, jnp.full(top.shape, fill, F32)], axis=0).astype(BF16)


def _ln_stats(x):
    m = jnp.mean(x, axis=-1, keepdims=True)
    m2 = jnp.mean(x * x, axis=-1, keepdims=True)
    v = jnp.maximum(m2 - m * m, 0.0)
    return m, lax.rsqrt(v + EPS)


def _round_bf16(x):
    return x.astype(BF16).astype(F32)


def _dot(a, b):
    return jnp.dot(a, b, preferred_element_type=F32)


def _make_kernel(sk, win, cfg):
    nj = win // 128
    j0 = (sk - win) // 128
    jq = nj // 4
    jx = list(cfg["jx"])
    qscale = DH ** -0.5 * 1.4426950408889634

    def kernel(x_hbm, k_hbm, v_hbm, wq_hbm, wo_hbm, w3_hbm, w4_hbm, o_ref,
               kbuf, vbuf, vx, wqbuf, wobuf, w3buf, w4buf, xin,
               xs, ulhs, qp0, qp1, qp2, qlhs, sx, sy, pbuf0, pbuf1, plhs, mbuf, lpart, abuf, olhs, gp,
               sems):
        qp = (qp0, qp1, qp2)
        pbuf = (pbuf0, pbuf1)
        ns = abuf.shape[0]


        def cps_w(hbm, buf, sem, lo=0, n=None):
            n = buf.shape[0] if n is None else n
            return [pltpu.make_async_copy(
                hbm.at[pl.ds(lo, n), e],
                buf.at[pl.ds(lo, n), :, pl.ds(e * 8, 8), :],
                sems.at[sem]) for e in range(2)]

        def cps_kv(hbm, buf, sem, u):
            return [pltpu.make_async_copy(
                hbm.at[pl.ds(u * UT, UT), e, pl.ds(j0, nj)],
                buf.at[pl.ds(u * UT, UT), :, pl.ds(e * 8, 8), :],
                sems.at[sem]) for e in range(2)]

        def cps_v(u, par):
            return [pltpu.make_async_copy(
                v_hbm.at[pl.ds(2 * u, 2), e, :, pl.ds(j0, nj)],
                vbuf.at[pl.ds(2 * u, 2), :, :, pl.ds(e * 8, 8), :],
                sems.at[2 + par]) for e in range(2)]

        def cps_wo():
            return [pltpu.make_async_copy(
                wo_hbm.at[:, e], wobuf.at[:, :, :, pl.ds(e * 8, 8), :],
                sems.at[4]) for e in range(2)]

        w4_a = cfg["w4_a"]
        cps_k = lambda u, par: cps_kv(k_hbm, kbuf, par, u)
        cps_x_wq = lambda: [pltpu.make_async_copy(x_hbm, xin, sems.at[4])] + cps_w(wq_hbm, wqbuf, 4)
        cps_w3 = lambda: cps_w(w3_hbm, w3buf, 0)
        cps_w4a = lambda: cps_w(w4_hbm, w4buf, 1, 0, w4_a)
        cps_w4b = lambda: cps_w(w4_hbm, w4buf, 4, w4_a, FF // 16 - w4_a)

        def start(cps):
            for c in cps:
                c.start()

        def wait(cps):
            for c in cps:
                c.wait()

        start(cps_x_wq())
        start(cps_k(0, 0))
        start(cps_k(1, 1))
        start(cps_v(0, 0))
        start(cps_v(1, 1))

        k32 = kbuf.bitcast(U32)
        v32 = vbuf.bitcast(U32)
        wq32 = wqbuf.bitcast(U32)
        wo32 = wobuf.bitcast(U32)
        w332 = w3buf.bitcast(U32)
        w432 = w4buf.bitcast(U32)

        def js(u):
            return cfg["js_at"].get(u, cfg["jsplit"])

        def nmx(u):
            return cfg["nm_at"].get(u, cfg["nm"])

        def st_qproj(u, zdyn):
            lhs = pltpu.bitcast(ulhs[...], BF16)
            toks = []
            for kt in range(D // 128):
                for nt in range(3):
                    w = _as_bf16(wq32[pl.ds(kt * 8, 8), u * 3 + nt])
                    r = _dot(lhs[:, kt * 128:(kt + 1) * 128], w)
                    toks.append(r[8:16])
                    qp[u % 3][zdyn, kt, :, nt * 128:(nt + 1) * 128] = r[0:8]
            return toks

        def pack_q(q, u):
            q = q * qscale
            lane = lax.broadcasted_iota(jnp.int32, (8, 128), 1)
            sub = lax.broadcasted_iota(jnp.int32, (8, 128), 0)
            keep = (lane < DH - 128) == (sub % 2 == 0)
            q = jnp.concatenate(
                [q[:, 0:128], jnp.where(keep, q[:, 128:256], 0.0), q[:, 256:384]], axis=1)
            qlhs.at[u % 8][:, 0:384] = pltpu.bitcast(_lhs(q), U32)

        def st_qpack(u):
            q = qp[u % 3][0, 0]
            for kt in range(1, D // 128):
                q = q + qp[u % 3][0, kt]
            pack_q(q, u)

        def st_qk(u, js):
            sl = u % 2
            lhs = pltpu.bitcast(qlhs[u % 8], BF16)
            toks = []
            for j in js:
                ra = 2 * (j // jq)
                cs = slice((j % jq) * 128, (j % jq + 1) * 128)
                for t in range(3):
                    w = _as_bf16(k32[pl.ds(u * UT + t * 8, 8), j])
                    r = _dot(lhs[:, t * 128:(t + 1) * 128], w)
                    toks.append(r[8:16])
                    if t == 0:
                        sx[sl, ra:ra + 1, cs] = r[0:1]
                    elif t == 1:
                        sy[sl, ra:ra + 2, cs] = r[ra:ra + 2]
                    else:
                        sx[sl, ra + 1:ra + 2, cs] = r[0:1]
            return toks

        def st_softmax(u, zdyn):
            sl = u % 2
            s = sx[sl] + sy[sl]
            m = s[:, 0:128]
            for c in range(1, jq):
                m = jnp.maximum(m, s[:, c * 128:(c + 1) * 128])
            m = jnp.maximum(m, pltpu.roll(m, 2, 0))
            m = jnp.maximum(m, pltpu.roll(m, 4, 0))
            m = jnp.max(m, axis=1, keepdims=True)
            p = jnp.exp2(s - m)
            pbuf[sl][zdyn] = p
            for i in range(nmx(u)):
                c = jq - 1 - i
                plhs.at[sl, i][:, 0:128] = pltpu.bitcast(_lhs(p[:, c * 128:(c + 1) * 128]), U32)

        def st_lsum(u):
            l = pbuf[u % 2][0, :, 0:128]
            for c in range(1, jq):
                l = l + pbuf[u % 2][0, :, c * 128:(c + 1) * 128]
            l = l + pltpu.roll(l, 2, 0)
            lpart[u % ns] = l + pltpu.roll(l, 4, 0)

        def st_pvm(u):
            toks = []
            for i in range(nmx(u)):
                lhs = pltpu.bitcast(plhs[u % 2, i], BF16)
                j = nj - 1 - i
                for t in range(3):
                    if t == 1:
                        w32 = jnp.concatenate(
                            [v32[2 * u, 8:12, j], v32[2 * u + 1, 0:4, j]], axis=0)
                    else:
                        w32 = v32[2 * u + t // 2, 2 * t:2 * t + 8, j]
                    if cfg["pretr"]:
                        r = _dot(lhs, _as_bf16(w32))
                    else:
                        r = lax.dot_general(lhs, _as_bf16(w32), (((1,), (1,)), ((), ())),
                                            preferred_element_type=F32)
                    toks.append(r[8:16])
                    mbuf[u % ns, i, t] = r[0:8]
            return toks

        def st_expand(u):
            def body(i, c):
                hd, dt = i // 12, i % 12
                for ix, j in enumerate(jx):
                    w = v32[2 * u + hd, dt, j]
                    vx[2 * u + hd, dt, ix] = pltpu.bitcast(w << 16, F32)
                    vbuf[2 * u + hd, dt, j] = pltpu.bitcast(w & jnp.uint32(0xFFFF0000), BF16)
                return c
            if jx:
                lax.fori_loop(0, UT, body, 0)
            for i in range(nmx(u) if cfg["pretr"] else 0):
                j = nj - 1 - i
                for t in range(3):
                    idx = [divmod(t * 8 + v, 12) for v in range(8)]
                    blk = jnp.concatenate([vbuf[2 * u + hd, dt, j] for hd, dt in idx], axis=0)
                    blk = blk.astype(F32).T.astype(BF16)
                    for v, (hd, dt) in enumerate(idx):
                        vbuf[2 * u + hd, dt, j] = blk[v * 16:(v + 1) * 16]

        def st_pv(u, toks, tok_map):
            nm, sl = nmx(u), u % ns
            for piece in range(NPIECE):
                hd, half = divmod(piece, NPIECE // 2)
                sub = len(tok_map) // NPIECE
                lo = hi = None
                for j in range(nj - nm):
                    row = 2 * (j // jq) + hd
                    cs = slice((j % jq) * 128, (j % jq + 1) * 128)
                    pb = jnp.broadcast_to(pbuf[u % 2][0, row:row + 1, cs], (8, 128))
                    k = piece * sub + j * sub // nj
                    ti = tok_map[k] if j % (nj // sub) == 0 else -1
                    if j > 0 and tok_map[k - 1] == ti:
                        ti = -1
                    if toks and ti >= 0:
                        pb = pb + toks[min(ti, len(toks) - 1)]
                    w = v32[2 * u + hd, pl.ds(half * 2, 2), j]
                    if j in jx:
                        a = vx[2 * u + hd, pl.ds(half * 2, 2), jx.index(j)] * pb
                        b = pltpu.bitcast(w, F32) * pb
                    else:
                        a = pltpu.bitcast(w << 16, F32) * pb
                        b = pltpu.bitcast(w & jnp.uint32(0xFFFF0000), F32) * pb
                    lo = a if lo is None else lo + a
                    hi = b if hi is None else hi + b
                for i in range(2):
                    base = (piece * 2 + i) * 16
                    abuf[sl, pl.ds(base, 8, stride=2), :] = lo[i]
                    abuf[sl, pl.ds(base + 1, 8, stride=2), :] = hi[i]

        def st_ored(u, ts=(0, 1, 2)):
            nm, sl = nmx(u), u % ns
            l = jnp.sum(lpart[sl], axis=1, keepdims=True)
            r0 = pl.reciprocal(l, approx=True)
            ia = jnp.broadcast_to(r0 * (2.0 - l * r0), (8, 128))
            ib = pltpu.roll(ia, 1, 0)
            lane = lax.broadcasted_iota(jnp.int32, (8, 128), 1)
            for t in ts:
                at = abuf[sl, t * 128:(t + 1) * 128, :].T
                o = at[0:8]
                for i in range(1, 16):
                    o = o + at[i * 8:(i + 1) * 8]
                if nm:
                    om = mbuf[sl, 0, t]
                    for i in range(1, nm):
                        om = om + mbuf[sl, i, t]
                    sub = lax.broadcasted_iota(jnp.int32, (8, 128), 0)
                    row = (6, jnp.where(lane < DH - 128, 6, 7), 7)[t]
                    o = o + jnp.where(sub == row, om, 0.0)
                o = o + pltpu.roll(o, 4, 0)
                o = o + pltpu.roll(o, 2, 0)
                o = o + pltpu.roll(o, 1, 0)
                o = o * (ia, jnp.where(lane < DH - 128, ia, ib), ib)[t]
                olhs.at[u][:, t * 128:(t + 1) * 128] = pltpu.bitcast(_lhs(o), U32)

        def st_oproj(u, ts=(0, 1, 2)):
            lhs = pltpu.bitcast(olhs[u], BF16)
            toks = []
            for t in ts:
                for n in range(D // 128):
                    if t == 1:
                        w32 = jnp.concatenate(
                            [wo32[2 * u, 8:12, n], wo32[2 * u + 1, 0:4, n]], axis=0)
                    else:
                        w32 = wo32[2 * u + t // 2, 2 * t:2 * t + 8, n]
                    r = _dot(lhs[:, t * 128:(t + 1) * 128], _as_bf16(w32))
                    toks.append(r[8:16])
                    gp[t, n, pl.ds(u, 1), :] = r[0:1]
            return toks

        def mlp(first):
            g = gp[0] + gp[1] + gp[2]
            g = g[:, 0:8] + g[:, 8:16]
            g = jnp.concatenate([g[n] for n in range(D // 128)], axis=1)
            g = g + pltpu.roll(g, 4, 0)
            g = g + pltpu.roll(g, 2, 0)
            g = g + pltpu.roll(g, 1, 0)
            x1 = _round_bf16(xs[...] + g)
            lhs = _lhs(x1, 1.0)
            m1, r1 = _ln_stats(x1)
            y = (x1 - m1) * r1
            m2, r2 = _ln_stats(y)
            a = r1 * r2
            b = (m1 * r1 + m2) * r2
            hl = []
            for n in range(FF // 128):
                r = _dot(lhs, _as_bf16(w332[:, n]))
                hl.append(_lhs(jax.nn.gelu(r[0:8] * a - r[8:16] * b, approximate=True)))
            acc = x1 + y
            acc = [acc[:, c * 128:(c + 1) * 128] for c in range(D // 128)]
            for kt in range(FF // 128):
                if first and kt == 0:
                    wait(cps_w4a())
                if first and kt * 8 == w4_a:
                    wait(cps_w4b())
                for c in range(D // 128):
                    w = _as_bf16(w432[pl.ds(kt * 8, 8), c])
                    acc[c] = acc[c] + _dot(hl[kt], w)[0:8]
            xs[...] = _round_bf16(jnp.concatenate(acc, axis=1))

        wait(cps_x_wq())
        start(cps_wo())
        wait(cps_k(0, 0))
        start(cps_k(2, 0))
        wait(cps_k(1, 1))
        wait(cps_v(0, 0))
        xs[...] = jnp.broadcast_to(xin[...].astype(F32), (8, D))

        def layer(li, carry):
            first = li == 0
            n_first = jnp.maximum(1 - li, 0)
            zdyn = li >> 4

            def block_dma(ua, ub):
                def last_wait(t):
                    wait(cps_v(t + 1, (t + 1) % 2) if t + 1 < NU else cps_w3())

                def dma_ops(_, c):
                    for t in range(ua, ub):
                        if t + 3 < NU:
                            start(cps_k(t + 3, (t + 3) % 2))
                        if t + 2 < NU:
                            start(cps_v(t + 2, t % 2))
                        if t == NU - 2:
                            start(cps_w3())
                            start(cps_w4a())
                            start(cps_w4b())
                        if t == 1:
                            wait(cps_wo())
                        if cfg.get("only") is None:
                            st_expand(t)
                        if t + 2 < NU:
                            wait(cps_k(t + 2, t % 2))
                        if t < ub - 1:
                            last_wait(t)
                    return c

                lax.fori_loop(0, n_first, dma_ops, 0)
                pl.when(first)(lambda: last_wait(ub - 1))

            def prologue():
                x = xs[...]
                m, r = _ln_stats(x)
                lhs = _lhs(x, 1.0)

                def q_direct(u):
                    qs = []
                    for nt in range(3):
                        qq = _dot(lhs, _as_bf16(wq32[:, u * 3 + nt]))
                        qs.append((qq[0:8] - qq[8:16] * m) * r)
                    pack_q(jnp.concatenate(qs, axis=1), u)

                q_direct(0)
                q_direct(1)
                ulhs[...] = pltpu.bitcast(_lhs((x - m) * r), U32)
                toks = st_qk(0, range(nj))
                st_softmax(0, zdyn)
                q_direct(2)
                pos = js(1) - cfg["pvm_back0"]
                toks += st_qk(1, range(pos))
                toks += st_pvm(0)
                toks += st_qk(1, range(pos, js(1)))
                return toks

            def block(bi):
                ua, ub = cfg["blocks"][bi]
                block_dma(ua, ub)
                toks = []
                if bi > 0:
                    for u in range(*cfg["blocks"][bi - 1]):
                        st_ored(u)
                else:
                    toks += prologue()
                for t in range(ua, ub):
                    base = len(toks)
                    if t == ua and bi > 0:
                        toks += st_pvm(t)
                    if t + 1 < NU:
                        toks += st_qk(t + 1, range(js(t + 1), nj))
                        st_softmax(t + 1, zdyn)
                    for u in cfg["qproj_at"].get(t, ()):
                        toks += st_qproj(u, zdyn)
                    for u in cfg["oproj_at"].get(t, ()):
                        toks += st_oproj(*u) if isinstance(u, tuple) else st_oproj(u)
                    pos = max(js(t + 2) - cfg["pvm_back"], 0)
                    if t + 2 < NU:
                        toks += st_qk(t + 2, range(pos))
                    if t + 1 < ub:
                        toks += st_pvm(t + 1)
                    if t + 2 < NU:
                        toks += st_qk(t + 2, range(pos, js(t + 2)))
                    tok_map = cfg["tok"].get(t)
                    if tok_map is None:
                        n = len(toks) - base
                        if t == ub - 1:
                            n += cfg["tok_lin"][1]
                        tok_map = [k * n // (4 * NPIECE) - cfg["tok_lin"][0]
                                   for k in range(4 * NPIECE)]
                    NTOK[t] = len(toks) - base
                    st_pv(t, toks, [base + i for i in tok_map])
                    st_lsum(t)
                    for u in cfg["qproj_at"].get(t, ()):
                        st_qpack(u)

            if cfg.get("only") is not None:
                for bi in cfg["only"]:
                    block(bi)
                lax.fori_loop(0, n_first, lambda i, c: c + 1, 0)
                pl.when(first)(lambda: wait(cps_w4a()))
                f = lambda v: pltpu.bitcast(v, F32)
                z8 = pl.multiple_of(zdyn * 8, 8)
                z128 = pl.multiple_of(zdyn * 128, 128)
                xs[:, 0:128] = (abuf[zdyn, pl.ds(z8, 8), :] + lpart[zdyn] + mbuf[zdyn, zdyn, zdyn]
                                + f(olhs[zdyn, :, pl.ds(z128, 128)]) + f(qlhs[zdyn, :, pl.ds(z128, 128)])
                                + sx[zdyn, :, pl.ds(z128, 128)] + sy[zdyn, :, pl.ds(z128, 128)]
                                + pbuf0[zdyn, :, pl.ds(z128, 128)] + pbuf1[zdyn, :, pl.ds(z128, 128)]
                                + gp[zdyn, zdyn, pl.ds(z8, 8), :] + f(plhs[zdyn, zdyn]))
                return carry

            for bi in range(len(cfg["blocks"])):
                block(bi)

            def tail(first_static):
                for u in range(*cfg["blocks"][-1]):
                    st_ored(u)
                seen = set()
                for us in cfg["oproj_at"].values():
                    for u in us:
                        uu, ts = u if isinstance(u, tuple) else (u, (0, 1, 2))
                        seen |= {(uu, t) for t in ts}
                for u in range(NU):
                    ts = tuple(t for t in range(3) if (u, t) not in seen)
                    if ts:
                        st_oproj(u, ts)
                mlp(first_static)

            pl.when(first)(lambda: tail(True))
            pl.when(jnp.logical_not(first))(lambda: tail(False))
            return carry

        lax.fori_loop(0, cfg["layers"], layer, 0)
        o_ref[...] = xs[0:1, :].astype(o_ref.dtype)

    return kernel


@jax.jit
def pallas_interleave_layers__sliding_block_cached__mixer_s_mlp__decode_kernel(
    A_x: jax.Array,
    A_k_cache: jax.Array,
    A_v_cache: jax.Array,
    A_wq: jax.Array,
    A_wo: jax.Array,
    B_x: jax.Array,
    B_w1: jax.Array,
    B_w2: jax.Array,
    B_w3: jax.Array,
    B_w4: jax.Array,
):
    b, sq, d = A_x.shape
    _, hkv, sk, dh = A_k_cache.shape
    assert (b, sq, d, hkv, dh) == (1, 1, D, H, DH)
    win = min(4096, max(256, sk // 4))
    assert win % 512 == 0 and sk % 128 == 0
    nj = win // 128

    kt = _tile_view(jnp.swapaxes(A_k_cache, 2, 3).reshape(H * DH, sk))
    vt = _head_view(jnp.swapaxes(A_v_cache, 2, 3).reshape(H * DH, sk))

    def buf(r, c):
        return pltpu.VMEM((r // 16, c // 128, 16, 128), BF16)

    def hbuf(c):
        return pltpu.VMEM((H, DH // 16, c // 128, 16, 128), BF16)

    bl = CFG["blocks"]
    ns = CFG.get("ns") or max(bl[i + 1][1] - bl[i][0] for i in range(len(bl) - 1))
    nm_max = max([1, CFG["nm"]] + list(CFG["nm_at"].values()))
    any_spec = pl.BlockSpec(memory_space=pl.ANY)
    out = pl.pallas_call(
        _make_kernel(sk, win, CFG),
        out_shape=jax.ShapeDtypeStruct((1, D), A_x.dtype),
        in_specs=[any_spec] * 7,
        out_specs=pl.BlockSpec(memory_space=pltpu.VMEM),
        scratch_shapes=[
            buf(H * DH, win), hbuf(win),
            pltpu.VMEM((H, DH // 16, max(len(CFG["jx"]), 1), 8, 128), F32),
            buf(D, H * DH), hbuf(D), buf(D, FF), buf(FF, D),
            pltpu.VMEM((1, D), BF16),
            pltpu.VMEM((8, D), F32),
            pltpu.VMEM((8, D), U32),
            pltpu.VMEM((1, D // 128, 8, 384), F32),
            pltpu.VMEM((1, D // 128, 8, 384), F32),
            pltpu.VMEM((1, D // 128, 8, 384), F32),
            pltpu.VMEM((8, 8, 384), U32),
            pltpu.VMEM((2, 8, win // 4), F32),
            pltpu.VMEM((2, 8, win // 4), F32),
            pltpu.VMEM((1, 8, win // 4), F32),
            pltpu.VMEM((1, 8, win // 4), F32),
            pltpu.VMEM((2, nm_max, 8, 128), U32),
            pltpu.VMEM((ns, nm_max, 3, 8, 128), F32),
            pltpu.VMEM((ns, 8, 128), F32),
            pltpu.VMEM((ns, 384, 128), F32),
            pltpu.VMEM((NU, 8, 384), U32),
            pltpu.VMEM((3, D // 128, NU, 128), F32),
            pltpu.SemaphoreType.DMA((5,)),
        ],
        compiler_params=pltpu.CompilerParams(vmem_limit_bytes=int(CFG["vmem_mb"] * 1024 * 1024)),
        name="interleave_decode",
    )(A_x.reshape(1, D), kt, vt, _tile_view(A_wq), _head_view(A_wo),
      _tile_view(B_w3), _tile_view(B_w4))
    return out.reshape(b, sq, d)
```

```python
import jax
import jax.numpy as jnp
from jax import lax
import jax.experimental.pallas as pl
import jax.experimental.pallas.tpu as pltpu

F32 = jnp.float32
BF16 = jnp.bfloat16
U32 = jnp.uint32

D = 640
H = 32
DH = 192
FF = 1536
NU = H // 2
UT = 2 * DH // 16
EPS = 1e-5
NPIECE = 12

NTOK = {}
CFG = dict(
    blocks=((0, 4), (4, 8), (8, 12), (12, 15), (15, 16)), ns=7,
    jsplit=8, js_at={},
    pvm_back=2, pvm_back0=0, pretr=1,
    nm=2, nm_at={0: 3, 1: 3, 2: 3, 3: 3, 14: 3, 15: 3},
    qproj_at={t: (t + 3,) for t in range(13)},
    oproj_at={4: ((0, (2,)),), 5: ((1, (2,)),), 6: ((2, (2,)),), 7: ((3, (2,)),),
              8: ((4, (2,)),), 9: ((5, (2,)),), 10: ((6, (2,)),), 11: ((7, (2,)),),
              12: ((8, (2,)),), 13: ((9, (2,)), (10, (2,)), (0, (0, 1))),
              14: ((11, (2,)), (1, (0, 1)), (2, (0, 1)), (3, (0, 1))),
              15: ((4, (0, 1)), (5, (0, 1)), (6, (0, 1)), (7, (0, 1)), (8, (0, 1)), (9, (0, 1)),
                   (10, (0, 1)), (11, (0, 1)), 12)},
    jx=(1, 5, 9, 13, 17, 21, 25), vmem_mb=128,
    tok={
        0: [-27,-24,-22,-20,-17,-15,-13,-11,-8,-6,-4,-1,1,3,6,8,10,13,16,19,21,24,27,30,33,35,38,41,44,47,49,52,55,58,61,63,66,69,72,75,77,80,83,86,88,91,94,97],
        1: [-21,-18,-16,-13,-11,-9,-6,-4,-2,1,3,5,8,10,12,15,17,19,22,25,27,30,32,35,37,40,42,45,48,50,53,55,58,60,63,65,68,71,73,76,78,81,83,86,88,91,94,96],
        2: [-21,-19,-16,-14,-11,-9,-6,-3,-1,2,4,7,9,12,14,17,20,22,25,27,30,32,35,37,40,43,45,48,50,53,55,58,60,63,66,68,71,73,76,78,81,83,86,89,91,94,96,99],
        3: [-19,-16,-14,-11,-8,-6,-3,-1,2,4,7,9,12,15,17,20,22,25,27,30,32,35,38,40,43,45,48,50,53,55,58,61,63,66,68,71,73,76,78,81,84,86,89,91,94,96,99,101],
        4: [-23,-21,-18,-16,-14,-12,-9,-7,-5,-3,0,2,4,6,8,11,13,16,19,21,24,27,30,33,36,38,41,44,47,50,53,55,58,61,64,67,70,72,75,78,81,84,87,89,92,95,98,101],
        5: [-24,-22,-19,-17,-14,-12,-9,-7,-4,-1,1,4,6,9,11,14,16,19,22,24,27,30,32,35,38,40,43,46,48,51,54,57,59,62,65,67,70,73,76,79,81,84,87,90,92,95,98,101],
        6: [-19,-16,-13,-11,-8,-5,-3,0,3,5,8,11,13,16,19,21,24,26,29,32,34,37,40,42,45,48,50,53,56,58,61,63,66,69,71,74,77,79,82,85,87,90,93,95,98,100,103,106],
        7: [-14,-11,-8,-6,-3,0,2,5,8,10,13,15,18,21,23,26,29,31,34,36,39,41,44,46,49,51,54,56,59,61,64,66,69,72,74,77,80,82,85,88,90,93,95,98,101,103,106,109],
        8: [-27,-25,-22,-20,-17,-15,-12,-10,-8,-5,-3,0,2,5,7,10,12,15,17,20,23,26,28,31,34,37,39,42,45,48,50,53,56,58,61,64,66,69,72,74,77,80,82,85,88,90,93,96],
        9: [-30,-27,-24,-22,-19,-17,-14,-11,-9,-6,-3,-1,2,5,7,10,13,15,18,20,23,26,28,31,34,36,39,41,44,47,49,52,54,57,60,62,65,68,70,73,75,78,81,83,86,89,91,94],
        10: [-26,-23,-20,-18,-15,-13,-10,-7,-5,-2,1,3,6,8,11,14,16,19,21,24,27,29,32,35,37,40,42,45,48,50,53,56,58,61,63,66,69,71,74,76,79,82,84,87,90,92,95,97],
        11: [-22,-19,-17,-14,-12,-9,-6,-4,-1,2,4,7,9,12,15,17,20,23,26,28,31,34,37,40,43,46,49,51,54,57,60,63,66,69,71,74,77,80,82,85,88,91,94,96,99,102,105,107],
        12: [-27,-25,-22,-20,-17,-15,-12,-10,-8,-5,-3,0,2,5,7,10,12,15,17,20,23,25,28,31,33,36,39,42,44,47,50,52,55,58,61,63,66,69,72,75,77,80,83,86,89,92,94,97],
        13: [-28,-25,-22,-20,-17,-14,-11,-8,-6,-3,0,3,6,9,11,14,17,20,22,25,27,30,33,35,38,41,43,46,48,51,54,56,59,62,65,67,70,73,76,79,81,84,87,90,93,96,98,101],
        14: [-21,-19,-16,-14,-11,-9,-6,-4,-2,1,3,6,8,11,13,16,18,21,23,26,28,31,34,36,39,42,44,47,49,52,55,57,60,63,65,68,70,73,76,78,81,84,86,89,91,94,97,99],
        15: [-33,-30,-26,-23,-20,-17,-14,-10,-7,-5,-2,1,3,6,9,11,14,17,19,22,24,27,30,32,35,38,40,43,46,48,51,53,56,60,63,66,70,73,77,80,84,86,89,91,94,97,99,102],
    },
    tok_lin=(24, 18),
    w4_cuts=(7, 11), layers=2)


def _tile_view(a):
    r, c = a.shape
    a = a.reshape(r // 16, 2, 8, c // 128, 128)
    return jnp.swapaxes(a, 2, 3)


def _head_view(a):
    c = a.shape[1]
    a = a.reshape(H, 2, DH // 16, 8, c // 128, 128)
    return jnp.swapaxes(a, 3, 4)


def _as_bf16(w32):
    n = w32.shape[0]
    return pltpu.bitcast(w32.reshape(n * 8, 128), BF16)


def _lhs(top, fill=0.0):
    return jnp.concatenate([top, jnp.full(top.shape, fill, F32)], axis=0).astype(BF16)


def _ln_stats(x):
    m = jnp.mean(x, axis=-1, keepdims=True)
    m2 = jnp.mean(x * x, axis=-1, keepdims=True)
    v = jnp.maximum(m2 - m * m, 0.0)
    return m, lax.rsqrt(v + EPS)


def _round_bf16(x):
    return x.astype(BF16).astype(F32)


def _dot(a, b):
    return jnp.dot(a, b, preferred_element_type=F32)


def _make_kernel(sk, win, cfg):
    nj = win // 128
    j0 = (sk - win) // 128
    jq = nj // 4
    jx = list(cfg["jx"])
    qscale = DH ** -0.5 * 1.4426950408889634

    def kernel(x_hbm, k_hbm, v_hbm, wq_hbm, wo_hbm, w3_hbm, w4_hbm, o_ref,
               kbuf, vbuf, vx, wqbuf, wobuf, w3buf, w4buf, xin,
               xs, ulhs, qp0, qp1, qp2, qlhs, sx, sy, pbuf0, pbuf1, plhs, mbuf, lpart, abuf, olhs, gp,
               sems):
        qp = (qp0, qp1, qp2)
        pbuf = (pbuf0, pbuf1)
        ns = abuf.shape[0]


        def cps_w(hbm, buf, sem, lo=0, n=None):
            n = buf.shape[0] if n is None else n
            return [pltpu.make_async_copy(
                hbm.at[pl.ds(lo, n), e],
                buf.at[pl.ds(lo, n), :, pl.ds(e * 8, 8), :],
                sems.at[sem]) for e in range(2)]

        def cps_kv(hbm, buf, sem, u):
            return [pltpu.make_async_copy(
                hbm.at[pl.ds(u * UT, UT), e, pl.ds(j0, nj)],
                buf.at[pl.ds(u * UT, UT), :, pl.ds(e * 8, 8), :],
                sems.at[sem]) for e in range(2)]

        def cps_v(u, par):
            return [pltpu.make_async_copy(
                v_hbm.at[pl.ds(2 * u, 2), e, :, pl.ds(j0, nj)],
                vbuf.at[pl.ds(2 * u, 2), :, :, pl.ds(e * 8, 8), :],
                sems.at[2 + par]) for e in range(2)]

        def cps_wo():
            return [pltpu.make_async_copy(
                wo_hbm.at[:, e], wobuf.at[:, :, :, pl.ds(e * 8, 8), :],
                sems.at[4]) for e in range(2)]

        cps_k = lambda u, par: cps_kv(k_hbm, kbuf, par, u)
        cps_x_wq = lambda: cps_w(wq_hbm, wqbuf, 4) + [pltpu.make_async_copy(x_hbm, xin, sems.at[4])]
        cps_w3 = lambda: cps_w(w3_hbm, w3buf, 0)
        w4_cuts = (0,) + tuple(cfg["w4_cuts"]) + (FF // 128,)
        cps_w4 = lambda i: cps_w(w4_hbm, w4buf, (1, 4, 2)[i], w4_cuts[i] * 8,
                                 (w4_cuts[i + 1] - w4_cuts[i]) * 8)

        def start(cps):
            for c in cps:
                c.start()

        def wait(cps):
            for c in cps:
                c.wait()

        start(cps_x_wq())
        start(cps_k(0, 0))
        start(cps_k(1, 1))
        start(cps_v(0, 0))
        start(cps_v(1, 1))

        k32 = kbuf.bitcast(U32)
        v32 = vbuf.bitcast(U32)
        wq32 = wqbuf.bitcast(U32)
        wo32 = wobuf.bitcast(U32)
        w332 = w3buf.bitcast(U32)
        w432 = w4buf.bitcast(U32)

        def js(u):
            return cfg["js_at"].get(u, cfg["jsplit"])

        def nmx(u):
            return cfg["nm_at"].get(u, cfg["nm"])

        def st_qproj(u, zdyn):
            lhs = pltpu.bitcast(ulhs[...], BF16)
            toks = []
            for kt in range(D // 128):
                for nt in range(3):
                    w = _as_bf16(wq32[pl.ds(kt * 8, 8), u * 3 + nt])
                    r = _dot(lhs[:, kt * 128:(kt + 1) * 128], w)
                    toks.append(r[8:16])
                    qp[u % 3][zdyn, kt, :, nt * 128:(nt + 1) * 128] = r[0:8]
            return toks

        def pack_q(q, u):
            q = q * qscale
            lane = lax.broadcasted_iota(jnp.int32, (8, 128), 1)
            sub = lax.broadcasted_iota(jnp.int32, (8, 128), 0)
            keep = (lane < DH - 128) == (sub % 2 == 0)
            q = jnp.concatenate(
                [q[:, 0:128], jnp.where(keep, q[:, 128:256], 0.0), q[:, 256:384]], axis=1)
            qlhs.at[u % 8][:, 0:384] = pltpu.bitcast(_lhs(q), U32)

        def st_qpack(u):
            q = qp[u % 3][0, 0]
            for kt in range(1, D // 128):
                q = q + qp[u % 3][0, kt]
            pack_q(q, u)

        def st_qk(u, js):
            sl = u % 2
            lhs = pltpu.bitcast(qlhs[u % 8], BF16)
            toks = []
            for j in js:
                ra = 2 * (j // jq)
                cs = slice((j % jq) * 128, (j % jq + 1) * 128)
                for t in range(3):
                    w = _as_bf16(k32[pl.ds(u * UT + t * 8, 8), j])
                    r = _dot(lhs[:, t * 128:(t + 1) * 128], w)
                    toks.append(r[8:16])
                    if t == 0:
                        sx[sl, ra:ra + 1, cs] = r[0:1]
                    elif t == 1:
                        sy[sl, ra:ra + 2, cs] = r[ra:ra + 2]
                    else:
                        sx[sl, ra + 1:ra + 2, cs] = r[0:1]
            return toks

        def st_softmax(u, zdyn):
            sl = u % 2
            s = sx[sl] + sy[sl]
            m = s[:, 0:128]
            for c in range(1, jq):
                m = jnp.maximum(m, s[:, c * 128:(c + 1) * 128])
            m = jnp.maximum(m, pltpu.roll(m, 2, 0))
            m = jnp.maximum(m, pltpu.roll(m, 4, 0))
            m = jnp.max(m, axis=1, keepdims=True)
            p = jnp.exp2(s - m)
            pbuf[sl][zdyn] = p
            for i in range(nmx(u)):
                c = jq - 1 - i
                plhs.at[sl, i][:, 0:128] = pltpu.bitcast(_lhs(p[:, c * 128:(c + 1) * 128]), U32)

        def inv_l(l):
            l = jnp.sum(l, axis=1, keepdims=True)
            r0 = pl.reciprocal(l, approx=True)
            return jnp.broadcast_to(r0 * (2.0 - l * r0), (8, 128))

        def st_lsum(u):
            l = pbuf[u % 2][0, :, 0:128]
            for c in range(1, jq):
                l = l + pbuf[u % 2][0, :, c * 128:(c + 1) * 128]
            l = l + pltpu.roll(l, 2, 0)
            l = l + pltpu.roll(l, 4, 0)
            lpart[u % ns] = inv_l(l) if u == NU - 1 else l

        def st_pvm(u):
            toks = []
            for i in range(nmx(u)):
                lhs = pltpu.bitcast(plhs[u % 2, i], BF16)
                j = nj - 1 - i
                for t in range(3):
                    if t == 1:
                        w32 = jnp.concatenate(
                            [v32[2 * u, 8:12, j], v32[2 * u + 1, 0:4, j]], axis=0)
                    else:
                        w32 = v32[2 * u + t // 2, 2 * t:2 * t + 8, j]
                    if cfg["pretr"]:
                        r = _dot(lhs, _as_bf16(w32))
                    else:
                        r = lax.dot_general(lhs, _as_bf16(w32), (((1,), (1,)), ((), ())),
                                            preferred_element_type=F32)
                    toks.append(r[8:16])
                    mbuf[u % ns, i, t] = r[0:8]
            return toks

        def st_expand(u):
            def body(i, c):
                hd, dt = i // 12, i % 12
                for ix, j in enumerate(jx):
                    w = v32[2 * u + hd, dt, j]
                    vx[2 * u + hd, dt, ix] = pltpu.bitcast(w << 16, F32)
                    vbuf[2 * u + hd, dt, j] = pltpu.bitcast(w & jnp.uint32(0xFFFF0000), BF16)
                return c
            if jx:
                lax.fori_loop(0, UT, body, 0)
            for i in range(nmx(u) if cfg["pretr"] else 0):
                j = nj - 1 - i
                for t in range(3):
                    idx = [divmod(t * 8 + v, 12) for v in range(8)]
                    blk = jnp.concatenate([vbuf[2 * u + hd, dt, j] for hd, dt in idx], axis=0)
                    blk = blk.astype(F32).T.astype(BF16)
                    for v, (hd, dt) in enumerate(idx):
                        vbuf[2 * u + hd, dt, j] = blk[v * 16:(v + 1) * 16]

        def st_pv(u, toks, tok_map):
            nm, sl = nmx(u), u % ns
            for piece in range(NPIECE):
                hd, half = divmod(piece, NPIECE // 2)
                sub = len(tok_map) // NPIECE
                lo = hi = None
                for j in range(nj - nm):
                    row = 2 * (j // jq) + hd
                    cs = slice((j % jq) * 128, (j % jq + 1) * 128)
                    pb = jnp.broadcast_to(pbuf[u % 2][0, row:row + 1, cs], (8, 128))
                    k = piece * sub + j * sub // nj
                    ti = tok_map[k] if j % (nj // sub) == 0 else -1
                    if j > 0 and tok_map[k - 1] == ti:
                        ti = -1
                    if toks and ti >= 0:
                        pb = pb + toks[min(ti, len(toks) - 1)]
                    w = v32[2 * u + hd, pl.ds(half * 2, 2), j]
                    if j in jx:
                        a = vx[2 * u + hd, pl.ds(half * 2, 2), jx.index(j)] * pb
                        b = pltpu.bitcast(w, F32) * pb
                    else:
                        a = pltpu.bitcast(w << 16, F32) * pb
                        b = pltpu.bitcast(w & jnp.uint32(0xFFFF0000), F32) * pb
                    lo = a if lo is None else lo + a
                    hi = b if hi is None else hi + b
                for i in range(2):
                    base = (piece * 2 + i) * 16
                    abuf[sl, pl.ds(base, 8, stride=2), :] = lo[i]
                    abuf[sl, pl.ds(base + 1, 8, stride=2), :] = hi[i]

        def st_ored(u, ts=(0, 1, 2), partial_rows=False):
            nm, sl = nmx(u), u % ns
            ia = lpart[sl] if u == NU - 1 else inv_l(lpart[sl])
            ib = pltpu.roll(ia, 1, 0)
            if partial_rows:
                even = lax.broadcasted_iota(jnp.int32, (8, 128), 0) % 2 == 0
                ia, ib = jnp.where(even, ia, ib), jnp.where(even, ib, ia)
            lane = lax.broadcasted_iota(jnp.int32, (8, 128), 1)
            for t in ts:
                at = abuf[sl, t * 128:(t + 1) * 128, :].T
                o = at[0:8]
                for i in range(1, 16):
                    o = o + at[i * 8:(i + 1) * 8]
                if nm:
                    om = mbuf[sl, 0, t]
                    for i in range(1, nm):
                        om = om + mbuf[sl, i, t]
                    sub = lax.broadcasted_iota(jnp.int32, (8, 128), 0)
                    row = (6, jnp.where(lane < DH - 128, 6, 7), 7)[t]
                    o = o + jnp.where(sub == row, om, 0.0)
                if not partial_rows:
                    o = o + pltpu.roll(o, 4, 0)
                    o = o + pltpu.roll(o, 2, 0)
                    o = o + pltpu.roll(o, 1, 0)
                o = o * (ia, jnp.where(lane < DH - 128, ia, ib), ib)[t]
                olhs.at[u][:, t * 128:(t + 1) * 128] = pltpu.bitcast(_lhs(o), U32)

        def st_oproj(u, ts=(0, 1, 2), out=None):
            lhs = pltpu.bitcast(olhs[u], BF16)
            toks = []
            for t in ts:
                for n in range(D // 128):
                    if t == 1:
                        w32 = jnp.concatenate(
                            [wo32[2 * u, 8:12, n], wo32[2 * u + 1, 0:4, n]], axis=0)
                    else:
                        w32 = wo32[2 * u + t // 2, 2 * t:2 * t + 8, n]
                    r = _dot(lhs[:, t * 128:(t + 1) * 128], _as_bf16(w32))
                    toks.append(r[8:16])
                    if out is None:
                        gp[t, n, pl.ds(u, 1), :] = r[0:1]
                    else:
                        out[n].append(r[0:8])
            return toks

        def mlp(first, extra):
            g = gp[0] + gp[1] + gp[2]
            sub = lax.broadcasted_iota(jnp.int32, (D // 128, 8, 128), 1)
            g = g[:, 0:8] + jnp.where(sub < 7, g[:, 8:16], 0.0)
            g = jnp.concatenate([g[n] + extra[n][0] + extra[n][1] + extra[n][2]
                                 for n in range(D // 128)], axis=1)
            g = g + pltpu.roll(g, 4, 0)
            g = g + pltpu.roll(g, 2, 0)
            g = g + pltpu.roll(g, 1, 0)
            x1 = _round_bf16(xs[...] + g)
            lhs = _lhs(x1, 1.0)
            m1, r1 = _ln_stats(x1)
            y = (x1 - m1) * r1
            m2, r2 = _ln_stats(y)
            a = r1 * r2
            b = (m1 * r1 + m2) * r2
            hl = []
            for n in range(FF // 128):
                r = _dot(lhs, _as_bf16(w332[:, n]))
                hl.append(_lhs(jax.nn.gelu(r[0:8] * a - r[8:16] * b, approximate=True)))
            acc = x1 + y
            acc = [acc[:, c * 128:(c + 1) * 128] for c in range(D // 128)]
            for kt in range(FF // 128):
                if first and kt in w4_cuts:
                    wait(cps_w4(w4_cuts.index(kt)))
                for c in range(D // 128):
                    w = _as_bf16(w432[pl.ds(kt * 8, 8), c])
                    acc[c] = acc[c] + _dot(hl[kt], w)[0:8]
            xs[...] = _round_bf16(jnp.concatenate(acc, axis=1))

        wait(cps_x_wq())
        start(cps_wo())
        wait(cps_k(0, 0))
        start(cps_k(2, 0))
        wait(cps_k(1, 1))
        wait(cps_v(0, 0))
        xs[...] = jnp.broadcast_to(xin[...].astype(F32), (8, D))

        def layer(li, carry):
            first = li == 0
            n_first = jnp.maximum(1 - li, 0)
            zdyn = li >> 4

            def block_dma(ua, ub):
                def last_wait(t):
                    wait(cps_v(t + 1, (t + 1) % 2) if t + 1 < NU else cps_w3())

                def dma_ops(_, c):
                    for t in range(ua, ub):
                        if t + 3 < NU:
                            start(cps_k(t + 3, (t + 3) % 2))
                        if t + 2 < NU:
                            start(cps_v(t + 2, t % 2))
                        if t == NU - 2:
                            start(cps_w3())
                            for i in range(len(w4_cuts) - 1):
                                start(cps_w4(i))
                        if t == 1:
                            wait(cps_wo())
                        if cfg.get("only") is None:
                            st_expand(t)
                        if t + 2 < NU:
                            wait(cps_k(t + 2, t % 2))
                        if t < ub - 1:
                            last_wait(t)
                    return c

                lax.fori_loop(0, n_first, dma_ops, 0)
                pl.when(first)(lambda: last_wait(ub - 1))

            def prologue():
                x = xs[...]
                m, r = _ln_stats(x)
                lhs = _lhs(x, 1.0)

                def q_direct(u):
                    qs = []
                    for nt in range(3):
                        qq = _dot(lhs, _as_bf16(wq32[:, u * 3 + nt]))
                        qs.append((qq[0:8] - qq[8:16] * m) * r)
                    pack_q(jnp.concatenate(qs, axis=1), u)

                q_direct(0)
                q_direct(1)
                ulhs[...] = pltpu.bitcast(_lhs((x - m) * r), U32)
                toks = st_qk(0, range(nj))
                st_softmax(0, zdyn)
                q_direct(2)
                pos = js(1) - cfg["pvm_back0"]
                toks += st_qk(1, range(pos))
                toks += st_pvm(0)
                toks += st_qk(1, range(pos, js(1)))
                return toks

            def block(bi):
                ua, ub = cfg["blocks"][bi]
                block_dma(ua, ub)
                toks = []
                if bi > 0:
                    for u in range(*cfg["blocks"][bi - 1]):
                        st_ored(u)
                else:
                    toks += prologue()
                for t in range(ua, ub):
                    base = len(toks)
                    if t == ua and bi > 0:
                        toks += st_pvm(t)
                    if t + 1 < NU:
                        toks += st_qk(t + 1, range(js(t + 1), nj))
                        st_softmax(t + 1, zdyn)
                    for u in cfg["qproj_at"].get(t, ()):
                        toks += st_qproj(u, zdyn)
                    for u in cfg["oproj_at"].get(t, ()):
                        toks += st_oproj(*u) if isinstance(u, tuple) else st_oproj(u)
                    pos = max(js(t + 2) - cfg["pvm_back"], 0)
                    if t + 2 < NU:
                        toks += st_qk(t + 2, range(pos))
                    if t + 1 < ub:
                        toks += st_pvm(t + 1)
                    if t + 2 < NU:
                        toks += st_qk(t + 2, range(pos, js(t + 2)))
                    tok_map = cfg["tok"].get(t)
                    if tok_map is None:
                        n = len(toks) - base
                        if t == ub - 1:
                            n += cfg["tok_lin"][1]
                        tok_map = [k * n // (4 * NPIECE) - cfg["tok_lin"][0]
                                   for k in range(4 * NPIECE)]
                    NTOK[t] = len(toks) - base
                    st_pv(t, toks, [base + i for i in tok_map])
                    st_lsum(t)
                    for u in cfg["qproj_at"].get(t, ()):
                        st_qpack(u)

            if cfg.get("only") is not None:
                for bi in cfg["only"]:
                    block(bi)
                lax.fori_loop(0, n_first, lambda i, c: c + 1, 0)
                pl.when(first)(lambda: wait(cps_w4(0)))
                f = lambda v: pltpu.bitcast(v, F32)
                z8 = pl.multiple_of(zdyn * 8, 8)
                z128 = pl.multiple_of(zdyn * 128, 128)
                xs[:, 0:128] = (abuf[zdyn, pl.ds(z8, 8), :] + lpart[zdyn] + mbuf[zdyn, zdyn, zdyn]
                                + f(olhs[zdyn, :, pl.ds(z128, 128)]) + f(qlhs[zdyn, :, pl.ds(z128, 128)])
                                + sx[zdyn, :, pl.ds(z128, 128)] + sy[zdyn, :, pl.ds(z128, 128)]
                                + pbuf0[zdyn, :, pl.ds(z128, 128)] + pbuf1[zdyn, :, pl.ds(z128, 128)]
                                + gp[zdyn, zdyn, pl.ds(z8, 8), :] + f(plhs[zdyn, zdyn]))
                return carry

            for bi in range(len(cfg["blocks"])):
                block(bi)

            def tail(first_static):
                for u in range(*cfg["blocks"][-1]):
                    st_ored(u, partial_rows=(u == NU - 1))
                seen = set()
                for us in cfg["oproj_at"].values():
                    for u in us:
                        uu, ts = u if isinstance(u, tuple) else (u, (0, 1, 2))
                        seen |= {(uu, t) for t in ts}
                for u in range(NU - 1):
                    ts = tuple(t for t in range(3) if (u, t) not in seen)
                    if ts:
                        st_oproj(u, ts)
                extra = [[] for _ in range(D // 128)]
                st_oproj(NU - 1, out=extra)
                mlp(first_static, extra)

            pl.when(first)(lambda: tail(True))
            pl.when(jnp.logical_not(first))(lambda: tail(False))
            return carry

        lax.fori_loop(0, cfg["layers"], layer, 0)
        o_ref[...] = xs[0:1, :].astype(o_ref.dtype)

    return kernel


@jax.jit
def pallas_interleave_layers__sliding_block_cached__mixer_s_mlp__decode_kernel(
    A_x: jax.Array,
    A_k_cache: jax.Array,
    A_v_cache: jax.Array,
    A_wq: jax.Array,
    A_wo: jax.Array,
    B_x: jax.Array,
    B_w1: jax.Array,
    B_w2: jax.Array,
    B_w3: jax.Array,
    B_w4: jax.Array,
):
    b, sq, d = A_x.shape
    _, hkv, sk, dh = A_k_cache.shape
    assert (b, sq, d, hkv, dh) == (1, 1, D, H, DH)
    win = min(4096, max(256, sk // 4))
    assert win % 512 == 0 and sk % 128 == 0
    nj = win // 128

    kt = _tile_view(jnp.swapaxes(A_k_cache, 2, 3).reshape(H * DH, sk))
    vt = _head_view(jnp.swapaxes(A_v_cache, 2, 3).reshape(H * DH, sk))

    def buf(r, c):
        return pltpu.VMEM((r // 16, c // 128, 16, 128), BF16)

    def hbuf(c):
        return pltpu.VMEM((H, DH // 16, c // 128, 16, 128), BF16)

    bl = CFG["blocks"]
    ns = CFG.get("ns") or max(bl[i + 1][1] - bl[i][0] for i in range(len(bl) - 1))
    nm_max = max([1, CFG["nm"]] + list(CFG["nm_at"].values()))
    any_spec = pl.BlockSpec(memory_space=pl.ANY)
    out = pl.pallas_call(
        _make_kernel(sk, win, CFG),
        out_shape=jax.ShapeDtypeStruct((1, D), A_x.dtype),
        in_specs=[any_spec] * 7,
        out_specs=pl.BlockSpec(memory_space=pltpu.VMEM),
        scratch_shapes=[
            buf(H * DH, win), hbuf(win),
            pltpu.VMEM((H, DH // 16, max(len(CFG["jx"]), 1), 8, 128), F32),
            buf(D, H * DH), hbuf(D), buf(D, FF), buf(FF, D),
            pltpu.VMEM((1, D), BF16),
            pltpu.VMEM((8, D), F32),
            pltpu.VMEM((8, D), U32),
            pltpu.VMEM((1, D // 128, 8, 384), F32),
            pltpu.VMEM((1, D // 128, 8, 384), F32),
            pltpu.VMEM((1, D // 128, 8, 384), F32),
            pltpu.VMEM((8, 8, 384), U32),
            pltpu.VMEM((2, 8, win // 4), F32),
            pltpu.VMEM((2, 8, win // 4), F32),
            pltpu.VMEM((1, 8, win // 4), F32),
            pltpu.VMEM((1, 8, win // 4), F32),
            pltpu.VMEM((2, nm_max, 8, 128), U32),
            pltpu.VMEM((ns, nm_max, 3, 8, 128), F32),
            pltpu.VMEM((ns, 8, 128), F32),
            pltpu.VMEM((ns, 384, 128), F32),
            pltpu.VMEM((NU, 8, 384), U32),
            pltpu.VMEM((3, D // 128, NU, 128), F32),
            pltpu.SemaphoreType.DMA((5,)),
        ],
        compiler_params=pltpu.CompilerParams(vmem_limit_bytes=int(CFG["vmem_mb"] * 1024 * 1024)),
        name="interleave_decode",
    )(A_x.reshape(1, D), kt, vt, _tile_view(A_wq), _head_view(A_wo),
      _tile_view(B_w3), _tile_view(B_w4))
    return out.reshape(b, sq, d)
```

```python
import jax
import jax.numpy as jnp
from jax import lax
import jax.experimental.pallas as pl
import jax.experimental.pallas.tpu as pltpu

F32 = jnp.float32
BF16 = jnp.bfloat16
U32 = jnp.uint32

D = 640
H = 32
DH = 192
FF = 1536
NU = H // 2
UT = 2 * DH // 16
EPS = 1e-5
NPIECE = 12

NTOK = {}
CFG = dict(
    blocks=((0, 4), (4, 8), (8, 12), (12, 15), (15, 16)), ns=7,
    jsplit=8, js_at={},
    gap=40, gap_at={0: 44, 1: 44, 2: 44}, pvm_back0=0, pretr=1,
    nm=3, nm_at={0: 2, 4: 2},
    va_units=(6, 7, 8, 9), va_force=(7, 16), va_tok=(10, 100),
    qproj_at={0: (3,), 1: (4,), 2: (5,), 3: (10,), 5: (11,), 6: (12,), 7: (13,), 10: (14,), 11: (15,)},
    ored_at={4: (0,), 5: (1,), 6: (2,), 7: (3,), 8: (4,), 9: (5,), 10: (6,), 11: (7,),
             12: (8,), 13: (9, 10), 14: (11,), 15: (12, 13, 14)},
    oproj_at={4: ((0, (2,)),), 5: ((1, (2,)),), 6: ((2, (2,)),), 7: ((3, (2,)),),
              8: ((4, (2,)), (0, (0,))), 9: ((5, (2,)), (0, (1,))), 10: ((6, (2,)),), 11: ((7, (2,)),),
              12: ((8, (2,)),), 13: ((9, (2,)), (10, (2,)), (4, (0, 1))),
              14: ((11, (2,)), (1, (0, 1)), (2, (0, 1)), (3, (0, 1))),
              15: ((5, (0, 1)), (6, (0, 1)), (7, (0, 1)), (8, (0, 1)), (9, (0, 1)),
                   (10, (0, 1)), (11, (0, 1)), 12, (13, (0, 1)))},
    jx=(1, 5, 9, 13, 17, 21, 25), vmem_mb=128,
    tok={
        0: [-22,-20,-18,-15,-13,-10,-8,-5,-3,-1,2,4,7,9,12,14,16,19,22,24,27,30,32,35,37,40,43,45,48,50,53,56,58,61,64,67,69,72,75,78,80,83,86,89,91,94,97,99],
        1: [-24,-21,-19,-17,-14,-12,-9,-7,-5,-2,0,3,5,7,10,12,15,17,20,22,25,28,30,33,35,38,40,43,46,48,51,53,56,59,61,64,67,69,72,75,77,80,83,85,88,91,93,96],
        2: [-21,-19,-16,-14,-12,-9,-7,-4,-2,0,3,5,8,10,12,15,17,20,22,25,28,30,33,36,38,41,43,46,49,51,54,56,59,62,64,67,69,72,74,77,79,82,84,86,89,91,94,96],
        3: [-21,-19,-16,-14,-11,-9,-6,-4,-1,1,4,6,8,11,13,16,18,21,24,26,29,32,34,37,40,42,45,47,50,53,55,58,61,63,65,68,70,72,75,77,79,82,84,86,89,91,93,96],
        4: [-25,-22,-20,-18,-15,-13,-11,-8,-6,-4,-1,1,3,5,8,10,12,15,18,21,24,26,29,32,35,38,40,43,46,49,52,55,57,60,63,66,69,72,75,77,80,83,86,89,92,95,98,100],
        5: [-19,-16,-14,-11,-9,-6,-4,-1,1,3,6,8,11,13,16,18,21,24,26,29,32,35,38,41,43,46,49,52,55,58,60,63,66,69,71,73,76,78,81,83,86,88,90,93,95,98,100,103],
        6: [-11,-8,-6,-3,0,2,5,7,10,13,15,18,21,23,26,28,31,34,36,39,42,44,47,49,52,55,57,60,63,65,68,70,73,76,78,81,83,86,89,91,94,97,99,102,104,107,110,112],
        7: [-10,-8,-5,-3,0,2,5,7,10,12,15,17,20,22,25,27,30,33,35,38,41,44,46,49,52,55,57,60,63,66,68,71,74,76,79,82,84,87,90,92,95,97,100,103,105,108,111,113],
        8: [-24,-21,-19,-17,-14,-12,-10,-7,-5,-2,1,3,6,9,12,15,17,20,23,25,28,30,33,35,38,40,43,45,48,50,53,55,57,60,63,66,69,72,74,77,80,83,86,89,92,94,97,100],
        9: [-18,-16,-13,-11,-9,-6,-4,-2,1,3,5,8,10,12,15,17,19,22,25,28,30,33,36,39,41,44,47,50,53,56,59,62,65,67,70,72,75,77,80,82,85,87,90,92,95,97,100,102],
        10: [-19,-17,-14,-12,-9,-6,-4,-1,1,4,7,9,12,14,17,20,22,25,27,30,32,35,37,40,42,45,48,51,54,56,59,62,65,67,70,73,76,78,81,84,87,89,92,95,98,100,103,106],
        11: [-7,-5,-3,-1,2,4,6,8,11,13,16,19,21,24,27,29,32,34,37,40,42,45,47,50,53,55,58,60,63,66,68,71,73,76,79,81,84,87,90,92,95,98,100,103,105,108,111,113],
        12: [-32,-28,-25,-21,-18,-14,-11,-8,-4,-2,-1,1,3,4,6,8,9,12,16,19,22,25,28,32,35,38,40,43,46,48,51,54,56,59,61,64,67,69,72,74,77,80,82,85,87,90,92,95],
        13: [-24,-22,-19,-17,-14,-11,-9,-6,-4,-1,2,4,7,9,12,15,17,20,23,25,28,31,33,36,39,42,45,48,50,53,56,59,62,65,67,70,72,75,77,80,82,85,87,89,92,94,96,99],
        14: [-18,-15,-13,-11,-8,-6,-4,-1,1,4,7,10,13,16,20,23,26,28,30,33,35,37,40,42,44,47,50,53,55,58,61,64,67,69,72,74,77,79,82,84,87,89,92,94,97,99,102,104],
        15: [-44,-41,-37,-34,-30,-27,-24,-20,-17,-14,-11,-7,-4,-1,2,5,8,11,14,18,21,24,27,31,34,36,38,41,43,45,47,49,52,56,59,63,67,71,75,79,83,83,84,84,85,85,86,86],
    },
    tok_lin=(24, 18),
    w4_cuts=(7, 11), layers=2)


def _tile_view(a):
    r, c = a.shape
    a = a.reshape(r // 16, 2, 8, c // 128, 128)
    return jnp.swapaxes(a, 2, 3)


def _head_view(a):
    c = a.shape[1]
    a = a.reshape(H, 2, DH // 16, 8, c // 128, 128)
    return jnp.swapaxes(a, 3, 4)


def _as_bf16(w32):
    n = w32.shape[0]
    return pltpu.bitcast(w32.reshape(n * 8, 128), BF16)


def _lhs(top, fill=0.0):
    return jnp.concatenate([top, jnp.full(top.shape, fill, F32)], axis=0).astype(BF16)


def _ln_stats(x):
    m = jnp.mean(x, axis=-1, keepdims=True)
    m2 = jnp.mean(x * x, axis=-1, keepdims=True)
    v = jnp.maximum(m2 - m * m, 0.0)
    return m, lax.rsqrt(v + EPS)


def _round_bf16(x):
    return x.astype(BF16).astype(F32)


def _dot(a, b):
    return jnp.dot(a, b, preferred_element_type=F32)


def _make_kernel(sk, win, cfg):
    nj = win // 128
    j0 = (sk - win) // 128
    jq = nj // 4
    jx = list(cfg["jx"])
    qscale = DH ** -0.5 * 1.4426950408889634

    def kernel(x_hbm, k_hbm, v_hbm, wq_hbm, wo_hbm, w3_hbm, w4_hbm, o_ref,
               kbuf, vbuf, vx, wqbuf, wobuf, w3buf, w4buf, xin,
               xs, ulhs, qp0, qp1, qlhs, ucol0, ucol1, sx, sy, pbuf0, pbuf1, plhs, mbuf, lpart, abuf, olhs, gp,
               sems):
        qp = (qp0, qp1)
        ucol = (ucol0, ucol1)
        pbuf = (pbuf0, pbuf1)
        ns = abuf.shape[0]


        def cps_w(hbm, buf, sem, lo=0, n=None):
            n = buf.shape[0] if n is None else n
            return [pltpu.make_async_copy(
                hbm.at[pl.ds(lo, n), e],
                buf.at[pl.ds(lo, n), :, pl.ds(e * 8, 8), :],
                sems.at[sem]) for e in range(2)]

        def cps_kv(hbm, buf, sem, u):
            return [pltpu.make_async_copy(
                hbm.at[pl.ds(u * UT, UT), e, pl.ds(j0, nj)],
                buf.at[pl.ds(u * UT, UT), :, pl.ds(e * 8, 8), :],
                sems.at[sem]) for e in range(2)]

        def cps_v(u, par):
            return [pltpu.make_async_copy(
                v_hbm.at[pl.ds(2 * u, 2), e, :, pl.ds(j0, nj)],
                vbuf.at[pl.ds(2 * u, 2), :, :, pl.ds(e * 8, 8), :],
                sems.at[2 + par]) for e in range(2)]

        def cps_wo():
            return [pltpu.make_async_copy(
                wo_hbm.at[:, e], wobuf.at[:, :, :, pl.ds(e * 8, 8), :],
                sems.at[4]) for e in range(2)]

        cps_k = lambda u, par: cps_kv(k_hbm, kbuf, par, u)
        cps_x_wq = lambda: cps_w(wq_hbm, wqbuf, 4) + [pltpu.make_async_copy(x_hbm, xin, sems.at[4])]
        cps_w3 = lambda: cps_w(w3_hbm, w3buf, 0)
        w4_cuts = (0,) + tuple(cfg["w4_cuts"]) + (FF // 128,)
        cps_w4 = lambda i: cps_w(w4_hbm, w4buf, (1, 4, 2)[i], w4_cuts[i] * 8,
                                 (w4_cuts[i + 1] - w4_cuts[i]) * 8)

        def start(cps):
            for c in cps:
                c.start()

        def wait(cps):
            for c in cps:
                c.wait()

        start(cps_x_wq())
        start(cps_k(0, 0))
        start(cps_k(1, 1))
        start(cps_v(0, 0))
        start(cps_v(1, 1))

        k32 = kbuf.bitcast(U32)
        v32 = vbuf.bitcast(U32)
        wq32 = wqbuf.bitcast(U32)
        wo32 = wobuf.bitcast(U32)
        w332 = w3buf.bitcast(U32)
        w432 = w4buf.bitcast(U32)

        def js(u):
            return cfg["js_at"].get(u, cfg["jsplit"])

        def qslot(u):
            va = cfg["va_units"]
            return 4 + va.index(u) if u in va else u % 4

        def jms(u):
            return [nj - 1 - jq * i for i in range(nmx(u))]

        def nmx(u):
            return cfg["nm_at"].get(u, cfg["nm"])

        def st_qproj(u, zdyn):
            lhs = pltpu.bitcast(ulhs[...], BF16)
            toks = []
            for kt in range(D // 128):
                for nt in range(3):
                    w = _as_bf16(wq32[pl.ds(kt * 8, 8), u * 3 + nt])
                    r = _dot(lhs[:, kt * 128:(kt + 1) * 128], w)
                    toks.append(r[8:16])
                    qp[u % 2][zdyn, kt, :, nt * 128:(nt + 1) * 128] = r[0:8]
            return toks

        def pack_q(q, u):
            q = q * qscale
            lane = lax.broadcasted_iota(jnp.int32, (8, 128), 1)
            sub = lax.broadcasted_iota(jnp.int32, (8, 128), 0)
            keep = (lane < DH - 128) == (sub % 2 == 0)
            q = jnp.concatenate(
                [q[:, 0:128], jnp.where(keep, q[:, 128:256], 0.0), q[:, 256:384]], axis=1)
            qlhs.at[qslot(u)][:, 0:384] = pltpu.bitcast(_lhs(q), U32)

        def st_qpack(u):
            q = qp[u % 2][0, 0]
            for kt in range(1, D // 128):
                q = q + qp[u % 2][0, kt]
            pack_q(q, u)

        def st_qk(u, js):
            sl = u % 2
            lhs = pltpu.bitcast(qlhs[qslot(u)], BF16)
            toks = []
            for j in js:
                ra = 2 * (j // jq)
                cs = slice((j % jq) * 128, (j % jq + 1) * 128)
                for t in range(3):
                    w = _as_bf16(k32[pl.ds(u * UT + t * 8, 8), j])
                    r = _dot(lhs[:, t * 128:(t + 1) * 128], w)
                    toks.append(r[8:16])
                    if t == 0:
                        sx[sl, ra:ra + 1, cs] = r[0:1]
                    elif t == 1:
                        sy[sl, ra:ra + 2, cs] = r[ra:ra + 2]
                    else:
                        sx[sl, ra + 1:ra + 2, cs] = r[0:1]
            return toks

        def st_softmax(u, zdyn):
            sl = u % 2
            s = sx[sl] + sy[sl]
            m = s
            while m.shape[1] > 128:
                h = m.shape[1] // 2
                m = jnp.maximum(m[:, :h], m[:, h:])
            m = jnp.maximum(m, pltpu.roll(m, 2, 0))
            m = jnp.maximum(m, pltpu.roll(m, 4, 0))
            m = jnp.max(m, axis=1, keepdims=True)
            p = jnp.exp2(s - m)
            pbuf[sl][zdyn] = p
            if nmx(u):
                plhs[:, sl * 128:(sl + 1) * 128] = pltpu.bitcast(_lhs(p[:, (jq - 1) * 128:jq * 128]), U32)

        def inv_l(l):
            l = jnp.sum(l, axis=1, keepdims=True)
            r0 = pl.reciprocal(l, approx=True)
            return jnp.broadcast_to(r0 * (2.0 - l * r0), (8, 128))

        def st_lsum(u):
            l = pbuf[u % 2][0, :, 0:128]
            for c in range(1, jq):
                l = l + pbuf[u % 2][0, :, c * 128:(c + 1) * 128]
            l = l + pltpu.roll(l, 2, 0)
            l = l + pltpu.roll(l, 4, 0)
            lpart[u % ns] = inv_l(l) if u == NU - 1 else l

        def st_pvm(u):
            toks = []
            for j in jms(u):
                lhs = pltpu.bitcast(plhs[:, u % 2 * 128:(u % 2 + 1) * 128], BF16)
                ra = 2 * (j // jq)
                for t in range(3):
                    if t == 1:
                        w32 = jnp.concatenate(
                            [v32[2 * u, 8:12, j], v32[2 * u + 1, 0:4, j]], axis=0)
                    else:
                        w32 = v32[2 * u + t // 2, 2 * t:2 * t + 8, j]
                    if cfg["pretr"]:
                        r = _dot(lhs, _as_bf16(w32))
                    else:
                        r = lax.dot_general(lhs, _as_bf16(w32), (((1,), (1,)), ((), ())),
                                            preferred_element_type=F32)
                    toks.append(r[8:16])
                    mbuf[u % ns, t, ra:ra + 2, :] = r[ra:ra + 2]
            return toks

        def st_expand(u):
            def body(i, c):
                hd, dt = i // 12, i % 12
                for ix, j in enumerate(jx):
                    w = v32[2 * u + hd, dt, j]
                    vx[2 * u + hd, dt, ix] = pltpu.bitcast(w << 16, F32)
                    vbuf[2 * u + hd, dt, j] = pltpu.bitcast(w & jnp.uint32(0xFFFF0000), BF16)
                return c
            if jx:
                lax.fori_loop(0, UT, body, 0)
            for j in (jms(u) if cfg["pretr"] else ()):
                for t in range(3):
                    idx = [divmod(t * 8 + v, 12) for v in range(8)]
                    blk = jnp.concatenate([vbuf[2 * u + hd, dt, j] for hd, dt in idx], axis=0)
                    blk = blk.astype(F32).T.astype(BF16)
                    for v, (hd, dt) in enumerate(idx):
                        vbuf[2 * u + hd, dt, j] = blk[v * 16:(v + 1) * 16]

        def st_pv(u, toks, tok_map):
            nm, sl = nmx(u), u % ns
            for piece in range(NPIECE):
                hd, half = divmod(piece, NPIECE // 2)
                sub = len(tok_map) // NPIECE
                lo = hi = None
                for j in range(nj):
                    if j in jms(u):
                        continue
                    row = 2 * (j // jq) + hd
                    cs = slice((j % jq) * 128, (j % jq + 1) * 128)
                    pb = jnp.broadcast_to(pbuf[u % 2][0, row:row + 1, cs], (8, 128))
                    k = piece * sub + j * sub // nj
                    ti = tok_map[k] if j % (nj // sub) == 0 else -1
                    if j > 0 and tok_map[k - 1] == ti:
                        ti = -1
                    if toks and ti >= 0:
                        pb = pb + toks[min(ti, len(toks) - 1)]
                    w = v32[2 * u + hd, pl.ds(half * 2, 2), j]
                    if j in jx:
                        a = vx[2 * u + hd, pl.ds(half * 2, 2), jx.index(j)] * pb
                        b = pltpu.bitcast(w, F32) * pb
                    else:
                        a = pltpu.bitcast(w << 16, F32) * pb
                        b = pltpu.bitcast(w & jnp.uint32(0xFFFF0000), F32) * pb
                    lo = a if lo is None else lo + a
                    hi = b if hi is None else hi + b
                for i in range(2):
                    base = (piece * 2 + i) * 16
                    abuf[sl, pl.ds(base, 8, stride=2), :] = lo[i]
                    abuf[sl, pl.ds(base + 1, 8, stride=2), :] = hi[i]

        def st_ored(u, ts=(0, 1, 2), partial_rows=False):
            nm, sl = nmx(u), u % ns
            ia = lpart[sl] if u == NU - 1 else inv_l(lpart[sl])
            ib = pltpu.roll(ia, 1, 0)
            if partial_rows:
                even = lax.broadcasted_iota(jnp.int32, (8, 128), 0) % 2 == 0
                ia, ib = jnp.where(even, ia, ib), jnp.where(even, ib, ia)
            lane = lax.broadcasted_iota(jnp.int32, (8, 128), 1)
            for t in ts:
                at = abuf[sl, t * 128:(t + 1) * 128, :].T
                o = at[0:8]
                for i in range(1, 16):
                    o = o + at[i * 8:(i + 1) * 8]
                if nm:
                    sub = lax.broadcasted_iota(jnp.int32, (8, 128), 0)
                    odd = (0, (lane >= DH - 128).astype(jnp.int32), 1)[t]
                    keep = (sub >= 8 - 2 * nm) & (sub % 2 == odd)
                    o = o + jnp.where(keep, mbuf[sl, t], 0.0)
                if not partial_rows:
                    o = o + pltpu.roll(o, 4, 0)
                    o = o + pltpu.roll(o, 2, 0)
                    o = o + pltpu.roll(o, 1, 0)
                o = o * (ia, jnp.where(lane < DH - 128, ia, ib), ib)[t]
                olhs.at[u][:, t * 128:(t + 1) * 128] = pltpu.bitcast(_lhs(o), U32)

        def st_oproj(u, ts=(0, 1, 2), out=None):
            lhs = pltpu.bitcast(olhs[u], BF16)
            toks = []
            for t in ts:
                for n in range(D // 128):
                    if t == 1:
                        w32 = jnp.concatenate(
                            [wo32[2 * u, 8:12, n], wo32[2 * u + 1, 0:4, n]], axis=0)
                    else:
                        w32 = wo32[2 * u + t // 2, 2 * t:2 * t + 8, n]
                    r = _dot(lhs[:, t * 128:(t + 1) * 128], _as_bf16(w32))
                    toks.append(r[8:16])
                    if out is None:
                        gp[t, n, pl.ds(u, 1), :] = r[0:1]
                    else:
                        out[n].append(r[0:8])
            return toks

        def mlp(first, extra):
            g = gp[0] + gp[1] + gp[2]
            sub = lax.broadcasted_iota(jnp.int32, (D // 128, 8, 128), 1)
            g = g[:, 0:8] + jnp.where(sub < 7, g[:, 8:16], 0.0)
            g = jnp.concatenate([g[n] + extra[n][0] + extra[n][1] + extra[n][2]
                                 for n in range(D // 128)], axis=1)
            g = g + pltpu.roll(g, 4, 0)
            g = g + pltpu.roll(g, 2, 0)
            g = g + pltpu.roll(g, 1, 0)
            x1 = _round_bf16(xs[...] + g)
            lhs = _lhs(x1, 1.0)
            m1, r1 = _ln_stats(x1)
            y = (x1 - m1) * r1
            m2, r2 = _ln_stats(y)
            a = r1 * r2
            b = (m1 * r1 + m2) * r2
            hl = []
            for n in range(FF // 128):
                r = _dot(lhs, _as_bf16(w332[:, n]))
                hl.append(_lhs(jax.nn.gelu(r[0:8] * a - r[8:16] * b, approximate=True)))
            acc = x1 + y
            acc = [acc[:, c * 128:(c + 1) * 128] for c in range(D // 128)]
            for kt in range(FF // 128):
                if first and kt in w4_cuts:
                    wait(cps_w4(w4_cuts.index(kt)))
                for c in range(D // 128):
                    w = _as_bf16(w432[pl.ds(kt * 8, 8), c])
                    acc[c] = acc[c] + _dot(hl[kt], w)[0:8]
            xs[...] = _round_bf16(jnp.concatenate(acc, axis=1))

        wait(cps_x_wq())
        start(cps_wo())
        wait(cps_k(0, 0))
        start(cps_k(2, 0))
        wait(cps_k(1, 1))
        wait(cps_v(0, 0))
        xs[...] = jnp.broadcast_to(xin[...].astype(F32), (8, D))

        def layer(li, carry):
            first = li == 0
            n_first = jnp.maximum(1 - li, 0)
            zdyn = li >> 4

            def block_dma(ua, ub):
                def last_wait(t):
                    wait(cps_v(t + 1, (t + 1) % 2) if t + 1 < NU else cps_w3())

                def dma_ops(_, c):
                    for t in range(ua, ub):
                        if t + 3 < NU:
                            start(cps_k(t + 3, (t + 3) % 2))
                        if t + 2 < NU:
                            start(cps_v(t + 2, t % 2))
                        if t == NU - 2:
                            start(cps_w3())
                            for i in range(len(w4_cuts) - 1):
                                start(cps_w4(i))
                        if t == 1:
                            wait(cps_wo())
                        if cfg.get("only") is None:
                            st_expand(t)
                        if t + 2 < NU:
                            wait(cps_k(t + 2, t % 2))
                        if t < ub - 1:
                            last_wait(t)
                    return c

                lax.fori_loop(0, n_first, dma_ops, 0)
                pl.when(first)(lambda: last_wait(ub - 1))

            def prologue():
                x = xs[...]
                m, r = _ln_stats(x)
                lhs = _lhs(x, 1.0)

                def q_direct(u):
                    qs = []
                    for nt in range(3):
                        qq = _dot(lhs, _as_bf16(wq32[:, u * 3 + nt]))
                        qs.append((qq[0:8] - qq[8:16] * m) * r)
                    pack_q(jnp.concatenate(qs, axis=1), u)

                q_direct(0)
                q_direct(1)
                un = (x - m) * r
                ulhs[...] = pltpu.bitcast(_lhs(un), U32)
                va = cfg["va_units"]
                f1, f2 = cfg["va_force"]
                toks = st_qk(0, range(f1 if va else nj))
                if va:
                    for kb in range(D // 128):
                        blk = jnp.broadcast_to(un[0:1, kb * 128:(kb + 1) * 128], (128, 128)).T
                        ucol[kb // 3][zdyn, (kb % 3) * 128:(kb % 3 + 1) * 128, :] = blk
                        qlhs[8 + zdyn, :, 0:128] = pltpu.bitcast(blk[120:128], U32)
                        if kb == 2:
                            toks += st_qk(0, range(f1, f2))
                    toks += st_qk(0, range(f2, nj))
                st_softmax(0, zdyn)
                toks += st_qproj(2, zdyn)
                st_qpack(2)
                pos = js(1) - cfg["pvm_back0"]
                toks += st_qk(1, range(pos))
                toks += st_pvm(0)
                toks += st_qk(1, range(pos, js(1)))
                if va:
                    acc = [None] * len(va)
                    t0, t1 = cfg["va_tok"]
                    nkt = D // 16
                    for kt in range(nkt):
                        lo = ucol[kt // 24][0, pl.ds(kt % 24 * 16, 8, stride=2), :]
                        hi = ucol[kt // 24][0, pl.ds(kt % 24 * 16 + 1, 8, stride=2), :]
                        tk = toks[t0 + kt * (t1 - t0) // nkt]
                        lo, hi = lo + tk, hi + tk
                        for i, u in enumerate(va):
                            w = wq32[kt, u * 3:u * 3 + 3]
                            pr = (pltpu.bitcast(w << 16, F32) * lo
                                  + pltpu.bitcast(w & jnp.uint32(0xFFFF0000), F32) * hi)
                            acc[i] = pr if acc[i] is None else acc[i] + pr
                    for i, u in enumerate(va):
                        q = jnp.concatenate([acc[i][n] for n in range(3)], axis=1)
                        q = q + pltpu.roll(q, 4, 0)
                        q = q + pltpu.roll(q, 2, 0)
                        q = q + pltpu.roll(q, 1, 0)
                        pack_q(q, u)
                return toks

            def block(bi):
                ua, ub = cfg["blocks"][bi]
                block_dma(ua, ub)
                toks = []
                if bi == 0:
                    toks += prologue()
                done = js(ua + 1)
                for t in range(ua, ub):
                    base = len(toks)
                    for u in cfg["ored_at"].get(t, ()):
                        st_ored(u)
                    if t + 1 < NU:
                        toks += st_qk(t + 1, range(done, nj))
                        st_softmax(t + 1, zdyn)
                    g0 = len(toks)
                    if t == ua and bi > 0:
                        toks += st_pvm(t)
                    for u in cfg["qproj_at"].get(t, ()):
                        toks += st_qproj(u, zdyn)
                    for u in cfg["oproj_at"].get(t, ()):
                        toks += st_oproj(*u) if isinstance(u, tuple) else st_oproj(u)
                    done = js(t + 2)
                    if t + 1 < ub:
                        gap = cfg["gap_at"].get(t, cfg["gap"])
                        done = max(-((len(toks) - g0 - gap) // 3), 0)
                    if t + 2 < NU:
                        toks += st_qk(t + 2, range(done))
                    if t + 1 < ub:
                        toks += st_pvm(t + 1)
                    tok_map = cfg["tok"].get(t)
                    if tok_map is None:
                        n = len(toks) - base
                        if t == ub - 1:
                            n += cfg["tok_lin"][1]
                        tok_map = [k * n // (4 * NPIECE) - cfg["tok_lin"][0]
                                   for k in range(4 * NPIECE)]
                    NTOK[t] = len(toks) - base
                    st_pv(t, toks, [base + i for i in tok_map])
                    st_lsum(t)
                    for u in cfg["qproj_at"].get(t, ()):
                        st_qpack(u)

            if cfg.get("only") is not None:
                for i in range(cfg.get("pad", 0)):
                    lp = pltpu.bitcast(qlhs[0, :, 0:128], BF16)
                    lpart[i] = _dot(lp, _as_bf16(k32[pl.ds(0, 8), i]))[0:8]
                for bi in cfg["only"]:
                    block(bi)
                lax.fori_loop(0, n_first, lambda i, c: c + 1, 0)
                pl.when(first)(lambda: wait(cps_w4(0)))
                f = lambda v: pltpu.bitcast(v, F32)
                z8 = pl.multiple_of(zdyn * 8, 8)
                z128 = pl.multiple_of(zdyn * 128, 128)
                xs[:, 0:128] = (abuf[zdyn, pl.ds(z8, 8), :] + lpart[zdyn] + mbuf[zdyn, zdyn]
                                + f(olhs[zdyn, :, pl.ds(z128, 128)]) + f(qlhs[zdyn, :, pl.ds(z128, 128)])
                                + sx[zdyn, :, pl.ds(z128, 128)] + sy[zdyn, :, pl.ds(z128, 128)]
                                + pbuf0[zdyn, :, pl.ds(z128, 128)] + pbuf1[zdyn, :, pl.ds(z128, 128)]
                                + gp[zdyn, zdyn, pl.ds(z8, 8), :] + f(plhs[:, pl.ds(z128, 128)]))
                return carry

            for bi in range(len(cfg["blocks"])):
                block(bi)

            def tail(first_static):
                for u in range(*cfg["blocks"][-1]):
                    st_ored(u, partial_rows=(u == NU - 1))
                seen = set()
                for us in cfg["oproj_at"].values():
                    for u in us:
                        uu, ts = u if isinstance(u, tuple) else (u, (0, 1, 2))
                        seen |= {(uu, t) for t in ts}
                for u in range(NU - 1):
                    ts = tuple(t for t in range(3) if (u, t) not in seen)
                    if ts:
                        st_oproj(u, ts)
                extra = [[] for _ in range(D // 128)]
                st_oproj(NU - 1, out=extra)
                mlp(first_static, extra)

            pl.when(first)(lambda: tail(True))
            pl.when(jnp.logical_not(first))(lambda: tail(False))
            return carry

        lax.fori_loop(0, cfg["layers"], layer, 0)
        o_ref[...] = xs[0:1, :].astype(o_ref.dtype)

    return kernel


@jax.jit
def pallas_interleave_layers__sliding_block_cached__mixer_s_mlp__decode_kernel(
    A_x: jax.Array,
    A_k_cache: jax.Array,
    A_v_cache: jax.Array,
    A_wq: jax.Array,
    A_wo: jax.Array,
    B_x: jax.Array,
    B_w1: jax.Array,
    B_w2: jax.Array,
    B_w3: jax.Array,
    B_w4: jax.Array,
):
    b, sq, d = A_x.shape
    _, hkv, sk, dh = A_k_cache.shape
    assert (b, sq, d, hkv, dh) == (1, 1, D, H, DH)
    win = min(4096, max(256, sk // 4))
    assert win % 512 == 0 and sk % 128 == 0
    nj = win // 128

    kt = _tile_view(jnp.swapaxes(A_k_cache, 2, 3).reshape(H * DH, sk))
    vt = _head_view(jnp.swapaxes(A_v_cache, 2, 3).reshape(H * DH, sk))

    def buf(r, c):
        return pltpu.VMEM((r // 16, c // 128, 16, 128), BF16)

    def hbuf(c):
        return pltpu.VMEM((H, DH // 16, c // 128, 16, 128), BF16)

    bl = CFG["blocks"]
    ns = CFG.get("ns") or max(bl[i + 1][1] - bl[i][0] for i in range(len(bl) - 1))
    any_spec = pl.BlockSpec(memory_space=pl.ANY)
    out = pl.pallas_call(
        _make_kernel(sk, win, CFG),
        out_shape=jax.ShapeDtypeStruct((1, D), A_x.dtype),
        in_specs=[any_spec] * 7,
        out_specs=pl.BlockSpec(memory_space=pltpu.VMEM),
        scratch_shapes=[
            buf(H * DH, win), hbuf(win),
            pltpu.VMEM((H, DH // 16, max(len(CFG["jx"]), 1), 8, 128), F32),
            buf(D, H * DH), hbuf(D), buf(D, FF), buf(FF, D),
            pltpu.VMEM((1, D), BF16),
            pltpu.VMEM((8, D), F32),
            pltpu.VMEM((8, D), U32),
            pltpu.VMEM((1, D // 128, 8, 384), F32),
            pltpu.VMEM((1, D // 128, 8, 384), F32),
            pltpu.VMEM((9, 8, 384), U32),
            pltpu.VMEM((1, 384, 128), F32),
            pltpu.VMEM((1, 256, 128), F32),
            pltpu.VMEM((2, 8, win // 4), F32),
            pltpu.VMEM((2, 8, win // 4), F32),
            pltpu.VMEM((1, 8, win // 4), F32),
            pltpu.VMEM((1, 8, win // 4), F32),
            pltpu.VMEM((8, 256), U32),
            pltpu.VMEM((ns, 3, 8, 128), F32),
            pltpu.VMEM((ns, 8, 128), F32),
            pltpu.VMEM((ns, 384, 128), F32),
            pltpu.VMEM((NU, 8, 384), U32),
            pltpu.VMEM((3, D // 128, NU, 128), F32),
            pltpu.SemaphoreType.DMA((5,)),
        ],
        compiler_params=pltpu.CompilerParams(vmem_limit_bytes=int(CFG["vmem_mb"] * 1024 * 1024)),
        name="interleave_decode",
    )(A_x.reshape(1, D), kt, vt, _tile_view(A_wq), _head_view(A_wo),
      _tile_view(B_w3), _tile_view(B_w4))
    return out.reshape(b, sq, d)
```

```python
import jax
import jax.numpy as jnp
from jax import lax
import jax.experimental.pallas as pl
import jax.experimental.pallas.tpu as pltpu

F32 = jnp.float32
BF16 = jnp.bfloat16
U32 = jnp.uint32

D = 640
H = 32
DH = 192
FF = 1536
NU = H // 2
UT = 2 * DH // 16
EPS = 1e-5
NPIECE = 12

CFG = dict(
    blocks=((0, 4), (4, 8), (8, 12), (12, 15), (15, 16)), ns=7,
    jsplit=8, js_at={},
    gap=40, gap_at={0: 44, 1: 44, 2: 44}, pvm_back0=0,
    nm=3, nm_at={0: 2, 4: 2},
    va_units=(6, 7, 8, 9), va_force=(7, 16), va_tok=(10, 100),
    qproj_at={0: (3,), 1: (4,), 2: (5,), 3: (10,), 5: (11,), 6: (12,), 7: (13,), 10: (14,), 11: (15,)},
    ored_at={4: (0,), 5: (1,), 6: (2,), 7: (3,), 8: (4,), 9: (5,), 10: (6,), 11: (7,),
             12: (8,), 13: (9, 10), 14: (11,), 15: (12, 13, 14)},
    oproj_at={4: ((0, (2,)),), 5: ((1, (2,)),), 6: ((2, (2,)),), 7: ((3, (2,)),),
              8: ((4, (2,)), (0, (0,))), 9: ((5, (2,)), (0, (1,))), 10: ((6, (2,)),), 11: ((7, (2,)),),
              12: ((8, (2,)),), 13: ((9, (2,)), (10, (2,)), (4, (0, 1))),
              14: ((11, (2,)), (1, (0, 1)), (2, (0, 1)), (3, (0, 1))),
              15: ((5, (0, 1)), (6, (0, 1)), (7, (0, 1)), (8, (0, 1)), (9, (0, 1)),
                   (10, (0, 1)), (11, (0, 1)), 12, (13, (0, 1)))},
    jx=(1, 5, 9, 13, 17, 21, 25), vmem_mb=128,
    tok={
        0: [-22,-20,-18,-15,-13,-10,-8,-5,-3,-1,2,4,7,9,12,14,16,19,22,24,27,30,32,35,37,40,43,45,48,50,53,56,58,61,64,67,69,72,75,78,80,83,86,89,91,94,97,99],
        1: [-24,-21,-19,-17,-14,-12,-9,-7,-5,-2,0,3,5,7,10,12,15,17,20,22,25,28,30,33,35,38,40,43,46,48,51,53,56,59,61,64,67,69,72,75,77,80,83,85,88,91,93,96],
        2: [-21,-19,-16,-14,-12,-9,-7,-4,-2,0,3,5,8,10,12,15,17,20,22,25,28,30,33,36,38,41,43,46,49,51,54,56,59,62,64,67,69,72,74,77,79,82,84,86,89,91,94,96],
        3: [-21,-19,-16,-14,-11,-9,-6,-4,-1,1,4,6,8,11,13,16,18,21,24,26,29,32,34,37,40,42,45,47,50,53,55,58,61,63,65,68,70,72,75,77,79,82,84,86,89,91,93,96],
        4: [-25,-22,-20,-18,-15,-13,-11,-8,-6,-4,-1,1,3,5,8,10,12,15,18,21,24,26,29,32,35,38,40,43,46,49,52,55,57,60,63,66,69,72,75,77,80,83,86,89,92,95,98,100],
        5: [-19,-16,-14,-11,-9,-6,-4,-1,1,3,6,8,11,13,16,18,21,24,26,29,32,35,38,41,43,46,49,52,55,58,60,63,66,69,71,73,76,78,81,83,86,88,90,93,95,98,100,103],
        6: [-11,-8,-6,-3,0,2,5,7,10,13,15,18,21,23,26,28,31,34,36,39,42,44,47,49,52,55,57,60,63,65,68,70,73,76,78,81,83,86,89,91,94,97,99,102,104,107,110,112],
        7: [-10,-8,-5,-3,0,2,5,7,10,12,15,17,20,22,25,27,30,33,35,38,41,44,46,49,52,55,57,60,63,66,68,71,74,76,79,82,84,87,90,92,95,97,100,103,105,108,111,113],
        8: [-24,-21,-19,-17,-14,-12,-10,-7,-5,-2,1,3,6,9,12,15,17,20,23,25,28,30,33,35,38,40,43,45,48,50,53,55,57,60,63,66,69,72,74,77,80,83,86,89,92,94,97,100],
        9: [-18,-16,-13,-11,-9,-6,-4,-2,1,3,5,8,10,12,15,17,19,22,25,28,30,33,36,39,41,44,47,50,53,56,59,62,65,67,70,72,75,77,80,82,85,87,90,92,95,97,100,102],
        10: [-19,-17,-14,-12,-9,-6,-4,-1,1,4,7,9,12,14,17,20,22,25,27,30,32,35,37,40,42,45,48,51,54,56,59,62,65,67,70,73,76,78,81,84,87,89,92,95,98,100,103,106],
        11: [-7,-5,-3,-1,2,4,6,8,11,13,16,19,21,24,27,29,32,34,37,40,42,45,47,50,53,55,58,60,63,66,68,71,73,76,79,81,84,87,90,92,95,98,100,103,105,108,111,113],
        12: [-32,-28,-25,-21,-18,-14,-11,-8,-4,-2,-1,1,3,4,6,8,9,12,16,19,22,25,28,32,35,38,40,43,46,48,51,54,56,59,61,64,67,69,72,74,77,80,82,85,87,90,92,95],
        13: [-24,-22,-19,-17,-14,-11,-9,-6,-4,-1,2,4,7,9,12,15,17,20,23,25,28,31,33,36,39,42,45,48,50,53,56,59,62,65,67,70,72,75,77,80,82,85,87,89,92,94,96,99],
        14: [-18,-15,-13,-11,-8,-6,-4,-1,1,4,7,10,13,16,20,23,26,28,30,33,35,37,40,42,44,47,50,53,55,58,61,64,67,69,72,74,77,79,82,84,87,89,92,94,97,99,102,104],
        15: [-44,-41,-37,-34,-30,-27,-24,-20,-17,-14,-11,-7,-4,-1,2,5,8,11,14,18,21,24,27,31,34,36,38,41,43,45,47,49,52,56,59,63,67,71,75,79,83,83,84,84,85,85,86,86],
    },
    w4_cuts=(7, 11))


def _tile_view(a):
    r, c = a.shape
    a = a.reshape(r // 16, 2, 8, c // 128, 128)
    return jnp.swapaxes(a, 2, 3)


def _head_view(a):
    c = a.shape[1]
    a = a.reshape(H, 2, DH // 16, 8, c // 128, 128)
    return jnp.swapaxes(a, 3, 4)


def _as_bf16(w32):
    n = w32.shape[0]
    return pltpu.bitcast(w32.reshape(n * 8, 128), BF16)


def _lhs(top, fill=0.0):
    return jnp.concatenate([top, jnp.full(top.shape, fill, F32)], axis=0).astype(BF16)


def _ln_stats(x):
    m = jnp.mean(x, axis=-1, keepdims=True)
    m2 = jnp.mean(x * x, axis=-1, keepdims=True)
    v = jnp.maximum(m2 - m * m, 0.0)
    return m, lax.rsqrt(v + EPS)


def _round_bf16(x):
    return x.astype(BF16).astype(F32)


def _dot(a, b):
    return jnp.dot(a, b, preferred_element_type=F32)


def _make_kernel(sk, win, cfg):
    nj = win // 128
    j0 = (sk - win) // 128
    jq = nj // 4
    jx = list(cfg["jx"])
    qscale = DH ** -0.5 * 1.4426950408889634

    def kernel(x_hbm, k_hbm, v_hbm, wq_hbm, wo_hbm, w3_hbm, w4_hbm, o_ref,
               kbuf, vbuf, vx, wqbuf, wobuf, w3buf, w4buf, xin,
               xs, ulhs, qp0, qp1, qlhs, ucol0, ucol1, sx, sy, pbuf0, pbuf1, plhs, mbuf, lpart, abuf, olhs, gp,
               sems):
        qp = (qp0, qp1)
        ucol = (ucol0, ucol1)
        pbuf = (pbuf0, pbuf1)
        ns = abuf.shape[0]


        def cps_w(hbm, buf, sem, lo=0, n=None):
            n = buf.shape[0] if n is None else n
            return [pltpu.make_async_copy(
                hbm.at[pl.ds(lo, n), e],
                buf.at[pl.ds(lo, n), :, pl.ds(e * 8, 8), :],
                sems.at[sem]) for e in range(2)]

        def cps_kv(hbm, buf, sem, u):
            return [pltpu.make_async_copy(
                hbm.at[pl.ds(u * UT, UT), e, pl.ds(j0, nj)],
                buf.at[pl.ds(u * UT, UT), :, pl.ds(e * 8, 8), :],
                sems.at[sem]) for e in range(2)]

        def cps_v(u, par):
            return [pltpu.make_async_copy(
                v_hbm.at[pl.ds(2 * u, 2), e, :, pl.ds(j0, nj)],
                vbuf.at[pl.ds(2 * u, 2), :, :, pl.ds(e * 8, 8), :],
                sems.at[2 + par]) for e in range(2)]

        def cps_wo():
            return [pltpu.make_async_copy(
                wo_hbm.at[:, e], wobuf.at[:, :, :, pl.ds(e * 8, 8), :],
                sems.at[4]) for e in range(2)]

        cps_k = lambda u, par: cps_kv(k_hbm, kbuf, par, u)
        cps_x_wq = lambda: cps_w(wq_hbm, wqbuf, 4) + [pltpu.make_async_copy(x_hbm, xin, sems.at[4])]
        cps_w3 = lambda: cps_w(w3_hbm, w3buf, 0)
        w4_cuts = (0,) + tuple(cfg["w4_cuts"]) + (FF // 128,)
        cps_w4 = lambda i: cps_w(w4_hbm, w4buf, (1, 4, 2)[i], w4_cuts[i] * 8,
                                 (w4_cuts[i + 1] - w4_cuts[i]) * 8)

        def start(cps):
            for c in cps:
                c.start()

        def wait(cps):
            for c in cps:
                c.wait()

        start(cps_x_wq())
        start(cps_k(0, 0))
        start(cps_k(1, 1))
        start(cps_v(0, 0))
        start(cps_v(1, 1))

        k32 = kbuf.bitcast(U32)
        v32 = vbuf.bitcast(U32)
        wq32 = wqbuf.bitcast(U32)
        wo32 = wobuf.bitcast(U32)
        w332 = w3buf.bitcast(U32)
        w432 = w4buf.bitcast(U32)

        def js(u):
            return cfg["js_at"].get(u, cfg["jsplit"])

        def qslot(u):
            va = cfg["va_units"]
            return 4 + va.index(u) if u in va else u % 4

        def jms(u):
            return [nj - 1 - jq * i for i in range(nmx(u))]

        def nmx(u):
            return cfg["nm_at"].get(u, cfg["nm"])

        def st_qproj(u, zdyn):
            lhs = pltpu.bitcast(ulhs[...], BF16)
            toks = []
            for kt in range(D // 128):
                for nt in range(3):
                    w = _as_bf16(wq32[pl.ds(kt * 8, 8), u * 3 + nt])
                    r = _dot(lhs[:, kt * 128:(kt + 1) * 128], w)
                    toks.append(r[8:16])
                    qp[u % 2][zdyn, kt, :, nt * 128:(nt + 1) * 128] = r[0:8]
            return toks

        def pack_q(q, u):
            q = q * qscale
            lane = lax.broadcasted_iota(jnp.int32, (8, 128), 1)
            sub = lax.broadcasted_iota(jnp.int32, (8, 128), 0)
            keep = (lane < DH - 128) == (sub % 2 == 0)
            q = jnp.concatenate(
                [q[:, 0:128], jnp.where(keep, q[:, 128:256], 0.0), q[:, 256:384]], axis=1)
            qlhs.at[qslot(u)][:, 0:384] = pltpu.bitcast(_lhs(q), U32)

        def st_qpack(u):
            q = qp[u % 2][0, 0]
            for kt in range(1, D // 128):
                q = q + qp[u % 2][0, kt]
            pack_q(q, u)

        def st_qk(u, js):
            sl = u % 2
            lhs = pltpu.bitcast(qlhs[qslot(u)], BF16)
            toks = []
            for j in js:
                ra = 2 * (j // jq)
                cs = slice((j % jq) * 128, (j % jq + 1) * 128)
                for t in range(3):
                    w = _as_bf16(k32[pl.ds(u * UT + t * 8, 8), j])
                    r = _dot(lhs[:, t * 128:(t + 1) * 128], w)
                    toks.append(r[8:16])
                    if t == 0:
                        sx[sl, ra:ra + 1, cs] = r[0:1]
                    elif t == 1:
                        sy[sl, ra:ra + 2, cs] = r[ra:ra + 2]
                    else:
                        sx[sl, ra + 1:ra + 2, cs] = r[0:1]
            return toks

        def st_softmax(u, zdyn):
            sl = u % 2
            s = sx[sl] + sy[sl]
            m = s
            while m.shape[1] > 128:
                h = m.shape[1] // 2
                m = jnp.maximum(m[:, :h], m[:, h:])
            m = jnp.maximum(m, pltpu.roll(m, 2, 0))
            m = jnp.maximum(m, pltpu.roll(m, 4, 0))
            m = jnp.max(m, axis=1, keepdims=True)
            p = jnp.exp2(s - m)
            pbuf[sl][zdyn] = p
            if nmx(u):
                plhs[:, sl * 128:(sl + 1) * 128] = pltpu.bitcast(_lhs(p[:, (jq - 1) * 128:jq * 128]), U32)

        def inv_l(l):
            l = jnp.sum(l, axis=1, keepdims=True)
            r0 = pl.reciprocal(l, approx=True)
            return jnp.broadcast_to(r0 * (2.0 - l * r0), (8, 128))

        def st_lsum(u):
            l = pbuf[u % 2][0, :, 0:128]
            for c in range(1, jq):
                l = l + pbuf[u % 2][0, :, c * 128:(c + 1) * 128]
            l = l + pltpu.roll(l, 2, 0)
            l = l + pltpu.roll(l, 4, 0)
            lpart[u % ns] = inv_l(l) if u == NU - 1 else l

        def st_pvm(u):
            toks = []
            for j in jms(u):
                lhs = pltpu.bitcast(plhs[:, u % 2 * 128:(u % 2 + 1) * 128], BF16)
                ra = 2 * (j // jq)
                for t in range(3):
                    if t == 1:
                        w32 = jnp.concatenate(
                            [v32[2 * u, 8:12, j], v32[2 * u + 1, 0:4, j]], axis=0)
                    else:
                        w32 = v32[2 * u + t // 2, 2 * t:2 * t + 8, j]
                    r = _dot(lhs, _as_bf16(w32))
                    toks.append(r[8:16])
                    mbuf[u % ns, t, ra:ra + 2, :] = r[ra:ra + 2]
            return toks

        def st_expand(u):
            def body(i, c):
                hd, dt = i // 12, i % 12
                for ix, j in enumerate(jx):
                    w = v32[2 * u + hd, dt, j]
                    vx[2 * u + hd, dt, ix] = pltpu.bitcast(w << 16, F32)
                    vbuf[2 * u + hd, dt, j] = pltpu.bitcast(w & jnp.uint32(0xFFFF0000), BF16)
                return c
            if jx:
                lax.fori_loop(0, UT, body, 0)
            for j in jms(u):
                for t in range(3):
                    idx = [divmod(t * 8 + v, 12) for v in range(8)]
                    blk = jnp.concatenate([vbuf[2 * u + hd, dt, j] for hd, dt in idx], axis=0)
                    blk = blk.astype(F32).T.astype(BF16)
                    for v, (hd, dt) in enumerate(idx):
                        vbuf[2 * u + hd, dt, j] = blk[v * 16:(v + 1) * 16]

        def st_pv(u, toks, tok_map):
            nm, sl = nmx(u), u % ns
            for piece in range(NPIECE):
                hd, half = divmod(piece, NPIECE // 2)
                sub = len(tok_map) // NPIECE
                lo = hi = None
                for j in range(nj):
                    if j in jms(u):
                        continue
                    row = 2 * (j // jq) + hd
                    cs = slice((j % jq) * 128, (j % jq + 1) * 128)
                    pb = jnp.broadcast_to(pbuf[u % 2][0, row:row + 1, cs], (8, 128))
                    k = piece * sub + j * sub // nj
                    ti = tok_map[k] if j % (nj // sub) == 0 else -1
                    if j > 0 and tok_map[k - 1] == ti:
                        ti = -1
                    if toks and ti >= 0:
                        pb = pb + toks[min(ti, len(toks) - 1)]
                    w = v32[2 * u + hd, pl.ds(half * 2, 2), j]
                    if j in jx:
                        a = vx[2 * u + hd, pl.ds(half * 2, 2), jx.index(j)] * pb
                        b = pltpu.bitcast(w, F32) * pb
                    else:
                        a = pltpu.bitcast(w << 16, F32) * pb
                        b = pltpu.bitcast(w & jnp.uint32(0xFFFF0000), F32) * pb
                    lo = a if lo is None else lo + a
                    hi = b if hi is None else hi + b
                for i in range(2):
                    base = (piece * 2 + i) * 16
                    abuf[sl, pl.ds(base, 8, stride=2), :] = lo[i]
                    abuf[sl, pl.ds(base + 1, 8, stride=2), :] = hi[i]

        def st_ored(u, ts=(0, 1, 2), partial_rows=False):
            nm, sl = nmx(u), u % ns
            ia = lpart[sl] if u == NU - 1 else inv_l(lpart[sl])
            ib = pltpu.roll(ia, 1, 0)
            if partial_rows:
                even = lax.broadcasted_iota(jnp.int32, (8, 128), 0) % 2 == 0
                ia, ib = jnp.where(even, ia, ib), jnp.where(even, ib, ia)
            lane = lax.broadcasted_iota(jnp.int32, (8, 128), 1)
            for t in ts:
                at = abuf[sl, t * 128:(t + 1) * 128, :].T
                o = at[0:8]
                for i in range(1, 16):
                    o = o + at[i * 8:(i + 1) * 8]
                if nm:
                    sub = lax.broadcasted_iota(jnp.int32, (8, 128), 0)
                    odd = (0, (lane >= DH - 128).astype(jnp.int32), 1)[t]
                    keep = (sub >= 8 - 2 * nm) & (sub % 2 == odd)
                    o = o + jnp.where(keep, mbuf[sl, t], 0.0)
                if not partial_rows:
                    o = o + pltpu.roll(o, 4, 0)
                    o = o + pltpu.roll(o, 2, 0)
                    o = o + pltpu.roll(o, 1, 0)
                o = o * (ia, jnp.where(lane < DH - 128, ia, ib), ib)[t]
                olhs.at[u][:, t * 128:(t + 1) * 128] = pltpu.bitcast(_lhs(o), U32)

        def st_oproj(u, ts=(0, 1, 2), out=None):
            lhs = pltpu.bitcast(olhs[u], BF16)
            toks = []
            for t in ts:
                for n in range(D // 128):
                    if t == 1:
                        w32 = jnp.concatenate(
                            [wo32[2 * u, 8:12, n], wo32[2 * u + 1, 0:4, n]], axis=0)
                    else:
                        w32 = wo32[2 * u + t // 2, 2 * t:2 * t + 8, n]
                    r = _dot(lhs[:, t * 128:(t + 1) * 128], _as_bf16(w32))
                    toks.append(r[8:16])
                    if out is None:
                        gp[t, n, pl.ds(u, 1), :] = r[0:1]
                    else:
                        out[n].append(r[0:8])
            return toks

        def mlp(first, extra):
            g = gp[0] + gp[1] + gp[2]
            g = g[:, 0:8] + g[:, 8:16]
            g = jnp.concatenate([g[n] + extra[n][0] + extra[n][1] + extra[n][2]
                                 for n in range(D // 128)], axis=1)
            g = g + pltpu.roll(g, 4, 0)
            g = g + pltpu.roll(g, 2, 0)
            g = g + pltpu.roll(g, 1, 0)
            x1 = _round_bf16(xs[...] + g)
            lhs = _lhs(x1, 1.0)
            m1, r1 = _ln_stats(x1)
            y = (x1 - m1) * r1
            m2, r2 = _ln_stats(y)
            a = r1 * r2
            b = (m1 * r1 + m2) * r2
            hl = []
            for n in range(FF // 128):
                r = _dot(lhs, _as_bf16(w332[:, n]))
                hl.append(_lhs(jax.nn.gelu(r[0:8] * a - r[8:16] * b, approximate=True)))
            acc = x1 + y
            acc = [acc[:, c * 128:(c + 1) * 128] for c in range(D // 128)]
            for kt in range(FF // 128):
                if first and kt in w4_cuts:
                    wait(cps_w4(w4_cuts.index(kt)))
                for c in range(D // 128):
                    w = _as_bf16(w432[pl.ds(kt * 8, 8), c])
                    acc[c] = acc[c] + _dot(hl[kt], w)[0:8]
            xs[...] = _round_bf16(jnp.concatenate(acc, axis=1))

        gp[...] = jnp.zeros_like(gp)
        mbuf[...] = jnp.zeros_like(mbuf)
        wait(cps_x_wq())
        start(cps_wo())
        wait(cps_k(0, 0))
        start(cps_k(2, 0))
        wait(cps_k(1, 1))
        wait(cps_v(0, 0))
        xs[...] = jnp.broadcast_to(xin[...].astype(F32), (8, D))

        def layer(li, carry):
            first = li == 0
            n_first = jnp.maximum(1 - li, 0)
            zdyn = li >> 4

            def block_dma(ua, ub):
                def last_wait(t):
                    wait(cps_v(t + 1, (t + 1) % 2) if t + 1 < NU else cps_w3())

                def dma_ops(_, c):
                    for t in range(ua, ub):
                        if t + 3 < NU:
                            start(cps_k(t + 3, (t + 3) % 2))
                        if t + 2 < NU:
                            start(cps_v(t + 2, t % 2))
                        if t == NU - 2:
                            start(cps_w3())
                            for i in range(len(w4_cuts) - 1):
                                start(cps_w4(i))
                        if t == 1:
                            wait(cps_wo())
                        st_expand(t)
                        if t + 2 < NU:
                            wait(cps_k(t + 2, t % 2))
                        if t < ub - 1:
                            last_wait(t)
                    return c

                lax.fori_loop(0, n_first, dma_ops, 0)
                pl.when(first)(lambda: last_wait(ub - 1))

            def prologue():
                x = xs[...]
                m, r = _ln_stats(x)
                lhs = _lhs(x, 1.0)

                def q_direct(u):
                    qs = []
                    for nt in range(3):
                        qq = _dot(lhs, _as_bf16(wq32[:, u * 3 + nt]))
                        qs.append((qq[0:8] - qq[8:16] * m) * r)
                    pack_q(jnp.concatenate(qs, axis=1), u)

                q_direct(0)
                q_direct(1)
                un = (x - m) * r
                ulhs[...] = pltpu.bitcast(_lhs(un), U32)
                va = cfg["va_units"]
                f1, f2 = cfg["va_force"]
                toks = st_qk(0, range(f1 if va else nj))
                if va:
                    for kb in range(D // 128):
                        blk = jnp.broadcast_to(un[0:1, kb * 128:(kb + 1) * 128], (128, 128)).T
                        ucol[kb // 3][zdyn, (kb % 3) * 128:(kb % 3 + 1) * 128, :] = blk
                        qlhs[8 + zdyn, :, 0:128] = pltpu.bitcast(blk[120:128], U32)
                        if kb == 2:
                            toks += st_qk(0, range(f1, f2))
                    toks += st_qk(0, range(f2, nj))
                st_softmax(0, zdyn)
                toks += st_qproj(2, zdyn)
                st_qpack(2)
                pos = js(1) - cfg["pvm_back0"]
                toks += st_qk(1, range(pos))
                toks += st_pvm(0)
                toks += st_qk(1, range(pos, js(1)))
                if va:
                    acc = [None] * len(va)
                    t0, t1 = cfg["va_tok"]
                    nkt = D // 16
                    for kt in range(nkt):
                        lo = ucol[kt // 24][0, pl.ds(kt % 24 * 16, 8, stride=2), :]
                        hi = ucol[kt // 24][0, pl.ds(kt % 24 * 16 + 1, 8, stride=2), :]
                        tk = toks[t0 + kt * (t1 - t0) // nkt]
                        lo, hi = lo + tk, hi + tk
                        for i, u in enumerate(va):
                            w = wq32[kt, u * 3:u * 3 + 3]
                            pr = (pltpu.bitcast(w << 16, F32) * lo
                                  + pltpu.bitcast(w & jnp.uint32(0xFFFF0000), F32) * hi)
                            acc[i] = pr if acc[i] is None else acc[i] + pr
                    for i, u in enumerate(va):
                        q = jnp.concatenate([acc[i][n] for n in range(3)], axis=1)
                        q = q + pltpu.roll(q, 4, 0)
                        q = q + pltpu.roll(q, 2, 0)
                        q = q + pltpu.roll(q, 1, 0)
                        pack_q(q, u)
                return toks

            def block(bi):
                ua, ub = cfg["blocks"][bi]
                block_dma(ua, ub)
                toks = []
                if bi == 0:
                    toks += prologue()
                done = js(ua + 1)
                for t in range(ua, ub):
                    base = len(toks)
                    for u in cfg["ored_at"].get(t, ()):
                        st_ored(u)
                    if t + 1 < NU:
                        toks += st_qk(t + 1, range(done, nj))
                        st_softmax(t + 1, zdyn)
                    g0 = len(toks)
                    if t == ua and bi > 0:
                        toks += st_pvm(t)
                    for u in cfg["qproj_at"].get(t, ()):
                        toks += st_qproj(u, zdyn)
                    for u in cfg["oproj_at"].get(t, ()):
                        toks += st_oproj(*u) if isinstance(u, tuple) else st_oproj(u)
                    done = js(t + 2)
                    if t + 1 < ub:
                        gap = cfg["gap_at"].get(t, cfg["gap"])
                        done = max(-((len(toks) - g0 - gap) // 3), 0)
                    if t + 2 < NU:
                        toks += st_qk(t + 2, range(done))
                    if t + 1 < ub:
                        toks += st_pvm(t + 1)
                    st_pv(t, toks, [base + i for i in cfg["tok"][t]])
                    st_lsum(t)
                    for u in cfg["qproj_at"].get(t, ()):
                        st_qpack(u)

            for bi in range(len(cfg["blocks"])):
                block(bi)

            def tail(first_static):
                for u in range(*cfg["blocks"][-1]):
                    st_ored(u, partial_rows=(u == NU - 1))
                seen = set()
                for us in cfg["oproj_at"].values():
                    for u in us:
                        uu, ts = u if isinstance(u, tuple) else (u, (0, 1, 2))
                        seen |= {(uu, t) for t in ts}
                for u in range(NU - 1):
                    ts = tuple(t for t in range(3) if (u, t) not in seen)
                    if ts:
                        st_oproj(u, ts)
                extra = [[] for _ in range(D // 128)]
                st_oproj(NU - 1, out=extra)
                mlp(first_static, extra)

            pl.when(first)(lambda: tail(True))
            pl.when(jnp.logical_not(first))(lambda: tail(False))
            return carry

        lax.fori_loop(0, 2, layer, 0)
        o_ref[...] = xs[0:1, :].astype(o_ref.dtype)

    return kernel


@jax.jit
def pallas_interleave_layers__sliding_block_cached__mixer_s_mlp__decode_kernel(
    A_x: jax.Array,
    A_k_cache: jax.Array,
    A_v_cache: jax.Array,
    A_wq: jax.Array,
    A_wo: jax.Array,
    B_x: jax.Array,
    B_w1: jax.Array,
    B_w2: jax.Array,
    B_w3: jax.Array,
    B_w4: jax.Array,
):
    b, sq, d = A_x.shape
    _, hkv, sk, dh = A_k_cache.shape
    assert (b, sq, d, hkv, dh) == (1, 1, D, H, DH)
    win = min(4096, max(256, sk // 4))
    assert win % 512 == 0 and sk % 128 == 0
    nj = win // 128

    kt = _tile_view(jnp.swapaxes(A_k_cache, 2, 3).reshape(H * DH, sk))
    vt = _head_view(jnp.swapaxes(A_v_cache, 2, 3).reshape(H * DH, sk))

    def buf(r, c):
        return pltpu.VMEM((r // 16, c // 128, 16, 128), BF16)

    def hbuf(c):
        return pltpu.VMEM((H, DH // 16, c // 128, 16, 128), BF16)

    bl = CFG["blocks"]
    ns = CFG.get("ns") or max(bl[i + 1][1] - bl[i][0] for i in range(len(bl) - 1))
    any_spec = pl.BlockSpec(memory_space=pl.ANY)
    out = pl.pallas_call(
        _make_kernel(sk, win, CFG),
        out_shape=jax.ShapeDtypeStruct((1, D), A_x.dtype),
        in_specs=[any_spec] * 7,
        out_specs=pl.BlockSpec(memory_space=pltpu.VMEM),
        scratch_shapes=[
            buf(H * DH, win), hbuf(win),
            pltpu.VMEM((H, DH // 16, max(len(CFG["jx"]), 1), 8, 128), F32),
            buf(D, H * DH), hbuf(D), buf(D, FF), buf(FF, D),
            pltpu.VMEM((1, D), BF16),
            pltpu.VMEM((8, D), F32),
            pltpu.VMEM((8, D), U32),
            pltpu.VMEM((1, D // 128, 8, 384), F32),
            pltpu.VMEM((1, D // 128, 8, 384), F32),
            pltpu.VMEM((9, 8, 384), U32),
            pltpu.VMEM((1, 384, 128), F32),
            pltpu.VMEM((1, 256, 128), F32),
            pltpu.VMEM((2, 8, win // 4), F32),
            pltpu.VMEM((2, 8, win // 4), F32),
            pltpu.VMEM((1, 8, win // 4), F32),
            pltpu.VMEM((1, 8, win // 4), F32),
            pltpu.VMEM((8, 256), U32),
            pltpu.VMEM((ns, 3, 8, 128), F32),
            pltpu.VMEM((ns, 8, 128), F32),
            pltpu.VMEM((ns, 384, 128), F32),
            pltpu.VMEM((NU, 8, 384), U32),
            pltpu.VMEM((3, D // 128, NU, 128), F32),
            pltpu.SemaphoreType.DMA((5,)),
        ],
        compiler_params=pltpu.CompilerParams(vmem_limit_bytes=int(CFG["vmem_mb"] * 1024 * 1024)),
        name="interleave_decode",
    )(A_x.reshape(1, D), kt, vt, _tile_view(A_wq), _head_view(A_wo),
      _tile_view(B_w3), _tile_view(B_w4))
    return out.reshape(b, sq, d)
```

```python
import jax
import jax.numpy as jnp
from jax import lax
import jax.experimental.pallas as pl
import jax.experimental.pallas.tpu as pltpu

F32 = jnp.float32
BF16 = jnp.bfloat16
U32 = jnp.uint32

D = 640
H = 32
DH = 192
FF = 1536
NU = H // 2
UT = 2 * DH // 16
EPS = 1e-5
NPIECE = 12

CFG = dict(
    blocks=((0, 4), (4, 8), (8, 12), (12, 15), (15, 16)), ns=7,
    jsplit=8, js_at={},
    gap=49, gap1=24, gap_at={0: 44, 1: 44, 2: 44}, gap1_at={0: 0, 1: 0, 2: 0, 3: 0}, ored_pin=(), ored_back=4, pvm_back0=0, pin0=0,
    nm=3, nm_at={0: 2, 4: 2},
    va_units=(6, 7, 8, 9), va_force=(7, 16), va_tok=(12, 108),
    qproj_at={0: (3,), 1: (4,), 2: (5,), 3: (10,), 5: (11,), 6: (12,), 7: (13,), 10: (14,), 11: (15,)},
    ored_at={4: (0,), 5: (1,), 6: (2,), 7: (3,), 8: (4,), 9: (5,), 10: (6,), 11: (7,),
             12: (8,), 13: (9, 10), 14: (11,), 15: (12, 13, 14)},
    oproj_at={4: ((0, (2,)),), 5: ((1, (2,)),), 6: ((2, (2,)),), 7: ((3, (2,)),),
              8: ((4, (2,)), (0, (0,))), 9: ((5, (2,)), (0, (1,))), 10: ((6, (2,)),), 11: ((7, (2,)),),
              12: ((8, (2,)),), 13: ((9, (2,)), (10, (2,)), (4, (0, 1))),
              14: ((11, (2,)), (1, (0, 1)), (2, (0, 1)), (3, (0, 1))),
              15: ((5, (0, 1)), (6, (0, 1)), (7, (0, 1)), (8, (0, 1)), (9, (0, 1)),
                   (10, (0, 1)), (11, (0, 1)), 12, (13, (0, 1)))},
    jx=(1, 5, 9, 13, 17, 21, 25), vmem_mb=128,
    tok={
        0: [-22,-18,-17,-15,-13,-10,-8,-5,-3,-1,-1,4,7,9,12,14,16,19,22,24,27,27,33,35,37,40,43,45,48,50,53,55,56,58,64,67,69,74,75,78,80,83,86,89,91,94,96,97],
        1: [-24,-21,-19,-17,-14,-12,-12,-7,-5,-2,0,3,5,7,10,12,15,17,20,22,25,28,30,33,34,37,39,42,45,47,51,53,56,59,61,64,68,69,72,75,77,80,83,85,88,91,93,96],
        2: [-21,-19,-16,-12,-11,-9,-7,-4,-2,0,3,5,8,10,12,15,17,20,22,25,28,30,33,36,38,41,43,45,49,51,54,56,59,62,64,67,69,72,74,74,79,82,84,86,86,93,94,96],
        3: [-21,-19,-16,-14,-11,-9,-6,-4,1,5,5,7,9,12,14,17,18,21,24,26,29,32,34,35,40,42,42,47,50,53,54,57,60,62,65,68,70,72,77,79,80,82,84,86,89,91,96,96],
        4: [-25,-22,-22,-20,-15,-13,-10,-8,-4,-2,-1,0,3,5,7,9,11,14,17,19,22,25,28,31,34,37,40,43,46,49,51,54,57,60,63,66,69,71,74,77,80,83,85,88,91,94,97,100],
        5: [-28,-26,-24,-21,-19,-17,-14,-12,-10,-8,-5,-3,0,2,5,7,9,12,15,17,20,23,25,28,31,33,35,38,40,43,45,46,50,52,55,58,60,63,65,68,70,73,76,78,81,83,86,89],
        6: [-25,-22,-19,-16,-14,-11,-8,-5,-3,0,3,6,9,11,14,17,20,22,25,27,30,33,35,38,39,43,46,48,51,53,56,59,61,64,67,70,73,75,78,81,84,86,88,90,93,95,97,99],
        7: [-24,-21,-19,-16,-13,-11,-8,-5,-3,0,3,5,8,11,13,16,19,21,26,27,29,31,34,37,39,42,45,48,50,53,56,59,61,64,68,71,74,77,80,84,87,89,91,93,95,97,99,101],
        8: [-26,-24,-22,-19,-17,-15,-12,-10,-8,-5,-3,-1,1,4,6,8,11,14,16,19,22,25,28,31,34,36,39,42,45,48,51,54,57,59,59,66,68,71,73,75,78,81,83,86,89,91,94,102],
        9: [-31,-28,-26,-23,-21,-18,-16,-14,-11,-9,-6,-4,-1,1,3,6,6,11,14,16,19,22,24,27,30,32,35,37,40,43,45,48,52,53,56,56,58,59,66,69,71,74,77,79,82,84,87,89],
        10: [-32,-29,-27,-24,-24,-21,-19,-16,-14,-9,-7,-4,-2,1,5,8,10,13,16,16,19,21,24,27,29,32,35,38,40,43,46,48,51,54,56,59,62,64,67,68,72,75,77,80,83,85,88,91],
        11: [-23,-20,-18,-15,-13,-10,-8,-5,-2,1,3,6,9,9,14,16,19,20,23,26,29,31,33,37,39,42,45,48,50,53,56,58,61,64,67,69,72,72,79,82,85,87,90,93,96,99,102,105],
        12: [-20,-18,-16,-14,-10,-8,-7,-3,-2,-1,-1,1,3,5,7,9,11,14,16,19,22,24,27,30,32,33,35,38,43,46,48,51,54,57,60,63,66,69,72,75,78,81,83,86,89,89,95,97],
        13: [-31,-28,-26,-21,-21,-19,-16,-13,-11,-8,-4,-2,1,4,6,9,12,14,17,19,22,24,27,29,32,34,37,40,42,46,47,50,53,55,58,61,64,64,70,72,75,77,80,82,84,87,89,91],
        14: [-25,-23,-20,-18,-15,-13,-10,-8,-5,-2,1,3,6,11,12,13,16,18,21,24,26,28,31,33,36,38,41,44,46,49,52,54,55,58,62,65,68,70,73,76,78,81,84,86,89,92,95,97],
        15: [-53,-52,-51,-48,-28,-20,-19,-19,-16,-14,-7,-7,-2,1,7,7,8,13,13,17,22,23,25,31,35,39,41,41,46,46,47,48,54,59,59,60,67,67,69,69,81,85,85,85,85,85,92,92],
    },
    w4_cuts=(7, 11))


def _tile_view(a):
    r, c = a.shape
    a = a.reshape(r // 16, 2, 8, c // 128, 128)
    return jnp.swapaxes(a, 2, 3)


def _head_view(a):
    c = a.shape[1]
    a = a.reshape(H, 2, DH // 16, 8, c // 128, 128)
    return jnp.swapaxes(a, 3, 4)


def _as_bf16(w32):
    n = w32.shape[0]
    return pltpu.bitcast(w32.reshape(n * 8, 128), BF16)


def _lhs(top, fill=0.0):
    return jnp.concatenate([top, jnp.full(top.shape, fill, F32)], axis=0).astype(BF16)


def _ln_stats(x):
    m = jnp.mean(x, axis=-1, keepdims=True)
    m2 = jnp.mean(x * x, axis=-1, keepdims=True)
    v = jnp.maximum(m2 - m * m, 0.0)
    return m, lax.rsqrt(v + EPS)


def _round_bf16(x):
    return x.astype(BF16).astype(F32)


def _dot(a, b):
    return jnp.dot(a, b, preferred_element_type=F32)


def _make_kernel(sk, win, cfg):
    nj = win // 128
    j0 = (sk - win) // 128
    jq = nj // 4
    jx = list(cfg["jx"])
    qscale = DH ** -0.5 * 1.4426950408889634

    def kernel(x_hbm, k_hbm, v_hbm, wq_hbm, wo_hbm, w3_hbm, w4_hbm, o_ref,
               kbuf, vbuf, vx, wqbuf, wobuf, w3buf, w4buf, xin,
               xs, ulhs, qp0, qp1, qlhs, ucol0, ucol1, sx, sy, pbuf0, pbuf1, plhs, mbuf, lpart, abuf, olhs, gp,
               sems):
        qp = (qp0, qp1)
        ucol = (ucol0, ucol1)
        pbuf = (pbuf0, pbuf1)
        ns = abuf.shape[0]


        def cps_w(hbm, buf, sem, lo=0, n=None):
            n = buf.shape[0] if n is None else n
            return [pltpu.make_async_copy(
                hbm.at[pl.ds(lo, n), e],
                buf.at[pl.ds(lo, n), :, pl.ds(e * 8, 8), :],
                sems.at[sem]) for e in range(2)]

        def cps_kv(hbm, buf, sem, u):
            return [pltpu.make_async_copy(
                hbm.at[pl.ds(u * UT, UT), e, pl.ds(j0, nj)],
                buf.at[pl.ds(u * UT, UT), :, pl.ds(e * 8, 8), :],
                sems.at[sem]) for e in range(2)]

        def cps_v(u, par):
            return [pltpu.make_async_copy(
                v_hbm.at[pl.ds(2 * u, 2), e, :, pl.ds(j0, nj)],
                vbuf.at[pl.ds(2 * u, 2), :, :, pl.ds(e * 8, 8), :],
                sems.at[2 + par]) for e in range(2)]

        def cps_wo():
            return [pltpu.make_async_copy(
                wo_hbm.at[:, e], wobuf.at[:, :, :, pl.ds(e * 8, 8), :],
                sems.at[4]) for e in range(2)]

        cps_k = lambda u, par: cps_kv(k_hbm, kbuf, par, u)
        cps_x_wq = lambda: cps_w(wq_hbm, wqbuf, 4) + [pltpu.make_async_copy(x_hbm, xin, sems.at[4])]
        cps_w3 = lambda: cps_w(w3_hbm, w3buf, 0)
        w4_cuts = (0,) + tuple(cfg["w4_cuts"]) + (FF // 128,)
        cps_w4 = lambda i: cps_w(w4_hbm, w4buf, (1, 4, 2)[i], w4_cuts[i] * 8,
                                 (w4_cuts[i + 1] - w4_cuts[i]) * 8)

        def start(cps):
            for c in cps:
                c.start()

        def wait(cps):
            for c in cps:
                c.wait()

        start(cps_x_wq())
        start(cps_k(0, 0))
        start(cps_k(1, 1))
        start(cps_v(0, 0))
        start(cps_v(1, 1))

        k32 = kbuf.bitcast(U32)
        v32 = vbuf.bitcast(U32)
        wq32 = wqbuf.bitcast(U32)
        wo32 = wobuf.bitcast(U32)
        w332 = w3buf.bitcast(U32)
        w432 = w4buf.bitcast(U32)

        def js(u):
            return cfg["js_at"].get(u, cfg["jsplit"])

        def qslot(u):
            va = cfg["va_units"]
            return 4 + va.index(u) if u in va else u % 4

        def jms(u):
            return [nj - 1 - jq * i for i in range(nmx(u))]

        def nmx(u):
            return cfg["nm_at"].get(u, cfg["nm"])

        def st_qproj(u, zdyn):
            lhs = pltpu.bitcast(ulhs[...], BF16)
            toks = []
            for kt in range(D // 128):
                for nt in range(3):
                    w = _as_bf16(wq32[pl.ds(kt * 8, 8), u * 3 + nt])
                    r = _dot(lhs[:, kt * 128:(kt + 1) * 128], w)
                    toks.append(r[8:16])
                    qp[u % 2][zdyn, kt, :, nt * 128:(nt + 1) * 128] = r[0:8]
            return toks

        def pack_q(q, u):
            q = q * qscale
            lane = lax.broadcasted_iota(jnp.int32, (8, 128), 1)
            sub = lax.broadcasted_iota(jnp.int32, (8, 128), 0)
            keep = (lane < DH - 128) == (sub % 2 == 0)
            q = jnp.concatenate(
                [q[:, 0:128], jnp.where(keep, q[:, 128:256], 0.0), q[:, 256:384]], axis=1)
            qlhs.at[qslot(u)][:, 0:384] = pltpu.bitcast(_lhs(q), U32)

        def st_qpack(u):
            q = qp[u % 2][0, 0]
            for kt in range(1, D // 128):
                q = q + qp[u % 2][0, kt]
            pack_q(q, u)

        def st_qk(u, js):
            sl = u % 2
            lhs = pltpu.bitcast(qlhs[qslot(u)], BF16)
            toks = []
            for j in js:
                ra = 2 * (j // jq)
                cs = slice((j % jq) * 128, (j % jq + 1) * 128)
                for t in range(3):
                    w = _as_bf16(k32[pl.ds(u * UT + t * 8, 8), j])
                    r = _dot(lhs[:, t * 128:(t + 1) * 128], w)
                    toks.append(r[8:16])
                    if t == 0:
                        sx[sl, ra:ra + 1, cs] = r[0:1]
                    elif t == 1:
                        sy[sl, ra:ra + 2, cs] = r[ra:ra + 2]
                    else:
                        sx[sl, ra + 1:ra + 2, cs] = r[0:1]
            return toks

        def st_softmax(u, zdyn, pin=False):
            sl = u % 2
            s = sx[sl] + sy[sl]
            m = s
            while m.shape[1] > 128:
                h = m.shape[1] // 2
                m = jnp.maximum(m[:, :h], m[:, h:])
            m = jnp.maximum(m, pltpu.roll(m, 2, 0))
            m = jnp.maximum(m, pltpu.roll(m, 4, 0))
            if pin:
                qlhs[9 + zdyn, :, 0:128] = pltpu.bitcast(m, U32)
            m = jnp.max(m, axis=1, keepdims=True)
            p = jnp.exp2(s - m)
            pbuf[sl][zdyn] = p
            if nmx(u):
                plhs[:, sl * 128:(sl + 1) * 128] = pltpu.bitcast(_lhs(p[:, (jq - 1) * 128:jq * 128]), U32)

        def inv_l(l):
            l = jnp.sum(l, axis=1, keepdims=True)
            r0 = pl.reciprocal(l, approx=True)
            return jnp.broadcast_to(r0 * (2.0 - l * r0), (8, 128))

        def st_lsum(u):
            l = pbuf[u % 2][0, :, 0:128]
            for c in range(1, jq):
                l = l + pbuf[u % 2][0, :, c * 128:(c + 1) * 128]
            l = l + pltpu.roll(l, 2, 0)
            l = l + pltpu.roll(l, 4, 0)
            lpart[u % ns] = inv_l(l) if u == NU - 1 else l

        def st_pvm(u):
            toks = []
            for j in jms(u):
                lhs = pltpu.bitcast(plhs[:, u % 2 * 128:(u % 2 + 1) * 128], BF16)
                ra = 2 * (j // jq)
                for t in range(3):
                    if t == 1:
                        w32 = jnp.concatenate(
                            [v32[2 * u, 8:12, j], v32[2 * u + 1, 0:4, j]], axis=0)
                    else:
                        w32 = v32[2 * u + t // 2, 2 * t:2 * t + 8, j]
                    r = _dot(lhs, _as_bf16(w32))
                    toks.append(r[8:16])
                    mbuf[u % ns, t, ra:ra + 2, :] = r[ra:ra + 2]
            return toks

        def st_expand(u):
            def body(i, c):
                hd, dt = i // 12, i % 12
                for ix, j in enumerate(jx):
                    w = v32[2 * u + hd, dt, j]
                    vx[2 * u + hd, dt, ix] = pltpu.bitcast(w << 16, F32)
                    vbuf[2 * u + hd, dt, j] = pltpu.bitcast(w & jnp.uint32(0xFFFF0000), BF16)
                return c
            if jx:
                lax.fori_loop(0, UT, body, 0)
            for j in jms(u):
                for t in range(3):
                    idx = [divmod(t * 8 + v, 12) for v in range(8)]
                    blk = jnp.concatenate([vbuf[2 * u + hd, dt, j] for hd, dt in idx], axis=0)
                    blk = blk.astype(F32).T.astype(BF16)
                    for v, (hd, dt) in enumerate(idx):
                        vbuf[2 * u + hd, dt, j] = blk[v * 16:(v + 1) * 16]

        def st_pv(u, toks, tok_map):
            nm, sl = nmx(u), u % ns
            for piece in range(NPIECE):
                hd, half = divmod(piece, NPIECE // 2)
                sub = len(tok_map) // NPIECE
                lo = hi = None
                for j in range(nj):
                    if j in jms(u):
                        continue
                    row = 2 * (j // jq) + hd
                    cs = slice((j % jq) * 128, (j % jq + 1) * 128)
                    pb = jnp.broadcast_to(pbuf[u % 2][0, row:row + 1, cs], (8, 128))
                    k = piece * sub + j * sub // nj
                    ti = tok_map[k] if j % (nj // sub) == 0 else -1
                    if j > 0 and tok_map[k - 1] == ti:
                        ti = -1
                    if toks and ti >= 0:
                        pb = pb + toks[min(ti, len(toks) - 1)]
                    w = v32[2 * u + hd, pl.ds(half * 2, 2), j]
                    if j in jx:
                        a = vx[2 * u + hd, pl.ds(half * 2, 2), jx.index(j)] * pb
                        b = pltpu.bitcast(w, F32) * pb
                    else:
                        a = pltpu.bitcast(w << 16, F32) * pb
                        b = pltpu.bitcast(w & jnp.uint32(0xFFFF0000), F32) * pb
                    lo = a if lo is None else lo + a
                    hi = b if hi is None else hi + b
                for i in range(2):
                    base = (piece * 2 + i) * 16
                    abuf[sl, pl.ds(base, 8, stride=2), :] = lo[i]
                    abuf[sl, pl.ds(base + 1, 8, stride=2), :] = hi[i]

        def st_ored(u, ts=(0, 1, 2), partial_rows=False, pin=None):
            nm, sl = nmx(u), u % ns
            ia = lpart[sl] if u == NU - 1 else inv_l(lpart[sl])
            ib = pltpu.roll(ia, 1, 0)
            if partial_rows:
                even = lax.broadcasted_iota(jnp.int32, (8, 128), 0) % 2 == 0
                ia, ib = jnp.where(even, ia, ib), jnp.where(even, ib, ia)
            lane = lax.broadcasted_iota(jnp.int32, (8, 128), 1)
            for t in ts:
                at = abuf[sl, t * 128:(t + 1) * 128, :].T
                if pin is not None:
                    qlhs[9 + pin, :, 0:128] = pltpu.bitcast(at[120:128], U32)
                o = at[0:8]
                for i in range(1, 16):
                    o = o + at[i * 8:(i + 1) * 8]
                if nm:
                    sub = lax.broadcasted_iota(jnp.int32, (8, 128), 0)
                    odd = (0, (lane >= DH - 128).astype(jnp.int32), 1)[t]
                    keep = (sub >= 8 - 2 * nm) & (sub % 2 == odd)
                    o = o + jnp.where(keep, mbuf[sl, t], 0.0)
                if not partial_rows:
                    o = o + pltpu.roll(o, 4, 0)
                    o = o + pltpu.roll(o, 2, 0)
                    o = o + pltpu.roll(o, 1, 0)
                o = o * (ia, jnp.where(lane < DH - 128, ia, ib), ib)[t]
                olhs.at[u][:, t * 128:(t + 1) * 128] = pltpu.bitcast(_lhs(o), U32)

        def st_oproj(u, ts=(0, 1, 2), out=None):
            lhs = pltpu.bitcast(olhs[u], BF16)
            toks = []
            for t in ts:
                for n in range(D // 128):
                    if t == 1:
                        w32 = jnp.concatenate(
                            [wo32[2 * u, 8:12, n], wo32[2 * u + 1, 0:4, n]], axis=0)
                    else:
                        w32 = wo32[2 * u + t // 2, 2 * t:2 * t + 8, n]
                    r = _dot(lhs[:, t * 128:(t + 1) * 128], _as_bf16(w32))
                    toks.append(r[8:16])
                    if out is None:
                        gp[t, n, pl.ds(u, 1), :] = r[0:1]
                    else:
                        out[n].append(r[0:8])
            return toks

        def mlp(first, extra):
            g = gp[0] + gp[1] + gp[2]
            g = g[:, 0:8] + g[:, 8:16]
            g = jnp.concatenate([g[n] + extra[n][0] + extra[n][1] + extra[n][2]
                                 for n in range(D // 128)], axis=1)
            g = g + pltpu.roll(g, 4, 0)
            g = g + pltpu.roll(g, 2, 0)
            g = g + pltpu.roll(g, 1, 0)
            x1 = _round_bf16(xs[...] + g)
            lhs = _lhs(x1, 1.0)
            m1, r1 = _ln_stats(x1)
            y = (x1 - m1) * r1
            m2, r2 = _ln_stats(y)
            a = r1 * r2
            b = (m1 * r1 + m2) * r2
            hl = []
            for n in range(FF // 128):
                r = _dot(lhs, _as_bf16(w332[:, n]))
                hl.append(_lhs(jax.nn.gelu(r[0:8] * a - r[8:16] * b, approximate=True)))
            acc = x1 + y
            acc = [acc[:, c * 128:(c + 1) * 128] for c in range(D // 128)]
            for kt in range(FF // 128):
                if first and kt in w4_cuts:
                    wait(cps_w4(w4_cuts.index(kt)))
                for c in range(D // 128):
                    w = _as_bf16(w432[pl.ds(kt * 8, 8), c])
                    acc[c] = acc[c] + _dot(hl[kt], w)[0:8]
            xs[...] = _round_bf16(jnp.concatenate(acc, axis=1))

        gp[...] = jnp.zeros_like(gp)
        mbuf[...] = jnp.zeros_like(mbuf)
        wait(cps_x_wq())
        start(cps_wo())
        wait(cps_k(0, 0))
        start(cps_k(2, 0))
        wait(cps_k(1, 1))
        wait(cps_v(0, 0))
        xs[...] = jnp.broadcast_to(xin[...].astype(F32), (8, D))

        def layer(li, carry):
            first = li == 0
            n_first = jnp.maximum(1 - li, 0)
            zdyn = li >> 4

            def block_dma(ua, ub):
                def last_wait(t):
                    wait(cps_v(t + 1, (t + 1) % 2) if t + 1 < NU else cps_w3())

                def dma_ops(_, c):
                    for t in range(ua, ub):
                        if t + 3 < NU:
                            start(cps_k(t + 3, (t + 3) % 2))
                        if t + 2 < NU:
                            start(cps_v(t + 2, t % 2))
                        if t == NU - 2:
                            start(cps_w3())
                            for i in range(len(w4_cuts) - 1):
                                start(cps_w4(i))
                        if t == 1:
                            wait(cps_wo())
                        st_expand(t)
                        if t + 2 < NU:
                            wait(cps_k(t + 2, t % 2))
                        if t < ub - 1:
                            last_wait(t)
                    return c

                lax.fori_loop(0, n_first, dma_ops, 0)
                pl.when(first)(lambda: last_wait(ub - 1))

            def prologue():
                x = xs[...]
                m, r = _ln_stats(x)
                lhs = _lhs(x, 1.0)

                def q_direct(u):
                    qs = []
                    for nt in range(3):
                        qq = _dot(lhs, _as_bf16(wq32[:, u * 3 + nt]))
                        qs.append((qq[0:8] - qq[8:16] * m) * r)
                    pack_q(jnp.concatenate(qs, axis=1), u)

                q_direct(0)
                q_direct(1)
                un = (x - m) * r
                ulhs[...] = pltpu.bitcast(_lhs(un), U32)
                va = cfg["va_units"]
                f1, f2 = cfg["va_force"]
                toks = st_qk(0, range(f1 if va else nj))
                if va:
                    for kb in range(D // 128):
                        blk = jnp.broadcast_to(un[0:1, kb * 128:(kb + 1) * 128], (128, 128)).T
                        ucol[kb // 3][zdyn, (kb % 3) * 128:(kb % 3 + 1) * 128, :] = blk
                        qlhs[9 + zdyn, :, 0:128] = pltpu.bitcast(blk[120:128], U32)
                        if kb == 2:
                            toks += st_qk(0, range(f1, f2))
                    toks += st_qk(0, range(f2, nj))
                toks += st_qproj(2, zdyn)
                st_qpack(2)
                pos = js(1) - cfg["pvm_back0"]
                toks += st_qk(1, range(cfg["pin0"]))
                st_softmax(0, zdyn, pin=cfg["pin0"] > 0)
                toks += st_qk(1, range(cfg["pin0"], pos))
                toks += st_pvm(0)
                toks += st_qk(1, range(pos, js(1)))
                if va:
                    acc = [None] * len(va)
                    t0, t1 = cfg["va_tok"]
                    nkt = D // 16
                    for kt in range(nkt):
                        lo = ucol[kt // 24][0, pl.ds(kt % 24 * 16, 8, stride=2), :]
                        hi = ucol[kt // 24][0, pl.ds(kt % 24 * 16 + 1, 8, stride=2), :]
                        tk = toks[t0 + kt * (t1 - t0) // nkt]
                        lo, hi = lo + tk, hi + tk
                        for i, u in enumerate(va):
                            w = wq32[kt, u * 3:u * 3 + 3]
                            pr = (pltpu.bitcast(w << 16, F32) * lo
                                  + pltpu.bitcast(w & jnp.uint32(0xFFFF0000), F32) * hi)
                            acc[i] = pr if acc[i] is None else acc[i] + pr
                    for i, u in enumerate(va):
                        q = jnp.concatenate([acc[i][n] for n in range(3)], axis=1)
                        q = q + pltpu.roll(q, 4, 0)
                        q = q + pltpu.roll(q, 2, 0)
                        q = q + pltpu.roll(q, 1, 0)
                        pack_q(q, u)
                return toks

            def block(bi):
                ua, ub = cfg["blocks"][bi]
                block_dma(ua, ub)
                toks = []
                if bi == 0:
                    toks += prologue()
                done = js(ua + 1)
                for t in range(ua, ub):
                    base = len(toks)
                    ous = cfg["ored_at"].get(t, ())
                    if t in cfg["ored_pin"]:
                        for i, u in enumerate(ous):
                            nxt = nj - cfg["ored_back"] - (len(ous) - 1 - i) * 11
                            toks += st_qk(t + 1, range(done, nxt))
                            done = max(done, nxt)
                            st_ored(u, pin=zdyn)
                    else:
                        for u in ous:
                            st_ored(u)
                    if t + 1 < NU:
                        toks += st_qk(t + 1, range(done, nj))
                    g0 = len(toks)
                    if t == ua and bi > 0:
                        toks += st_pvm(t)
                    for u in cfg["qproj_at"].get(t, ()):
                        toks += st_qproj(u, zdyn)
                    for u in cfg["oproj_at"].get(t, ()):
                        toks += st_oproj(*u) if isinstance(u, tuple) else st_oproj(u)
                    done = js(t + 2)
                    if t + 1 < ub:
                        gap = cfg["gap_at"].get(t, cfg["gap"])
                        done = max(-((len(toks) - g0 - gap) // 3), 0)
                    gap1 = cfg["gap1_at"].get(t, cfg["gap1"])
                    d1 = min(max(-((len(toks) - g0 - gap1) // 3), 0), done)
                    if t + 2 < NU:
                        toks += st_qk(t + 2, range(d1))
                    if t + 1 < NU:
                        st_softmax(t + 1, zdyn, pin=gap1 > 0 and t + 2 < NU and d1 < done)
                    if t + 2 < NU:
                        toks += st_qk(t + 2, range(d1, done))
                    if t + 1 < ub:
                        toks += st_pvm(t + 1)
                    st_pv(t, toks, [base + i for i in cfg["tok"][t]])
                    st_lsum(t)
                    for u in cfg["qproj_at"].get(t, ()):
                        st_qpack(u)

            for bi in range(len(cfg["blocks"])):
                block(bi)

            def tail(first_static):
                for u in range(*cfg["blocks"][-1]):
                    st_ored(u, partial_rows=(u == NU - 1))
                seen = set()
                for us in cfg["oproj_at"].values():
                    for u in us:
                        uu, ts = u if isinstance(u, tuple) else (u, (0, 1, 2))
                        seen |= {(uu, t) for t in ts}
                for u in range(NU - 1):
                    ts = tuple(t for t in range(3) if (u, t) not in seen)
                    if ts:
                        st_oproj(u, ts)
                extra = [[] for _ in range(D // 128)]
                st_oproj(NU - 1, out=extra)
                mlp(first_static, extra)

            pl.when(first)(lambda: tail(True))
            pl.when(jnp.logical_not(first))(lambda: tail(False))
            return carry

        lax.fori_loop(0, 2, layer, 0)
        o_ref[...] = xs[0:1, :].astype(o_ref.dtype)

    return kernel


@jax.jit
def pallas_interleave_layers__sliding_block_cached__mixer_s_mlp__decode_kernel(
    A_x: jax.Array,
    A_k_cache: jax.Array,
    A_v_cache: jax.Array,
    A_wq: jax.Array,
    A_wo: jax.Array,
    B_x: jax.Array,
    B_w1: jax.Array,
    B_w2: jax.Array,
    B_w3: jax.Array,
    B_w4: jax.Array,
):
    b, sq, d = A_x.shape
    _, hkv, sk, dh = A_k_cache.shape
    assert (b, sq, d, hkv, dh) == (1, 1, D, H, DH)
    win = min(4096, max(256, sk // 4))
    assert win % 512 == 0 and sk % 128 == 0
    nj = win // 128

    kt = _tile_view(jnp.swapaxes(A_k_cache, 2, 3).reshape(H * DH, sk))
    vt = _head_view(jnp.swapaxes(A_v_cache, 2, 3).reshape(H * DH, sk))

    def buf(r, c):
        return pltpu.VMEM((r // 16, c // 128, 16, 128), BF16)

    def hbuf(c):
        return pltpu.VMEM((H, DH // 16, c // 128, 16, 128), BF16)

    bl = CFG["blocks"]
    ns = CFG.get("ns") or max(bl[i + 1][1] - bl[i][0] for i in range(len(bl) - 1))
    any_spec = pl.BlockSpec(memory_space=pl.ANY)
    out = pl.pallas_call(
        _make_kernel(sk, win, CFG),
        out_shape=jax.ShapeDtypeStruct((1, D), A_x.dtype),
        in_specs=[any_spec] * 7,
        out_specs=pl.BlockSpec(memory_space=pltpu.VMEM),
        scratch_shapes=[
            buf(H * DH, win), hbuf(win),
            pltpu.VMEM((H, DH // 16, max(len(CFG["jx"]), 1), 8, 128), F32),
            buf(D, H * DH), hbuf(D), buf(D, FF), buf(FF, D),
            pltpu.VMEM((1, D), BF16),
            pltpu.VMEM((8, D), F32),
            pltpu.VMEM((8, D), U32),
            pltpu.VMEM((1, D // 128, 8, 384), F32),
            pltpu.VMEM((1, D // 128, 8, 384), F32),
            pltpu.VMEM((10, 8, 384), U32),
            pltpu.VMEM((1, 384, 128), F32),
            pltpu.VMEM((1, 256, 128), F32),
            pltpu.VMEM((2, 8, win // 4), F32),
            pltpu.VMEM((2, 8, win // 4), F32),
            pltpu.VMEM((1, 8, win // 4), F32),
            pltpu.VMEM((1, 8, win // 4), F32),
            pltpu.VMEM((8, 256), U32),
            pltpu.VMEM((ns, 3, 8, 128), F32),
            pltpu.VMEM((ns, 8, 128), F32),
            pltpu.VMEM((ns, 384, 128), F32),
            pltpu.VMEM((NU, 8, 384), U32),
            pltpu.VMEM((3, D // 128, NU, 128), F32),
            pltpu.SemaphoreType.DMA((5,)),
        ],
        compiler_params=pltpu.CompilerParams(vmem_limit_bytes=int(CFG["vmem_mb"] * 1024 * 1024)),
        name="interleave_decode",
    )(A_x.reshape(1, D), kt, vt, _tile_view(A_wq), _head_view(A_wo),
      _tile_view(B_w3), _tile_view(B_w4))
    return out.reshape(b, sq, d)
```

```python
import jax
import jax.numpy as jnp
from jax import lax
import jax.experimental.pallas as pl
import jax.experimental.pallas.tpu as pltpu

F32 = jnp.float32
BF16 = jnp.bfloat16
U32 = jnp.uint32

D = 640
H = 32
DH = 192
FF = 1536
NU = H // 2
UT = 2 * DH // 16
EPS = 1e-5
NPIECE = 12

CFG = dict(
    blocks=((0, 4), (4, 8), (8, 12), (12, 15), (15, 16)), ns=7,
    jsplit=8, js_at={},
    gap=49, gap1=24, gap_at={0: 44, 1: 44, 2: 44}, gap1_at={0: 0, 1: 0, 2: 0, 3: 0}, ored_pin=(), ored_back=4, pvm_back0=0, pin0=0,
    nm=3, nm_at={0: 2, 4: 2},
    va_units=(6, 7, 8, 9), va_force=(7, 16), va_tok=(12, 108),
    qproj_at={0: (3,), 1: (4,), 2: (5,), 3: (10,), 5: (11,), 6: (12,), 7: (13,), 10: (14,), 11: (15,)},
    ored_at={4: (0,), 5: (1,), 6: (2,), 7: (3,), 8: (4,), 9: (5,), 10: (6,), 11: (7,),
             12: (8,), 13: (9, 10), 14: (11,), 15: (12, 13, 14)},
    oproj_at={4: ((0, (2,)),), 5: ((1, (2,)),), 6: ((2, (2,)),), 7: ((3, (2,)),),
              8: ((4, (2,)), (0, (0,))), 9: ((5, (2,)), (0, (1,))), 10: ((6, (2,)),), 11: ((7, (2,)),),
              12: ((8, (2,)),), 13: ((9, (2,)), (10, (2,)), (4, (0, 1))),
              14: ((11, (2,)), (1, (0, 1)), (2, (0, 1)), (3, (0, 1))),
              15: ((5, (0, 1)), (6, (0, 1)), (7, (0, 1)), (8, (0, 1)), (9, (0, 1)),
                   (10, (0, 1)), (11, (0, 1)), 12, (13, (0, 1)))},
    jx=(1, 5, 9, 13, 17, 21, 25), vmem_mb=128,
    tok={
        0: [-22,-18,-17,-15,-13,-10,-8,-5,-3,-1,-1,4,7,9,12,14,16,19,22,24,27,27,33,35,37,40,43,45,48,50,53,55,56,58,64,67,69,74,75,78,80,83,86,89,91,94,96,97],
        1: [-24,-21,-19,-17,-14,-12,-12,-7,-5,-2,0,3,5,7,10,12,15,17,20,22,25,28,30,33,34,37,39,42,45,47,51,53,56,59,61,64,68,69,72,75,77,80,83,85,88,91,93,96],
        2: [-21,-19,-16,-12,-11,-9,-7,-4,-2,0,3,5,8,10,12,15,17,20,22,25,28,30,33,36,38,41,43,45,49,51,54,56,59,62,64,67,69,72,74,74,79,82,84,86,86,93,94,96],
        3: [-21,-19,-16,-14,-11,-9,-6,-4,1,5,5,7,9,12,14,17,18,21,24,26,29,32,34,35,40,42,42,47,50,53,54,57,60,62,65,68,70,72,77,79,80,82,84,86,89,91,96,96],
        4: [-25,-22,-22,-20,-15,-13,-10,-8,-4,-2,-1,0,3,5,7,9,11,14,17,19,22,25,28,31,34,37,40,43,46,49,51,54,57,60,63,66,69,71,74,77,80,83,85,88,91,94,97,100],
        5: [-28,-26,-24,-21,-19,-17,-14,-12,-10,-8,-5,-3,0,2,5,7,9,12,15,17,20,23,25,28,31,33,35,38,40,43,45,46,50,52,55,58,60,63,65,68,70,73,76,78,81,83,86,89],
        6: [-25,-22,-19,-16,-14,-11,-8,-5,-3,0,3,6,9,11,14,17,20,22,25,27,30,33,35,38,39,43,46,48,51,53,56,59,61,64,67,70,73,75,78,81,84,86,88,90,93,95,97,99],
        7: [-24,-21,-19,-16,-13,-11,-8,-5,-3,0,3,5,8,11,13,16,19,21,26,27,29,31,34,37,39,42,45,48,50,53,56,59,61,64,68,71,74,77,80,84,87,89,91,93,95,97,99,101],
        8: [-26,-24,-22,-19,-17,-15,-12,-10,-8,-5,-3,-1,1,4,6,8,11,14,16,19,22,25,28,31,34,36,39,42,45,48,51,54,57,59,59,66,68,71,73,75,78,81,83,86,89,91,94,102],
        9: [-31,-28,-26,-23,-21,-18,-16,-14,-11,-9,-6,-4,-1,1,3,6,6,11,14,16,19,22,24,27,30,32,35,37,40,43,45,48,52,53,56,56,58,59,66,69,71,74,77,79,82,84,87,89],
        10: [-32,-29,-27,-24,-24,-21,-19,-16,-14,-9,-7,-4,-2,1,5,8,10,13,16,16,19,21,24,27,29,32,35,38,40,43,46,48,51,54,56,59,62,64,67,68,72,75,77,80,83,85,88,91],
        11: [-23,-20,-18,-15,-13,-10,-8,-5,-2,1,3,6,9,9,14,16,19,20,23,26,29,31,33,37,39,42,45,48,50,53,56,58,61,64,67,69,72,72,79,82,85,87,90,93,96,99,102,105],
        12: [-20,-18,-16,-14,-10,-8,-7,-3,-2,-1,-1,1,3,5,7,9,11,14,16,19,22,24,27,30,32,33,35,38,43,46,48,51,54,57,60,63,66,69,72,75,78,81,83,86,89,89,95,97],
        13: [-31,-28,-26,-21,-21,-19,-16,-13,-11,-8,-4,-2,1,4,6,9,12,14,17,19,22,24,27,29,32,34,37,40,42,46,47,50,53,55,58,61,64,64,70,72,75,77,80,82,84,87,89,91],
        14: [-25,-23,-20,-18,-15,-13,-10,-8,-5,-2,1,3,6,11,12,13,16,18,21,24,26,28,31,33,36,38,41,44,46,49,52,54,55,58,62,65,68,70,73,76,78,81,84,86,89,92,95,97],
        15: [-53,-52,-51,-48,-28,-20,-19,-19,-16,-14,-7,-7,-2,1,7,7,8,13,13,17,22,23,25,31,35,39,41,41,46,46,47,48,54,59,59,60,67,67,69,69,81,85,85,85,85,85,92,92],
    },
    w4_cuts=(9, 11))


def _tile_view(a):
    r, c = a.shape
    a = a.reshape(r // 16, 2, 8, c // 128, 128)
    return jnp.swapaxes(a, 2, 3)


def _head_view(a):
    c = a.shape[1]
    a = a.reshape(H, 2, DH // 16, 8, c // 128, 128)
    return jnp.swapaxes(a, 3, 4)


def _as_bf16(w32):
    n = w32.shape[0]
    return pltpu.bitcast(w32.reshape(n * 8, 128), BF16)


def _lhs(top, fill=0.0):
    return jnp.concatenate([top, jnp.full(top.shape, fill, F32)], axis=0).astype(BF16)


def _ln_stats(x):
    m = jnp.mean(x, axis=-1, keepdims=True)
    m2 = jnp.mean(x * x, axis=-1, keepdims=True)
    v = jnp.maximum(m2 - m * m, 0.0)
    return m, lax.rsqrt(v + EPS)


def _round_bf16(x):
    return x.astype(BF16).astype(F32)


def _dot(a, b):
    return jnp.dot(a, b, preferred_element_type=F32)


def _make_kernel(sk, win, cfg):
    nj = win // 128
    j0 = (sk - win) // 128
    jq = nj // 4
    jx = list(cfg["jx"])
    assert nj == 32 and cfg["blocks"][-2][0] <= NU - 3 and cfg["blocks"][-1] == (NU - 1, NU)
    qscale = DH ** -0.5 * 1.4426950408889634

    def kernel(x_hbm, k_hbm, v_hbm, wq_hbm, wo_hbm, w3_hbm, w4_hbm, o_ref,
               kbuf, vbuf, vx, wqbuf, wobuf, w3buf, w4buf, xin,
               xs, ulhs, qp0, qp1, qlhs, ucol0, ucol1, sx, sy, pbuf0, pbuf1, plhs, mbuf, lpart, abuf, olhs, gp,
               sems):
        qp = (qp0, qp1)
        ucol = (ucol0, ucol1)
        pbuf = (pbuf0, pbuf1)
        ns = abuf.shape[0]


        def cps_w(hbm, buf, sem, lo=0, n=None):
            n = buf.shape[0] if n is None else n
            return [pltpu.make_async_copy(
                hbm.at[pl.ds(lo, n), e],
                buf.at[pl.ds(lo, n), :, pl.ds(e * 8, 8), :],
                sems.at[sem]) for e in range(2)]

        def cps_kv(hbm, buf, sem, u):
            return [pltpu.make_async_copy(
                hbm.at[pl.ds(u * UT, UT), e, pl.ds(j0, nj)],
                buf.at[pl.ds(u * UT, UT), :, pl.ds(e * 8, 8), :],
                sems.at[sem]) for e in range(2)]

        def cps_v(u, par):
            return [pltpu.make_async_copy(
                v_hbm.at[pl.ds(2 * u, 2), e, :, pl.ds(j0, nj)],
                vbuf.at[pl.ds(2 * u, 2), :, :, pl.ds(e * 8, 8), :],
                sems.at[2 + par]) for e in range(2)]

        def cps_wo():
            return [pltpu.make_async_copy(
                wo_hbm.at[:, e], wobuf.at[:, :, :, pl.ds(e * 8, 8), :],
                sems.at[4]) for e in range(2)]

        cps_k = lambda u, par: cps_kv(k_hbm, kbuf, par, u)
        cps_x_wq = lambda: cps_w(wq_hbm, wqbuf, 4) + [pltpu.make_async_copy(x_hbm, xin, sems.at[4])]
        cps_w3 = lambda: cps_w(w3_hbm, w3buf, 0)
        w4_cuts = (0,) + tuple(cfg["w4_cuts"]) + (FF // 128,)
        cps_w4 = lambda i: cps_w(w4_hbm, w4buf, (4, 2, 1)[i], w4_cuts[i] * 8,
                                 (w4_cuts[i + 1] - w4_cuts[i]) * 8)

        def start(cps):
            for c in cps:
                c.start()

        def wait(cps):
            for c in cps:
                c.wait()

        start(cps_x_wq())
        start(cps_k(0, 0))
        start(cps_k(1, 1))
        start(cps_v(0, 0))
        start(cps_v(1, 1))

        k32 = kbuf.bitcast(U32)
        v32 = vbuf.bitcast(U32)
        wq32 = wqbuf.bitcast(U32)
        wo32 = wobuf.bitcast(U32)
        w332 = w3buf.bitcast(U32)
        w432 = w4buf.bitcast(U32)

        def js(u):
            return cfg["js_at"].get(u, cfg["jsplit"])

        def qslot(u):
            va = cfg["va_units"]
            return 4 + va.index(u) if u in va else u % 4

        def jms(u):
            return [nj - 1 - jq * i for i in range(nmx(u))]

        def nmx(u):
            return cfg["nm_at"].get(u, cfg["nm"])

        def st_qproj(u, zdyn):
            lhs = pltpu.bitcast(ulhs[...], BF16)
            toks = []
            for kt in range(D // 128):
                for nt in range(3):
                    w = _as_bf16(wq32[pl.ds(kt * 8, 8), u * 3 + nt])
                    r = _dot(lhs[:, kt * 128:(kt + 1) * 128], w)
                    toks.append(r[8:16])
                    qp[u % 2][zdyn, kt, :, nt * 128:(nt + 1) * 128] = r[0:8]
            return toks

        def pack_q(q, u):
            q = q * qscale
            lane = lax.broadcasted_iota(jnp.int32, (8, 128), 1)
            sub = lax.broadcasted_iota(jnp.int32, (8, 128), 0)
            keep = (lane < DH - 128) == (sub % 2 == 0)
            q = jnp.concatenate(
                [q[:, 0:128], jnp.where(keep, q[:, 128:256], 0.0), q[:, 256:384]], axis=1)
            qlhs.at[qslot(u)][:, 0:384] = pltpu.bitcast(_lhs(q), U32)

        def st_qpack(u):
            q = qp[u % 2][0, 0]
            for kt in range(1, D // 128):
                q = q + qp[u % 2][0, kt]
            pack_q(q, u)

        def st_qk(u, js):
            sl = u % 2
            lhs = pltpu.bitcast(qlhs[qslot(u)], BF16)
            toks = []
            for j in js:
                ra = 2 * (j // jq)
                cs = slice((j % jq) * 128, (j % jq + 1) * 128)
                for t in range(3):
                    w = _as_bf16(k32[pl.ds(u * UT + t * 8, 8), j])
                    r = _dot(lhs[:, t * 128:(t + 1) * 128], w)
                    toks.append(r[8:16])
                    if t == 0:
                        sx[sl, ra:ra + 1, cs] = r[0:1]
                    elif t == 1:
                        sy[sl, ra:ra + 2, cs] = r[ra:ra + 2]
                    else:
                        sx[sl, ra + 1:ra + 2, cs] = r[0:1]
            return toks

        def st_softmax(u, zdyn, pin=False):
            sl = u % 2
            s = sx[sl] + sy[sl]
            m = s
            while m.shape[1] > 128:
                h = m.shape[1] // 2
                m = jnp.maximum(m[:, :h], m[:, h:])
            m = jnp.maximum(m, pltpu.roll(m, 2, 0))
            m = jnp.maximum(m, pltpu.roll(m, 4, 0))
            if pin:
                qlhs[9 + zdyn, :, 0:128] = pltpu.bitcast(m, U32)
            m = jnp.max(m, axis=1, keepdims=True)
            p = jnp.exp2(s - m)
            pbuf[sl][zdyn] = p
            if nmx(u):
                plhs[:, sl * 128:(sl + 1) * 128] = pltpu.bitcast(_lhs(p[:, (jq - 1) * 128:jq * 128]), U32)

        def inv_l(l):
            l = jnp.sum(l, axis=1, keepdims=True)
            r0 = pl.reciprocal(l, approx=True)
            return jnp.broadcast_to(r0 * (2.0 - l * r0), (8, 128))

        def st_lsum(u):
            l = pbuf[u % 2][0, :, 0:128]
            for c in range(1, jq):
                l = l + pbuf[u % 2][0, :, c * 128:(c + 1) * 128]
            l = l + pltpu.roll(l, 2, 0)
            l = l + pltpu.roll(l, 4, 0)
            lpart[u % ns] = inv_l(l) if u == NU - 1 else l

        def st_pvm(u):
            toks = []
            for j in jms(u):
                lhs = pltpu.bitcast(plhs[:, u % 2 * 128:(u % 2 + 1) * 128], BF16)
                ra = 2 * (j // jq)
                for t in range(3):
                    if t == 1:
                        w32 = jnp.concatenate(
                            [v32[2 * u, 8:12, j], v32[2 * u + 1, 0:4, j]], axis=0)
                    else:
                        w32 = v32[2 * u + t // 2, 2 * t:2 * t + 8, j]
                    r = _dot(lhs, _as_bf16(w32))
                    toks.append(r[8:16])
                    mbuf[u % ns, t, ra:ra + 2, :] = r[ra:ra + 2]
            return toks

        def st_expand(u):
            def body(i, c):
                hd, dt = i // 12, i % 12
                for ix, j in enumerate(jx):
                    w = v32[2 * u + hd, dt, j]
                    vx[2 * u + hd, dt, ix] = pltpu.bitcast(w << 16, F32)
                    vbuf[2 * u + hd, dt, j] = pltpu.bitcast(w & jnp.uint32(0xFFFF0000), BF16)
                return c
            if jx:
                lax.fori_loop(0, UT, body, 0)
            for j in jms(u):
                for t in range(3):
                    idx = [divmod(t * 8 + v, 12) for v in range(8)]
                    blk = jnp.concatenate([vbuf[2 * u + hd, dt, j] for hd, dt in idx], axis=0)
                    blk = blk.astype(F32).T.astype(BF16)
                    for v, (hd, dt) in enumerate(idx):
                        vbuf[2 * u + hd, dt, j] = blk[v * 16:(v + 1) * 16]

        def st_pv(u, toks, tok_map):
            nm, sl = nmx(u), u % ns
            for piece in range(NPIECE):
                hd, half = divmod(piece, NPIECE // 2)
                sub = len(tok_map) // NPIECE
                lo = hi = None
                for j in range(nj):
                    if j in jms(u):
                        continue
                    row = 2 * (j // jq) + hd
                    cs = slice((j % jq) * 128, (j % jq + 1) * 128)
                    pb = jnp.broadcast_to(pbuf[u % 2][0, row:row + 1, cs], (8, 128))
                    k = piece * sub + j * sub // nj
                    ti = tok_map[k] if j % (nj // sub) == 0 else -1
                    if j > 0 and tok_map[k - 1] == ti:
                        ti = -1
                    if toks and ti >= 0:
                        pb = pb + toks[min(ti, len(toks) - 1)]
                    w = v32[2 * u + hd, pl.ds(half * 2, 2), j]
                    if j in jx:
                        a = vx[2 * u + hd, pl.ds(half * 2, 2), jx.index(j)] * pb
                        b = pltpu.bitcast(w, F32) * pb
                    else:
                        a = pltpu.bitcast(w << 16, F32) * pb
                        b = pltpu.bitcast(w & jnp.uint32(0xFFFF0000), F32) * pb
                    lo = a if lo is None else lo + a
                    hi = b if hi is None else hi + b
                for i in range(2):
                    base = (piece * 2 + i) * 16
                    abuf[sl, pl.ds(base, 8, stride=2), :] = lo[i]
                    abuf[sl, pl.ds(base + 1, 8, stride=2), :] = hi[i]

        def st_ored(u, ts=(0, 1, 2), partial_rows=False, pin=None):
            nm, sl = nmx(u), u % ns
            ia = lpart[sl] if u == NU - 1 else inv_l(lpart[sl])
            ib = pltpu.roll(ia, 1, 0)
            if partial_rows:
                even = lax.broadcasted_iota(jnp.int32, (8, 128), 0) % 2 == 0
                ia, ib = jnp.where(even, ia, ib), jnp.where(even, ib, ia)
            lane = lax.broadcasted_iota(jnp.int32, (8, 128), 1)
            for t in ts:
                at = abuf[sl, t * 128:(t + 1) * 128, :].T
                if pin is not None:
                    qlhs[9 + pin, :, 0:128] = pltpu.bitcast(at[120:128], U32)
                o = at[0:8]
                for i in range(1, 16):
                    o = o + at[i * 8:(i + 1) * 8]
                if nm:
                    sub = lax.broadcasted_iota(jnp.int32, (8, 128), 0)
                    odd = (0, (lane >= DH - 128).astype(jnp.int32), 1)[t]
                    keep = (sub >= 8 - 2 * nm) & (sub % 2 == odd)
                    o = o + jnp.where(keep, mbuf[sl, t], 0.0)
                if not partial_rows:
                    o = o + pltpu.roll(o, 4, 0)
                    o = o + pltpu.roll(o, 2, 0)
                    o = o + pltpu.roll(o, 1, 0)
                o = o * (ia, jnp.where(lane < DH - 128, ia, ib), ib)[t]
                olhs.at[u][:, t * 128:(t + 1) * 128] = pltpu.bitcast(_lhs(o), U32)

        def st_oproj(u, ts=(0, 1, 2), out=None):
            lhs = pltpu.bitcast(olhs[u], BF16)
            toks = []
            for t in ts:
                for n in range(D // 128):
                    if t == 1:
                        w32 = jnp.concatenate(
                            [wo32[2 * u, 8:12, n], wo32[2 * u + 1, 0:4, n]], axis=0)
                    else:
                        w32 = wo32[2 * u + t // 2, 2 * t:2 * t + 8, n]
                    r = _dot(lhs[:, t * 128:(t + 1) * 128], _as_bf16(w32))
                    toks.append(r[8:16])
                    if out is None:
                        gp[t, n, pl.ds(u, 1), :] = r[0:1]
                    else:
                        out[n].append(r[0:8])
            return toks

        def mlp(first, extra):
            g = gp[0] + gp[1] + gp[2]
            g = g[:, 0:8] + g[:, 8:16]
            g = jnp.concatenate([g[n] + extra[n][0] + extra[n][1] + extra[n][2]
                                 for n in range(D // 128)], axis=1)
            g = g + pltpu.roll(g, 4, 0)
            g = g + pltpu.roll(g, 2, 0)
            g = g + pltpu.roll(g, 1, 0)
            x1 = _round_bf16(xs[...] + g)
            lhs = _lhs(x1, 1.0)
            m1, r1 = _ln_stats(x1)
            y = (x1 - m1) * r1
            m2, r2 = _ln_stats(y)
            a = r1 * r2
            b = (m1 * r1 + m2) * r2
            hl = []
            for n in range(FF // 128):
                r = _dot(lhs, _as_bf16(w332[:, n]))
                hn = jax.nn.gelu(r[0:8] * a - r[8:16] * b, approximate=True)
                hl.append(_lhs(hn))
            if first:
                ucol0[0, 0:128, :] = jnp.broadcast_to(_round_bf16(hn[0:1]), (128, 128)).T
            acc = x1 + y
            acc = [acc[:, c * 128:(c + 1) * 128] for c in range(D // 128)]
            for kt in range(FF // 128):
                if first and kt in w4_cuts:
                    wait(cps_w4(w4_cuts.index(kt)))
                if first and kt == FF // 128 - 1:
                    pa = None
                    for dt in range(8):
                        w = w432[kt * 8 + dt]
                        pr = (pltpu.bitcast(w << 16, F32) * ucol0[0, pl.ds(dt * 16, 8, stride=2), :]
                              + pltpu.bitcast(w & jnp.uint32(0xFFFF0000), F32)
                              * ucol0[0, pl.ds(dt * 16 + 1, 8, stride=2), :])
                        pa = pr if pa is None else pa + pr
                    for c in range(D // 128):
                        pc = pa[c]
                        pc = pc + pltpu.roll(pc, 4, 0)
                        pc = pc + pltpu.roll(pc, 2, 0)
                        acc[c] = acc[c] + (pc + pltpu.roll(pc, 1, 0))
                    continue
                for c in range(D // 128):
                    w = _as_bf16(w432[pl.ds(kt * 8, 8), c])
                    acc[c] = acc[c] + _dot(hl[kt], w)[0:8]
            xs[...] = _round_bf16(jnp.concatenate(acc, axis=1))

        gp[...] = jnp.zeros_like(gp)
        mbuf[...] = jnp.zeros_like(mbuf)
        wait(cps_x_wq())
        start(cps_wo())
        wait(cps_k(0, 0))
        start(cps_k(2, 0))
        wait(cps_k(1, 1))
        wait(cps_v(0, 0))
        xs[...] = jnp.broadcast_to(xin[...].astype(F32), (8, D))

        def layer(li, carry):
            first = li == 0
            n_first = jnp.maximum(1 - li, 0)
            zdyn = li >> 4

            def block_dma(ua, ub):
                def last_wait(t):
                    if t == NU - 2:
                        wait(cps_k(NU - 1, (NU - 1) % 2))
                    else:
                        wait(cps_v(t + 1, (t + 1) % 2) if t + 1 < NU else cps_w3())

                def dma_ops(_, c):
                    for t in range(ua, ub):
                        if t + 3 < NU:
                            start(cps_k(t + 3, (t + 3) % 2))
                        if t + 2 < NU:
                            start(cps_v(t + 2, t % 2))
                        if t == NU - 2:
                            start(cps_w3())
                            start(cps_w4(0))
                            start(cps_w4(1))
                        if t == NU - 1:
                            start(cps_w4(2))
                            wait(cps_v(t, t % 2))
                        if t == 1:
                            wait(cps_wo())
                        st_expand(t)
                        if t + 2 < NU - 1:
                            wait(cps_k(t + 2, t % 2))
                        if t < ub - 1:
                            last_wait(t)
                    return c

                lax.fori_loop(0, n_first, dma_ops, 0)
                pl.when(first)(lambda: last_wait(ub - 1))

            def prologue():
                x = xs[...]
                m, r = _ln_stats(x)
                lhs = _lhs(x, 1.0)

                def q_direct(u):
                    qs = []
                    for nt in range(3):
                        qq = _dot(lhs, _as_bf16(wq32[:, u * 3 + nt]))
                        qs.append((qq[0:8] - qq[8:16] * m) * r)
                    pack_q(jnp.concatenate(qs, axis=1), u)

                q_direct(0)
                q_direct(1)
                un = (x - m) * r
                ulhs[...] = pltpu.bitcast(_lhs(un), U32)
                va = cfg["va_units"]
                f1, f2 = cfg["va_force"]
                toks = st_qk(0, range(f1 if va else nj))
                if va:
                    for kb in range(D // 128):
                        blk = jnp.broadcast_to(un[0:1, kb * 128:(kb + 1) * 128], (128, 128)).T
                        ucol[kb // 3][zdyn, (kb % 3) * 128:(kb % 3 + 1) * 128, :] = blk
                        qlhs[9 + zdyn, :, 0:128] = pltpu.bitcast(blk[120:128], U32)
                        if kb == 2:
                            toks += st_qk(0, range(f1, f2))
                    toks += st_qk(0, range(f2, nj))
                toks += st_qproj(2, zdyn)
                st_qpack(2)
                pos = js(1) - cfg["pvm_back0"]
                toks += st_qk(1, range(cfg["pin0"]))
                st_softmax(0, zdyn, pin=cfg["pin0"] > 0)
                toks += st_qk(1, range(cfg["pin0"], pos))
                toks += st_pvm(0)
                toks += st_qk(1, range(pos, js(1)))
                if va:
                    acc = [None] * len(va)
                    t0, t1 = cfg["va_tok"]
                    nkt = D // 16
                    for kt in range(nkt):
                        lo = ucol[kt // 24][0, pl.ds(kt % 24 * 16, 8, stride=2), :]
                        hi = ucol[kt // 24][0, pl.ds(kt % 24 * 16 + 1, 8, stride=2), :]
                        tk = toks[t0 + kt * (t1 - t0) // nkt]
                        lo, hi = lo + tk, hi + tk
                        for i, u in enumerate(va):
                            w = wq32[kt, u * 3:u * 3 + 3]
                            pr = (pltpu.bitcast(w << 16, F32) * lo
                                  + pltpu.bitcast(w & jnp.uint32(0xFFFF0000), F32) * hi)
                            acc[i] = pr if acc[i] is None else acc[i] + pr
                    for i, u in enumerate(va):
                        q = jnp.concatenate([acc[i][n] for n in range(3)], axis=1)
                        q = q + pltpu.roll(q, 4, 0)
                        q = q + pltpu.roll(q, 2, 0)
                        q = q + pltpu.roll(q, 1, 0)
                        pack_q(q, u)
                return toks

            def block(bi):
                ua, ub = cfg["blocks"][bi]
                block_dma(ua, ub)
                toks = []
                if bi == 0:
                    toks += prologue()
                done = js(ua + 1)
                for t in range(ua, ub):
                    base = len(toks)
                    ous = cfg["ored_at"].get(t, ())
                    if t in cfg["ored_pin"]:
                        for i, u in enumerate(ous):
                            nxt = nj - cfg["ored_back"] - (len(ous) - 1 - i) * 11
                            toks += st_qk(t + 1, range(done, nxt))
                            done = max(done, nxt)
                            st_ored(u, pin=zdyn)
                    else:
                        for u in ous:
                            st_ored(u)
                    if t + 1 < NU:
                        toks += st_qk(t + 1, range(done, nj))
                    g0 = len(toks)
                    if t == ua and bi > 0:
                        toks += st_pvm(t)
                    for u in cfg["qproj_at"].get(t, ()):
                        toks += st_qproj(u, zdyn)
                    for u in cfg["oproj_at"].get(t, ()):
                        toks += st_oproj(*u) if isinstance(u, tuple) else st_oproj(u)
                    done = js(t + 2)
                    if t + 1 < ub:
                        gap = cfg["gap_at"].get(t, cfg["gap"])
                        done = max(-((len(toks) - g0 - gap) // 3), 0)
                    gap1 = cfg["gap1_at"].get(t, cfg["gap1"])
                    d1 = min(max(-((len(toks) - g0 - gap1) // 3), 0), done)
                    if t + 2 < NU:
                        toks += st_qk(t + 2, range(d1))
                    if t + 1 < NU:
                        st_softmax(t + 1, zdyn, pin=gap1 > 0 and t + 2 < NU and d1 < done)
                    if t + 2 < NU:
                        toks += st_qk(t + 2, range(d1, done))
                    if t + 1 < ub:
                        toks += st_pvm(t + 1)
                    st_pv(t, toks, [base + i for i in cfg["tok"][t]])
                    st_lsum(t)
                    for u in cfg["qproj_at"].get(t, ()):
                        st_qpack(u)

            for bi in range(len(cfg["blocks"])):
                block(bi)

            def tail(first_static):
                for u in range(*cfg["blocks"][-1]):
                    st_ored(u, partial_rows=(u == NU - 1))
                seen = set()
                for us in cfg["oproj_at"].values():
                    for u in us:
                        uu, ts = u if isinstance(u, tuple) else (u, (0, 1, 2))
                        seen |= {(uu, t) for t in ts}
                for u in range(NU - 1):
                    ts = tuple(t for t in range(3) if (u, t) not in seen)
                    if ts:
                        st_oproj(u, ts)
                extra = [[] for _ in range(D // 128)]
                st_oproj(NU - 1, out=extra)
                mlp(first_static, extra)

            pl.when(first)(lambda: tail(True))
            pl.when(jnp.logical_not(first))(lambda: tail(False))
            return carry

        lax.fori_loop(0, 2, layer, 0)
        o_ref[...] = xs[0:1, :].astype(o_ref.dtype)

    return kernel


@jax.jit
def pallas_interleave_layers__sliding_block_cached__mixer_s_mlp__decode_kernel(
    A_x: jax.Array,
    A_k_cache: jax.Array,
    A_v_cache: jax.Array,
    A_wq: jax.Array,
    A_wo: jax.Array,
    B_x: jax.Array,
    B_w1: jax.Array,
    B_w2: jax.Array,
    B_w3: jax.Array,
    B_w4: jax.Array,
):
    b, sq, d = A_x.shape
    _, hkv, sk, dh = A_k_cache.shape
    assert (b, sq, d, hkv, dh) == (1, 1, D, H, DH)
    win = min(4096, max(256, sk // 4))
    assert win % 512 == 0 and sk % 128 == 0
    nj = win // 128

    kt = _tile_view(jnp.swapaxes(A_k_cache, 2, 3).reshape(H * DH, sk))
    vt = _head_view(jnp.swapaxes(A_v_cache, 2, 3).reshape(H * DH, sk))

    def buf(r, c):
        return pltpu.VMEM((r // 16, c // 128, 16, 128), BF16)

    def hbuf(c):
        return pltpu.VMEM((H, DH // 16, c // 128, 16, 128), BF16)

    bl = CFG["blocks"]
    ns = CFG.get("ns") or max(bl[i + 1][1] - bl[i][0] for i in range(len(bl) - 1))
    any_spec = pl.BlockSpec(memory_space=pl.ANY)
    out = pl.pallas_call(
        _make_kernel(sk, win, CFG),
        out_shape=jax.ShapeDtypeStruct((1, D), A_x.dtype),
        in_specs=[any_spec] * 7,
        out_specs=pl.BlockSpec(memory_space=pltpu.VMEM),
        scratch_shapes=[
            buf(H * DH, win), hbuf(win),
            pltpu.VMEM((H, DH // 16, max(len(CFG["jx"]), 1), 8, 128), F32),
            buf(D, H * DH), hbuf(D), buf(D, FF), buf(FF, D),
            pltpu.VMEM((1, D), BF16),
            pltpu.VMEM((8, D), F32),
            pltpu.VMEM((8, D), U32),
            pltpu.VMEM((1, D // 128, 8, 384), F32),
            pltpu.VMEM((1, D // 128, 8, 384), F32),
            pltpu.VMEM((10, 8, 384), U32),
            pltpu.VMEM((1, 384, 128), F32),
            pltpu.VMEM((1, 256, 128), F32),
            pltpu.VMEM((2, 8, win // 4), F32),
            pltpu.VMEM((2, 8, win // 4), F32),
            pltpu.VMEM((1, 8, win // 4), F32),
            pltpu.VMEM((1, 8, win // 4), F32),
            pltpu.VMEM((8, 256), U32),
            pltpu.VMEM((ns, 3, 8, 128), F32),
            pltpu.VMEM((ns, 8, 128), F32),
            pltpu.VMEM((ns, 384, 128), F32),
            pltpu.VMEM((NU, 8, 384), U32),
            pltpu.VMEM((3, D // 128, NU, 128), F32),
            pltpu.SemaphoreType.DMA((5,)),
        ],
        compiler_params=pltpu.CompilerParams(vmem_limit_bytes=int(CFG["vmem_mb"] * 1024 * 1024)),
        name="interleave_decode",
    )(A_x.reshape(1, D), kt, vt, _tile_view(A_wq), _head_view(A_wo),
      _tile_view(B_w3), _tile_view(B_w4))
    return out.reshape(b, sq, d)
```

```python
import jax
import jax.numpy as jnp
from jax import lax
import jax.experimental.pallas as pl
import jax.experimental.pallas.tpu as pltpu

F32 = jnp.float32
BF16 = jnp.bfloat16
U32 = jnp.uint32

D = 640
H = 32
DH = 192
FF = 1536
NU = H // 2
UT = 2 * DH // 16
EPS = 1e-5
NPIECE = 12

CFG = dict(
    blocks=((0, 4), (4, 8), (8, 12), (12, 15), (15, 16)), ns=7,
    jsplit=10, js_at={1: 13, 5: 19, 9: 19, 13: 16},
    gap=49, gap1=24, gap_at={}, gap1_at={}, ored_pin=(), ored_back=4,
    nm=4, nm_at={15: 3},
    va_groups=((6, 7, 8, 9), (10, 11, 12, 13, 14), (15,)), va_force=7,
    va_tok=((6, 43), (48, 94), (102, 112)),
    ored_at={4: (0,), 5: (1,), 6: (2,), 7: (3,), 8: (4,), 9: (5,), 10: (6,), 11: (7,),
             12: (8,), 13: (9, 10), 14: (11,), 15: (12, 13, 14)},
    oproj_at={4: ((0, (2,)),), 5: ((1, (2,)),), 6: ((2, (2,)),), 7: ((3, (2,)),),
              8: ((4, (2,)), (0, (0,))), 9: ((5, (2,)), (0, (1,))), 10: ((6, (2,)),), 11: ((7, (2,)),),
              12: ((8, (2,)),), 13: ((9, (2,)), (10, (2,)), (4, (0, 1))),
              14: ((11, (2,)), (1, (0, 1)), (2, (0, 1)), (3, (0, 1))),
              15: ((5, (0, 1)), (6, (0, 1)), (7, (0, 1)), (8, (0, 1)), (9, (0, 1)),
                   (10, (0, 1)), (11, (0, 1)), 12, (13, (0, 1)))},
    jx=(1, 5, 9, 13, 17, 21, 25), vmem_mb=128,
    tok={
        0: [-26,-24,-22,-19,-17,-14,-12,-10,-7,-5,-2,0,2,5,7,9,12,14,17,19,21,24,26,29,31,33,36,38,41,43,45,48,50,52,55,57,60,62,64,67,69,72,74,76,79,81,84,86],
        1: [-32,-29,-27,-25,-22,-20,-17,-15,-13,-10,-8,-5,-3,-1,2,4,7,9,11,14,16,18,21,23,26,28,30,33,35,38,40,42,45,47,49,51,54,56,58,60,62,65,67,69,71,73,76,78],
        2: [-28,-26,-23,-21,-18,-16,-14,-11,-9,-7,-4,-2,1,3,5,8,10,13,15,18,20,23,25,28,30,33,35,38,40,42,45,47,50,52,55,57,59,62,64,67,69,71,74,76,79,81,83,86],
        3: [-20,-17,-15,-13,-10,-8,-6,-3,-1,2,4,6,9,11,14,16,18,21,24,26,29,31,34,37,39,42,44,47,50,52,55,58,60,63,65,67,70,72,75,77,79,82,84,87,89,92,94,96],
        4: [-27,-24,-22,-19,-17,-15,-12,-10,-7,-5,-3,0,2,5,7,9,12,14,17,19,22,24,27,29,32,34,37,39,42,44,46,49,51,54,56,59,61,64,66,69,71,74,76,79,81,84,86,88],
        5: [-10,-8,-5,-2,0,3,5,8,10,13,15,18,20,23,25,28,30,33,35,38,40,43,45,48,50,53,55,58,60,63,65,68,70,72,75,77,80,82,85,87,90,92,95,97,100,102,105,107],
        6: [-15,-13,-11,-8,-6,-3,-1,2,4,7,9,12,14,17,19,22,24,27,29,31,34,36,39,41,44,46,49,51,54,56,59,61,64,66,69,71,73,76,78,81,83,86,88,91,93,96,98,101],
        7: [-10,-7,-5,-2,0,2,5,7,10,12,15,17,20,22,25,27,30,32,35,37,40,42,44,47,49,52,54,57,59,62,64,67,69,72,74,77,79,82,84,86,89,91,94,96,99,101,104,106],
        8: [-25,-22,-20,-17,-15,-12,-10,-7,-5,-2,0,3,5,8,10,13,15,17,20,22,25,27,30,32,35,37,40,42,45,47,50,52,55,57,60,62,65,67,70,72,74,77,79,82,84,87,89,92],
        9: [-6,-3,-1,2,4,7,9,12,14,17,19,22,24,27,29,31,34,36,39,41,44,46,49,51,54,56,59,61,64,66,69,71,74,76,78,80,83,85,87,89,91,94,96,98,100,103,105,107],
        10: [-21,-18,-15,-13,-10,-7,-4,-2,1,4,7,9,12,15,17,20,23,25,28,30,33,35,38,40,43,45,48,50,53,55,58,60,63,65,68,70,72,75,77,80,82,85,87,90,92,95,97,100],
        11: [-17,-14,-12,-9,-7,-4,-2,1,3,6,8,10,13,15,18,20,23,25,28,31,33,36,38,41,43,46,48,51,53,56,58,61,64,66,68,71,73,76,78,80,83,85,88,90,93,95,97,100],
        12: [-26,-24,-21,-18,-16,-13,-11,-8,-6,-3,0,2,5,7,10,12,15,18,20,23,25,28,30,33,36,38,41,43,46,48,51,54,56,59,61,64,66,68,71,73,76,78,81,83,86,88,90,93],
        13: [-15,-12,-10,-8,-5,-3,0,2,4,7,9,12,14,16,19,21,23,26,29,31,34,37,39,42,45,47,50,52,55,58,60,63,66,68,71,73,75,78,80,83,85,88,90,93,95,97,100,102],
        14: [-20,-18,-15,-13,-10,-8,-6,-3,-1,2,4,7,9,12,14,16,19,21,24,26,29,31,34,36,38,41,43,46,48,51,53,56,58,60,63,65,67,70,72,74,77,79,81,84,86,88,91,93],
        15: [-33,-31,-30,-28,-27,-26,-24,-23,-21,-18,-14,-10,-7,-3,1,4,8,11,15,18,22,25,29,32,35,37,39,41,43,46,48,50,52,56,59,63,67,71,75,79,83,84,84,85,86,86,87,88],
    },
    w4_k=6, nq_mxu=6)


def _tile_view(a):
    r, c = a.shape
    a = a.reshape(r // 16, 2, 8, c // 128, 128)
    return jnp.swapaxes(a, 2, 3)


def _head_view(a):
    c = a.shape[1]
    a = a.reshape(H, 2, DH // 16, 8, c // 128, 128)
    return jnp.swapaxes(a, 3, 4)


def _as_bf16(w32):
    n = w32.shape[0]
    return pltpu.bitcast(w32.reshape(n * 8, 128), BF16)


def _lhs(top, fill=0.0):
    return jnp.concatenate([top, jnp.full(top.shape, fill, F32)], axis=0).astype(BF16)


def _ln_stats(x):
    m = jnp.mean(x, axis=-1, keepdims=True)
    m2 = jnp.mean(x * x, axis=-1, keepdims=True)
    v = jnp.maximum(m2 - m * m, 0.0)
    return m, lax.rsqrt(v + EPS)


def _round_bf16(x):
    return x.astype(BF16).astype(F32)


def _dot(a, b):
    return jnp.dot(a, b, preferred_element_type=F32)


def _make_kernel(sk, win, cfg):
    nj = win // 128
    j0 = (sk - win) // 128
    jq = nj // 4
    jx = list(cfg["jx"])
    assert nj == 32 and cfg["blocks"][-2][0] <= NU - 3 and cfg["blocks"][-1] == (NU - 1, NU)
    qscale = DH ** -0.5 * 1.4426950408889634

    def kernel(x_hbm, k_hbm, v_hbm, wq_hbm, wo_hbm, w3_hbm, w4_hbm, o_ref,
               kbuf, vbuf, vx, wqbuf, wobuf, w3buf, w4buf, xin,
               xs, qacc, qlhs, sx, sy, pbuf0, pbuf1, plhs, mbuf, lpart, abuf, olhs, gp,
               sems):
        pbuf = (pbuf0, pbuf1)
        ns = abuf.shape[0]


        def cps_w(hbm, buf, sem, lo=0, n=None):
            n = buf.shape[0] if n is None else n
            return [pltpu.make_async_copy(
                hbm.at[pl.ds(lo, n), e],
                buf.at[pl.ds(lo, n), :, pl.ds(e * 8, 8), :],
                sems.at[sem]) for e in range(2)]

        def cps_kv(hbm, buf, sem, u):
            return [pltpu.make_async_copy(
                hbm.at[pl.ds(u * UT, UT), e, pl.ds(j0, nj)],
                buf.at[pl.ds(u * UT, UT), :, pl.ds(e * 8, 8), :],
                sems.at[sem]) for e in range(2)]

        def cps_v(u, par):
            return [pltpu.make_async_copy(
                v_hbm.at[pl.ds(2 * u, 2), e, :, pl.ds(j0, nj)],
                vbuf.at[pl.ds(2 * u, 2), :, :, pl.ds(e * 8, 8), :],
                sems.at[2 + par]) for e in range(2)]

        def cps_wo(part):
            lo, n = ((0, H - 8), (H - 8, 8))[part]
            return [pltpu.make_async_copy(
                wo_hbm.at[pl.ds(lo, n), e], wobuf.at[pl.ds(lo, n), :, :, pl.ds(e * 8, 8), :],
                sems.at[4]) for e in range(2)]

        cps_k = lambda u, par: cps_kv(k_hbm, kbuf, par, u)
        cps_x_wq = lambda: cps_w(wq_hbm, wqbuf, 4) + [pltpu.make_async_copy(x_hbm, xin, sems.at[4])]
        cps_w3 = lambda: cps_w(w3_hbm, w3buf, 0)
        w4_k = cfg["w4_k"] * 128
        w4_parts = [(c, 0, FF) for c in range(D // 128 - 1)]
        w4_parts += [(D // 128 - 1, 0, w4_k), (D // 128 - 1, w4_k, FF - w4_k)]

        def cps_w4(i):
            c, lo, n = w4_parts[i]
            return [pltpu.make_async_copy(
                w4_hbm.at[pl.ds(lo, n), pl.ds(c * 128, 128)], w4buf.at[c, pl.ds(lo, n), :],
                sems.at[(2, 1, 3, 0, 4, 2)[i]])]

        def start(cps):
            for c in cps:
                c.start()

        def wait(cps):
            for c in cps:
                c.wait()

        start(cps_x_wq())
        start(cps_k(0, 0))
        start(cps_k(1, 1))
        start(cps_v(0, 0))
        start(cps_v(1, 1))

        k32 = kbuf.bitcast(U32)
        v32 = vbuf.bitcast(U32)
        wq32 = wqbuf.bitcast(U32)
        wo32 = wobuf.bitcast(U32)
        w332 = w3buf.bitcast(U32)
        w432 = w4buf.bitcast(U32)

        def js(u):
            return cfg["js_at"].get(u, cfg["jsplit"])

        def jms(u):
            return [nj - 1 - jq * (i % 4) - i // 4 for i in range(nmx(u))]

        def early_tiles(kb):
            return ((H * DH // 128,) * 3 + (3 * cfg["nq_mxu"], 0))[kb]

        def nmx(u):
            return cfg["nm_at"].get(u, cfg["nm"])

        def pack_q(q, u):
            q = q * qscale
            lane = lax.broadcasted_iota(jnp.int32, (8, 128), 1)
            sub = lax.broadcasted_iota(jnp.int32, (8, 128), 0)
            keep = (lane < DH - 128) == (sub % 2 == 0)
            q = jnp.concatenate(
                [q[:, 0:128], jnp.where(keep, q[:, 128:256], 0.0), q[:, 256:384]], axis=1)
            qlhs.at[u][:, 0:384] = pltpu.bitcast(_lhs(q), U32)

        def st_qk(u, js):
            sl = u % 2
            lhs = pltpu.bitcast(qlhs[u], BF16)
            toks = []
            for j in js:
                ra = 2 * (j // jq)
                cs = slice((j % jq) * 128, (j % jq + 1) * 128)
                for t in range(3):
                    w = _as_bf16(k32[pl.ds(u * UT + t * 8, 8), j])
                    r = _dot(lhs[:, t * 128:(t + 1) * 128], w)
                    toks.append(r[8:16])
                    if t == 0:
                        sx[sl, ra:ra + 1, cs] = r[0:1]
                    elif t == 1:
                        sy[sl, ra:ra + 2, cs] = r[ra:ra + 2]
                    else:
                        sx[sl, ra + 1:ra + 2, cs] = r[0:1]
            return toks

        def st_softmax(u, zdyn, pin=False):
            sl = u % 2
            s = sx[sl] + sy[sl]
            m = s
            while m.shape[1] > 128:
                h = m.shape[1] // 2
                m = jnp.maximum(m[:, :h], m[:, h:])
            m = jnp.maximum(m, pltpu.roll(m, 2, 0))
            m = jnp.maximum(m, pltpu.roll(m, 4, 0))
            if pin:
                qlhs[NU + zdyn, :, 0:128] = pltpu.bitcast(m, U32)
            m = jnp.max(m, axis=1, keepdims=True)
            p = jnp.exp2(s - m)
            pbuf[sl][zdyn] = p
            for g in range((nmx(u) + 3) // 4):
                c = jq - 1 - g
                plhs[:, (2 * sl + g) * 128:(2 * sl + g + 1) * 128] = pltpu.bitcast(
                    _lhs(p[:, c * 128:(c + 1) * 128]), U32)

        def inv_l(l):
            l = jnp.sum(l, axis=1, keepdims=True)
            r0 = pl.reciprocal(l, approx=True)
            return jnp.broadcast_to(r0 * (2.0 - l * r0), (8, 128))

        def st_lsum(u):
            l = pbuf[u % 2][0, :, 0:128]
            for c in range(1, jq):
                l = l + pbuf[u % 2][0, :, c * 128:(c + 1) * 128]
            l = l + pltpu.roll(l, 2, 0)
            l = l + pltpu.roll(l, 4, 0)
            lpart[u % ns] = inv_l(l) if u == NU - 1 else l

        def st_pvm(u):
            toks = []
            for j in jms(u):
                g = jq - 1 - j % jq
                pc = 2 * (u % 2) + g
                lhs = pltpu.bitcast(plhs[:, pc * 128:(pc + 1) * 128], BF16)
                ra = 2 * (j // jq)
                for t in range(3):
                    if t == 1:
                        w32 = jnp.concatenate(
                            [v32[2 * u, 8:12, j], v32[2 * u + 1, 0:4, j]], axis=0)
                    else:
                        w32 = v32[2 * u + t // 2, 2 * t:2 * t + 8, j]
                    r = _dot(lhs, _as_bf16(w32))
                    toks.append(r[8:16])
                    mbuf[u % ns, g, t, ra:ra + 2, :] = r[ra:ra + 2]
            return toks

        def st_expand(u):
            def body(i, c):
                hd, dt = i // 12, i % 12
                for ix, j in enumerate(jx):
                    w = v32[2 * u + hd, dt, j]
                    vx[2 * u + hd, dt, ix] = pltpu.bitcast(w << 16, F32)
                    vbuf[2 * u + hd, dt, j] = pltpu.bitcast(w & jnp.uint32(0xFFFF0000), BF16)
                return c
            if jx:
                lax.fori_loop(0, UT, body, 0)
            for j in jms(u):
                for t in range(3):
                    idx = [divmod(t * 8 + v, 12) for v in range(8)]
                    blk = jnp.concatenate([vbuf[2 * u + hd, dt, j] for hd, dt in idx], axis=0)
                    blk = blk.astype(F32).T.astype(BF16)
                    for v, (hd, dt) in enumerate(idx):
                        vbuf[2 * u + hd, dt, j] = blk[v * 16:(v + 1) * 16]

        def st_pv(u, toks, tok_map):
            nm, sl = nmx(u), u % ns
            for piece in range(NPIECE):
                hd, half = divmod(piece, NPIECE // 2)
                sub = len(tok_map) // NPIECE
                lo = hi = None
                for j in range(nj):
                    if j in jms(u):
                        continue
                    row = 2 * (j // jq) + hd
                    cs = slice((j % jq) * 128, (j % jq + 1) * 128)
                    pb = jnp.broadcast_to(pbuf[u % 2][0, row:row + 1, cs], (8, 128))
                    k = piece * sub + j * sub // nj
                    ti = tok_map[k] if j % (nj // sub) == 0 else -1
                    if j > 0 and tok_map[k - 1] == ti:
                        ti = -1
                    if toks and ti >= 0:
                        pb = pb + toks[min(ti, len(toks) - 1)]
                    w = v32[2 * u + hd, pl.ds(half * 2, 2), j]
                    if j in jx:
                        a = vx[2 * u + hd, pl.ds(half * 2, 2), jx.index(j)] * pb
                        b = pltpu.bitcast(w, F32) * pb
                    else:
                        a = pltpu.bitcast(w << 16, F32) * pb
                        b = pltpu.bitcast(w & jnp.uint32(0xFFFF0000), F32) * pb
                    lo = a if lo is None else lo + a
                    hi = b if hi is None else hi + b
                for i in range(2):
                    base = (piece * 2 + i) * 16
                    abuf[sl, pl.ds(base, 8, stride=2), :] = lo[i]
                    abuf[sl, pl.ds(base + 1, 8, stride=2), :] = hi[i]

        def st_ored(u, ts=(0, 1, 2), partial_rows=False, pin=None):
            nm, sl = nmx(u), u % ns
            ia = lpart[sl] if u == NU - 1 else inv_l(lpart[sl])
            ib = pltpu.roll(ia, 1, 0)
            if partial_rows:
                even = lax.broadcasted_iota(jnp.int32, (8, 128), 0) % 2 == 0
                ia, ib = jnp.where(even, ia, ib), jnp.where(even, ib, ia)
            lane = lax.broadcasted_iota(jnp.int32, (8, 128), 1)
            for t in ts:
                at = abuf[sl, t * 128:(t + 1) * 128, :].T
                if pin is not None:
                    qlhs[NU + pin, :, 0:128] = pltpu.bitcast(at[120:128], U32)
                o = at[0:8]
                for i in range(1, 16):
                    o = o + at[i * 8:(i + 1) * 8]
                if nm:
                    sub = lax.broadcasted_iota(jnp.int32, (8, 128), 0)
                    odd = (0, (lane >= DH - 128).astype(jnp.int32), 1)[t]
                    for g in range((nm + 3) // 4):
                        keep = (sub >= 8 - 2 * min(nm - 4 * g, 4)) & (sub % 2 == odd)
                        o = o + jnp.where(keep, mbuf[sl, g, t], 0.0)
                if not partial_rows:
                    o = o + pltpu.roll(o, 4, 0)
                    o = o + pltpu.roll(o, 2, 0)
                    o = o + pltpu.roll(o, 1, 0)
                o = o * (ia, jnp.where(lane < DH - 128, ia, ib), ib)[t]
                olhs.at[u][:, t * 128:(t + 1) * 128] = pltpu.bitcast(_lhs(o), U32)

        def st_oproj(u, ts=(0, 1, 2), out=None):
            lhs = pltpu.bitcast(olhs[u], BF16)
            toks = []
            for t in ts:
                for n in range(D // 128):
                    if t == 1:
                        w32 = jnp.concatenate(
                            [wo32[2 * u, 8:12, n], wo32[2 * u + 1, 0:4, n]], axis=0)
                    else:
                        w32 = wo32[2 * u + t // 2, 2 * t:2 * t + 8, n]
                    r = _dot(lhs[:, t * 128:(t + 1) * 128], _as_bf16(w32))
                    toks.append(r[8:16])
                    if out is None:
                        gp[t, n, pl.ds(u, 1), :] = r[0:1]
                    else:
                        out[n].append(r[0:8])
            return toks

        def mlp(first, extra):
            g = gp[0] + gp[1] + gp[2]
            g = g[:, 0:8] + g[:, 8:16]
            g = jnp.concatenate([g[n] + extra[n][0] + extra[n][1] + extra[n][2]
                                 for n in range(D // 128)], axis=1)
            g = g + pltpu.roll(g, 4, 0)
            g = g + pltpu.roll(g, 2, 0)
            g = g + pltpu.roll(g, 1, 0)
            x1 = _round_bf16(xs[...] + g)
            lhs = _lhs(x1, 1.0)
            m1, r1 = _ln_stats(x1)
            y = (x1 - m1) * r1
            m2, r2 = _ln_stats(y)
            a = r1 * r2
            b = (m1 * r1 + m2) * r2
            if first:
                wait(cps_w3())
                start(cps_w4(3))
                start(cps_w4(4))
            hl, hs = [], []
            for n in range(FF // 128):
                r = _dot(lhs, _as_bf16(w332[:, n]))
                hn = jax.nn.gelu(r[0:8] * a - r[8:16] * b, approximate=True)
                hl.append(_lhs(hn))
                hs.append(hn)
            acc = x1 + y
            acc = [acc[:, c * 128:(c + 1) * 128] for c in range(D // 128)]

            def w4_dot(kt, c):
                return _dot(hl[kt], pltpu.bitcast(w432[c, kt * 64:(kt + 1) * 64, :], BF16))[0:8]

            if not first:
                for kt in range(FF // 128):
                    for c in range(D // 128):
                        acc[c] = acc[c] + w4_dot(kt, c)
                xs[...] = _round_bf16(jnp.concatenate(acc, axis=1))
                return
            for i, (c, lo, n) in enumerate(w4_parts):
                wait(cps_w4(i))
                if i == 0:
                    start(cps_w4(5))
                    for k, hn in enumerate(hs[cfg["w4_k"]:]):
                        abuf[k // 3, (k % 3) * 128:(k % 3 + 1) * 128, :] = jnp.broadcast_to(
                            _round_bf16(hn[0:1]), (128, 128)).T
                if lo == 0:
                    for kt in range(n // 128):
                        acc[c] = acc[c] + w4_dot(kt, c)
                else:
                    pa = None
                    for dt in range(n // 16):
                        w = w432[c, lo // 2 + dt * 8:lo // 2 + (dt + 1) * 8, :]
                        sl, r0 = dt // 24, dt % 24 * 16
                        pr = (pltpu.bitcast(w << 16, F32) * abuf[sl, pl.ds(r0, 8, stride=2), :]
                              + pltpu.bitcast(w & jnp.uint32(0xFFFF0000), F32)
                              * abuf[sl, pl.ds(r0 + 1, 8, stride=2), :])
                        pa = pr if pa is None else pa + pr
                    pa = pa + pltpu.roll(pa, 4, 0)
                    pa = pa + pltpu.roll(pa, 2, 0)
                    acc[c] = acc[c] + (pa + pltpu.roll(pa, 1, 0))
                if lo + n == FF:
                    xc = _round_bf16(acc[c])
                    xs[:, c * 128:(c + 1) * 128] = xc
                    lhs = _lhs(xc)
                    for nt in range(early_tiles(c)):
                        r = _dot(lhs, _as_bf16(wq32[pl.ds(c * 8, 8), nt]))[0:4]
                        qacc[nt, 0:4, :] = r if c == 0 else qacc[nt, 0:4, :] + r

        gp[...] = jnp.zeros_like(gp)
        mbuf[...] = jnp.zeros_like(mbuf)
        wait(cps_x_wq())
        start(cps_wo(0))
        x0 = jnp.broadcast_to(xin[...].astype(F32), (8, D))
        sub0 = lax.broadcasted_iota(jnp.int32, (8, D), 0)
        lane0 = lax.broadcasted_iota(jnp.int32, (8, D), 1)
        for nkb, n0, n1 in ((4, 0, early_tiles(3)), (3, early_tiles(3), early_tiles(0))):
            lhs0 = _lhs(jnp.where(sub0 < 4, jnp.where(lane0 < nkb * 128, x0, 0.0), 1.0))

            def q0_body(nt, c, lhs0=lhs0):
                qacc[nt] = _dot(lhs0, _as_bf16(wq32[:, nt]))[0:8]
                return c
            lax.fori_loop(n0, n1, q0_body, 0)
        wait(cps_k(0, 0))
        start(cps_k(2, 0))
        wait(cps_k(1, 1))
        wait(cps_v(0, 0))
        xs[...] = x0

        def layer(li, carry):
            first = li == 0
            n_first = jnp.maximum(1 - li, 0)
            zdyn = li >> 4

            def block_dma(ua, ub):
                def last_wait(t):
                    if t == NU - 2:
                        wait(cps_k(NU - 1, (NU - 1) % 2))
                    else:
                        wait(cps_v(t + 1, (t + 1) % 2) if t + 1 < NU else cps_wo(1))

                def dma_ops(_, c):
                    for t in range(ua, ub):
                        if t + 3 < NU:
                            start(cps_k(t + 3, (t + 3) % 2))
                        if t + 2 < NU:
                            start(cps_v(t + 2, t % 2))
                        if t == NU - 2:
                            start(cps_w3())
                            start(cps_w4(0))
                        if t == NU - 1:
                            start(cps_w4(1))
                            wait(cps_v(t, t % 2))
                            start(cps_w4(2))
                        if t == 1:
                            wait(cps_wo(0))
                            start(cps_wo(1))
                        st_expand(t)
                        if t + 2 < NU - 1:
                            wait(cps_k(t + 2, t % 2))
                        if t < ub - 1:
                            last_wait(t)
                    return c

                lax.fori_loop(0, n_first, dma_ops, 0)
                pl.when(first)(lambda: last_wait(ub - 1))

            def prologue():
                x = xs[...]
                m, r = _ln_stats(x)
                nq = cfg["nq_mxu"]

                def finish_q(u, late):
                    qs = []
                    for nt in range(3):
                        qx = jnp.broadcast_to(qacc[u * 3 + nt, 0:1, :], (8, 128))
                        cs = jnp.broadcast_to(qacc[u * 3 + nt, 4:5, :], (8, 128))
                        qs.append((qx + late[nt] - cs * m) * r)
                    pack_q(jnp.concatenate(qs, axis=1), u)

                lhs = _lhs(x[:, D - 128:D])
                for u in range(nq):
                    finish_q(u, [_dot(lhs, _as_bf16(wq32[pl.ds(32, 8), u * 3 + nt]))[0:8]
                                 for nt in range(3)])
                f1 = cfg["va_force"]
                toks = st_qk(0, range(f1))
                for kb in range(2):
                    cs = slice((3 + kb) * 128, (4 + kb) * 128)
                    blk = jnp.broadcast_to(x[0:1, cs], (128, 128)).T
                    abuf[ns - 1 + zdyn, kb * 128:(kb + 1) * 128, :] = blk
                    qlhs[NU + zdyn, :, 0:128] = pltpu.bitcast(blk[120:128], U32)
                toks += st_qk(0, range(f1, nj))
                st_softmax(0, zdyn)
                toks += st_qk(1, range(js(1)))
                toks += st_pvm(0)
                for va, (t0, t1) in zip(cfg["va_groups"], cfg["va_tok"]):
                    acc = [None] * len(va)
                    for kt in range(16):
                        lo = abuf[ns - 1, pl.ds(kt * 16, 8, stride=2), :]
                        hi = abuf[ns - 1, pl.ds(kt * 16 + 1, 8, stride=2), :]
                        tk = toks[t0 + kt * (t1 - t0) // 16]
                        lo, hi = lo + tk, hi + tk
                        for i, u in enumerate(va):
                            w = wq32[24 + kt, u * 3:u * 3 + 3]
                            pr = (pltpu.bitcast(w << 16, F32) * lo
                                  + pltpu.bitcast(w & jnp.uint32(0xFFFF0000), F32) * hi)
                            acc[i] = pr if acc[i] is None else acc[i] + pr
                    for i, u in enumerate(va):
                        late = []
                        for nt in range(3):
                            q = acc[i][nt]
                            q = q + pltpu.roll(q, 4, 0)
                            q = q + pltpu.roll(q, 2, 0)
                            late.append(q + pltpu.roll(q, 1, 0))
                        finish_q(u, late)
                return toks

            def block(bi):
                ua, ub = cfg["blocks"][bi]
                block_dma(ua, ub)
                toks = []
                if bi == 0:
                    toks += prologue()
                done = js(ua + 1)
                for t in range(ua, ub):
                    base = len(toks)
                    ous = cfg["ored_at"].get(t, ())
                    if t in cfg["ored_pin"]:
                        for i, u in enumerate(ous):
                            nxt = nj - cfg["ored_back"] - (len(ous) - 1 - i) * 11
                            toks += st_qk(t + 1, range(done, nxt))
                            done = max(done, nxt)
                            st_ored(u, pin=zdyn)
                    else:
                        for u in ous:
                            st_ored(u)
                    if t + 1 < NU:
                        toks += st_qk(t + 1, range(done, nj))
                    g0 = len(toks)
                    if t == ua and bi > 0:
                        toks += st_pvm(t)
                    for u in cfg["oproj_at"].get(t, ()):
                        toks += st_oproj(*u) if isinstance(u, tuple) else st_oproj(u)
                    done = js(t + 2)
                    if t + 1 < ub:
                        gap = cfg["gap_at"].get(t, cfg["gap"])
                        done = max(-((len(toks) - g0 - gap) // 3), 0)
                    gap1 = cfg["gap1_at"].get(t, cfg["gap1"])
                    d1 = min(max(-((len(toks) - g0 - gap1) // 3), 0), done)
                    if t + 2 < NU:
                        toks += st_qk(t + 2, range(d1))
                    if t + 1 < NU:
                        st_softmax(t + 1, zdyn, pin=gap1 > 0 and t + 2 < NU and d1 < done)
                    if t + 2 < NU:
                        toks += st_qk(t + 2, range(d1, done))
                    if t + 1 < ub:
                        toks += st_pvm(t + 1)
                    st_pv(t, toks, [base + i for i in cfg["tok"][t]])
                    st_lsum(t)

            for bi in range(len(cfg["blocks"])):
                block(bi)

            def tail(first_static):
                for u in range(*cfg["blocks"][-1]):
                    st_ored(u, partial_rows=(u == NU - 1))
                seen = set()
                for us in cfg["oproj_at"].values():
                    for u in us:
                        uu, ts = u if isinstance(u, tuple) else (u, (0, 1, 2))
                        seen |= {(uu, t) for t in ts}
                for u in range(NU - 1):
                    ts = tuple(t for t in range(3) if (u, t) not in seen)
                    if ts:
                        st_oproj(u, ts)
                extra = [[] for _ in range(D // 128)]
                st_oproj(NU - 1, out=extra)
                mlp(first_static, extra)

            pl.when(first)(lambda: tail(True))
            pl.when(jnp.logical_not(first))(lambda: tail(False))
            return carry

        lax.fori_loop(0, 2, layer, 0)
        o_ref[...] = xs[0:1, :].astype(o_ref.dtype)

    return kernel


@jax.jit
def pallas_interleave_layers__sliding_block_cached__mixer_s_mlp__decode_kernel(
    A_x: jax.Array,
    A_k_cache: jax.Array,
    A_v_cache: jax.Array,
    A_wq: jax.Array,
    A_wo: jax.Array,
    B_x: jax.Array,
    B_w1: jax.Array,
    B_w2: jax.Array,
    B_w3: jax.Array,
    B_w4: jax.Array,
):
    b, sq, d = A_x.shape
    _, hkv, sk, dh = A_k_cache.shape
    assert (b, sq, d, hkv, dh) == (1, 1, D, H, DH)
    win = min(4096, max(256, sk // 4))
    assert win % 512 == 0 and sk % 128 == 0
    nj = win // 128

    kt = _tile_view(jnp.swapaxes(A_k_cache, 2, 3).reshape(H * DH, sk))
    vt = _head_view(jnp.swapaxes(A_v_cache, 2, 3).reshape(H * DH, sk))

    def buf(r, c):
        return pltpu.VMEM((r // 16, c // 128, 16, 128), BF16)

    def hbuf(c):
        return pltpu.VMEM((H, DH // 16, c // 128, 16, 128), BF16)

    bl = CFG["blocks"]
    ns = CFG.get("ns") or max(bl[i + 1][1] - bl[i][0] for i in range(len(bl) - 1))
    any_spec = pl.BlockSpec(memory_space=pl.ANY)
    out = pl.pallas_call(
        _make_kernel(sk, win, CFG),
        out_shape=jax.ShapeDtypeStruct((1, D), A_x.dtype),
        in_specs=[any_spec] * 7,
        out_specs=pl.BlockSpec(memory_space=pltpu.VMEM),
        scratch_shapes=[
            buf(H * DH, win), hbuf(win),
            pltpu.VMEM((H, DH // 16, max(len(CFG["jx"]), 1), 8, 128), F32),
            buf(D, H * DH), hbuf(D), buf(D, FF),
            pltpu.VMEM((D // 128, FF, 128), BF16),
            pltpu.VMEM((1, D), BF16),
            pltpu.VMEM((8, D), F32),
            pltpu.VMEM((H * DH // 128, 8, 128), F32),
            pltpu.VMEM((NU + 1, 8, 384), U32),
            pltpu.VMEM((2, 8, win // 4), F32),
            pltpu.VMEM((2, 8, win // 4), F32),
            pltpu.VMEM((1, 8, win // 4), F32),
            pltpu.VMEM((1, 8, win // 4), F32),
            pltpu.VMEM((8, 512), U32),
            pltpu.VMEM((ns, 2, 3, 8, 128), F32),
            pltpu.VMEM((ns, 8, 128), F32),
            pltpu.VMEM((ns, 384, 128), F32),
            pltpu.VMEM((NU, 8, 384), U32),
            pltpu.VMEM((3, D // 128, NU, 128), F32),
            pltpu.SemaphoreType.DMA((5,)),
        ],
        compiler_params=pltpu.CompilerParams(vmem_limit_bytes=int(CFG["vmem_mb"] * 1024 * 1024)),
        name="interleave_decode",
    )(A_x.reshape(1, D), kt, vt, _tile_view(A_wq), _head_view(A_wo),
      _tile_view(B_w3), B_w4)
    return out.reshape(b, sq, d)
```

```python
import jax
import jax.numpy as jnp
from jax import lax
import jax.experimental.pallas as pl
import jax.experimental.pallas.tpu as pltpu

F32 = jnp.float32
BF16 = jnp.bfloat16
U32 = jnp.uint32

D = 640
H = 32
DH = 192
FF = 1536
NU = H // 2
UT = 2 * DH // 16
EPS = 1e-5
NPIECE = 12

CFG = dict(
    blocks=((0, 4), (4, 8), (8, 12), (12, 15), (15, 16)), ns=7,
    jsplit=10, js_at={1: 13, 5: 19, 9: 19, 13: 16},
    gap=49, gap1=24, gap_at={}, gap1_at={}, ored_pin=(), ored_back=4,
    nm=4, nm_at={15: 3},
    va_groups=((6, 7, 8, 9), (10, 11, 12, 13, 14), (15,)), va_force=7,
    va_tok=((6, 43), (48, 94), (102, 112)),
    ored_at={4: (0,), 5: (1,), 6: (2,), 7: (3,), 8: (4,), 9: (5,), 10: (6,), 11: (7,),
             12: (8,), 13: (9, 10), 14: (11,), 15: (12, 13, 14)},
    oproj_at={4: ((0, (2,)),), 5: ((1, (2,)),), 6: ((2, (2,)),), 7: ((3, (2,)),),
              8: ((4, (0,)), (0, (0,))), 9: ((5, (0,)), (0, (1,))), 10: ((6, (0,)),), 11: ((7, (0,)),),
              12: ((8, (0,)),), 13: ((9, (0,)), (10, (0,)), (4, (1, 2))),
              14: ((11, (0,)), (1, (0, 1)), (2, (0, 1)), (3, (0, 1))),
              15: ((5, (1, 2)), (6, (1, 2)), (7, (1, 2)), (8, (1, 2)), (9, (1, 2)),
                   (10, (1, 2)), (11, (1, 2)), 12, (13, (0, 1)))},
    jx=(1, 5, 9, 13, 17, 21, 25), vmem_mb=128,
    tok={
        0: [-26,-24,-22,-19,-17,-14,-12,-10,-7,-5,-2,0,2,4,5,9,12,14,17,19,21,24,26,29,31,33,36,38,41,43,45,48,50,52,55,57,60,62,64,67,69,72,74,76,79,81,84,86],
        1: [-32,-29,-27,-25,-22,-18,-17,-15,-13,-10,-8,-5,-3,-1,2,4,7,9,9,11,16,18,21,23,26,28,30,33,38,38,40,42,45,47,49,54,56,57,58,60,62,65,67,69,71,73,76,78],
        2: [-28,-26,-23,-21,-18,-16,-14,-11,-9,-8,-4,-2,0,1,3,8,10,13,15,18,19,22,24,27,29,33,35,38,40,42,45,47,50,52,55,57,59,62,64,67,69,71,74,76,79,81,83,86],
        3: [-20,-17,-13,-11,-10,-8,-6,-3,-3,-1,4,6,9,11,14,16,18,21,24,26,29,31,34,37,39,42,44,47,50,52,52,55,57,63,65,67,70,72,75,77,79,82,84,87,89,91,93,95],
        4: [-27,-24,-22,-19,-17,-15,-12,-10,-7,-5,-3,0,2,5,7,9,12,14,17,19,22,24,27,29,32,34,37,39,42,44,46,49,51,54,56,59,61,64,66,69,71,74,76,79,81,84,86,88],
        5: [-10,-8,-5,-2,0,3,5,8,10,13,15,18,20,23,25,28,30,33,35,38,40,43,45,48,50,53,55,58,60,63,65,68,70,72,75,77,80,82,85,87,90,92,95,97,100,102,105,107],
        6: [-15,-13,-11,-9,-7,-4,-2,0,2,5,8,10,13,16,19,21,24,27,29,31,34,36,39,41,44,46,49,51,54,56,59,61,64,66,69,71,73,76,78,81,83,86,88,91,93,96,98,101],
        7: [-10,-7,-5,-2,0,2,5,7,10,12,15,17,20,22,25,27,30,32,35,38,41,43,46,49,51,54,56,58,60,63,65,67,69,72,74,77,79,82,84,86,89,91,94,96,99,101,104,106],
        8: [-22,-20,-18,-16,-14,-13,-11,-9,-7,-5,-2,0,2,4,6,8,11,13,16,18,21,24,26,29,32,34,37,40,42,45,48,50,53,55,58,60,63,65,67,70,72,75,77,79,82,84,86,89],
        9: [-9,-6,-4,-1,1,4,7,9,12,14,16,19,21,23,26,28,30,33,36,38,41,44,47,49,52,55,57,59,62,64,67,69,72,74,77,79,82,84,87,89,92,94,97,99,102,104,106,109],
        10: [-19,-16,-14,-11,-9,-7,-4,-2,1,3,6,8,10,13,15,18,20,23,25,28,30,33,35,38,40,43,45,48,50,53,56,58,61,63,66,68,70,73,75,78,80,83,85,87,89,92,94,96],
        11: [-21,-18,-16,-13,-10,-8,-5,-2,0,3,5,7,10,12,15,17,19,22,24,27,30,32,35,37,40,43,45,48,51,54,56,59,62,64,67,69,71,74,76,79,81,83,85,87,89,92,94,96],
        12: [-25,-23,-20,-18,-15,-13,-10,-8,-5,-3,0,2,5,7,10,13,15,18,20,23,26,28,31,33,36,39,41,44,47,49,52,55,57,60,62,64,67,69,71,74,76,79,81,83,86,88,91,93],
        13: [-15,-12,-10,-7,-5,-2,0,2,5,7,10,12,15,17,20,22,24,27,30,32,35,37,40,42,45,48,50,53,55,58,60,63,66,68,70,73,75,78,80,82,85,87,89,92,94,97,99,101],
        14: [-21,-19,-16,-14,-12,-9,-7,-5,-2,0,3,5,7,10,12,15,17,19,22,24,27,29,32,34,37,40,42,45,47,50,52,55,57,59,62,64,67,69,71,74,76,79,81,83,86,88,90,93],
        15: [-33,-31,-30,-28,-27,-26,-24,-23,-21,-18,-14,-10,-7,-3,1,4,8,11,15,18,22,25,29,32,35,37,39,41,43,46,48,50,52,56,59,63,67,71,75,79,83,84,84,85,86,86,87,88],
    },
    w4_k=8, nq_mxu=6)


def _tile_view(a):
    r, c = a.shape
    a = a.reshape(r // 16, 2, 8, c // 128, 128)
    return jnp.swapaxes(a, 2, 3)


def _head_view(a):
    c = a.shape[1]
    a = a.reshape(H, 2, DH // 16, 8, c // 128, 128)
    return jnp.swapaxes(a, 3, 4)


def _as_bf16(w32):
    n = w32.shape[0]
    return pltpu.bitcast(w32.reshape(n * 8, 128), BF16)


def _lhs(top, fill=0.0):
    return jnp.concatenate([top, jnp.full(top.shape, fill, F32)], axis=0).astype(BF16)


def _ln_stats(x):
    m = jnp.mean(x, axis=-1, keepdims=True)
    m2 = jnp.mean(x * x, axis=-1, keepdims=True)
    v = jnp.maximum(m2 - m * m, 0.0)
    return m, lax.rsqrt(v + EPS)


def _round_bf16(x):
    return x.astype(BF16).astype(F32)


def _dot(a, b):
    return jnp.dot(a, b, preferred_element_type=F32)


def _make_kernel(sk, win, cfg):
    nj = win // 128
    j0 = (sk - win) // 128
    jq = nj // 4
    jx = list(cfg["jx"])
    assert nj == 32 and cfg["blocks"][-2][0] <= NU - 3 and cfg["blocks"][-1] == (NU - 1, NU)
    qscale = DH ** -0.5 * 1.4426950408889634

    def kernel(x_hbm, k_hbm, v_hbm, wq_hbm, wo_hbm, w3_hbm, w4_hbm, o_ref,
               kbuf, vbuf, vx, wqbuf, wobuf, w3buf, w4buf, xin,
               xs, qacc, qlhs, sx, sy, pbuf0, pbuf1, plhs, mbuf, lpart, abuf, olhs, gp,
               sems):
        pbuf = (pbuf0, pbuf1)
        ns = abuf.shape[0]


        def cps_w(hbm, buf, sem, lo=0, n=None):
            n = buf.shape[0] if n is None else n
            return [pltpu.make_async_copy(
                hbm.at[pl.ds(lo, n), e],
                buf.at[pl.ds(lo, n), :, pl.ds(e * 8, 8), :],
                sems.at[sem]) for e in range(2)]

        def cps_kv(hbm, buf, sem, u):
            return [pltpu.make_async_copy(
                hbm.at[pl.ds(u * UT, UT), e, pl.ds(j0, nj)],
                buf.at[pl.ds(u * UT, UT), :, pl.ds(e * 8, 8), :],
                sems.at[sem]) for e in range(2)]

        def cps_v(u, par):
            return [pltpu.make_async_copy(
                v_hbm.at[pl.ds(2 * u, 2), e, :, pl.ds(j0, nj)],
                vbuf.at[pl.ds(2 * u, 2), :, :, pl.ds(e * 8, 8), :],
                sems.at[2 + par]) for e in range(2)]

        def cps_wo(part):
            lo, n = ((0, H - 8), (H - 8, 8))[part]
            return [pltpu.make_async_copy(
                wo_hbm.at[pl.ds(lo, n), e], wobuf.at[pl.ds(lo, n), :, :, pl.ds(e * 8, 8), :],
                sems.at[4]) for e in range(2)]

        cps_k = lambda u, par: cps_kv(k_hbm, kbuf, par, u)
        cps_x_wq = lambda: cps_w(wq_hbm, wqbuf, 4) + [pltpu.make_async_copy(x_hbm, xin, sems.at[4])]
        cps_w3 = lambda: cps_w(w3_hbm, w3buf, 0)
        w4_k = cfg["w4_k"] * 128
        w4_parts = [(c, 0, FF) for c in range(D // 128 - 1)]
        w4_parts += [(D // 128 - 1, 0, w4_k), (D // 128 - 1, w4_k, FF - w4_k)]

        def cps_w4(i):
            c, lo, n = w4_parts[i]
            return [pltpu.make_async_copy(
                w4_hbm.at[pl.ds(lo, n), pl.ds(c * 128, 128)], w4buf.at[c, pl.ds(lo, n), :],
                sems.at[(2, 1, 3, 0, 4, 2)[i]])]

        def start(cps):
            for c in cps:
                c.start()

        def wait(cps):
            for c in cps:
                c.wait()

        start(cps_x_wq())
        start(cps_k(0, 0))
        start(cps_k(1, 1))
        start(cps_v(0, 0))
        start(cps_v(1, 1))

        k32 = kbuf.bitcast(U32)
        v32 = vbuf.bitcast(U32)
        wq32 = wqbuf.bitcast(U32)
        wo32 = wobuf.bitcast(U32)
        w332 = w3buf.bitcast(U32)
        w432 = w4buf.bitcast(U32)

        def js(u):
            return cfg["js_at"].get(u, cfg["jsplit"])

        def jms(u):
            return [nj - 1 - jq * (i % 4) - i // 4 for i in range(nmx(u))]

        def early_tiles(kb):
            return ((H * DH // 128,) * 3 + (3 * cfg["nq_mxu"], 0))[kb]

        def nmx(u):
            return cfg["nm_at"].get(u, cfg["nm"])

        def pack_q(q, u):
            q = q * qscale
            lane = lax.broadcasted_iota(jnp.int32, (8, 128), 1)
            sub = lax.broadcasted_iota(jnp.int32, (8, 128), 0)
            keep = (lane < DH - 128) == (sub % 2 == 0)
            q = jnp.concatenate(
                [q[:, 0:128], jnp.where(keep, q[:, 128:256], 0.0), q[:, 256:384]], axis=1)
            qlhs.at[u][:, 0:384] = pltpu.bitcast(_lhs(q), U32)

        def st_qk(u, js):
            sl = u % 2
            lhs = pltpu.bitcast(qlhs[u], BF16)
            toks = []
            for j in js:
                ra = 2 * (j // jq)
                cs = slice((j % jq) * 128, (j % jq + 1) * 128)
                for t in range(3):
                    w = _as_bf16(k32[pl.ds(u * UT + t * 8, 8), j])
                    r = _dot(lhs[:, t * 128:(t + 1) * 128], w)
                    toks.append(r[8:16])
                    if t == 0:
                        sx[sl, ra:ra + 1, cs] = r[0:1]
                    elif t == 1:
                        sy[sl, ra:ra + 2, cs] = r[ra:ra + 2]
                    else:
                        sx[sl, ra + 1:ra + 2, cs] = r[0:1]
            return toks

        def st_softmax(u, zdyn, pin=False):
            sl = u % 2
            s = sx[sl] + sy[sl]
            m = s
            while m.shape[1] > 128:
                h = m.shape[1] // 2
                m = jnp.maximum(m[:, :h], m[:, h:])
            m = jnp.maximum(m, pltpu.roll(m, 2, 0))
            m = jnp.maximum(m, pltpu.roll(m, 4, 0))
            if pin:
                qlhs[NU + zdyn, :, 0:128] = pltpu.bitcast(m, U32)
            m = jnp.max(m, axis=1, keepdims=True)
            p = jnp.exp2(s - m)
            pbuf[sl][zdyn] = p
            for g in range((nmx(u) + 3) // 4):
                c = jq - 1 - g
                plhs[:, (2 * sl + g) * 128:(2 * sl + g + 1) * 128] = pltpu.bitcast(
                    _lhs(p[:, c * 128:(c + 1) * 128]), U32)

        def inv_l(l):
            l = jnp.sum(l, axis=1, keepdims=True)
            r0 = pl.reciprocal(l, approx=True)
            return jnp.broadcast_to(r0 * (2.0 - l * r0), (8, 128))

        def st_lsum(u):
            l = pbuf[u % 2][0, :, 0:128]
            for c in range(1, jq):
                l = l + pbuf[u % 2][0, :, c * 128:(c + 1) * 128]
            l = l + pltpu.roll(l, 2, 0)
            l = l + pltpu.roll(l, 4, 0)
            lpart[u % ns] = inv_l(l) if u == NU - 1 else l

        def st_pvm(u):
            toks = []
            for j in jms(u):
                g = jq - 1 - j % jq
                pc = 2 * (u % 2) + g
                lhs = pltpu.bitcast(plhs[:, pc * 128:(pc + 1) * 128], BF16)
                ra = 2 * (j // jq)
                for t in range(3):
                    if t == 1:
                        w32 = jnp.concatenate(
                            [v32[2 * u, 8:12, j], v32[2 * u + 1, 0:4, j]], axis=0)
                    else:
                        w32 = v32[2 * u + t // 2, 2 * t:2 * t + 8, j]
                    r = _dot(lhs, _as_bf16(w32))
                    toks.append(r[8:16])
                    mbuf[u % ns, g, t, ra:ra + 2, :] = r[ra:ra + 2]
            return toks

        def st_expand(u):
            def body(dt, c):
                for hd in range(2):
                    for ix, j in enumerate(jx):
                        w = v32[2 * u + hd, dt, j]
                        vx[2 * u + hd, dt, ix] = pltpu.bitcast(w << 16, F32)
                        vbuf[2 * u + hd, dt, j] = pltpu.bitcast(w & jnp.uint32(0xFFFF0000), BF16)
                return c
            lax.fori_loop(0, UT // 2, body, 0)
            for j in jms(u):
                for t in range(3):
                    idx = [divmod(t * 8 + v, 12) for v in range(8)]
                    blk = jnp.concatenate([vbuf[2 * u + hd, dt, j] for hd, dt in idx], axis=0)
                    blk = blk.astype(F32).T.astype(BF16)
                    for v, (hd, dt) in enumerate(idx):
                        vbuf[2 * u + hd, dt, j] = blk[v * 16:(v + 1) * 16]

        def st_pv(u, toks, tok_map):
            nm, sl = nmx(u), u % ns
            for piece in range(NPIECE):
                hd, half = divmod(piece, NPIECE // 2)
                sub = len(tok_map) // NPIECE
                lo = hi = None
                for j in range(nj):
                    if j in jms(u):
                        continue
                    row = 2 * (j // jq) + hd
                    cs = slice((j % jq) * 128, (j % jq + 1) * 128)
                    pb = jnp.broadcast_to(pbuf[u % 2][0, row:row + 1, cs], (8, 128))
                    k = piece * sub + j * sub // nj
                    ti = tok_map[k] if j % (nj // sub) == 0 else -1
                    if j > 0 and tok_map[k - 1] == ti:
                        ti = -1
                    if toks and ti >= 0:
                        pb = pb + toks[min(ti, len(toks) - 1)]
                    w = v32[2 * u + hd, pl.ds(half * 2, 2), j]
                    if j in jx:
                        a = vx[2 * u + hd, pl.ds(half * 2, 2), jx.index(j)] * pb
                        b = pltpu.bitcast(w, F32) * pb
                    else:
                        a = pltpu.bitcast(w << 16, F32) * pb
                        b = pltpu.bitcast(w & jnp.uint32(0xFFFF0000), F32) * pb
                    lo = a if lo is None else lo + a
                    hi = b if hi is None else hi + b
                for i in range(2):
                    base = (piece * 2 + i) * 16
                    abuf[sl, pl.ds(base, 8, stride=2), :] = lo[i]
                    abuf[sl, pl.ds(base + 1, 8, stride=2), :] = hi[i]

        def st_ored(u, ts=(0, 1, 2), partial_rows=False, pin=None):
            nm, sl = nmx(u), u % ns
            ia = lpart[sl] if u == NU - 1 else inv_l(lpart[sl])
            ib = pltpu.roll(ia, 1, 0)
            if partial_rows:
                even = lax.broadcasted_iota(jnp.int32, (8, 128), 0) % 2 == 0
                ia, ib = jnp.where(even, ia, ib), jnp.where(even, ib, ia)
            lane = lax.broadcasted_iota(jnp.int32, (8, 128), 1)
            for t in ts:
                at = abuf[sl, t * 128:(t + 1) * 128, :].T
                if pin is not None:
                    qlhs[NU + pin, :, 0:128] = pltpu.bitcast(at[120:128], U32)
                o = at[0:8]
                for i in range(1, 16):
                    o = o + at[i * 8:(i + 1) * 8]
                if nm:
                    sub = lax.broadcasted_iota(jnp.int32, (8, 128), 0)
                    odd = (0, (lane >= DH - 128).astype(jnp.int32), 1)[t]
                    for g in range((nm + 3) // 4):
                        keep = (sub >= 8 - 2 * min(nm - 4 * g, 4)) & (sub % 2 == odd)
                        o = o + jnp.where(keep, mbuf[sl, g, t], 0.0)
                if not partial_rows:
                    o = o + pltpu.roll(o, 4, 0)
                    o = o + pltpu.roll(o, 2, 0)
                    o = o + pltpu.roll(o, 1, 0)
                o = o * (ia, jnp.where(lane < DH - 128, ia, ib), ib)[t]
                olhs.at[u][:, t * 128:(t + 1) * 128] = pltpu.bitcast(_lhs(o), U32)

        def st_oproj(u, ts=(0, 1, 2), out=None):
            lhs = pltpu.bitcast(olhs[u], BF16)
            toks = []
            for t in ts:
                for n in range(D // 128):
                    if t == 1:
                        w32 = jnp.concatenate(
                            [wo32[2 * u, 8:12, n], wo32[2 * u + 1, 0:4, n]], axis=0)
                    else:
                        w32 = wo32[2 * u + t // 2, 2 * t:2 * t + 8, n]
                    r = _dot(lhs[:, t * 128:(t + 1) * 128], _as_bf16(w32))
                    toks.append(r[8:16])
                    if out is None:
                        gp[t, n, pl.ds(u, 1), :] = r[0:1]
                    else:
                        out[n].append(r[0:8])
            return toks

        def mlp(first, extra):
            g = gp[0] + gp[1] + gp[2]
            g = g[:, 0:8] + g[:, 8:16]
            g = jnp.concatenate([g[n] + extra[n][0] + extra[n][1] + extra[n][2]
                                 for n in range(D // 128)], axis=1)
            g = g + pltpu.roll(g, 4, 0)
            g = g + pltpu.roll(g, 2, 0)
            g = g + pltpu.roll(g, 1, 0)
            x1 = _round_bf16(xs[...] + g)
            lhs = _lhs(x1, 1.0)
            m1, r1 = _ln_stats(x1)
            y = (x1 - m1) * r1
            m2, r2 = _ln_stats(y)
            a = r1 * r2
            b = (m1 * r1 + m2) * r2
            if first:
                wait(cps_w3())
                start(cps_w4(3))
                start(cps_w4(4))
            hl, hs = [], []
            for n in range(FF // 128):
                r = _dot(lhs, _as_bf16(w332[:, n]))
                hn = jax.nn.gelu(r[0:8] * a - r[8:16] * b, approximate=True)
                hl.append(_lhs(hn))
                hs.append(hn)
            acc = x1 + y
            acc = [acc[:, c * 128:(c + 1) * 128] for c in range(D // 128)]

            def w4_dot(kt, c):
                return _dot(hl[kt], pltpu.bitcast(w432[c, kt * 64:(kt + 1) * 64, :], BF16))[0:8]

            if not first:
                for kt in range(FF // 128):
                    for c in range(D // 128):
                        acc[c] = acc[c] + w4_dot(kt, c)
                xs[...] = _round_bf16(jnp.concatenate(acc, axis=1))
                return
            for i, (c, lo, n) in enumerate(w4_parts):
                wait(cps_w4(i))
                if i == 0:
                    start(cps_w4(5))
                    for k, hn in enumerate(hs[cfg["w4_k"]:]):
                        abuf[k // 3, (k % 3) * 128:(k % 3 + 1) * 128, :] = jnp.broadcast_to(
                            _round_bf16(hn[0:1]), (128, 128)).T
                if lo == 0:
                    for kt in range(n // 128):
                        acc[c] = acc[c] + w4_dot(kt, c)
                else:
                    pa = None
                    for dt in range(n // 16):
                        w = w432[c, lo // 2 + dt * 8:lo // 2 + (dt + 1) * 8, :]
                        sl, r0 = dt // 24, dt % 24 * 16
                        pr = (pltpu.bitcast(w << 16, F32) * abuf[sl, pl.ds(r0, 8, stride=2), :]
                              + pltpu.bitcast(w & jnp.uint32(0xFFFF0000), F32)
                              * abuf[sl, pl.ds(r0 + 1, 8, stride=2), :])
                        pa = pr if pa is None else pa + pr
                    pa = pa + pltpu.roll(pa, 4, 0)
                    pa = pa + pltpu.roll(pa, 2, 0)
                    acc[c] = acc[c] + (pa + pltpu.roll(pa, 1, 0))
                if lo + n == FF:
                    xc = _round_bf16(acc[c])
                    xs[:, c * 128:(c + 1) * 128] = xc
                    lhs = _lhs(xc)
                    for nt in range(early_tiles(c)):
                        r = _dot(lhs, _as_bf16(wq32[pl.ds(c * 8, 8), nt]))[0:4]
                        qacc[nt, 0:4, :] = r if c == 0 else qacc[nt, 0:4, :] + r

        gp[...] = jnp.zeros_like(gp)
        mbuf[...] = jnp.zeros_like(mbuf)
        wait(cps_x_wq())
        start(cps_wo(0))
        x0 = jnp.broadcast_to(xin[...].astype(F32), (8, D))
        sub0 = lax.broadcasted_iota(jnp.int32, (8, D), 0)
        lane0 = lax.broadcasted_iota(jnp.int32, (8, D), 1)
        for nkb, n0, n1 in ((4, 0, early_tiles(3)), (3, early_tiles(3), early_tiles(0))):
            lhs0 = _lhs(jnp.where(sub0 < 4, jnp.where(lane0 < nkb * 128, x0, 0.0), 1.0))

            def q0_body(nt, c, lhs0=lhs0):
                qacc[nt] = _dot(lhs0, _as_bf16(wq32[:, nt]))[0:8]
                return c
            lax.fori_loop(n0, n1, q0_body, 0)
        wait(cps_k(0, 0))
        start(cps_k(2, 0))
        wait(cps_k(1, 1))
        wait(cps_v(0, 0))
        xs[...] = x0

        def layer(li, carry):
            first = li == 0
            n_first = jnp.maximum(1 - li, 0)
            zdyn = li >> 4

            def block_dma(ua, ub):
                def last_wait(t):
                    if t == NU - 2:
                        wait(cps_k(NU - 1, (NU - 1) % 2))
                    else:
                        wait(cps_v(t + 1, (t + 1) % 2) if t + 1 < NU else cps_wo(1))

                def dma_ops(_, c):
                    for t in range(ua, ub):
                        if t + 3 < NU:
                            start(cps_k(t + 3, (t + 3) % 2))
                        if t + 2 < NU:
                            start(cps_v(t + 2, t % 2))
                        if t == NU - 2:
                            start(cps_w3())
                            start(cps_w4(0))
                        if t == NU - 1:
                            start(cps_w4(1))
                            wait(cps_v(t, t % 2))
                            start(cps_w4(2))
                        if t == 1:
                            wait(cps_wo(0))
                            start(cps_wo(1))
                        st_expand(t)
                        if t + 2 < NU - 1:
                            wait(cps_k(t + 2, t % 2))
                        if t < ub - 1:
                            last_wait(t)
                    return c

                lax.fori_loop(0, n_first, dma_ops, 0)
                pl.when(first)(lambda: last_wait(ub - 1))

            def prologue():
                x = xs[...]
                m, r = _ln_stats(x)
                nq = cfg["nq_mxu"]

                def finish_q(u, late):
                    qs = []
                    for nt in range(3):
                        qx = jnp.broadcast_to(qacc[u * 3 + nt, 0:1, :], (8, 128))
                        cs = jnp.broadcast_to(qacc[u * 3 + nt, 4:5, :], (8, 128))
                        qs.append((qx + late[nt] - cs * m) * r)
                    pack_q(jnp.concatenate(qs, axis=1), u)

                lhs = _lhs(x[:, D - 128:D])
                for u in range(nq):
                    finish_q(u, [_dot(lhs, _as_bf16(wq32[pl.ds(32, 8), u * 3 + nt]))[0:8]
                                 for nt in range(3)])
                f1 = cfg["va_force"]
                toks = st_qk(0, range(f1))
                for kb in range(2):
                    cs = slice((3 + kb) * 128, (4 + kb) * 128)
                    blk = jnp.broadcast_to(x[0:1, cs], (128, 128)).T
                    abuf[ns - 1 + zdyn, kb * 128:(kb + 1) * 128, :] = blk
                    qlhs[NU + zdyn, :, 0:128] = pltpu.bitcast(blk[120:128], U32)
                toks += st_qk(0, range(f1, nj))
                st_softmax(0, zdyn)
                toks += st_qk(1, range(js(1)))
                toks += st_pvm(0)
                for va, (t0, t1) in zip(cfg["va_groups"], cfg["va_tok"]):
                    acc = [None] * len(va)
                    for kt in range(16):
                        lo = abuf[ns - 1, pl.ds(kt * 16, 8, stride=2), :]
                        hi = abuf[ns - 1, pl.ds(kt * 16 + 1, 8, stride=2), :]
                        tk = toks[t0 + kt * (t1 - t0) // 16]
                        lo, hi = lo + tk, hi + tk
                        for i, u in enumerate(va):
                            w = wq32[24 + kt, u * 3:u * 3 + 3]
                            pr = (pltpu.bitcast(w << 16, F32) * lo
                                  + pltpu.bitcast(w & jnp.uint32(0xFFFF0000), F32) * hi)
                            acc[i] = pr if acc[i] is None else acc[i] + pr
                    for i, u in enumerate(va):
                        late = []
                        for nt in range(3):
                            q = acc[i][nt]
                            q = q + pltpu.roll(q, 4, 0)
                            q = q + pltpu.roll(q, 2, 0)
                            late.append(q + pltpu.roll(q, 1, 0))
                        finish_q(u, late)
                return toks

            def block(bi):
                ua, ub = cfg["blocks"][bi]
                block_dma(ua, ub)
                toks = []
                if bi == 0:
                    toks += prologue()
                done = js(ua + 1)
                for t in range(ua, ub):
                    base = len(toks)
                    ous = cfg["ored_at"].get(t, ())
                    if t in cfg["ored_pin"]:
                        for i, u in enumerate(ous):
                            nxt = nj - cfg["ored_back"] - (len(ous) - 1 - i) * 11
                            toks += st_qk(t + 1, range(done, nxt))
                            done = max(done, nxt)
                            st_ored(u, pin=zdyn)
                    else:
                        for u in ous:
                            st_ored(u)
                    if t + 1 < NU:
                        toks += st_qk(t + 1, range(done, nj))
                    g0 = len(toks)
                    if t == ua and bi > 0:
                        toks += st_pvm(t)
                    for u in cfg["oproj_at"].get(t, ()):
                        toks += st_oproj(*u) if isinstance(u, tuple) else st_oproj(u)
                    done = js(t + 2)
                    if t + 1 < ub:
                        gap = cfg["gap_at"].get(t, cfg["gap"])
                        done = max(-((len(toks) - g0 - gap) // 3), 0)
                    gap1 = cfg["gap1_at"].get(t, cfg["gap1"])
                    d1 = min(max(-((len(toks) - g0 - gap1) // 3), 0), done)
                    if t + 2 < NU:
                        toks += st_qk(t + 2, range(d1))
                    if t + 1 < NU:
                        st_softmax(t + 1, zdyn, pin=gap1 > 0 and t + 2 < NU and d1 < done)
                    if t + 2 < NU:
                        toks += st_qk(t + 2, range(d1, done))
                    if t + 1 < ub:
                        toks += st_pvm(t + 1)
                    st_pv(t, toks, [base + i for i in cfg["tok"][t]])
                    st_lsum(t)

            for bi in range(len(cfg["blocks"])):
                block(bi)

            def tail(first_static):
                for u in range(*cfg["blocks"][-1]):
                    st_ored(u, partial_rows=(u == NU - 1))
                seen = set()
                for us in cfg["oproj_at"].values():
                    for u in us:
                        uu, ts = u if isinstance(u, tuple) else (u, (0, 1, 2))
                        seen |= {(uu, t) for t in ts}
                for u in range(NU - 1):
                    ts = tuple(t for t in range(3) if (u, t) not in seen)
                    if ts:
                        st_oproj(u, ts)
                extra = [[] for _ in range(D // 128)]
                st_oproj(NU - 1, out=extra)
                mlp(first_static, extra)

            pl.when(first)(lambda: tail(True))
            pl.when(jnp.logical_not(first))(lambda: tail(False))
            return carry

        lax.fori_loop(0, 2, layer, 0)
        o_ref[...] = xs[0:1, :].astype(o_ref.dtype)

    return kernel


@jax.jit
def pallas_interleave_layers__sliding_block_cached__mixer_s_mlp__decode_kernel(
    A_x: jax.Array,
    A_k_cache: jax.Array,
    A_v_cache: jax.Array,
    A_wq: jax.Array,
    A_wo: jax.Array,
    B_x: jax.Array,
    B_w1: jax.Array,
    B_w2: jax.Array,
    B_w3: jax.Array,
    B_w4: jax.Array,
):
    b, sq, d = A_x.shape
    _, hkv, sk, dh = A_k_cache.shape
    assert (b, sq, d, hkv, dh) == (1, 1, D, H, DH)
    win = min(4096, max(256, sk // 4))
    assert win % 512 == 0 and sk % 128 == 0
    nj = win // 128

    kt = _tile_view(jnp.swapaxes(A_k_cache, 2, 3).reshape(H * DH, sk))
    vt = _head_view(jnp.swapaxes(A_v_cache, 2, 3).reshape(H * DH, sk))

    def buf(r, c):
        return pltpu.VMEM((r // 16, c // 128, 16, 128), BF16)

    def hbuf(c):
        return pltpu.VMEM((H, DH // 16, c // 128, 16, 128), BF16)

    bl = CFG["blocks"]
    ns = CFG.get("ns") or max(bl[i + 1][1] - bl[i][0] for i in range(len(bl) - 1))
    any_spec = pl.BlockSpec(memory_space=pl.ANY)
    out = pl.pallas_call(
        _make_kernel(sk, win, CFG),
        out_shape=jax.ShapeDtypeStruct((1, D), A_x.dtype),
        in_specs=[any_spec] * 7,
        out_specs=pl.BlockSpec(memory_space=pltpu.VMEM),
        scratch_shapes=[
            buf(H * DH, win), hbuf(win),
            pltpu.VMEM((H, DH // 16, max(len(CFG["jx"]), 1), 8, 128), F32),
            buf(D, H * DH), hbuf(D), buf(D, FF),
            pltpu.VMEM((D // 128, FF, 128), BF16),
            pltpu.VMEM((1, D), BF16),
            pltpu.VMEM((8, D), F32),
            pltpu.VMEM((H * DH // 128, 8, 128), F32),
            pltpu.VMEM((NU + 1, 8, 384), U32),
            pltpu.VMEM((2, 8, win // 4), F32),
            pltpu.VMEM((2, 8, win // 4), F32),
            pltpu.VMEM((1, 8, win // 4), F32),
            pltpu.VMEM((1, 8, win // 4), F32),
            pltpu.VMEM((8, 512), U32),
            pltpu.VMEM((ns, 2, 3, 8, 128), F32),
            pltpu.VMEM((ns, 8, 128), F32),
            pltpu.VMEM((ns, 384, 128), F32),
            pltpu.VMEM((NU, 8, 384), U32),
            pltpu.VMEM((3, D // 128, NU, 128), F32),
            pltpu.SemaphoreType.DMA((5,)),
        ],
        compiler_params=pltpu.CompilerParams(vmem_limit_bytes=int(CFG["vmem_mb"] * 1024 * 1024)),
        name="interleave_decode",
    )(A_x.reshape(1, D), kt, vt, _tile_view(A_wq), _head_view(A_wo),
      _tile_view(B_w3), B_w4)
    return out.reshape(b, sq, d)
```

```python
import jax
import jax.numpy as jnp
from jax import lax
import jax.experimental.pallas as pl
import jax.experimental.pallas.tpu as pltpu

F32 = jnp.float32
BF16 = jnp.bfloat16
U32 = jnp.uint32

D = 640
H = 32
DH = 192
FF = 1536
NU = H // 2
UT = 2 * DH // 16
EPS = 1e-5
NPIECE = 12

CFG = dict(
    blocks=((0, 4), (4, 8), (8, 12), (12, 15), (15, 16)), ns=7,
    jsplit=10, js_at={1: 13, 5: 19, 9: 19, 13: 16},
    gap=49, gap1=24, gap_at={}, gap1_at={}, ored_pin=(), ored_back=4,
    nm=4, nm_at={12: 5, 13: 5, 14: 5, 15: 0},
    va_groups=((6, 7, 8, 9), (10, 11, 12, 13, 14), (15,)), va_force=7,
    va_tok=((6, 43), (48, 94), (102, 112)),
    ored_at={4: (0,), 5: (1,), 6: (2,), 7: (3,), 8: (4,), 9: (5,), 10: (6,), 11: (7,),
             12: (8,), 13: (9,), 14: (10, 11), 15: (12, 13, 14)},
    oproj_at={4: ((0, (2,)),), 5: ((1, (2,)),), 6: ((2, (2,)),), 7: ((3, (2,)),),
              8: ((4, (0,)), (0, (0,))), 9: ((5, (0,)), (0, (1,))), 10: ((6, (0,)),), 11: ((7, (0,)),),
              12: ((8, (0,)),), 13: ((9, (0,)),),
              14: ((4, (1, 2)), (10, (0,)), (1, (0, 1)), (11, (0,))),
              15: ((2, (0, 1)), (3, (0, 1)), (5, (1, 2)), (6, (1, 2)), (7, (1, 2)), (8, (1, 2)), (9, (1, 2)),
                   (10, (1, 2)), (11, (1, 2)), 12, (13, (0, 1)))},
    jx=(1, 5, 9, 13, 17, 21, 25), vmem_mb=128,
    tok={
        0: [-26,-24,-22,-19,-17,-14,-12,-10,-7,-5,-2,0,2,4,5,9,12,14,17,19,21,24,26,29,31,33,36,38,41,43,45,48,50,52,55,57,60,62,64,67,69,72,74,76,79,81,84,86],
        1: [-32,-29,-27,-25,-22,-18,-17,-15,-13,-10,-8,-5,-3,-1,2,4,7,9,9,11,16,18,21,23,26,28,30,33,38,38,40,42,45,47,49,54,56,57,58,60,62,65,67,69,71,73,76,78],
        2: [-28,-26,-23,-21,-18,-16,-14,-11,-9,-8,-4,-2,0,1,3,8,10,13,15,18,19,22,24,27,29,33,35,38,40,42,45,47,50,52,55,57,59,62,64,67,69,71,74,76,79,81,83,86],
        3: [-20,-17,-13,-11,-10,-8,-6,-3,-3,-1,4,6,9,11,14,16,18,21,24,26,29,31,34,37,39,42,44,47,50,52,52,55,57,63,65,67,70,72,75,77,79,82,84,87,89,91,93,95],
        4: [-27,-24,-22,-19,-17,-15,-12,-10,-7,-5,-3,0,2,5,7,9,12,14,17,19,22,24,27,29,32,34,37,39,42,44,46,49,51,54,56,59,61,64,66,69,71,74,76,79,81,84,86,88],
        5: [-10,-8,-5,-2,0,3,5,8,10,13,15,18,20,23,25,28,30,33,35,38,40,43,45,48,50,53,55,58,60,63,65,68,70,72,75,77,80,82,85,87,90,92,95,97,100,102,105,107],
        6: [-15,-13,-11,-9,-7,-4,-2,0,2,5,8,10,13,16,19,21,24,27,29,31,34,36,39,41,44,46,49,51,54,56,59,61,64,66,69,71,73,76,78,81,83,86,88,91,93,96,98,101],
        7: [-10,-7,-5,-2,0,2,5,7,10,12,15,17,20,22,25,27,30,32,35,38,41,43,46,49,51,54,56,58,60,63,65,67,69,72,74,77,79,82,84,86,89,91,94,96,99,101,104,106],
        8: [-22,-20,-18,-16,-14,-13,-11,-9,-7,-5,-2,0,2,4,6,8,11,13,16,18,21,24,26,29,32,34,37,40,42,45,48,50,53,55,58,60,63,65,67,70,72,75,77,79,82,84,86,89],
        9: [-9,-6,-4,-1,1,4,7,9,12,14,16,19,21,23,26,28,30,33,36,38,41,44,47,49,52,55,57,59,62,64,67,69,72,74,77,79,82,84,87,89,92,94,97,99,102,104,106,109],
        10: [-19,-16,-14,-11,-9,-7,-4,-2,1,3,6,8,10,13,15,18,20,23,25,28,30,33,35,38,40,43,45,48,50,53,56,58,61,63,66,68,70,73,75,78,80,83,85,87,89,92,94,96],
        11: [-21,-18,-16,-13,-10,-8,-5,-2,0,3,5,7,10,12,15,17,19,22,24,27,30,32,35,37,40,43,45,48,51,54,56,59,62,64,67,69,71,74,76,79,81,83,85,87,89,92,94,96],
        12: [-30,-27,-24,-22,-19,-16,-14,-11,-8,-6,-3,-1,2,5,7,10,13,15,18,20,23,25,28,31,33,36,38,41,43,46,48,51,53,56,58,61,63,66,68,71,73,76,78,81,83,86,88,91],
        13: [-20,-18,-15,-13,-10,-8,-6,-3,-1,2,4,7,9,11,14,16,19,21,23,26,28,31,33,35,38,40,43,45,48,50,52,55,57,60,62,64,67,69,72,74,76,79,81,84,86,89,91,93],
        14: [-35,-33,-31,-28,-26,-23,-21,-19,-16,-14,-12,-9,-7,-5,-2,0,2,5,7,10,12,15,17,20,22,25,27,30,32,35,37,40,42,44,47,49,52,54,56,59,61,64,66,69,71,73,76,78],
        15: [-27,-25,-23,-21,-19,-16,-14,-12,-10,-7,-4,0,3,6,9,12,16,19,22,25,29,32,35,38,42,44,46,48,51,53,55,57,59,64,68,73,77,82,86,91,95,96,96,96,96,96,96,96],
    },
    w4_k=8, w4_nv=3, w4_pin=10, w4_tok=(14, 36), nq_mxu=6)


def _tile_view(a):
    r, c = a.shape
    a = a.reshape(r // 16, 2, 8, c // 128, 128)
    return jnp.swapaxes(a, 2, 3)


def _head_view(a):
    c = a.shape[1]
    a = a.reshape(H, 2, DH // 16, 8, c // 128, 128)
    return jnp.swapaxes(a, 3, 4)


def _as_bf16(w32):
    n = w32.shape[0]
    return pltpu.bitcast(w32.reshape(n * 8, 128), BF16)


def _lhs(top, fill=0.0):
    return jnp.concatenate([top, jnp.full(top.shape, fill, F32)], axis=0).astype(BF16)


def _ln_stats(x):
    m = jnp.mean(x, axis=-1, keepdims=True)
    m2 = jnp.mean(x * x, axis=-1, keepdims=True)
    v = jnp.maximum(m2 - m * m, 0.0)
    return m, lax.rsqrt(v + EPS)


def _round_bf16(x):
    return x.astype(BF16).astype(F32)


def _dot(a, b):
    return jnp.dot(a, b, preferred_element_type=F32)


def _make_kernel(sk, win, cfg):
    nj = win // 128
    j0 = (sk - win) // 128
    jq = nj // 4
    jx = list(cfg["jx"])
    assert nj == 32 and cfg["blocks"][-2][0] <= NU - 3 and cfg["blocks"][-1] == (NU - 1, NU)
    qscale = DH ** -0.5 * 1.4426950408889634

    def kernel(x_hbm, k_hbm, v_hbm, wq_hbm, wo_hbm, w3_hbm, w4_hbm, o_ref,
               kbuf, vbuf, vx, wqbuf, wobuf, w3buf, w4buf, xin,
               xs, qacc, qlhs, sx, sy, pbuf0, pbuf1, plhs, mbuf, lpart, abuf, olhs, gp,
               sems):
        pbuf = (pbuf0, pbuf1)
        ns = abuf.shape[0]


        def cps_w(hbm, buf, sem, lo=0, n=None):
            n = buf.shape[0] if n is None else n
            return [pltpu.make_async_copy(
                hbm.at[pl.ds(lo, n), e],
                buf.at[pl.ds(lo, n), :, pl.ds(e * 8, 8), :],
                sems.at[sem]) for e in range(2)]

        def cps_kv(hbm, buf, sem, u):
            return [pltpu.make_async_copy(
                hbm.at[pl.ds(u * UT, UT), e, pl.ds(j0, nj)],
                buf.at[pl.ds(u * UT, UT), :, pl.ds(e * 8, 8), :],
                sems.at[sem]) for e in range(2)]

        def cps_v(u, par):
            return [pltpu.make_async_copy(
                v_hbm.at[pl.ds(2 * u, 2), e, :, pl.ds(j0, nj)],
                vbuf.at[pl.ds(2 * u, 2), :, :, pl.ds(e * 8, 8), :],
                sems.at[2 + par]) for e in range(2)]

        def cps_wo(part):
            lo, n = ((0, H - 8), (H - 8, 8))[part]
            return [pltpu.make_async_copy(
                wo_hbm.at[pl.ds(lo, n), e], wobuf.at[pl.ds(lo, n), :, :, pl.ds(e * 8, 8), :],
                sems.at[4]) for e in range(2)]

        cps_k = lambda u, par: cps_kv(k_hbm, kbuf, par, u)
        cps_x_wq = lambda: cps_w(wq_hbm, wqbuf, 4) + [pltpu.make_async_copy(x_hbm, xin, sems.at[4])]
        cps_w3 = lambda: cps_w(w3_hbm, w3buf, 0)
        w4_k = cfg["w4_k"] * 128
        w4_parts = [(c, 0, FF) for c in range(D // 128 - 1)]
        w4_parts += [(D // 128 - 1, 0, w4_k), (D // 128 - 1, w4_k, FF - w4_k)]

        def cps_w4(i):
            c, lo, n = w4_parts[i]
            return [pltpu.make_async_copy(
                w4_hbm.at[pl.ds(lo, n), pl.ds(c * 128, 128)], w4buf.at[c, pl.ds(lo, n), :],
                sems.at[(2, 1, 3, 0, 4, 2)[i]])]

        def start(cps):
            for c in cps:
                c.start()

        def wait(cps):
            for c in cps:
                c.wait()

        start(cps_x_wq())
        start(cps_k(0, 0))
        start(cps_k(1, 1))
        start(cps_v(0, 0))
        start(cps_v(1, 1))

        k32 = kbuf.bitcast(U32)
        v32 = vbuf.bitcast(U32)
        wq32 = wqbuf.bitcast(U32)
        wo32 = wobuf.bitcast(U32)
        w332 = w3buf.bitcast(U32)
        w432 = w4buf.bitcast(U32)

        def js(u):
            return cfg["js_at"].get(u, cfg["jsplit"])

        def jms(u):
            return [nj - 1 - jq * (i % 4) - i // 4 for i in range(nmx(u))]

        def early_tiles(kb):
            return ((H * DH // 128,) * 3 + (3 * cfg["nq_mxu"], 0))[kb]

        def nmx(u):
            return cfg["nm_at"].get(u, cfg["nm"])

        def pack_q(q, u):
            q = q * qscale
            lane = lax.broadcasted_iota(jnp.int32, (8, 128), 1)
            sub = lax.broadcasted_iota(jnp.int32, (8, 128), 0)
            keep = (lane < DH - 128) == (sub % 2 == 0)
            q = jnp.concatenate(
                [q[:, 0:128], jnp.where(keep, q[:, 128:256], 0.0), q[:, 256:384]], axis=1)
            qlhs.at[u][:, 0:384] = pltpu.bitcast(_lhs(q), U32)

        def st_qk(u, js):
            sl = u % 2
            lhs = pltpu.bitcast(qlhs[u], BF16)
            toks = []
            for j in js:
                ra = 2 * (j // jq)
                cs = slice((j % jq) * 128, (j % jq + 1) * 128)
                for t in range(3):
                    w = _as_bf16(k32[pl.ds(u * UT + t * 8, 8), j])
                    r = _dot(lhs[:, t * 128:(t + 1) * 128], w)
                    toks.append(r[8:16])
                    if t == 0:
                        sx[sl, ra:ra + 1, cs] = r[0:1]
                    elif t == 1:
                        sy[sl, ra:ra + 2, cs] = r[ra:ra + 2]
                    else:
                        sx[sl, ra + 1:ra + 2, cs] = r[0:1]
            return toks

        def st_softmax(u, zdyn, pin=False):
            sl = u % 2
            s = sx[sl] + sy[sl]
            m = s
            while m.shape[1] > 128:
                h = m.shape[1] // 2
                m = jnp.maximum(m[:, :h], m[:, h:])
            m = jnp.maximum(m, pltpu.roll(m, 2, 0))
            m = jnp.maximum(m, pltpu.roll(m, 4, 0))
            if pin:
                qlhs[NU + zdyn, :, 0:128] = pltpu.bitcast(m, U32)
            m = jnp.max(m, axis=1, keepdims=True)
            p = jnp.exp2(s - m)
            pbuf[sl][zdyn] = p
            for g in range((nmx(u) + 3) // 4):
                c = jq - 1 - g
                plhs[:, (2 * sl + g) * 128:(2 * sl + g + 1) * 128] = pltpu.bitcast(
                    _lhs(p[:, c * 128:(c + 1) * 128]), U32)

        def inv_l(l):
            l = jnp.sum(l, axis=1, keepdims=True)
            r0 = pl.reciprocal(l, approx=True)
            return jnp.broadcast_to(r0 * (2.0 - l * r0), (8, 128))

        def st_lsum(u):
            l = pbuf[u % 2][0, :, 0:128]
            for c in range(1, jq):
                l = l + pbuf[u % 2][0, :, c * 128:(c + 1) * 128]
            l = l + pltpu.roll(l, 2, 0)
            l = l + pltpu.roll(l, 4, 0)
            lpart[u % ns] = inv_l(l) if u == NU - 1 else l

        def st_pvm(u):
            toks = []
            for j in jms(u):
                g = jq - 1 - j % jq
                pc = 2 * (u % 2) + g
                lhs = pltpu.bitcast(plhs[:, pc * 128:(pc + 1) * 128], BF16)
                ra = 2 * (j // jq)
                for t in range(3):
                    if t == 1:
                        w32 = jnp.concatenate(
                            [v32[2 * u, 8:12, j], v32[2 * u + 1, 0:4, j]], axis=0)
                    else:
                        w32 = v32[2 * u + t // 2, 2 * t:2 * t + 8, j]
                    r = _dot(lhs, _as_bf16(w32))
                    toks.append(r[8:16])
                    mbuf[u % ns, g, t, ra:ra + 2, :] = r[ra:ra + 2]
            return toks

        def st_expand(u):
            def body(dt, c):
                for hd in range(2):
                    for ix, j in enumerate(jx):
                        w = v32[2 * u + hd, dt, j]
                        vx[2 * u + hd, dt, ix] = pltpu.bitcast(w << 16, F32)
                        vbuf[2 * u + hd, dt, j] = pltpu.bitcast(w & jnp.uint32(0xFFFF0000), BF16)
                return c
            lax.fori_loop(0, UT // 2, body, 0)
            for j in jms(u):
                for t in range(3):
                    idx = [divmod(t * 8 + v, 12) for v in range(8)]
                    blk = jnp.concatenate([vbuf[2 * u + hd, dt, j] for hd, dt in idx], axis=0)
                    blk = blk.astype(F32).T.astype(BF16)
                    for v, (hd, dt) in enumerate(idx):
                        vbuf[2 * u + hd, dt, j] = blk[v * 16:(v + 1) * 16]

        def st_pv(u, toks, tok_map):
            nm, sl = nmx(u), u % ns
            for piece in range(NPIECE):
                hd, half = divmod(piece, NPIECE // 2)
                sub = len(tok_map) // NPIECE
                lo = hi = None
                for j in range(nj):
                    if j in jms(u):
                        continue
                    row = 2 * (j // jq) + hd
                    cs = slice((j % jq) * 128, (j % jq + 1) * 128)
                    pb = jnp.broadcast_to(pbuf[u % 2][0, row:row + 1, cs], (8, 128))
                    k = piece * sub + j * sub // nj
                    ti = tok_map[k] if j % (nj // sub) == 0 else -1
                    if j > 0 and tok_map[k - 1] == ti:
                        ti = -1
                    if toks and ti >= 0:
                        pb = pb + toks[min(ti, len(toks) - 1)]
                    w = v32[2 * u + hd, pl.ds(half * 2, 2), j]
                    if j in jx:
                        a = vx[2 * u + hd, pl.ds(half * 2, 2), jx.index(j)] * pb
                        b = pltpu.bitcast(w, F32) * pb
                    else:
                        a = pltpu.bitcast(w << 16, F32) * pb
                        b = pltpu.bitcast(w & jnp.uint32(0xFFFF0000), F32) * pb
                    lo = a if lo is None else lo + a
                    hi = b if hi is None else hi + b
                for i in range(2):
                    base = (piece * 2 + i) * 16
                    abuf[sl, pl.ds(base, 8, stride=2), :] = lo[i]
                    abuf[sl, pl.ds(base + 1, 8, stride=2), :] = hi[i]

        def st_ored(u, ts=(0, 1, 2), pin=None):
            nm, sl = nmx(u), u % ns
            ia = inv_l(lpart[sl])
            ib = pltpu.roll(ia, 1, 0)
            lane = lax.broadcasted_iota(jnp.int32, (8, 128), 1)
            for t in ts:
                at = abuf[sl, t * 128:(t + 1) * 128, :].T
                if pin is not None:
                    qlhs[NU + pin, :, 0:128] = pltpu.bitcast(at[120:128], U32)
                o = at[0:8]
                for i in range(1, 16):
                    o = o + at[i * 8:(i + 1) * 8]
                if nm:
                    sub = lax.broadcasted_iota(jnp.int32, (8, 128), 0)
                    odd = (0, (lane >= DH - 128).astype(jnp.int32), 1)[t]
                    for g in range((nm + 3) // 4):
                        keep = (sub >= 8 - 2 * min(nm - 4 * g, 4)) & (sub % 2 == odd)
                        o = o + jnp.where(keep, mbuf[sl, g, t], 0.0)
                o = o + pltpu.roll(o, 4, 0)
                o = o + pltpu.roll(o, 2, 0)
                o = o + pltpu.roll(o, 1, 0)
                o = o * (ia, jnp.where(lane < DH - 128, ia, ib), ib)[t]
                olhs.at[u][:, t * 128:(t + 1) * 128] = pltpu.bitcast(_lhs(o), U32)

        def st_olast(u, out):
            sl = u % ns
            for hd in range(2):
                pa = [None, None]
                for dt in range(12):
                    base = (hd * 12 + dt) * 16
                    lo = jnp.sum(abuf[sl, pl.ds(base, 8, stride=2), :], axis=1, keepdims=True)
                    hi = jnp.sum(abuf[sl, pl.ds(base + 1, 8, stride=2), :], axis=1, keepdims=True)
                    w = wo32[2 * u + hd, dt]
                    pr = (pltpu.bitcast(w << 16, F32) * lo
                          + pltpu.bitcast(w & jnp.uint32(0xFFFF0000), F32) * hi)
                    pa[dt % 2] = pr if pa[dt % 2] is None else pa[dt % 2] + pr
                inv = jnp.broadcast_to(lpart[sl, hd:hd + 1, :], (8, 128))
                tot = (pa[0] + pa[1]) * inv
                for n in range(D // 128):
                    out[n].append(tot[n])

        def st_oproj(u, ts=(0, 1, 2)):
            lhs = pltpu.bitcast(olhs[u], BF16)
            toks = []
            for t in ts:
                for n in range(D // 128):
                    if t == 1:
                        w32 = jnp.concatenate(
                            [wo32[2 * u, 8:12, n], wo32[2 * u + 1, 0:4, n]], axis=0)
                    else:
                        w32 = wo32[2 * u + t // 2, 2 * t:2 * t + 8, n]
                    r = _dot(lhs[:, t * 128:(t + 1) * 128], _as_bf16(w32))
                    toks.append(r[8:16])
                    gp[t, n, pl.ds(u, 1), :] = r[0:1]
            return toks

        def mlp(first, extra, zdyn):
            g = gp[0] + gp[1] + gp[2]
            g = g[:, 0:8] + g[:, 8:16]
            g = jnp.concatenate([sum(extra[n], g[n]) for n in range(D // 128)], axis=1)
            g = g + pltpu.roll(g, 4, 0)
            g = g + pltpu.roll(g, 2, 0)
            g = g + pltpu.roll(g, 1, 0)
            x1 = _round_bf16(xs[...] + g)
            lhs = _lhs(x1, 1.0)
            m1, r1 = _ln_stats(x1)
            y = (x1 - m1) * r1
            m2, r2 = _ln_stats(y)
            a = r1 * r2
            b = (m1 * r1 + m2) * r2
            if first:
                wait(cps_w3())
                start(cps_w4(3))
                start(cps_w4(4))
            hl, hs = [], []
            for n in range(FF // 128):
                r = _dot(lhs, _as_bf16(w332[:, n]))
                hn = jax.nn.gelu(r[0:8] * a - r[8:16] * b, approximate=True)
                hl.append(_lhs(hn))
                hs.append(hn)
            acc = x1 + y
            acc = [acc[:, c * 128:(c + 1) * 128] for c in range(D // 128)]

            def w4_dot(kt, c):
                return _dot(hl[kt], pltpu.bitcast(w432[c, kt * 64:(kt + 1) * 64, :], BF16))[0:8]

            if not first:
                nv, kpin, (t0, t1) = cfg["w4_nv"], cfg["w4_pin"], cfg["w4_tok"]
                toks = []
                for kt in range(nv, FF // 128):
                    if nv and kt == kpin:
                        for k in range(nv):
                            blk = jnp.broadcast_to(_round_bf16(hs[k][0:1]), (128, 128)).T
                            abuf[zdyn, k * 128:(k + 1) * 128, :] = blk
                            qlhs[NU + zdyn, :, 0:128] = pltpu.bitcast(blk[120:128], U32)
                        hl[kt] = pltpu.bitcast(qlhs[0, :, 0:128], BF16)
                    if nv and kt + 1 == kpin:
                        qlhs.at[0][:, 0:128] = pltpu.bitcast(hl[kpin], U32)
                    for c in range(D // 128):
                        r = _dot(hl[kt], pltpu.bitcast(w432[c, kt * 64:(kt + 1) * 64, :], BF16))
                        toks.append(r[8:16])
                        acc[c] = acc[c] + r[0:8]
                pa = None
                for dt in range(nv * 8):
                    tk = toks[t0 + dt * (t1 - t0) // (nv * 8)]
                    lo = abuf[0, pl.ds(dt * 16, 8, stride=2), :] + tk
                    hi = abuf[0, pl.ds(dt * 16 + 1, 8, stride=2), :] + tk
                    w = w432[:, dt * 8:(dt + 1) * 8, :]
                    pr = (pltpu.bitcast(w << 16, F32) * lo
                          + pltpu.bitcast(w & jnp.uint32(0xFFFF0000), F32) * hi)
                    pa = pr if pa is None else pa + pr
                for c in range(D // 128 if nv else 0):
                    pc = pa[c]
                    pc = pc + pltpu.roll(pc, 4, 0)
                    pc = pc + pltpu.roll(pc, 2, 0)
                    acc[c] = (pc + pltpu.roll(pc, 1, 0)) + acc[c]
                xs[...] = _round_bf16(jnp.concatenate(acc, axis=1))
                return
            for i, (c, lo, n) in enumerate(w4_parts):
                wait(cps_w4(i))
                if i == 0:
                    start(cps_w4(5))
                    for k, hn in enumerate(hs[cfg["w4_k"]:]):
                        abuf[k // 3, (k % 3) * 128:(k % 3 + 1) * 128, :] = jnp.broadcast_to(
                            _round_bf16(hn[0:1]), (128, 128)).T
                if lo == 0:
                    for kt in range(n // 128):
                        acc[c] = acc[c] + w4_dot(kt, c)
                else:
                    pas = [None] * 4
                    for dt in range(n // 16):
                        w = w432[c, lo // 2 + dt * 8:lo // 2 + (dt + 1) * 8, :]
                        sl, r0 = dt // 24, dt % 24 * 16
                        pr = (pltpu.bitcast(w << 16, F32) * abuf[sl, pl.ds(r0, 8, stride=2), :]
                              + pltpu.bitcast(w & jnp.uint32(0xFFFF0000), F32)
                              * abuf[sl, pl.ds(r0 + 1, 8, stride=2), :])
                        pas[dt % 4] = pr if pas[dt % 4] is None else pas[dt % 4] + pr
                    pa = (pas[0] + pas[1]) + (pas[2] + pas[3])
                    pa = pa + pltpu.roll(pa, 4, 0)
                    pa = pa + pltpu.roll(pa, 2, 0)
                    acc[c] = acc[c] + (pa + pltpu.roll(pa, 1, 0))
                if lo + n == FF:
                    xc = _round_bf16(acc[c])
                    xs[:, c * 128:(c + 1) * 128] = xc
                    lhs = _lhs(xc)
                    for nt in range(early_tiles(c)):
                        r = _dot(lhs, _as_bf16(wq32[pl.ds(c * 8, 8), nt]))[0:4]
                        qacc[nt, 0:4, :] = r if c == 0 else qacc[nt, 0:4, :] + r

        gp[...] = jnp.zeros_like(gp)
        mbuf[...] = jnp.zeros_like(mbuf)
        wait(cps_x_wq())
        start(cps_wo(0))
        x0 = jnp.broadcast_to(xin[...].astype(F32), (8, D))
        sub0 = lax.broadcasted_iota(jnp.int32, (8, D), 0)
        lane0 = lax.broadcasted_iota(jnp.int32, (8, D), 1)
        for nkb, n0, n1 in ((4, 0, early_tiles(3)), (3, early_tiles(3), early_tiles(0))):
            lhs0 = _lhs(jnp.where(sub0 < 4, jnp.where(lane0 < nkb * 128, x0, 0.0), 1.0))

            def q0_body(nt, c, lhs0=lhs0):
                qacc[nt] = _dot(lhs0, _as_bf16(wq32[:, nt]))[0:8]
                return c
            lax.fori_loop(n0, n1, q0_body, 0)
        wait(cps_k(0, 0))
        start(cps_k(2, 0))
        wait(cps_k(1, 1))
        wait(cps_v(0, 0))
        xs[...] = x0

        def layer(li, carry):
            first = li == 0
            n_first = jnp.maximum(1 - li, 0)
            zdyn = li >> 4

            def block_dma(ua, ub):
                def last_wait(t):
                    if t == NU - 2:
                        wait(cps_k(NU - 1, (NU - 1) % 2))
                    else:
                        wait(cps_v(t + 1, (t + 1) % 2) if t + 1 < NU else cps_wo(1))

                def dma_ops(_, c):
                    for t in range(ua, ub):
                        if t + 3 < NU:
                            start(cps_k(t + 3, (t + 3) % 2))
                        if t + 2 < NU:
                            start(cps_v(t + 2, t % 2))
                        if t == NU - 2:
                            start(cps_w3())
                            start(cps_w4(0))
                        if t == NU - 1:
                            start(cps_w4(1))
                            wait(cps_v(t, t % 2))
                            start(cps_w4(2))
                        if t == 1:
                            wait(cps_wo(0))
                            start(cps_wo(1))
                        st_expand(t)
                        if t + 2 < NU - 1:
                            wait(cps_k(t + 2, t % 2))
                        if t < ub - 1:
                            last_wait(t)
                    return c

                lax.fori_loop(0, n_first, dma_ops, 0)
                pl.when(first)(lambda: last_wait(ub - 1))

            def prologue():
                x = xs[...]
                m, r = _ln_stats(x)
                nq = cfg["nq_mxu"]

                def finish_q(u, late):
                    qs = []
                    for nt in range(3):
                        qx = jnp.broadcast_to(qacc[u * 3 + nt, 0:1, :], (8, 128))
                        cs = jnp.broadcast_to(qacc[u * 3 + nt, 4:5, :], (8, 128))
                        qs.append((qx + late[nt] - cs * m) * r)
                    pack_q(jnp.concatenate(qs, axis=1), u)

                lhs = _lhs(x[:, D - 128:D])
                for u in range(nq):
                    finish_q(u, [_dot(lhs, _as_bf16(wq32[pl.ds(32, 8), u * 3 + nt]))[0:8]
                                 for nt in range(3)])
                f1 = cfg["va_force"]
                toks = st_qk(0, range(f1))
                for kb in range(2):
                    cs = slice((3 + kb) * 128, (4 + kb) * 128)
                    blk = jnp.broadcast_to(x[0:1, cs], (128, 128)).T
                    abuf[ns - 1 + zdyn, kb * 128:(kb + 1) * 128, :] = blk
                    qlhs[NU + zdyn, :, 0:128] = pltpu.bitcast(blk[120:128], U32)
                toks += st_qk(0, range(f1, nj))
                st_softmax(0, zdyn)
                toks += st_qk(1, range(js(1)))
                toks += st_pvm(0)
                for va, (t0, t1) in zip(cfg["va_groups"], cfg["va_tok"]):
                    acc = [None] * len(va)
                    for kt in range(16):
                        lo = abuf[ns - 1, pl.ds(kt * 16, 8, stride=2), :]
                        hi = abuf[ns - 1, pl.ds(kt * 16 + 1, 8, stride=2), :]
                        tk = toks[t0 + kt * (t1 - t0) // 16]
                        lo, hi = lo + tk, hi + tk
                        for i, u in enumerate(va):
                            w = wq32[24 + kt, u * 3:u * 3 + 3]
                            pr = (pltpu.bitcast(w << 16, F32) * lo
                                  + pltpu.bitcast(w & jnp.uint32(0xFFFF0000), F32) * hi)
                            acc[i] = pr if acc[i] is None else acc[i] + pr
                    for i, u in enumerate(va):
                        late = []
                        for nt in range(3):
                            q = acc[i][nt]
                            q = q + pltpu.roll(q, 4, 0)
                            q = q + pltpu.roll(q, 2, 0)
                            late.append(q + pltpu.roll(q, 1, 0))
                        finish_q(u, late)
                return toks

            def block(bi):
                ua, ub = cfg["blocks"][bi]
                block_dma(ua, ub)
                toks = []
                if bi == 0:
                    toks += prologue()
                done = js(ua + 1)
                for t in range(ua, ub):
                    base = len(toks)
                    ous = cfg["ored_at"].get(t, ())
                    if t in cfg["ored_pin"]:
                        for i, u in enumerate(ous):
                            nxt = nj - cfg["ored_back"] - (len(ous) - 1 - i) * 11
                            toks += st_qk(t + 1, range(done, nxt))
                            done = max(done, nxt)
                            st_ored(u, pin=zdyn)
                    else:
                        for u in ous:
                            st_ored(u)
                    if t + 1 < NU:
                        toks += st_qk(t + 1, range(done, nj))
                    g0 = len(toks)
                    if t == ua and bi > 0:
                        toks += st_pvm(t)
                    for u in cfg["oproj_at"].get(t, ()):
                        toks += st_oproj(*u) if isinstance(u, tuple) else st_oproj(u)
                    done = js(t + 2)
                    if t + 1 < ub:
                        gap = cfg["gap_at"].get(t, cfg["gap"])
                        done = max(-((len(toks) - g0 - gap) // 3), 0)
                    gap1 = cfg["gap1_at"].get(t, cfg["gap1"])
                    d1 = min(max(-((len(toks) - g0 - gap1) // 3), 0), done)
                    if t + 2 < NU:
                        toks += st_qk(t + 2, range(d1))
                    if t + 1 < NU:
                        st_softmax(t + 1, zdyn, pin=gap1 > 0 and t + 2 < NU and d1 < done)
                    if t + 2 < NU:
                        toks += st_qk(t + 2, range(d1, done))
                    if t + 1 < ub:
                        toks += st_pvm(t + 1)
                    st_pv(t, toks, [base + i for i in cfg["tok"][t]])
                    st_lsum(t)

            def tail(first_static):
                seen = set()
                for us in cfg["oproj_at"].values():
                    for u in us:
                        uu, ts = u if isinstance(u, tuple) else (u, (0, 1, 2))
                        seen |= {(uu, t) for t in ts}
                for u in range(NU - 1):
                    ts = tuple(t for t in range(3) if (u, t) not in seen)
                    if ts:
                        st_oproj(u, ts)
                extra = [[] for _ in range(D // 128)]
                st_olast(NU - 1, extra)
                mlp(first_static, extra, zdyn)

            for bi in range(len(cfg["blocks"])):
                block(bi)

            pl.when(first)(lambda: tail(True))
            pl.when(jnp.logical_not(first))(lambda: tail(False))
            return carry

        lax.fori_loop(0, 2, layer, 0)
        o_ref[...] = xs[0:1, :].astype(o_ref.dtype)

    return kernel


@jax.jit
def pallas_interleave_layers__sliding_block_cached__mixer_s_mlp__decode_kernel(
    A_x: jax.Array,
    A_k_cache: jax.Array,
    A_v_cache: jax.Array,
    A_wq: jax.Array,
    A_wo: jax.Array,
    B_x: jax.Array,
    B_w1: jax.Array,
    B_w2: jax.Array,
    B_w3: jax.Array,
    B_w4: jax.Array,
):
    b, sq, d = A_x.shape
    _, hkv, sk, dh = A_k_cache.shape
    assert (b, sq, d, hkv, dh) == (1, 1, D, H, DH)
    win = min(4096, max(256, sk // 4))
    assert win % 512 == 0 and sk % 128 == 0
    nj = win // 128

    kt = _tile_view(jnp.swapaxes(A_k_cache, 2, 3).reshape(H * DH, sk))
    vt = _head_view(jnp.swapaxes(A_v_cache, 2, 3).reshape(H * DH, sk))

    def buf(r, c):
        return pltpu.VMEM((r // 16, c // 128, 16, 128), BF16)

    def hbuf(c):
        return pltpu.VMEM((H, DH // 16, c // 128, 16, 128), BF16)

    bl = CFG["blocks"]
    ns = CFG.get("ns") or max(bl[i + 1][1] - bl[i][0] for i in range(len(bl) - 1))
    any_spec = pl.BlockSpec(memory_space=pl.ANY)
    out = pl.pallas_call(
        _make_kernel(sk, win, CFG),
        out_shape=jax.ShapeDtypeStruct((1, D), A_x.dtype),
        in_specs=[any_spec] * 7,
        out_specs=pl.BlockSpec(memory_space=pltpu.VMEM),
        scratch_shapes=[
            buf(H * DH, win), hbuf(win),
            pltpu.VMEM((H, DH // 16, max(len(CFG["jx"]), 1), 8, 128), F32),
            buf(D, H * DH), hbuf(D), buf(D, FF),
            pltpu.VMEM((D // 128, FF, 128), BF16),
            pltpu.VMEM((1, D), BF16),
            pltpu.VMEM((8, D), F32),
            pltpu.VMEM((H * DH // 128, 8, 128), F32),
            pltpu.VMEM((NU + 1, 8, 384), U32),
            pltpu.VMEM((2, 8, win // 4), F32),
            pltpu.VMEM((2, 8, win // 4), F32),
            pltpu.VMEM((1, 8, win // 4), F32),
            pltpu.VMEM((1, 8, win // 4), F32),
            pltpu.VMEM((8, 512), U32),
            pltpu.VMEM((ns, 2, 3, 8, 128), F32),
            pltpu.VMEM((ns, 8, 128), F32),
            pltpu.VMEM((ns, 384, 128), F32),
            pltpu.VMEM((NU, 8, 384), U32),
            pltpu.VMEM((3, D // 128, NU, 128), F32),
            pltpu.SemaphoreType.DMA((5,)),
        ],
        compiler_params=pltpu.CompilerParams(vmem_limit_bytes=int(CFG["vmem_mb"] * 1024 * 1024)),
        name="interleave_decode",
    )(A_x.reshape(1, D), kt, vt, _tile_view(A_wq), _head_view(A_wo),
      _tile_view(B_w3), B_w4)
    return out.reshape(b, sq, d)
```

```python
import jax
import jax.numpy as jnp
from jax import lax
import jax.experimental.pallas as pl
import jax.experimental.pallas.tpu as pltpu

F32 = jnp.float32
BF16 = jnp.bfloat16
U32 = jnp.uint32

D = 640
H = 32
DH = 192
FF = 1536
NU = H // 2
UT = 2 * DH // 16
EPS = 1e-5
NPIECE = 12

CFG = dict(
    blocks=((0, 4), (4, 8), (8, 12), (12, 15), (15, 16)), ns=7,
    jsplit=10, js_at={1: 13, 5: 19, 9: 19, 13: 16},
    gap=49, gap1=24, gap_at={}, gap1_at={}, ored_pin=(), ored_back=4,
    nm=4, nm_at={12: 5, 13: 5, 14: 5, 15: 0},
    va_groups=((6, 7, 8, 9), (10, 11, 12, 13, 14), (15,)), va_force=7,
    va_tok=((6, 43), (48, 94), (102, 112)),
    ored_at={4: (0,), 5: (1,), 6: (2,), 7: (3,), 8: (4,), 9: (5,), 10: (6,), 11: (7,),
             12: (8,), 13: (9,), 14: (10, 11), 15: (12, 13, 14)},
    oproj_at={4: ((0, (2,)),), 5: ((1, (2,)),), 6: ((2, (2,)),), 7: ((3, (2,)),),
              8: ((4, (0,)), (0, (0,))), 9: ((5, (0,)), (0, (1,))), 10: ((6, (0,)),), 11: ((7, (0,)),),
              12: ((8, (0,)),), 13: ((9, (0,)),),
              14: ((4, (1, 2)), (10, (0,)), (1, (0, 1)), (11, (0,))),
              15: ((2, (0, 1)), (3, (0, 1)), (5, (1, 2)), (6, (1, 2)), (7, (1, 2)), (8, (1, 2)), (9, (1, 2)),
                   (10, (1, 2)), (11, (1, 2)), 12, (13, (0, 1)))},
    jx=(1, 5, 9, 13, 17, 21, 25), vmem_mb=128,
    tok={
        0: [-26,-24,-22,-19,-17,-15,-13,-10,-8,-6,-3,-1,1,4,6,9,11,14,16,19,21,24,26,28,31,34,36,39,41,44,46,49,51,54,57,59,62,64,66,68,71,73,75,77,79,82,84,86],
        1: [-32,-29,-27,-25,-22,-20,-17,-15,-13,-10,-8,-5,-3,-1,2,4,7,9,11,14,16,18,21,23,26,28,30,33,35,37,40,42,44,47,49,51,54,56,58,60,62,65,67,69,71,73,76,78],
        2: [-28,-26,-23,-21,-18,-16,-14,-11,-9,-7,-4,-2,1,3,6,8,10,13,15,18,20,23,25,28,30,33,35,37,40,42,45,47,50,52,55,57,59,62,65,67,70,73,75,78,81,83,86,89],
        3: [-17,-15,-13,-10,-8,-6,-4,-2,0,2,5,7,9,11,14,16,19,22,24,27,29,32,34,37,39,42,44,47,49,52,55,57,60,62,65,67,70,72,74,77,79,81,84,86,88,90,93,95],
        4: [-27,-24,-22,-19,-17,-15,-12,-10,-7,-5,-4,-2,0,2,4,6,8,11,14,17,20,23,26,29,32,34,37,39,42,44,46,49,51,54,56,59,61,64,66,69,71,74,76,79,81,84,86,88],
        5: [-10,-8,-5,-2,0,3,5,8,10,13,15,18,20,23,25,28,30,33,35,38,40,43,45,48,50,53,56,58,61,64,66,69,71,74,76,78,80,82,84,87,89,91,94,97,99,102,104,107],
        6: [-15,-13,-11,-9,-7,-4,-2,0,2,5,8,10,13,16,19,21,24,27,29,31,34,36,39,41,44,46,49,51,54,56,59,61,64,66,69,71,73,76,78,81,83,86,88,91,93,96,98,101],
        7: [-10,-7,-5,-2,0,2,5,7,10,12,15,17,20,22,25,27,30,32,35,38,41,43,46,49,51,54,56,58,60,63,65,67,69,72,74,77,79,82,84,86,89,91,94,96,98,100,103,105],
        8: [-23,-21,-19,-17,-15,-14,-12,-10,-8,-6,-3,-1,1,3,5,7,10,12,15,17,20,23,25,28,31,33,36,39,41,44,47,49,52,54,57,59,62,64,66,69,71,74,76,79,81,84,87,89],
        9: [-8,-6,-4,-1,1,4,6,8,11,13,16,18,21,24,26,29,31,34,36,39,42,44,47,49,52,55,57,59,62,64,67,69,72,74,77,79,82,84,87,89,92,94,97,99,102,104,106,109],
        10: [-19,-16,-14,-11,-9,-7,-4,-2,1,3,6,8,10,13,15,18,20,23,25,28,30,33,35,38,40,43,45,48,50,53,56,58,61,63,66,68,70,73,75,78,80,83,85,88,90,93,95,98],
        11: [-19,-16,-14,-11,-8,-6,-3,0,2,5,7,9,12,14,17,19,21,24,26,29,32,34,37,39,42,45,47,50,53,56,58,61,64,66,69,71,73,76,78,81,83,85,88,90,92,94,97,99],
        12: [-29,-27,-24,-21,-19,-16,-14,-11,-8,-6,-3,-1,2,5,7,10,13,15,18,20,23,25,28,31,33,35,38,40,43,45,47,50,52,55,57,60,63,66,68,71,74,76,78,80,83,85,87,89],
        13: [-21,-19,-17,-14,-12,-9,-7,-5,-2,0,3,5,7,10,12,15,17,19,21,23,25,27,29,31,33,36,39,42,45,47,50,53,56,58,61,63,65,68,70,73,75,77,80,82,84,86,89,91],
        14: [-38,-36,-34,-32,-30,-28,-26,-24,-22,-19,-16,-13,-11,-8,-5,-2,1,3,6,8,11,13,16,18,21,23,26,28,31,33,36,38,40,43,45,48,50,53,55,57,60,63,65,68,71,74,77,79],
        15: [-27,-25,-23,-21,-19,-16,-14,-12,-10,-7,-4,0,3,6,9,12,16,19,22,25,29,32,35,38,42,44,46,48,51,53,55,57,59,64,68,73,77,82,86,91,95,96,96,96,96,96,96,96],
    },
    w4_k=8, w4_nv=3, w4_pin=10, w4_tok=(14, 36), nq_mxu=6)


def _tile_view(a):
    r, c = a.shape
    a = a.reshape(r // 16, 2, 8, c // 128, 128)
    return jnp.swapaxes(a, 2, 3)


def _head_view(a):
    c = a.shape[1]
    a = a.reshape(H, 2, DH // 16, 8, c // 128, 128)
    return jnp.swapaxes(a, 3, 4)


def _as_bf16(w32):
    n = w32.shape[0]
    return pltpu.bitcast(w32.reshape(n * 8, 128), BF16)


def _lhs(top, fill=0.0):
    return jnp.concatenate([top, jnp.full(top.shape, fill, F32)], axis=0).astype(BF16)


def _ln_stats(x):
    m = jnp.mean(x, axis=-1, keepdims=True)
    m2 = jnp.mean(x * x, axis=-1, keepdims=True)
    v = jnp.maximum(m2 - m * m, 0.0)
    return m, lax.rsqrt(v + EPS)


def _round_bf16(x):
    return x.astype(BF16).astype(F32)


def _dot(a, b):
    return jnp.dot(a, b, preferred_element_type=F32)


def _make_kernel(sk, win, cfg):
    nj = win // 128
    j0 = (sk - win) // 128
    jq = nj // 4
    jx = list(cfg["jx"])
    assert nj == 32 and cfg["blocks"][-2][0] <= NU - 3 and cfg["blocks"][-1] == (NU - 1, NU)
    qscale = DH ** -0.5 * 1.4426950408889634

    def kernel(x_hbm, k_hbm, v_hbm, wq_hbm, wo_hbm, w3_hbm, w4_hbm, o_ref,
               kbuf, vbuf, vx, wqbuf, wobuf, w3buf, w4buf, xin,
               xs, qacc, qlhs, sx, sy, pbuf0, pbuf1, plhs, mbuf, lpart, abuf, olhs, gp,
               sems):
        pbuf = (pbuf0, pbuf1)
        ns = abuf.shape[0]


        def cps_w(hbm, buf, sem, lo=0, n=None):
            n = buf.shape[0] if n is None else n
            return [pltpu.make_async_copy(
                hbm.at[pl.ds(lo, n), e],
                buf.at[pl.ds(lo, n), :, pl.ds(e * 8, 8), :],
                sems.at[sem]) for e in range(2)]

        def cps_kv(hbm, buf, sem, u):
            return [pltpu.make_async_copy(
                hbm.at[pl.ds(u * UT, UT), e, pl.ds(j0, nj)],
                buf.at[pl.ds(u * UT, UT), :, pl.ds(e * 8, 8), :],
                sems.at[sem]) for e in range(2)]

        def cps_v(u, par):
            return [pltpu.make_async_copy(
                v_hbm.at[pl.ds(2 * u, 2), e, :, pl.ds(j0, nj)],
                vbuf.at[pl.ds(2 * u, 2), :, :, pl.ds(e * 8, 8), :],
                sems.at[2 + par]) for e in range(2)]

        def cps_wo(part):
            lo, n = ((0, H - 8), (H - 8, 8))[part]
            return [pltpu.make_async_copy(
                wo_hbm.at[pl.ds(lo, n), e], wobuf.at[pl.ds(lo, n), :, :, pl.ds(e * 8, 8), :],
                sems.at[4]) for e in range(2)]

        cps_k = lambda u, par: cps_kv(k_hbm, kbuf, par, u)
        cps_x_wq = lambda: cps_w(wq_hbm, wqbuf, 4) + [pltpu.make_async_copy(x_hbm, xin, sems.at[4])]
        cps_w3 = lambda: cps_w(w3_hbm, w3buf, 0)
        w4_k = cfg["w4_k"] * 128
        w4_parts = [(c, 0, FF) for c in range(D // 128 - 1)]
        w4_parts += [(D // 128 - 1, 0, w4_k), (D // 128 - 1, w4_k, FF - w4_k)]

        def cps_w4(i):
            c, lo, n = w4_parts[i]
            return [pltpu.make_async_copy(
                w4_hbm.at[pl.ds(lo, n), pl.ds(c * 128, 128)], w4buf.at[c, pl.ds(lo, n), :],
                sems.at[(2, 1, 3, 0, 4, 2)[i]])]

        def start(cps):
            for c in cps:
                c.start()

        def wait(cps):
            for c in cps:
                c.wait()

        start(cps_x_wq())
        start(cps_k(0, 0))
        start(cps_k(1, 1))
        start(cps_v(0, 0))
        start(cps_v(1, 1))

        k32 = kbuf.bitcast(U32)
        v32 = vbuf.bitcast(U32)
        wq32 = wqbuf.bitcast(U32)
        wo32 = wobuf.bitcast(U32)
        w332 = w3buf.bitcast(U32)
        w432 = w4buf.bitcast(U32)

        def js(u):
            return cfg["js_at"].get(u, cfg["jsplit"])

        def jms(u):
            return [nj - 1 - jq * (i % 4) - i // 4 for i in range(nmx(u))]

        def early_tiles(kb):
            return ((H * DH // 128,) * 3 + (3 * cfg["nq_mxu"], 0))[kb]

        def nmx(u):
            return cfg["nm_at"].get(u, cfg["nm"])

        def pack_q(q, u):
            q = q * qscale
            lane = lax.broadcasted_iota(jnp.int32, (8, 128), 1)
            sub = lax.broadcasted_iota(jnp.int32, (8, 128), 0)
            keep = (lane < DH - 128) == (sub % 2 == 0)
            q = jnp.concatenate(
                [q[:, 0:128], jnp.where(keep, q[:, 128:256], 0.0), q[:, 256:384]], axis=1)
            qlhs.at[u][:, 0:384] = pltpu.bitcast(_lhs(q), U32)

        def st_qk(u, js):
            sl = u % 2
            lhs = pltpu.bitcast(qlhs[u], BF16)
            toks = []
            for j in js:
                ra = 2 * (j // jq)
                cs = slice((j % jq) * 128, (j % jq + 1) * 128)
                for t in range(3):
                    w = _as_bf16(k32[pl.ds(u * UT + t * 8, 8), j])
                    r = _dot(lhs[:, t * 128:(t + 1) * 128], w)
                    toks.append(r[8:16])
                    if t == 0:
                        sx[sl, ra:ra + 1, cs] = r[0:1]
                    elif t == 1:
                        sy[sl, ra:ra + 2, cs] = r[ra:ra + 2]
                    else:
                        sx[sl, ra + 1:ra + 2, cs] = r[0:1]
            return toks

        def st_softmax(u, zdyn, pin=False):
            sl = u % 2
            s = sx[sl] + sy[sl]
            m = s
            while m.shape[1] > 128:
                h = m.shape[1] // 2
                m = jnp.maximum(m[:, :h], m[:, h:])
            m = jnp.maximum(m, pltpu.roll(m, 2, 0))
            m = jnp.maximum(m, pltpu.roll(m, 4, 0))
            if pin:
                qlhs[NU + zdyn, :, 0:128] = pltpu.bitcast(m, U32)
            m = jnp.max(m, axis=1, keepdims=True)
            p = jnp.exp2(s - m)
            pbuf[sl][zdyn] = p
            for g in range((nmx(u) + 3) // 4):
                c = jq - 1 - g
                plhs[:, (2 * sl + g) * 128:(2 * sl + g + 1) * 128] = pltpu.bitcast(
                    _lhs(p[:, c * 128:(c + 1) * 128]), U32)

        def inv_l(l):
            l = jnp.sum(l, axis=1, keepdims=True)
            r0 = pl.reciprocal(l, approx=True)
            return jnp.broadcast_to(r0 * (2.0 - l * r0), (8, 128))

        def st_lsum(u):
            l = pbuf[u % 2][0, :, 0:128]
            for c in range(1, jq):
                l = l + pbuf[u % 2][0, :, c * 128:(c + 1) * 128]
            l = l + pltpu.roll(l, 2, 0)
            l = l + pltpu.roll(l, 4, 0)
            lpart[u % ns] = inv_l(l) if u == NU - 1 else l

        def st_pvm(u):
            toks = []
            for j in jms(u):
                g = jq - 1 - j % jq
                pc = 2 * (u % 2) + g
                lhs = pltpu.bitcast(plhs[:, pc * 128:(pc + 1) * 128], BF16)
                ra = 2 * (j // jq)
                for t in range(3):
                    if t == 1:
                        w32 = jnp.concatenate(
                            [v32[2 * u, 8:12, j], v32[2 * u + 1, 0:4, j]], axis=0)
                    else:
                        w32 = v32[2 * u + t // 2, 2 * t:2 * t + 8, j]
                    r = _dot(lhs, _as_bf16(w32))
                    toks.append(r[8:16])
                    mbuf[u % ns, g, t, ra:ra + 2, :] = r[ra:ra + 2]
            return toks

        def st_expand(u):
            def body(dt, c):
                for hd in range(2):
                    for ix, j in enumerate(jx):
                        w = v32[2 * u + hd, dt, j]
                        vx[2 * u + hd, dt, ix] = pltpu.bitcast(w << 16, F32)
                        vbuf[2 * u + hd, dt, j] = pltpu.bitcast(w & jnp.uint32(0xFFFF0000), BF16)
                return c
            lax.fori_loop(0, UT // 2, body, 0)
            for j in jms(u):
                for t in range(3):
                    idx = [divmod(t * 8 + v, 12) for v in range(8)]
                    blk = jnp.concatenate([vbuf[2 * u + hd, dt, j] for hd, dt in idx], axis=0)
                    blk = blk.astype(F32).T.astype(BF16)
                    for v, (hd, dt) in enumerate(idx):
                        vbuf[2 * u + hd, dt, j] = blk[v * 16:(v + 1) * 16]

        def st_pv(u, toks, tok_map):
            nm, sl = nmx(u), u % ns
            for piece in range(NPIECE):
                hd, half = divmod(piece, NPIECE // 2)
                sub = len(tok_map) // NPIECE
                lo = hi = None
                for j in range(nj):
                    if j in jms(u):
                        continue
                    row = 2 * (j // jq) + hd
                    cs = slice((j % jq) * 128, (j % jq + 1) * 128)
                    pb = jnp.broadcast_to(pbuf[u % 2][0, row:row + 1, cs], (8, 128))
                    k = piece * sub + j * sub // nj
                    ti = tok_map[k] if j % (nj // sub) == 0 else -1
                    if j > 0 and tok_map[k - 1] == ti:
                        ti = -1
                    if toks and ti >= 0:
                        pb = pb + toks[min(ti, len(toks) - 1)]
                    w = v32[2 * u + hd, pl.ds(half * 2, 2), j]
                    if j in jx:
                        a = vx[2 * u + hd, pl.ds(half * 2, 2), jx.index(j)] * pb
                        b = pltpu.bitcast(w, F32) * pb
                    else:
                        a = pltpu.bitcast(w << 16, F32) * pb
                        b = pltpu.bitcast(w & jnp.uint32(0xFFFF0000), F32) * pb
                    lo = a if lo is None else lo + a
                    hi = b if hi is None else hi + b
                for i in range(2):
                    base = (piece * 2 + i) * 16
                    abuf[sl, pl.ds(base, 8, stride=2), :] = lo[i]
                    abuf[sl, pl.ds(base + 1, 8, stride=2), :] = hi[i]

        def st_ored(u, ts=(0, 1, 2), pin=None):
            nm, sl = nmx(u), u % ns
            ia = inv_l(lpart[sl])
            ib = pltpu.roll(ia, 1, 0)
            lane = lax.broadcasted_iota(jnp.int32, (8, 128), 1)
            for t in ts:
                at = abuf[sl, t * 128:(t + 1) * 128, :].T
                if pin is not None:
                    qlhs[NU + pin, :, 0:128] = pltpu.bitcast(at[120:128], U32)
                o = at[0:8]
                for i in range(1, 16):
                    o = o + at[i * 8:(i + 1) * 8]
                if nm:
                    sub = lax.broadcasted_iota(jnp.int32, (8, 128), 0)
                    odd = (0, (lane >= DH - 128).astype(jnp.int32), 1)[t]
                    for g in range((nm + 3) // 4):
                        keep = (sub >= 8 - 2 * min(nm - 4 * g, 4)) & (sub % 2 == odd)
                        o = o + jnp.where(keep, mbuf[sl, g, t], 0.0)
                o = o + pltpu.roll(o, 4, 0)
                o = o + pltpu.roll(o, 2, 0)
                o = o + pltpu.roll(o, 1, 0)
                o = o * (ia, jnp.where(lane < DH - 128, ia, ib), ib)[t]
                olhs.at[u][:, t * 128:(t + 1) * 128] = pltpu.bitcast(_lhs(o), U32)

        def st_olast(u, out):
            sl = u % ns
            for hd in range(2):
                pa = [None, None]
                for dt in range(12):
                    base = (hd * 12 + dt) * 16
                    lo = jnp.sum(abuf[sl, pl.ds(base, 8, stride=2), :], axis=1, keepdims=True)
                    hi = jnp.sum(abuf[sl, pl.ds(base + 1, 8, stride=2), :], axis=1, keepdims=True)
                    w = wo32[2 * u + hd, dt]
                    pr = (pltpu.bitcast(w << 16, F32) * lo
                          + pltpu.bitcast(w & jnp.uint32(0xFFFF0000), F32) * hi)
                    pa[dt % 2] = pr if pa[dt % 2] is None else pa[dt % 2] + pr
                inv = jnp.broadcast_to(lpart[sl, hd:hd + 1, :], (8, 128))
                tot = (pa[0] + pa[1]) * inv
                for n in range(D // 128):
                    out[n].append(tot[n])

        def st_oproj(u, ts=(0, 1, 2)):
            lhs = pltpu.bitcast(olhs[u], BF16)
            toks = []
            for t in ts:
                for n in range(D // 128):
                    if t == 1:
                        w32 = jnp.concatenate(
                            [wo32[2 * u, 8:12, n], wo32[2 * u + 1, 0:4, n]], axis=0)
                    else:
                        w32 = wo32[2 * u + t // 2, 2 * t:2 * t + 8, n]
                    r = _dot(lhs[:, t * 128:(t + 1) * 128], _as_bf16(w32))
                    toks.append(r[8:16])
                    gp[t, n, pl.ds(u, 1), :] = r[0:1]
            return toks

        def mlp(first, extra, zdyn):
            g = gp[0] + gp[1] + gp[2]
            g = g[:, 0:8] + g[:, 8:16]
            g = jnp.concatenate([sum(extra[n], g[n]) for n in range(D // 128)], axis=1)
            g = g + pltpu.roll(g, 4, 0)
            g = g + pltpu.roll(g, 2, 0)
            g = g + pltpu.roll(g, 1, 0)
            x1 = _round_bf16(xs[...] + g)
            lhs = _lhs(x1, 1.0)
            m1, r1 = _ln_stats(x1)
            y = (x1 - m1) * r1
            m2, r2 = _ln_stats(y)
            a = r1 * r2
            b = (m1 * r1 + m2) * r2
            if first:
                wait(cps_w3())
                start(cps_w4(3))
                start(cps_w4(4))
            hl, hs = [], []
            for n in range(FF // 128):
                r = _dot(lhs, _as_bf16(w332[:, n]))
                hn = jax.nn.gelu(r[0:8] * a - r[8:16] * b, approximate=True)
                hl.append(_lhs(hn))
                hs.append(hn)
            acc = x1 + y
            acc = [acc[:, c * 128:(c + 1) * 128] for c in range(D // 128)]

            def w4_dot(kt, c):
                return _dot(hl[kt], pltpu.bitcast(w432[c, kt * 64:(kt + 1) * 64, :], BF16))[0:8]

            if not first:
                nv, kpin, (t0, t1) = cfg["w4_nv"], cfg["w4_pin"], cfg["w4_tok"]
                toks = []
                for kt in range(nv, FF // 128):
                    if nv and kt == kpin:
                        for k in range(nv):
                            blk = jnp.broadcast_to(_round_bf16(hs[k][0:1]), (128, 128)).T
                            abuf[zdyn, k * 128:(k + 1) * 128, :] = blk
                            qlhs[NU + zdyn, :, 0:128] = pltpu.bitcast(blk[120:128], U32)
                        hl[kt] = pltpu.bitcast(qlhs[0, :, 0:128], BF16)
                    if nv and kt + 1 == kpin:
                        qlhs.at[0][:, 0:128] = pltpu.bitcast(hl[kpin], U32)
                    for c in range(D // 128):
                        r = _dot(hl[kt], pltpu.bitcast(w432[c, kt * 64:(kt + 1) * 64, :], BF16))
                        toks.append(r[8:16])
                        acc[c] = acc[c] + r[0:8]
                pa = None
                for dt in range(nv * 8):
                    tk = toks[t0 + dt * (t1 - t0) // (nv * 8)]
                    lo = abuf[0, pl.ds(dt * 16, 8, stride=2), :] + tk
                    hi = abuf[0, pl.ds(dt * 16 + 1, 8, stride=2), :] + tk
                    w = w432[:, dt * 8:(dt + 1) * 8, :]
                    pr = (pltpu.bitcast(w << 16, F32) * lo
                          + pltpu.bitcast(w & jnp.uint32(0xFFFF0000), F32) * hi)
                    pa = pr if pa is None else pa + pr
                for c in range(D // 128 if nv else 0):
                    pc = pa[c]
                    pc = pc + pltpu.roll(pc, 4, 0)
                    pc = pc + pltpu.roll(pc, 2, 0)
                    acc[c] = (pc + pltpu.roll(pc, 1, 0)) + acc[c]
                xs[...] = _round_bf16(jnp.concatenate(acc, axis=1))
                return
            for i, (c, lo, n) in enumerate(w4_parts):
                wait(cps_w4(i))
                if i == 0:
                    start(cps_w4(5))
                    for k, hn in enumerate(hs[cfg["w4_k"]:]):
                        abuf[k // 3, (k % 3) * 128:(k % 3 + 1) * 128, :] = jnp.broadcast_to(
                            _round_bf16(hn[0:1]), (128, 128)).T
                if lo == 0:
                    for kt in range(n // 128):
                        acc[c] = acc[c] + w4_dot(kt, c)
                else:
                    pas = [None] * 4
                    for dt in range(n // 16):
                        w = w432[c, lo // 2 + dt * 8:lo // 2 + (dt + 1) * 8, :]
                        sl, r0 = dt // 24, dt % 24 * 16
                        pr = (pltpu.bitcast(w << 16, F32) * abuf[sl, pl.ds(r0, 8, stride=2), :]
                              + pltpu.bitcast(w & jnp.uint32(0xFFFF0000), F32)
                              * abuf[sl, pl.ds(r0 + 1, 8, stride=2), :])
                        pas[dt % 4] = pr if pas[dt % 4] is None else pas[dt % 4] + pr
                    pa = (pas[0] + pas[1]) + (pas[2] + pas[3])
                    pa = pa + pltpu.roll(pa, 4, 0)
                    pa = pa + pltpu.roll(pa, 2, 0)
                    acc[c] = acc[c] + (pa + pltpu.roll(pa, 1, 0))
                if lo + n == FF:
                    xc = _round_bf16(acc[c])
                    xs[:, c * 128:(c + 1) * 128] = xc
                    lhs = _lhs(xc)
                    for nt in range(early_tiles(c)):
                        r = _dot(lhs, _as_bf16(wq32[pl.ds(c * 8, 8), nt]))[0:4]
                        qacc[nt, 0:4, :] = r if c == 0 else qacc[nt, 0:4, :] + r

        gp[...] = jnp.zeros_like(gp)
        mbuf[...] = jnp.zeros_like(mbuf)
        wait(cps_x_wq())
        start(cps_wo(0))
        x0 = jnp.broadcast_to(xin[...].astype(F32), (8, D))
        sub0 = lax.broadcasted_iota(jnp.int32, (8, D), 0)
        lane0 = lax.broadcasted_iota(jnp.int32, (8, D), 1)
        for nkb, n0, n1 in ((4, 0, early_tiles(3)), (3, early_tiles(3), early_tiles(0))):
            lhs0 = _lhs(jnp.where(sub0 < 4, jnp.where(lane0 < nkb * 128, x0, 0.0), 1.0))

            def q0_body(nt, c, lhs0=lhs0):
                qacc[nt] = _dot(lhs0, _as_bf16(wq32[:, nt]))[0:8]
                return c
            lax.fori_loop(n0, n1, q0_body, 0)
        wait(cps_k(0, 0))
        start(cps_k(2, 0))
        wait(cps_k(1, 1))
        wait(cps_v(0, 0))
        xs[...] = x0

        def layer(li, carry):
            first = li == 0
            n_first = jnp.maximum(1 - li, 0)
            zdyn = li >> 4

            def block_dma(ua, ub):
                def last_wait(t):
                    if t == NU - 2:
                        wait(cps_k(NU - 1, (NU - 1) % 2))
                    else:
                        wait(cps_v(t + 1, (t + 1) % 2) if t + 1 < NU else cps_wo(1))

                def dma_ops(_, c):
                    for t in range(ua, ub):
                        if t + 3 < NU:
                            start(cps_k(t + 3, (t + 3) % 2))
                        if t + 2 < NU:
                            start(cps_v(t + 2, t % 2))
                        if t == NU - 2:
                            start(cps_w3())
                            start(cps_w4(0))
                        if t == NU - 1:
                            start(cps_w4(1))
                            wait(cps_v(t, t % 2))
                            start(cps_w4(2))
                        if t == 1:
                            wait(cps_wo(0))
                            start(cps_wo(1))
                        st_expand(t)
                        if t + 2 < NU - 1:
                            wait(cps_k(t + 2, t % 2))
                        if t < ub - 1:
                            last_wait(t)
                    return c

                lax.fori_loop(0, n_first, dma_ops, 0)
                pl.when(first)(lambda: last_wait(ub - 1))

            def prologue():
                x = xs[...]
                m, r = _ln_stats(x)
                nq = cfg["nq_mxu"]

                def finish_q(u, late):
                    qs = []
                    for nt in range(3):
                        qx = jnp.broadcast_to(qacc[u * 3 + nt, 0:1, :], (8, 128))
                        cs = jnp.broadcast_to(qacc[u * 3 + nt, 4:5, :], (8, 128))
                        qs.append((qx + late[nt] - cs * m) * r)
                    pack_q(jnp.concatenate(qs, axis=1), u)

                lhs = _lhs(x[:, D - 128:D])
                for u in range(nq):
                    finish_q(u, [_dot(lhs, _as_bf16(wq32[pl.ds(32, 8), u * 3 + nt]))[0:8]
                                 for nt in range(3)])
                f1 = cfg["va_force"]
                toks = st_qk(0, range(f1))
                for kb in range(2):
                    cs = slice((3 + kb) * 128, (4 + kb) * 128)
                    blk = jnp.broadcast_to(x[0:1, cs], (128, 128)).T
                    abuf[ns - 1 + zdyn, kb * 128:(kb + 1) * 128, :] = blk
                    qlhs[NU + zdyn, :, 0:128] = pltpu.bitcast(blk[120:128], U32)
                toks += st_qk(0, range(f1, nj))
                st_softmax(0, zdyn)
                toks += st_qk(1, range(js(1)))
                toks += st_pvm(0)
                for va, (t0, t1) in zip(cfg["va_groups"], cfg["va_tok"]):
                    acc = [None] * len(va)
                    for kt in range(16):
                        lo = abuf[ns - 1, pl.ds(kt * 16, 8, stride=2), :]
                        hi = abuf[ns - 1, pl.ds(kt * 16 + 1, 8, stride=2), :]
                        tk = toks[t0 + kt * (t1 - t0) // 16]
                        lo, hi = lo + tk, hi + tk
                        for i, u in enumerate(va):
                            w = wq32[24 + kt, u * 3:u * 3 + 3]
                            pr = (pltpu.bitcast(w << 16, F32) * lo
                                  + pltpu.bitcast(w & jnp.uint32(0xFFFF0000), F32) * hi)
                            acc[i] = pr if acc[i] is None else acc[i] + pr
                    for i, u in enumerate(va):
                        late = []
                        for nt in range(3):
                            q = acc[i][nt]
                            q = q + pltpu.roll(q, 4, 0)
                            q = q + pltpu.roll(q, 2, 0)
                            late.append(q + pltpu.roll(q, 1, 0))
                        finish_q(u, late)
                return toks

            def block(bi):
                ua, ub = cfg["blocks"][bi]
                block_dma(ua, ub)
                toks = []
                if bi == 0:
                    toks += prologue()
                done = js(ua + 1)
                for t in range(ua, ub):
                    base = len(toks)
                    ous = cfg["ored_at"].get(t, ())
                    if t in cfg["ored_pin"]:
                        for i, u in enumerate(ous):
                            nxt = nj - cfg["ored_back"] - (len(ous) - 1 - i) * 11
                            toks += st_qk(t + 1, range(done, nxt))
                            done = max(done, nxt)
                            st_ored(u, pin=zdyn)
                    else:
                        for u in ous:
                            st_ored(u)
                    if t + 1 < NU:
                        toks += st_qk(t + 1, range(done, nj))
                    g0 = len(toks)
                    if t == ua and bi > 0:
                        toks += st_pvm(t)
                    for u in cfg["oproj_at"].get(t, ()):
                        toks += st_oproj(*u) if isinstance(u, tuple) else st_oproj(u)
                    done = js(t + 2)
                    if t + 1 < ub:
                        gap = cfg["gap_at"].get(t, cfg["gap"])
                        done = max(-((len(toks) - g0 - gap) // 3), 0)
                    gap1 = cfg["gap1_at"].get(t, cfg["gap1"])
                    d1 = min(max(-((len(toks) - g0 - gap1) // 3), 0), done)
                    if t + 2 < NU:
                        toks += st_qk(t + 2, range(d1))
                    if t + 1 < NU:
                        st_softmax(t + 1, zdyn, pin=gap1 > 0 and t + 2 < NU and d1 < done)
                    if t + 2 < NU:
                        toks += st_qk(t + 2, range(d1, done))
                    if t + 1 < ub:
                        toks += st_pvm(t + 1)
                    st_pv(t, toks, [base + i for i in cfg["tok"][t]])
                    st_lsum(t)

            def tail(first_static):
                seen = set()
                for us in cfg["oproj_at"].values():
                    for u in us:
                        uu, ts = u if isinstance(u, tuple) else (u, (0, 1, 2))
                        seen |= {(uu, t) for t in ts}
                for u in range(NU - 1):
                    ts = tuple(t for t in range(3) if (u, t) not in seen)
                    if ts:
                        st_oproj(u, ts)
                extra = [[] for _ in range(D // 128)]
                st_olast(NU - 1, extra)
                mlp(first_static, extra, zdyn)

            for bi in range(len(cfg["blocks"])):
                block(bi)

            pl.when(first)(lambda: tail(True))
            pl.when(jnp.logical_not(first))(lambda: tail(False))
            return carry

        lax.fori_loop(0, 2, layer, 0)
        o_ref[...] = xs[0:1, :].astype(o_ref.dtype)

    return kernel


@jax.jit
def pallas_interleave_layers__sliding_block_cached__mixer_s_mlp__decode_kernel(
    A_x: jax.Array,
    A_k_cache: jax.Array,
    A_v_cache: jax.Array,
    A_wq: jax.Array,
    A_wo: jax.Array,
    B_x: jax.Array,
    B_w1: jax.Array,
    B_w2: jax.Array,
    B_w3: jax.Array,
    B_w4: jax.Array,
):
    b, sq, d = A_x.shape
    _, hkv, sk, dh = A_k_cache.shape
    assert (b, sq, d, hkv, dh) == (1, 1, D, H, DH)
    win = min(4096, max(256, sk // 4))
    assert win % 512 == 0 and sk % 128 == 0
    nj = win // 128

    kt = _tile_view(jnp.swapaxes(A_k_cache, 2, 3).reshape(H * DH, sk))
    vt = _head_view(jnp.swapaxes(A_v_cache, 2, 3).reshape(H * DH, sk))

    def buf(r, c):
        return pltpu.VMEM((r // 16, c // 128, 16, 128), BF16)

    def hbuf(c):
        return pltpu.VMEM((H, DH // 16, c // 128, 16, 128), BF16)

    bl = CFG["blocks"]
    ns = CFG.get("ns") or max(bl[i + 1][1] - bl[i][0] for i in range(len(bl) - 1))
    any_spec = pl.BlockSpec(memory_space=pl.ANY)
    out = pl.pallas_call(
        _make_kernel(sk, win, CFG),
        out_shape=jax.ShapeDtypeStruct((1, D), A_x.dtype),
        in_specs=[any_spec] * 7,
        out_specs=pl.BlockSpec(memory_space=pltpu.VMEM),
        scratch_shapes=[
            buf(H * DH, win), hbuf(win),
            pltpu.VMEM((H, DH // 16, max(len(CFG["jx"]), 1), 8, 128), F32),
            buf(D, H * DH), hbuf(D), buf(D, FF),
            pltpu.VMEM((D // 128, FF, 128), BF16),
            pltpu.VMEM((1, D), BF16),
            pltpu.VMEM((8, D), F32),
            pltpu.VMEM((H * DH // 128, 8, 128), F32),
            pltpu.VMEM((NU + 1, 8, 384), U32),
            pltpu.VMEM((2, 8, win // 4), F32),
            pltpu.VMEM((2, 8, win // 4), F32),
            pltpu.VMEM((1, 8, win // 4), F32),
            pltpu.VMEM((1, 8, win // 4), F32),
            pltpu.VMEM((8, 512), U32),
            pltpu.VMEM((ns, 2, 3, 8, 128), F32),
            pltpu.VMEM((ns, 8, 128), F32),
            pltpu.VMEM((ns, 384, 128), F32),
            pltpu.VMEM((NU, 8, 384), U32),
            pltpu.VMEM((3, D // 128, NU, 128), F32),
            pltpu.SemaphoreType.DMA((5,)),
        ],
        compiler_params=pltpu.CompilerParams(vmem_limit_bytes=int(CFG["vmem_mb"] * 1024 * 1024)),
        name="interleave_decode",
    )(A_x.reshape(1, D), kt, vt, _tile_view(A_wq), _head_view(A_wo),
      _tile_view(B_w3), B_w4)
    return out.reshape(b, sq, d)
```

```python
import jax
import jax.numpy as jnp
from jax import lax
import jax.experimental.pallas as pl
import jax.experimental.pallas.tpu as pltpu

F32 = jnp.float32
BF16 = jnp.bfloat16
U32 = jnp.uint32

D = 640
H = 32
DH = 192
FF = 1536
NU = H // 2
UT = 2 * DH // 16
EPS = 1e-5
NPIECE = 12

CFG = dict(
    blocks=((0, 4), (4, 8), (8, 12), (12, 15), (15, 16)), ns=7,
    jsplit=10, js_at={1: 13, 5: 19, 9: 19, 13: 16},
    gap=49, gap1=24, gap_at={}, gap1_at={}, ored_pin=(), ored_back=4,
    nm=4, nm_at={12: 5, 13: 5, 14: 5, 15: 0},
    va_groups=((6, 7, 8, 9), (10, 11, 12, 13, 14), (15,)), va_force=7,
    va_tok=((6, 43), (48, 94), (102, 112)),
    ored_at={4: (0,), 5: (1,), 6: (2,), 7: (3,), 8: (4,), 9: (5,), 10: (6,), 11: (7,),
             12: (8,), 13: (9,), 14: (10, 11), 15: (12, 13, 14)},
    oproj_at={4: ((0, (2,)),), 5: ((1, (2,)),), 6: ((2, (2,)),), 7: ((3, (2,)),),
              8: ((4, (0,)), (0, (0,))), 9: ((5, (0,)), (0, (1,))), 10: ((6, (0,)),), 11: ((7, (0,)),),
              12: ((8, (0,)),), 13: ((9, (0,)),),
              14: ((4, (1, 2)), (10, (0,)), (1, (0, 1)), (11, (0,))),
              15: ((2, (0, 1)), (3, (0, 1)), (5, (1, 2)), (6, (1, 2)), (7, (1, 2)), (8, (1, 2)), (9, (1, 2)),
                   (10, (1, 2)), (11, (1, 2)), 12, (13, (0, 1)))},
    jx=(1, 5, 9, 13, 17, 21, 25), vmem_mb=128,
    tok={
        0: [-26,-24,-22,-19,-17,-15,-13,-10,-8,-6,-3,-1,1,4,6,9,11,14,16,19,21,24,26,28,31,34,36,39,41,44,46,49,51,54,57,59,62,64,66,68,71,73,75,77,79,82,84,86],
        1: [-32,-29,-27,-25,-22,-20,-17,-15,-13,-10,-8,-5,-3,-1,2,4,7,9,11,14,16,18,21,23,26,28,30,33,35,37,40,42,44,47,49,51,54,56,58,60,62,65,67,69,71,73,76,78],
        2: [-28,-26,-23,-21,-18,-16,-14,-11,-9,-7,-4,-2,1,3,6,8,10,13,15,18,20,23,25,28,30,33,35,37,40,42,45,47,50,52,55,57,59,62,65,67,70,73,75,78,81,83,86,89],
        3: [-17,-15,-13,-10,-8,-6,-4,-2,0,2,5,7,9,11,14,16,19,22,24,27,29,32,34,37,39,42,44,47,49,52,55,57,60,62,65,67,70,72,74,77,79,81,84,86,88,90,93,95],
        4: [-27,-24,-22,-19,-17,-15,-12,-10,-7,-5,-4,-2,0,2,4,6,8,11,14,17,20,23,26,29,32,34,37,39,42,44,46,49,51,54,56,59,61,64,66,69,71,74,76,79,81,84,86,88],
        5: [-10,-8,-5,-2,0,3,5,8,10,13,15,18,20,23,25,28,30,33,35,38,40,43,45,48,50,53,56,58,61,64,66,69,71,74,76,78,80,82,84,87,89,91,94,97,99,102,104,107],
        6: [-15,-13,-11,-9,-7,-4,-2,0,2,5,8,10,13,16,19,21,24,27,29,31,34,36,39,41,44,46,49,51,54,56,59,61,64,66,69,71,73,76,78,81,83,86,88,91,93,96,98,101],
        7: [-10,-7,-5,-2,0,2,5,7,10,12,15,17,20,22,25,27,30,32,35,38,41,43,46,49,51,54,56,58,60,63,65,67,69,72,74,77,79,82,84,86,89,91,94,96,98,100,103,105],
        8: [-23,-21,-19,-17,-15,-14,-12,-10,-8,-6,-3,-1,1,3,5,7,10,12,15,17,20,23,25,28,31,33,36,39,41,44,47,49,52,54,57,59,62,64,66,69,71,74,76,79,81,84,87,89],
        9: [-8,-6,-4,-1,1,4,6,8,11,13,16,18,21,24,26,29,31,34,36,39,42,44,47,49,52,55,57,59,62,64,67,69,72,74,77,79,82,84,87,89,92,94,97,99,102,104,106,109],
        10: [-19,-16,-14,-11,-9,-7,-4,-2,1,3,6,8,10,13,15,18,20,23,25,28,30,33,35,38,40,43,45,48,50,53,56,58,61,63,66,68,70,73,75,78,80,83,85,88,90,93,95,98],
        11: [-19,-16,-14,-11,-8,-6,-3,0,2,5,7,9,12,14,17,19,21,24,26,29,32,34,37,39,42,45,47,50,53,56,58,61,64,66,69,71,73,76,78,81,83,85,88,90,92,94,97,99],
        12: [-29,-27,-24,-21,-19,-16,-14,-11,-8,-6,-3,-1,2,5,7,10,13,15,18,20,23,25,28,31,33,35,38,40,43,45,47,50,52,55,57,60,63,66,68,71,74,76,78,80,83,85,87,89],
        13: [-21,-19,-17,-14,-12,-9,-7,-5,-2,0,3,5,7,10,12,15,17,19,21,23,25,27,29,31,33,36,39,42,45,47,50,53,56,58,61,63,65,68,70,73,75,77,80,82,84,86,89,91],
        14: [-38,-36,-34,-32,-30,-28,-26,-24,-22,-19,-16,-13,-11,-8,-5,-2,1,3,6,8,11,13,16,18,21,23,26,28,31,33,36,38,40,43,45,48,50,53,55,57,60,63,65,68,71,74,77,79],
        15: [-27,-25,-23,-21,-19,-16,-14,-12,-10,-7,-4,0,3,6,9,12,16,19,22,25,29,32,35,38,42,44,46,48,51,53,55,57,59,64,68,73,77,82,86,91,95,96,96,96,96,96,96,96],
    },
    w4_k=8, w4_nv=3, w4_pin=10, w4_tok=(14, 36), nq_mxu=6)


def _tile_view(a):
    r, c = a.shape
    a = a.reshape(r // 16, 2, 8, c // 128, 128)
    return jnp.swapaxes(a, 2, 3)


def _head_view(a):
    c = a.shape[1]
    a = a.reshape(H, 2, DH // 16, 8, c // 128, 128)
    return jnp.swapaxes(a, 3, 4)


def _as_bf16(w32):
    n = w32.shape[0]
    return pltpu.bitcast(w32.reshape(n * 8, 128), BF16)


def _lhs(top, fill=0.0):
    return jnp.concatenate([top, jnp.full(top.shape, fill, F32)], axis=0).astype(BF16)


def _ln_stats(x):
    m = jnp.mean(x, axis=-1, keepdims=True)
    m2 = jnp.mean(x * x, axis=-1, keepdims=True)
    v = jnp.maximum(m2 - m * m, 0.0)
    return m, lax.rsqrt(v + EPS)


def _round_bf16(x):
    return x.astype(BF16).astype(F32)


def _dot(a, b):
    return jnp.dot(a, b, preferred_element_type=F32)


def _make_kernel(sk, win, cfg):
    nj = win // 128
    j0 = (sk - win) // 128
    jq = nj // 4
    jx = list(cfg["jx"])
    assert nj == 32 and cfg["blocks"][-2][0] <= NU - 3 and cfg["blocks"][-1] == (NU - 1, NU)
    qscale = DH ** -0.5 * 1.4426950408889634

    def kernel(x_hbm, k_hbm, v_hbm, wq_hbm, wo_hbm, w3_hbm, w4_hbm, o_ref,
               kbuf, vbuf, vx, wqbuf, wobuf, w3buf, w4buf, xin,
               xs, qacc, qlhs, sx, sy, pbuf0, pbuf1, plhs, mbuf, lpart, abuf, olhs, gp,
               sems):
        pbuf = (pbuf0, pbuf1)
        ns = abuf.shape[0]


        def cps_w(hbm, buf, sem, lo=0, n=None):
            n = buf.shape[0] if n is None else n
            return [pltpu.make_async_copy(
                hbm.at[pl.ds(lo, n), e],
                buf.at[pl.ds(lo, n), :, pl.ds(e * 8, 8), :],
                sems.at[sem]) for e in range(2)]

        def cps_kv(hbm, buf, sem, u):
            return [pltpu.make_async_copy(
                hbm.at[pl.ds(u * UT, UT), e, pl.ds(j0, nj)],
                buf.at[pl.ds(u * UT, UT), :, pl.ds(e * 8, 8), :],
                sems.at[sem]) for e in range(2)]

        def cps_v(u, par):
            return [pltpu.make_async_copy(
                v_hbm.at[pl.ds(2 * u, 2), e, :, pl.ds(j0, nj)],
                vbuf.at[pl.ds(2 * u, 2), :, :, pl.ds(e * 8, 8), :],
                sems.at[2 + par]) for e in range(2)]

        def cps_wo(part):
            lo, n = ((0, H - 8), (H - 8, 8))[part]
            return [pltpu.make_async_copy(
                wo_hbm.at[pl.ds(lo, n), e], wobuf.at[pl.ds(lo, n), :, :, pl.ds(e * 8, 8), :],
                sems.at[4]) for e in range(2)]

        cps_k = lambda u, par: cps_kv(k_hbm, kbuf, par, u)
        cps_x_wq = lambda: cps_w(wq_hbm, wqbuf, 4) + [pltpu.make_async_copy(x_hbm, xin, sems.at[4])]
        cps_w3 = lambda: cps_w(w3_hbm, w3buf, 0)
        w4_k = cfg["w4_k"] * 128
        w4_parts = [(c, 0, FF) for c in range(D // 128 - 1)]
        w4_parts += [(D // 128 - 1, 0, w4_k), (D // 128 - 1, w4_k, FF - w4_k)]

        def cps_w4(i):
            c, lo, n = w4_parts[i]
            return [pltpu.make_async_copy(
                w4_hbm.at[pl.ds(lo // 16, n // 16), e, pl.ds(c, 1)],
                w4buf.at[pl.ds(lo // 16, n // 16), pl.ds(c, 1), pl.ds(e * 8, 8), :],
                sems.at[(2, 1, 3, 0, 4, 2)[i]]) for e in range(2)]

        def start(cps):
            for c in cps:
                c.start()

        def wait(cps):
            for c in cps:
                c.wait()

        start(cps_x_wq())
        start(cps_k(0, 0))
        start(cps_k(1, 1))
        start(cps_v(0, 0))
        start(cps_v(1, 1))

        k32 = kbuf.bitcast(U32)
        v32 = vbuf.bitcast(U32)
        wq32 = wqbuf.bitcast(U32)
        wo32 = wobuf.bitcast(U32)
        w332 = w3buf.bitcast(U32)
        w432 = w4buf.bitcast(U32)

        def js(u):
            return cfg["js_at"].get(u, cfg["jsplit"])

        def jms(u):
            return [nj - 1 - jq * (i % 4) - i // 4 for i in range(nmx(u))]

        def early_tiles(kb):
            return ((H * DH // 128,) * 3 + (3 * cfg["nq_mxu"], 0))[kb]

        def nmx(u):
            return cfg["nm_at"].get(u, cfg["nm"])

        def pack_q(q, u):
            q = q * qscale
            lane = lax.broadcasted_iota(jnp.int32, (8, 128), 1)
            sub = lax.broadcasted_iota(jnp.int32, (8, 128), 0)
            keep = (lane < DH - 128) == (sub % 2 == 0)
            q = jnp.concatenate(
                [q[:, 0:128], jnp.where(keep, q[:, 128:256], 0.0), q[:, 256:384]], axis=1)
            qlhs.at[u][:, 0:384] = pltpu.bitcast(_lhs(q), U32)

        def st_qk(u, js):
            sl = u % 2
            lhs = pltpu.bitcast(qlhs[u], BF16)
            toks = []
            for j in js:
                ra = 2 * (j // jq)
                cs = slice((j % jq) * 128, (j % jq + 1) * 128)
                for t in range(3):
                    w = _as_bf16(k32[pl.ds(u * UT + t * 8, 8), j])
                    r = _dot(lhs[:, t * 128:(t + 1) * 128], w)
                    toks.append(r[8:16])
                    if t == 0:
                        sx[sl, ra:ra + 1, cs] = r[0:1]
                    elif t == 1:
                        sy[sl, ra:ra + 2, cs] = r[ra:ra + 2]
                    else:
                        sx[sl, ra + 1:ra + 2, cs] = r[0:1]
            return toks

        def st_softmax(u, zdyn, pin=False):
            sl = u % 2
            s = sx[sl] + sy[sl]
            m = s
            while m.shape[1] > 128:
                h = m.shape[1] // 2
                m = jnp.maximum(m[:, :h], m[:, h:])
            m = jnp.maximum(m, pltpu.roll(m, 2, 0))
            m = jnp.maximum(m, pltpu.roll(m, 4, 0))
            if pin:
                qlhs[NU + zdyn, :, 0:128] = pltpu.bitcast(m, U32)
            m = jnp.max(m, axis=1, keepdims=True)
            p = jnp.exp2(s - m)
            pbuf[sl][zdyn] = p
            for g in range((nmx(u) + 3) // 4):
                c = jq - 1 - g
                plhs[:, (2 * sl + g) * 128:(2 * sl + g + 1) * 128] = pltpu.bitcast(
                    _lhs(p[:, c * 128:(c + 1) * 128]), U32)

        def inv_l(l):
            l = jnp.sum(l, axis=1, keepdims=True)
            r0 = pl.reciprocal(l, approx=True)
            return jnp.broadcast_to(r0 * (2.0 - l * r0), (8, 128))

        def st_lsum(u):
            l = pbuf[u % 2][0, :, 0:128]
            for c in range(1, jq):
                l = l + pbuf[u % 2][0, :, c * 128:(c + 1) * 128]
            l = l + pltpu.roll(l, 2, 0)
            l = l + pltpu.roll(l, 4, 0)
            lpart[u % ns] = inv_l(l) if u == NU - 1 else l

        def st_pvm(u):
            toks = []
            for j in jms(u):
                g = jq - 1 - j % jq
                pc = 2 * (u % 2) + g
                lhs = pltpu.bitcast(plhs[:, pc * 128:(pc + 1) * 128], BF16)
                ra = 2 * (j // jq)
                for t in range(3):
                    if t == 1:
                        w32 = jnp.concatenate(
                            [v32[2 * u, 8:12, j], v32[2 * u + 1, 0:4, j]], axis=0)
                    else:
                        w32 = v32[2 * u + t // 2, 2 * t:2 * t + 8, j]
                    r = _dot(lhs, _as_bf16(w32))
                    toks.append(r[8:16])
                    mbuf[u % ns, g, t, ra:ra + 2, :] = r[ra:ra + 2]
            return toks

        def st_expand(u):
            def body(dt, c):
                for hd in range(2):
                    for ix, j in enumerate(jx):
                        w = v32[2 * u + hd, dt, j]
                        vx[2 * u + hd, dt, ix] = pltpu.bitcast(w << 16, F32)
                        vbuf[2 * u + hd, dt, j] = pltpu.bitcast(w & jnp.uint32(0xFFFF0000), BF16)
                return c
            lax.fori_loop(0, UT // 2, body, 0)
            for j in jms(u):
                for t in range(3):
                    idx = [divmod(t * 8 + v, 12) for v in range(8)]
                    blk = jnp.concatenate([vbuf[2 * u + hd, dt, j] for hd, dt in idx], axis=0)
                    blk = blk.astype(F32).T.astype(BF16)
                    for v, (hd, dt) in enumerate(idx):
                        vbuf[2 * u + hd, dt, j] = blk[v * 16:(v + 1) * 16]

        def st_pv(u, toks, tok_map):
            nm, sl = nmx(u), u % ns
            for piece in range(NPIECE):
                hd, half = divmod(piece, NPIECE // 2)
                sub = len(tok_map) // NPIECE
                lo = hi = None
                for j in range(nj):
                    if j in jms(u):
                        continue
                    row = 2 * (j // jq) + hd
                    cs = slice((j % jq) * 128, (j % jq + 1) * 128)
                    pb = jnp.broadcast_to(pbuf[u % 2][0, row:row + 1, cs], (8, 128))
                    k = piece * sub + j * sub // nj
                    ti = tok_map[k] if j % (nj // sub) == 0 else -1
                    if j > 0 and tok_map[k - 1] == ti:
                        ti = -1
                    if toks and ti >= 0:
                        pb = pb + toks[min(ti, len(toks) - 1)]
                    w = v32[2 * u + hd, pl.ds(half * 2, 2), j]
                    if j in jx:
                        a = vx[2 * u + hd, pl.ds(half * 2, 2), jx.index(j)] * pb
                        b = pltpu.bitcast(w, F32) * pb
                    else:
                        a = pltpu.bitcast(w << 16, F32) * pb
                        b = pltpu.bitcast(w & jnp.uint32(0xFFFF0000), F32) * pb
                    lo = a if lo is None else lo + a
                    hi = b if hi is None else hi + b
                for i in range(2):
                    base = (piece * 2 + i) * 16
                    abuf[sl, pl.ds(base, 8, stride=2), :] = lo[i]
                    abuf[sl, pl.ds(base + 1, 8, stride=2), :] = hi[i]

        def st_ored(u, ts=(0, 1, 2), pin=None):
            nm, sl = nmx(u), u % ns
            ia = inv_l(lpart[sl])
            ib = pltpu.roll(ia, 1, 0)
            lane = lax.broadcasted_iota(jnp.int32, (8, 128), 1)
            for t in ts:
                at = abuf[sl, t * 128:(t + 1) * 128, :].T
                if pin is not None:
                    qlhs[NU + pin, :, 0:128] = pltpu.bitcast(at[120:128], U32)
                o = at[0:8]
                for i in range(1, 16):
                    o = o + at[i * 8:(i + 1) * 8]
                if nm:
                    sub = lax.broadcasted_iota(jnp.int32, (8, 128), 0)
                    odd = (0, (lane >= DH - 128).astype(jnp.int32), 1)[t]
                    for g in range((nm + 3) // 4):
                        keep = (sub >= 8 - 2 * min(nm - 4 * g, 4)) & (sub % 2 == odd)
                        o = o + jnp.where(keep, mbuf[sl, g, t], 0.0)
                o = o + pltpu.roll(o, 4, 0)
                o = o + pltpu.roll(o, 2, 0)
                o = o + pltpu.roll(o, 1, 0)
                o = o * (ia, jnp.where(lane < DH - 128, ia, ib), ib)[t]
                olhs.at[u][:, t * 128:(t + 1) * 128] = pltpu.bitcast(_lhs(o), U32)

        def st_olast(u, out):
            sl = u % ns
            for hd in range(2):
                pa = [None, None]
                for dt in range(12):
                    base = (hd * 12 + dt) * 16
                    lo = jnp.sum(abuf[sl, pl.ds(base, 8, stride=2), :], axis=1, keepdims=True)
                    hi = jnp.sum(abuf[sl, pl.ds(base + 1, 8, stride=2), :], axis=1, keepdims=True)
                    w = wo32[2 * u + hd, dt]
                    pr = (pltpu.bitcast(w << 16, F32) * lo
                          + pltpu.bitcast(w & jnp.uint32(0xFFFF0000), F32) * hi)
                    pa[dt % 2] = pr if pa[dt % 2] is None else pa[dt % 2] + pr
                inv = jnp.broadcast_to(lpart[sl, hd:hd + 1, :], (8, 128))
                tot = (pa[0] + pa[1]) * inv
                for n in range(D // 128):
                    out[n].append(tot[n])

        def st_oproj(u, ts=(0, 1, 2)):
            lhs = pltpu.bitcast(olhs[u], BF16)
            toks = []
            for t in ts:
                for n in range(D // 128):
                    if t == 1:
                        w32 = jnp.concatenate(
                            [wo32[2 * u, 8:12, n], wo32[2 * u + 1, 0:4, n]], axis=0)
                    else:
                        w32 = wo32[2 * u + t // 2, 2 * t:2 * t + 8, n]
                    r = _dot(lhs[:, t * 128:(t + 1) * 128], _as_bf16(w32))
                    toks.append(r[8:16])
                    gp[t, n, pl.ds(u, 1), :] = r[0:1]
            return toks

        def mlp(first, extra, zdyn):
            g = gp[0] + gp[1] + gp[2]
            g = g[:, 0:8] + g[:, 8:16]
            g = jnp.concatenate([sum(extra[n], g[n]) for n in range(D // 128)], axis=1)
            g = g + pltpu.roll(g, 4, 0)
            g = g + pltpu.roll(g, 2, 0)
            g = g + pltpu.roll(g, 1, 0)
            x1 = _round_bf16(xs[...] + g)
            lhs = _lhs(x1, 1.0)
            m1, r1 = _ln_stats(x1)
            y = (x1 - m1) * r1
            m2, r2 = _ln_stats(y)
            a = r1 * r2
            b = (m1 * r1 + m2) * r2
            if first:
                wait(cps_w3())
                start(cps_w4(3))
                start(cps_w4(4))
            hl, hs = [], []
            for n in range(FF // 128):
                r = _dot(lhs, _as_bf16(w332[:, n]))
                hn = jax.nn.gelu(r[0:8] * a - r[8:16] * b, approximate=True)
                hl.append(_lhs(hn))
                hs.append(hn)
            acc = x1 + y
            acc = [acc[:, c * 128:(c + 1) * 128] for c in range(D // 128)]

            def w4_dot(kt, c):
                return _dot(hl[kt], _as_bf16(w432[pl.ds(kt * 8, 8), c]))[0:8]

            if not first:
                nv, kpin, (t0, t1) = cfg["w4_nv"], cfg["w4_pin"], cfg["w4_tok"]
                toks = []
                for kt in range(nv, FF // 128):
                    if nv and kt == kpin:
                        for k in range(nv):
                            blk = jnp.broadcast_to(_round_bf16(hs[k][0:1]), (128, 128)).T
                            abuf[zdyn, k * 128:(k + 1) * 128, :] = blk
                            qlhs[NU + zdyn, :, 0:128] = pltpu.bitcast(blk[120:128], U32)
                        hl[kt] = pltpu.bitcast(qlhs[0, :, 0:128], BF16)
                    if nv and kt + 1 == kpin:
                        qlhs.at[0][:, 0:128] = pltpu.bitcast(hl[kpin], U32)
                    for c in range(D // 128):
                        r = _dot(hl[kt], _as_bf16(w432[pl.ds(kt * 8, 8), c]))
                        toks.append(r[8:16])
                        acc[c] = acc[c] + r[0:8]
                pa = None
                for dt in range(nv * 8):
                    tk = toks[t0 + dt * (t1 - t0) // (nv * 8)]
                    lo = abuf[0, pl.ds(dt * 16, 8, stride=2), :] + tk
                    hi = abuf[0, pl.ds(dt * 16 + 1, 8, stride=2), :] + tk
                    w = w432[dt]
                    pr = (pltpu.bitcast(w << 16, F32) * lo
                          + pltpu.bitcast(w & jnp.uint32(0xFFFF0000), F32) * hi)
                    pa = pr if pa is None else pa + pr
                for c in range(D // 128 if nv else 0):
                    pc = pa[c]
                    pc = pc + pltpu.roll(pc, 4, 0)
                    pc = pc + pltpu.roll(pc, 2, 0)
                    acc[c] = (pc + pltpu.roll(pc, 1, 0)) + acc[c]
                xs[...] = _round_bf16(jnp.concatenate(acc, axis=1))
                return
            for i, (c, lo, n) in enumerate(w4_parts):
                wait(cps_w4(i))
                if i == 0:
                    start(cps_w4(5))
                    for k, hn in enumerate(hs[cfg["w4_k"]:]):
                        abuf[k // 3, (k % 3) * 128:(k % 3 + 1) * 128, :] = jnp.broadcast_to(
                            _round_bf16(hn[0:1]), (128, 128)).T
                if lo == 0:
                    for kt in range(n // 128):
                        acc[c] = acc[c] + w4_dot(kt, c)
                else:
                    pas = [None] * 4
                    for dt in range(n // 16):
                        w = w432[lo // 16 + dt, c]
                        sl, r0 = dt // 24, dt % 24 * 16
                        pr = (pltpu.bitcast(w << 16, F32) * abuf[sl, pl.ds(r0, 8, stride=2), :]
                              + pltpu.bitcast(w & jnp.uint32(0xFFFF0000), F32)
                              * abuf[sl, pl.ds(r0 + 1, 8, stride=2), :])
                        pas[dt % 4] = pr if pas[dt % 4] is None else pas[dt % 4] + pr
                    pa = (pas[0] + pas[1]) + (pas[2] + pas[3])
                    pa = pa + pltpu.roll(pa, 4, 0)
                    pa = pa + pltpu.roll(pa, 2, 0)
                    acc[c] = acc[c] + (pa + pltpu.roll(pa, 1, 0))
                if lo + n == FF:
                    xc = _round_bf16(acc[c])
                    xs[:, c * 128:(c + 1) * 128] = xc
                    lhs = _lhs(xc)
                    for nt in range(early_tiles(c)):
                        r = _dot(lhs, _as_bf16(wq32[pl.ds(c * 8, 8), nt]))[0:4]
                        qacc[nt, 0:4, :] = r if c == 0 else qacc[nt, 0:4, :] + r

        gp[...] = jnp.zeros_like(gp)
        mbuf[...] = jnp.zeros_like(mbuf)
        wait(cps_x_wq())
        start(cps_wo(0))
        x0 = jnp.broadcast_to(xin[...].astype(F32), (8, D))
        sub0 = lax.broadcasted_iota(jnp.int32, (8, D), 0)
        lane0 = lax.broadcasted_iota(jnp.int32, (8, D), 1)
        for nkb, n0, n1 in ((4, 0, early_tiles(3)), (3, early_tiles(3), early_tiles(0))):
            lhs0 = _lhs(jnp.where(sub0 < 4, jnp.where(lane0 < nkb * 128, x0, 0.0), 1.0))

            def q0_body(nt, c, lhs0=lhs0):
                qacc[nt] = _dot(lhs0, _as_bf16(wq32[:, nt]))[0:8]
                return c
            lax.fori_loop(n0, n1, q0_body, 0)
        wait(cps_k(0, 0))
        start(cps_k(2, 0))
        wait(cps_k(1, 1))
        wait(cps_v(0, 0))
        xs[...] = x0

        def layer(li, carry):
            first = li == 0
            n_first = jnp.maximum(1 - li, 0)
            zdyn = li >> 4

            def block_dma(ua, ub):
                def last_wait(t):
                    if t == NU - 2:
                        wait(cps_k(NU - 1, (NU - 1) % 2))
                    else:
                        wait(cps_v(t + 1, (t + 1) % 2) if t + 1 < NU else cps_wo(1))

                def dma_ops(_, c):
                    for t in range(ua, ub):
                        if t + 3 < NU:
                            start(cps_k(t + 3, (t + 3) % 2))
                        if t + 2 < NU:
                            start(cps_v(t + 2, t % 2))
                        if t == NU - 2:
                            start(cps_w3())
                            start(cps_w4(0))
                        if t == NU - 1:
                            start(cps_w4(1))
                            wait(cps_v(t, t % 2))
                            start(cps_w4(2))
                        if t == 1:
                            wait(cps_wo(0))
                            start(cps_wo(1))
                        st_expand(t)
                        if t + 2 < NU - 1:
                            wait(cps_k(t + 2, t % 2))
                        if t < ub - 1:
                            last_wait(t)
                    return c

                lax.fori_loop(0, n_first, dma_ops, 0)
                pl.when(first)(lambda: last_wait(ub - 1))

            def prologue():
                x = xs[...]
                m, r = _ln_stats(x)
                nq = cfg["nq_mxu"]

                def finish_q(u, late):
                    qs = []
                    for nt in range(3):
                        qx = jnp.broadcast_to(qacc[u * 3 + nt, 0:1, :], (8, 128))
                        cs = jnp.broadcast_to(qacc[u * 3 + nt, 4:5, :], (8, 128))
                        qs.append((qx + late[nt] - cs * m) * r)
                    pack_q(jnp.concatenate(qs, axis=1), u)

                lhs = _lhs(x[:, D - 128:D])
                for u in range(nq):
                    finish_q(u, [_dot(lhs, _as_bf16(wq32[pl.ds(32, 8), u * 3 + nt]))[0:8]
                                 for nt in range(3)])
                f1 = cfg["va_force"]
                toks = st_qk(0, range(f1))
                for kb in range(2):
                    cs = slice((3 + kb) * 128, (4 + kb) * 128)
                    blk = jnp.broadcast_to(x[0:1, cs], (128, 128)).T
                    abuf[ns - 1 + zdyn, kb * 128:(kb + 1) * 128, :] = blk
                    qlhs[NU + zdyn, :, 0:128] = pltpu.bitcast(blk[120:128], U32)
                toks += st_qk(0, range(f1, nj))
                st_softmax(0, zdyn)
                toks += st_qk(1, range(js(1)))
                toks += st_pvm(0)
                for va, (t0, t1) in zip(cfg["va_groups"], cfg["va_tok"]):
                    acc = [None] * len(va)
                    for kt in range(16):
                        lo = abuf[ns - 1, pl.ds(kt * 16, 8, stride=2), :]
                        hi = abuf[ns - 1, pl.ds(kt * 16 + 1, 8, stride=2), :]
                        tk = toks[t0 + kt * (t1 - t0) // 16]
                        lo, hi = lo + tk, hi + tk
                        for i, u in enumerate(va):
                            w = wq32[24 + kt, u * 3:u * 3 + 3]
                            pr = (pltpu.bitcast(w << 16, F32) * lo
                                  + pltpu.bitcast(w & jnp.uint32(0xFFFF0000), F32) * hi)
                            acc[i] = pr if acc[i] is None else acc[i] + pr
                    for i, u in enumerate(va):
                        late = []
                        for nt in range(3):
                            q = acc[i][nt]
                            q = q + pltpu.roll(q, 4, 0)
                            q = q + pltpu.roll(q, 2, 0)
                            late.append(q + pltpu.roll(q, 1, 0))
                        finish_q(u, late)
                return toks

            def block(bi):
                ua, ub = cfg["blocks"][bi]
                block_dma(ua, ub)
                toks = []
                if bi == 0:
                    toks += prologue()
                done = js(ua + 1)
                for t in range(ua, ub):
                    base = len(toks)
                    ous = cfg["ored_at"].get(t, ())
                    if t in cfg["ored_pin"]:
                        for i, u in enumerate(ous):
                            nxt = nj - cfg["ored_back"] - (len(ous) - 1 - i) * 11
                            toks += st_qk(t + 1, range(done, nxt))
                            done = max(done, nxt)
                            st_ored(u, pin=zdyn)
                    else:
                        for u in ous:
                            st_ored(u)
                    if t + 1 < NU:
                        toks += st_qk(t + 1, range(done, nj))
                    g0 = len(toks)
                    if t == ua and bi > 0:
                        toks += st_pvm(t)
                    for u in cfg["oproj_at"].get(t, ()):
                        toks += st_oproj(*u) if isinstance(u, tuple) else st_oproj(u)
                    done = js(t + 2)
                    if t + 1 < ub:
                        gap = cfg["gap_at"].get(t, cfg["gap"])
                        done = max(-((len(toks) - g0 - gap) // 3), 0)
                    gap1 = cfg["gap1_at"].get(t, cfg["gap1"])
                    d1 = min(max(-((len(toks) - g0 - gap1) // 3), 0), done)
                    if t + 2 < NU:
                        toks += st_qk(t + 2, range(d1))
                    if t + 1 < NU:
                        st_softmax(t + 1, zdyn, pin=gap1 > 0 and t + 2 < NU and d1 < done)
                    if t + 2 < NU:
                        toks += st_qk(t + 2, range(d1, done))
                    if t + 1 < ub:
                        toks += st_pvm(t + 1)
                    st_pv(t, toks, [base + i for i in cfg["tok"][t]])
                    st_lsum(t)

            def tail(first_static):
                seen = set()
                for us in cfg["oproj_at"].values():
                    for u in us:
                        uu, ts = u if isinstance(u, tuple) else (u, (0, 1, 2))
                        seen |= {(uu, t) for t in ts}
                for u in range(NU - 1):
                    ts = tuple(t for t in range(3) if (u, t) not in seen)
                    if ts:
                        st_oproj(u, ts)
                extra = [[] for _ in range(D // 128)]
                st_olast(NU - 1, extra)
                mlp(first_static, extra, zdyn)

            for bi in range(len(cfg["blocks"])):
                block(bi)

            pl.when(first)(lambda: tail(True))
            pl.when(jnp.logical_not(first))(lambda: tail(False))
            return carry

        lax.fori_loop(0, 2, layer, 0)
        o_ref[...] = xs[0:1, :].astype(o_ref.dtype)

    return kernel


@jax.jit
def pallas_interleave_layers__sliding_block_cached__mixer_s_mlp__decode_kernel(
    A_x: jax.Array,
    A_k_cache: jax.Array,
    A_v_cache: jax.Array,
    A_wq: jax.Array,
    A_wo: jax.Array,
    B_x: jax.Array,
    B_w1: jax.Array,
    B_w2: jax.Array,
    B_w3: jax.Array,
    B_w4: jax.Array,
):
    b, sq, d = A_x.shape
    _, hkv, sk, dh = A_k_cache.shape
    assert (b, sq, d, hkv, dh) == (1, 1, D, H, DH)
    win = min(4096, max(256, sk // 4))
    assert win % 512 == 0 and sk % 128 == 0
    nj = win // 128

    kt = _tile_view(jnp.swapaxes(A_k_cache, 2, 3).reshape(H * DH, sk))
    vt = _head_view(jnp.swapaxes(A_v_cache, 2, 3).reshape(H * DH, sk))

    def buf(r, c):
        return pltpu.VMEM((r // 16, c // 128, 16, 128), BF16)

    def hbuf(c):
        return pltpu.VMEM((H, DH // 16, c // 128, 16, 128), BF16)

    bl = CFG["blocks"]
    ns = CFG.get("ns") or max(bl[i + 1][1] - bl[i][0] for i in range(len(bl) - 1))
    any_spec = pl.BlockSpec(memory_space=pl.ANY)
    out = pl.pallas_call(
        _make_kernel(sk, win, CFG),
        out_shape=jax.ShapeDtypeStruct((1, D), A_x.dtype),
        in_specs=[any_spec] * 7,
        out_specs=pl.BlockSpec(memory_space=pltpu.VMEM),
        scratch_shapes=[
            buf(H * DH, win), hbuf(win),
            pltpu.VMEM((H, DH // 16, max(len(CFG["jx"]), 1), 8, 128), F32),
            buf(D, H * DH), hbuf(D), buf(D, FF), buf(FF, D),
            pltpu.VMEM((1, D), BF16),
            pltpu.VMEM((8, D), F32),
            pltpu.VMEM((H * DH // 128, 8, 128), F32),
            pltpu.VMEM((NU + 1, 8, 384), U32),
            pltpu.VMEM((2, 8, win // 4), F32),
            pltpu.VMEM((2, 8, win // 4), F32),
            pltpu.VMEM((1, 8, win // 4), F32),
            pltpu.VMEM((1, 8, win // 4), F32),
            pltpu.VMEM((8, 512), U32),
            pltpu.VMEM((ns, 2, 3, 8, 128), F32),
            pltpu.VMEM((ns, 8, 128), F32),
            pltpu.VMEM((ns, 384, 128), F32),
            pltpu.VMEM((NU, 8, 384), U32),
            pltpu.VMEM((3, D // 128, NU, 128), F32),
            pltpu.SemaphoreType.DMA((5,)),
        ],
        compiler_params=pltpu.CompilerParams(vmem_limit_bytes=int(CFG["vmem_mb"] * 1024 * 1024)),
        name="interleave_decode",
    )(A_x.reshape(1, D), kt, vt, _tile_view(A_wq), _head_view(A_wo),
      _tile_view(B_w3), _tile_view(B_w4))
    return out.reshape(b, sq, d)
```

```python
import jax
import jax.numpy as jnp
from jax import lax
import jax.experimental.pallas as pl
import jax.experimental.pallas.tpu as pltpu

F32 = jnp.float32
BF16 = jnp.bfloat16
U32 = jnp.uint32

D = 640
H = 32
DH = 192
FF = 1536
NU = H // 2
UT = 2 * DH // 16
EPS = 1e-5
NPIECE = 12

CFG = dict(
    blocks=((0, 4), (4, 8), (8, 12), (12, 15), (15, 16)),
    ns=7,
    jsplit=10, js_at={1: 13, 5: 19, 9: 19, 13: 16},
    gap=49, gap1=24,
    nm=4, nm_at={12: 5, 13: 5, 14: 5, 15: 0},
    va_groups=((6, 7, 8, 9), (10, 11, 12, 13, 14), (15,)), va_force=7,
    va_tok=((6, 43), (48, 94), (102, 112)),
    ored_at={4: (0,), 5: (1,), 6: (2,), 7: (3,), 8: (4,), 9: (5,), 10: (6,), 11: (7,),
             12: (8,), 13: (9,), 14: (10, 11), 15: (12, 13, 14)},
    oproj_at={4: ((0, (2,)),), 5: ((1, (2,)),), 6: ((2, (2,)),), 7: ((3, (2,)),),
              8: ((4, (0,)), (0, (0,))), 9: ((5, (0,)), (0, (1,))), 10: ((6, (0,)),), 11: ((7, (0,)),),
              12: ((8, (0,)),), 13: ((9, (0,)),),
              14: ((4, (1, 2)), (10, (0,)), (1, (0, 1)), (11, (0,))),
              15: ((2, (0, 1)), (3, (0, 1)), (5, (1, 2)), (6, (1, 2)), (7, (1, 2)), (8, (1, 2)), (9, (1, 2)),
                   (10, (1, 2)), (11, (1, 2)), 12, (13, (0, 1)))},
    jx=(1, 5, 9, 13, 17, 21, 25),
    vmem_mb=128,
    tok={
        0: [-26,-24,-22,-19,-17,-15,-13,-10,-8,-6,-3,-1,1,4,6,9,11,14,16,19,21,24,26,28,31,34,36,39,41,44,46,49,51,54,57,59,62,64,66,68,71,73,75,77,79,82,84,86],
        1: [-32,-29,-27,-25,-22,-20,-17,-15,-13,-10,-8,-5,-3,-1,2,4,7,9,11,14,16,18,21,23,26,28,30,33,35,37,40,42,44,47,49,51,54,56,58,60,62,65,67,69,71,73,76,78],
        2: [-28,-26,-23,-21,-18,-16,-14,-11,-9,-7,-4,-2,1,3,6,8,10,13,15,18,20,23,25,28,30,33,35,37,40,42,45,47,50,52,55,57,59,62,65,67,70,73,75,78,81,83,86,89],
        3: [-17,-15,-13,-10,-8,-6,-4,-2,0,2,5,7,9,11,14,16,19,22,24,27,29,32,34,37,39,42,44,47,49,52,55,57,60,62,65,67,70,72,74,77,79,81,84,86,88,90,93,95],
        4: [-27,-24,-22,-19,-17,-15,-12,-10,-7,-5,-4,-2,0,2,4,6,8,11,14,17,20,23,26,29,32,34,37,39,42,44,46,49,51,54,56,59,61,64,66,69,71,74,76,79,81,84,86,88],
        5: [-10,-8,-5,-2,0,3,5,8,10,13,15,18,20,23,25,28,30,33,35,38,40,43,45,48,50,53,56,58,61,64,66,69,71,74,76,78,80,82,84,87,89,91,94,97,99,102,104,107],
        6: [-15,-13,-11,-9,-7,-4,-2,0,2,5,8,10,13,16,19,21,24,27,29,31,34,36,39,41,44,46,49,51,54,56,59,61,64,66,69,71,73,76,78,81,83,86,88,91,93,96,98,101],
        7: [-10,-7,-5,-2,0,2,5,7,10,12,15,17,20,22,25,27,30,32,35,38,41,43,46,49,51,54,56,58,60,63,65,67,69,72,74,77,79,82,84,86,89,91,94,96,98,100,103,105],
        8: [-23,-21,-19,-17,-15,-14,-12,-10,-8,-6,-3,-1,1,3,5,7,10,12,15,17,20,23,25,28,31,33,36,39,41,44,47,49,52,54,57,59,62,64,66,69,71,74,76,79,81,84,87,89],
        9: [-8,-6,-4,-1,1,4,6,8,11,13,16,18,21,24,26,29,31,34,36,39,42,44,47,49,52,55,57,59,62,64,67,69,72,74,77,79,82,84,87,89,92,94,97,99,102,104,106,109],
        10: [-19,-16,-14,-11,-9,-7,-4,-2,1,3,6,8,10,13,15,18,20,23,25,28,30,33,35,38,40,43,45,48,50,53,56,58,61,63,66,68,70,73,75,78,80,83,85,88,90,93,95,98],
        11: [-19,-16,-14,-11,-8,-6,-3,0,2,5,7,9,12,14,17,19,21,24,26,29,32,34,37,39,42,45,47,50,53,56,58,61,64,66,69,71,73,76,78,81,83,85,88,90,92,94,97,99],
        12: [-29,-27,-24,-21,-19,-16,-14,-11,-8,-6,-3,-1,2,5,7,10,13,15,18,20,23,25,28,31,33,35,38,40,43,45,47,50,52,55,57,60,63,66,68,71,74,76,78,80,83,85,87,89],
        13: [-21,-19,-17,-14,-12,-9,-7,-5,-2,0,3,5,7,10,12,15,17,19,21,23,25,27,29,31,33,36,39,42,45,47,50,53,56,58,61,63,65,68,70,73,75,77,80,82,84,86,89,91],
        14: [-38,-36,-34,-32,-30,-28,-26,-24,-22,-19,-16,-13,-11,-8,-5,-2,1,3,6,8,11,13,16,18,21,23,26,28,31,33,36,38,40,43,45,48,50,53,55,57,60,63,65,68,71,74,77,79],
        15: [-27,-25,-23,-21,-19,-16,-14,-12,-10,-7,-4,0,3,6,9,12,16,19,22,25,29,32,35,38,42,44,46,48,51,53,55,57,59,64,68,73,77,82,86,91,95,96,96,96,96,96,96,96],
    },
    w4_k=8, w4_nv=3, w4_pin=10, w4_tok=(14, 36), nq_mxu=6)


def _tile_view(a):
    r, c = a.shape
    a = a.reshape(r // 16, 2, 8, c // 128, 128)
    return jnp.swapaxes(a, 2, 3)


def _head_view(a):
    c = a.shape[1]
    a = a.reshape(H, 2, DH // 16, 8, c // 128, 128)
    return jnp.swapaxes(a, 3, 4)


def _as_bf16(w32):
    n = w32.shape[0]
    return pltpu.bitcast(w32.reshape(n * 8, 128), BF16)


def _lhs(top, fill=0.0):
    return jnp.concatenate([top, jnp.full(top.shape, fill, F32)], axis=0).astype(BF16)


def _ln_stats(x):
    m = jnp.mean(x, axis=-1, keepdims=True)
    m2 = jnp.mean(x * x, axis=-1, keepdims=True)
    v = jnp.maximum(m2 - m * m, 0.0)
    return m, lax.rsqrt(v + EPS)


def _round_bf16(x):
    return x.astype(BF16).astype(F32)


def _dot(a, b):
    return jnp.dot(a, b, preferred_element_type=F32)


def _make_kernel(sk, win, cfg):
    nj = win // 128
    j0 = (sk - win) // 128
    jq = nj // 4
    jx = list(cfg["jx"])
    assert nj == 32 and cfg["blocks"][-2][0] <= NU - 3 and cfg["blocks"][-1] == (NU - 1, NU)
    qscale = DH ** -0.5 * 1.4426950408889634

    def kernel(x_hbm, k_hbm, v_hbm, wq_hbm, wo_hbm, w3_hbm, w4_hbm, o_ref,
               kbuf, vbuf, wobuf, w4buf, vx, wqbuf, w3buf, xin,
               xs, qacc, qlhs, sx, sy, pbuf0, pbuf1, plhs, mbuf, lpart, abuf, olhs, gp,
               sems):
        pbuf = (pbuf0, pbuf1)
        ns = abuf.shape[0]


        def cps_w(hbm, buf, sem, lo=0, n=None):
            n = buf.shape[0] if n is None else n
            return [pltpu.make_async_copy(
                hbm.at[pl.ds(lo, n), e],
                buf.at[pl.ds(lo, n), :, pl.ds(e * 8, 8), :],
                sems.at[sem]) for e in range(2)]

        def cps_k(u, par):
            return [pltpu.make_async_copy(
                k_hbm.at[pl.ds(u * UT, UT), e, pl.ds(j0, nj)],
                kbuf[u].at[:, :, pl.ds(e * 8, 8), :],
                sems.at[par]) for e in range(2)]

        def cps_v(u, par):
            return [pltpu.make_async_copy(
                v_hbm.at[pl.ds(2 * u, 2), e, :, pl.ds(j0, nj)],
                vbuf[u].at[:, :, :, pl.ds(e * 8, 8), :],
                sems.at[2 + par]) for e in range(2)]

        def cps_wo(part):
            lo, n = ((0, H - 8), (H - 8, 8))[part]
            return [pltpu.make_async_copy(
                wo_hbm.at[pl.ds(lo, n), e], wobuf[part].at[:, :, :, pl.ds(e * 8, 8), :],
                sems.at[4]) for e in range(2)]

        cps_x_wq = lambda: cps_w(wq_hbm, wqbuf, 4) + [pltpu.make_async_copy(x_hbm, xin, sems.at[4])]
        cps_w3 = lambda: cps_w(w3_hbm, w3buf, 0)
        w4_k = cfg["w4_k"] * 128
        w4_parts = [(c, 0, FF) for c in range(D // 128 - 1)]
        w4_parts += [(D // 128 - 1, 0, w4_k), (D // 128 - 1, w4_k, FF - w4_k)]

        def cps_w4(i):
            c, lo, n = w4_parts[i]
            return [pltpu.make_async_copy(
                w4_hbm.at[pl.ds(lo // 16, n // 16), e, c],
                w4buf[i].at[:, pl.ds(e * 8, 8), :],
                sems.at[(2, 1, 3, 0, 4, 2)[i]]) for e in range(2)]

        def start(cps):
            for c in cps:
                c.start()

        def wait(cps):
            for c in cps:
                c.wait()

        start(cps_x_wq())
        start(cps_k(0, 0))
        start(cps_k(1, 1))
        start(cps_v(0, 0))
        start(cps_v(1, 1))

        k32 = [b.bitcast(U32) for b in kbuf]
        v32 = [b.bitcast(U32) for b in vbuf]
        wq32 = wqbuf.bitcast(U32)
        wo32p = [b.bitcast(U32) for b in wobuf]
        w332 = w3buf.bitcast(U32)
        w432p = [b.bitcast(U32) for b in w4buf]

        def wo32(h):
            return wo32p[0].at[h] if h < H - 8 else wo32p[1].at[h - (H - 8)]

        def w4_words(c, t0, n):
            i = c if t0 * 16 < w4_parts[c][2] else c + 1
            return w432p[i][pl.ds(t0 - w4_parts[i][1] // 16, n)]

        def js(u):
            return cfg["js_at"].get(u, cfg["jsplit"])

        def jms(u):
            return [nj - 1 - jq * (i % 4) - i // 4 for i in range(nmx(u))]

        def early_tiles(kb):
            return ((H * DH // 128,) * 3 + (3 * cfg["nq_mxu"], 0))[kb]

        def nmx(u):
            return cfg["nm_at"].get(u, cfg["nm"])

        def pack_q(q, u):
            q = q * qscale
            lane = lax.broadcasted_iota(jnp.int32, (8, 128), 1)
            sub = lax.broadcasted_iota(jnp.int32, (8, 128), 0)
            keep = (lane < DH - 128) == (sub % 2 == 0)
            q = jnp.concatenate(
                [q[:, 0:128], jnp.where(keep, q[:, 128:256], 0.0), q[:, 256:384]], axis=1)
            qlhs.at[u][:, 0:384] = pltpu.bitcast(_lhs(q), U32)

        def st_qk(u, js):
            sl = u % 2
            lhs = pltpu.bitcast(qlhs[u], BF16)
            toks = []
            for j in js:
                ra = 2 * (j // jq)
                cs = slice((j % jq) * 128, (j % jq + 1) * 128)
                for t in range(3):
                    w = _as_bf16(k32[u][pl.ds(t * 8, 8), j])
                    r = _dot(lhs[:, t * 128:(t + 1) * 128], w)
                    toks.append(r[8:16])
                    if t == 0:
                        sx[sl, ra:ra + 1, cs] = r[0:1]
                    elif t == 1:
                        sy[sl, ra:ra + 2, cs] = r[ra:ra + 2]
                    else:
                        sx[sl, ra + 1:ra + 2, cs] = r[0:1]
            return toks

        def st_softmax(u, zdyn, pin=False):
            sl = u % 2
            s = sx[sl] + sy[sl]
            m = s
            while m.shape[1] > 128:
                h = m.shape[1] // 2
                m = jnp.maximum(m[:, :h], m[:, h:])
            m = jnp.maximum(m, pltpu.roll(m, 2, 0))
            m = jnp.maximum(m, pltpu.roll(m, 4, 0))
            if pin:
                qlhs[NU + zdyn, :, 0:128] = pltpu.bitcast(m, U32)
            m = jnp.max(m, axis=1, keepdims=True)
            p = jnp.exp2(s - m)
            pbuf[sl][zdyn] = p
            for g in range((nmx(u) + 3) // 4):
                c = jq - 1 - g
                plhs[:, (2 * sl + g) * 128:(2 * sl + g + 1) * 128] = pltpu.bitcast(
                    _lhs(p[:, c * 128:(c + 1) * 128]), U32)

        def inv_l(l):
            l = jnp.sum(l, axis=1, keepdims=True)
            r0 = pl.reciprocal(l, approx=True)
            return jnp.broadcast_to(r0 * (2.0 - l * r0), (8, 128))

        def st_lsum(u):
            l = pbuf[u % 2][0, :, 0:128]
            for c in range(1, jq):
                l = l + pbuf[u % 2][0, :, c * 128:(c + 1) * 128]
            l = l + pltpu.roll(l, 2, 0)
            l = l + pltpu.roll(l, 4, 0)
            lpart[u % ns] = inv_l(l) if u == NU - 1 else l

        def st_pvm(u):
            toks = []
            for j in jms(u):
                g = jq - 1 - j % jq
                pc = 2 * (u % 2) + g
                lhs = pltpu.bitcast(plhs[:, pc * 128:(pc + 1) * 128], BF16)
                ra = 2 * (j // jq)
                for t in range(3):
                    if t == 1:
                        w32 = jnp.concatenate(
                            [v32[u][0, 8:12, j], v32[u][1, 0:4, j]], axis=0)
                    else:
                        w32 = v32[u][t // 2, 2 * t:2 * t + 8, j]
                    r = _dot(lhs, _as_bf16(w32))
                    toks.append(r[8:16])
                    mbuf[u % ns, g, t, ra:ra + 2, :] = r[ra:ra + 2]
            return toks

        def st_expand(u):
            def body(dt, c):
                for hd in range(2):
                    for ix, j in enumerate(jx):
                        w = v32[u][hd, dt, j]
                        vx[2 * u + hd, dt, ix] = pltpu.bitcast(w << 16, F32)
                        vbuf[u][hd, dt, j] = pltpu.bitcast(w & jnp.uint32(0xFFFF0000), BF16)
                return c
            lax.fori_loop(0, UT // 2, body, 0)
            for j in jms(u):
                for t in range(3):
                    idx = [divmod(t * 8 + v, 12) for v in range(8)]
                    blk = jnp.concatenate([vbuf[u][hd, dt, j] for hd, dt in idx], axis=0)
                    blk = blk.astype(F32).T.astype(BF16)
                    for v, (hd, dt) in enumerate(idx):
                        vbuf[u][hd, dt, j] = blk[v * 16:(v + 1) * 16]

        def st_pv(u, toks, tok_map):
            nm, sl = nmx(u), u % ns
            for piece in range(NPIECE):
                hd, half = divmod(piece, NPIECE // 2)
                sub = len(tok_map) // NPIECE
                lo = hi = None
                for j in range(nj):
                    if j in jms(u):
                        continue
                    row = 2 * (j // jq) + hd
                    cs = slice((j % jq) * 128, (j % jq + 1) * 128)
                    pb = jnp.broadcast_to(pbuf[u % 2][0, row:row + 1, cs], (8, 128))
                    k = piece * sub + j * sub // nj
                    ti = tok_map[k] if j % (nj // sub) == 0 else -1
                    if j > 0 and tok_map[k - 1] == ti:
                        ti = -1
                    if toks and ti >= 0:
                        pb = pb + toks[min(ti, len(toks) - 1)]
                    w = v32[u][hd, pl.ds(half * 2, 2), j]
                    if j in jx:
                        a = vx[2 * u + hd, pl.ds(half * 2, 2), jx.index(j)] * pb
                        b = pltpu.bitcast(w, F32) * pb
                    else:
                        a = pltpu.bitcast(w << 16, F32) * pb
                        b = pltpu.bitcast(w & jnp.uint32(0xFFFF0000), F32) * pb
                    lo = a if lo is None else lo + a
                    hi = b if hi is None else hi + b
                for i in range(2):
                    base = (piece * 2 + i) * 16
                    abuf[sl, pl.ds(base, 8, stride=2), :] = lo[i]
                    abuf[sl, pl.ds(base + 1, 8, stride=2), :] = hi[i]

        def st_ored(u):
            nm, sl = nmx(u), u % ns
            ia = inv_l(lpart[sl])
            ib = pltpu.roll(ia, 1, 0)
            lane = lax.broadcasted_iota(jnp.int32, (8, 128), 1)
            for t in range(3):
                at = abuf[sl, t * 128:(t + 1) * 128, :].T
                o = at[0:8]
                for i in range(1, 16):
                    o = o + at[i * 8:(i + 1) * 8]
                if nm:
                    sub = lax.broadcasted_iota(jnp.int32, (8, 128), 0)
                    odd = (0, (lane >= DH - 128).astype(jnp.int32), 1)[t]
                    for g in range((nm + 3) // 4):
                        keep = (sub >= 8 - 2 * min(nm - 4 * g, 4)) & (sub % 2 == odd)
                        o = o + jnp.where(keep, mbuf[sl, g, t], 0.0)
                o = o + pltpu.roll(o, 4, 0)
                o = o + pltpu.roll(o, 2, 0)
                o = o + pltpu.roll(o, 1, 0)
                o = o * (ia, jnp.where(lane < DH - 128, ia, ib), ib)[t]
                olhs.at[u][:, t * 128:(t + 1) * 128] = pltpu.bitcast(_lhs(o), U32)

        def st_olast(u, out):
            sl = u % ns
            for hd in range(2):
                pa = [None, None]
                for dt in range(12):
                    base = (hd * 12 + dt) * 16
                    lo = jnp.sum(abuf[sl, pl.ds(base, 8, stride=2), :], axis=1, keepdims=True)
                    hi = jnp.sum(abuf[sl, pl.ds(base + 1, 8, stride=2), :], axis=1, keepdims=True)
                    w = wo32(2 * u + hd)[dt]
                    pr = (pltpu.bitcast(w << 16, F32) * lo
                          + pltpu.bitcast(w & jnp.uint32(0xFFFF0000), F32) * hi)
                    pa[dt % 2] = pr if pa[dt % 2] is None else pa[dt % 2] + pr
                inv = jnp.broadcast_to(lpart[sl, hd:hd + 1, :], (8, 128))
                tot = (pa[0] + pa[1]) * inv
                for n in range(D // 128):
                    out[n].append(tot[n])

        def st_oproj(u, ts=(0, 1, 2)):
            lhs = pltpu.bitcast(olhs[u], BF16)
            toks = []
            for t in ts:
                for n in range(D // 128):
                    if t == 1:
                        w32 = jnp.concatenate(
                            [wo32(2 * u)[8:12, n], wo32(2 * u + 1)[0:4, n]], axis=0)
                    else:
                        w32 = wo32(2 * u + t // 2)[2 * t:2 * t + 8, n]
                    r = _dot(lhs[:, t * 128:(t + 1) * 128], _as_bf16(w32))
                    toks.append(r[8:16])
                    gp[t, n, pl.ds(u, 1), :] = r[0:1]
            return toks

        def mlp(first, extra, zdyn):
            g = gp[0] + gp[1] + gp[2]
            g = g[:, 0:8] + g[:, 8:16]
            g = jnp.concatenate([sum(extra[n], g[n]) for n in range(D // 128)], axis=1)
            g = g + pltpu.roll(g, 4, 0)
            g = g + pltpu.roll(g, 2, 0)
            g = g + pltpu.roll(g, 1, 0)
            x1 = _round_bf16(xs[...] + g)
            lhs = _lhs(x1, 1.0)
            m1, r1 = _ln_stats(x1)
            y = (x1 - m1) * r1
            m2, r2 = _ln_stats(y)
            a = r1 * r2
            b = (m1 * r1 + m2) * r2
            if first:
                wait(cps_w3())
                start(cps_w4(3))
                start(cps_w4(4))
            hl, hs = [], []
            for n in range(FF // 128):
                r = _dot(lhs, _as_bf16(w332[:, n]))
                hn = jax.nn.gelu(r[0:8] * a - r[8:16] * b, approximate=True)
                hl.append(_lhs(hn))
                hs.append(hn)
            acc = x1 + y
            acc = [acc[:, c * 128:(c + 1) * 128] for c in range(D // 128)]

            def w4_dot(kt, c):
                return _dot(hl[kt], _as_bf16(w4_words(c, kt * 8, 8)))[0:8]

            if not first:
                nv, kpin, (t0, t1) = cfg["w4_nv"], cfg["w4_pin"], cfg["w4_tok"]
                toks = []
                for kt in range(nv, FF // 128):
                    if nv and kt == kpin:
                        for k in range(nv):
                            blk = jnp.broadcast_to(_round_bf16(hs[k][0:1]), (128, 128)).T
                            abuf[zdyn, k * 128:(k + 1) * 128, :] = blk
                            qlhs[NU + zdyn, :, 0:128] = pltpu.bitcast(blk[120:128], U32)
                        hl[kt] = pltpu.bitcast(qlhs[0, :, 0:128], BF16)
                    if nv and kt + 1 == kpin:
                        qlhs.at[0][:, 0:128] = pltpu.bitcast(hl[kpin], U32)
                    for c in range(D // 128):
                        r = _dot(hl[kt], _as_bf16(w4_words(c, kt * 8, 8)))
                        toks.append(r[8:16])
                        acc[c] = acc[c] + r[0:8]
                pa = None
                for dt in range(nv * 8):
                    tk = toks[t0 + dt * (t1 - t0) // (nv * 8)]
                    lo = abuf[0, pl.ds(dt * 16, 8, stride=2), :] + tk
                    hi = abuf[0, pl.ds(dt * 16 + 1, 8, stride=2), :] + tk
                    w = jnp.concatenate([w4_words(c, dt, 1) for c in range(D // 128)], axis=0)
                    pr = (pltpu.bitcast(w << 16, F32) * lo
                          + pltpu.bitcast(w & jnp.uint32(0xFFFF0000), F32) * hi)
                    pa = pr if pa is None else pa + pr
                for c in range(D // 128 if nv else 0):
                    pc = pa[c]
                    pc = pc + pltpu.roll(pc, 4, 0)
                    pc = pc + pltpu.roll(pc, 2, 0)
                    acc[c] = (pc + pltpu.roll(pc, 1, 0)) + acc[c]
                xs[...] = _round_bf16(jnp.concatenate(acc, axis=1))
                return
            for i, (c, lo, n) in enumerate(w4_parts):
                wait(cps_w4(i))
                if i == 0:
                    start(cps_w4(5))
                    for k, hn in enumerate(hs[cfg["w4_k"]:]):
                        abuf[k // 3, (k % 3) * 128:(k % 3 + 1) * 128, :] = jnp.broadcast_to(
                            _round_bf16(hn[0:1]), (128, 128)).T
                if lo == 0:
                    for kt in range(n // 128):
                        acc[c] = acc[c] + w4_dot(kt, c)
                else:
                    pas = [None] * 4
                    for dt in range(n // 16):
                        w = w4_words(c, lo // 16 + dt, 1)[0]
                        sl, r0 = dt // 24, dt % 24 * 16
                        pr = (pltpu.bitcast(w << 16, F32) * abuf[sl, pl.ds(r0, 8, stride=2), :]
                              + pltpu.bitcast(w & jnp.uint32(0xFFFF0000), F32)
                              * abuf[sl, pl.ds(r0 + 1, 8, stride=2), :])
                        pas[dt % 4] = pr if pas[dt % 4] is None else pas[dt % 4] + pr
                    pa = (pas[0] + pas[1]) + (pas[2] + pas[3])
                    pa = pa + pltpu.roll(pa, 4, 0)
                    pa = pa + pltpu.roll(pa, 2, 0)
                    acc[c] = acc[c] + (pa + pltpu.roll(pa, 1, 0))
                if lo + n == FF:
                    xc = _round_bf16(acc[c])
                    xs[:, c * 128:(c + 1) * 128] = xc
                    lhs = _lhs(xc)
                    for nt in range(early_tiles(c)):
                        r = _dot(lhs, _as_bf16(wq32[pl.ds(c * 8, 8), nt]))[0:4]
                        qacc[nt, 0:4, :] = r if c == 0 else qacc[nt, 0:4, :] + r

        gp[...] = jnp.zeros_like(gp)
        mbuf[...] = jnp.zeros_like(mbuf)
        wait(cps_x_wq())
        start(cps_wo(0))
        x0 = jnp.broadcast_to(xin[...].astype(F32), (8, D))
        sub0 = lax.broadcasted_iota(jnp.int32, (8, D), 0)
        lane0 = lax.broadcasted_iota(jnp.int32, (8, D), 1)
        for nkb, n0, n1 in ((4, 0, early_tiles(3)), (3, early_tiles(3), early_tiles(0))):
            lhs0 = _lhs(jnp.where(sub0 < 4, jnp.where(lane0 < nkb * 128, x0, 0.0), 1.0))

            def q0_body(nt, c, lhs0=lhs0):
                qacc[nt] = _dot(lhs0, _as_bf16(wq32[:, nt]))[0:8]
                return c
            lax.fori_loop(n0, n1, q0_body, 0)
        wait(cps_k(0, 0))
        start(cps_k(2, 0))
        wait(cps_k(1, 1))
        wait(cps_v(0, 0))
        xs[...] = x0

        def layer(li, carry):
            first = li == 0
            n_first = jnp.maximum(1 - li, 0)
            zdyn = li >> 4

            def block_dma(ua, ub):
                def last_wait(t):
                    if t == NU - 2:
                        wait(cps_k(NU - 1, (NU - 1) % 2))
                    else:
                        wait(cps_v(t + 1, (t + 1) % 2) if t + 1 < NU else cps_wo(1))

                def dma_ops(_, c):
                    for t in range(ua, ub):
                        if t + 3 < NU:
                            start(cps_k(t + 3, (t + 3) % 2))
                        if t + 2 < NU:
                            start(cps_v(t + 2, t % 2))
                        if t == NU - 2:
                            start(cps_w3())
                            start(cps_w4(0))
                        if t == NU - 1:
                            start(cps_w4(1))
                            wait(cps_v(t, t % 2))
                            start(cps_w4(2))
                        if t == 1:
                            wait(cps_wo(0))
                            start(cps_wo(1))
                        st_expand(t)
                        if t + 2 < NU - 1:
                            wait(cps_k(t + 2, t % 2))
                        if t < ub - 1:
                            last_wait(t)
                    return c

                lax.fori_loop(0, n_first, dma_ops, 0)
                pl.when(first)(lambda: last_wait(ub - 1))

            def prologue():
                x = xs[...]
                m, r = _ln_stats(x)
                nq = cfg["nq_mxu"]

                def finish_q(u, late):
                    qs = []
                    for nt in range(3):
                        qx = jnp.broadcast_to(qacc[u * 3 + nt, 0:1, :], (8, 128))
                        cs = jnp.broadcast_to(qacc[u * 3 + nt, 4:5, :], (8, 128))
                        qs.append((qx + late[nt] - cs * m) * r)
                    pack_q(jnp.concatenate(qs, axis=1), u)

                lhs = _lhs(x[:, D - 128:D])
                for u in range(nq):
                    finish_q(u, [_dot(lhs, _as_bf16(wq32[pl.ds(32, 8), u * 3 + nt]))[0:8]
                                 for nt in range(3)])
                f1 = cfg["va_force"]
                toks = st_qk(0, range(f1))
                for kb in range(2):
                    cs = slice((3 + kb) * 128, (4 + kb) * 128)
                    blk = jnp.broadcast_to(x[0:1, cs], (128, 128)).T
                    abuf[ns - 1 + zdyn, kb * 128:(kb + 1) * 128, :] = blk
                    qlhs[NU + zdyn, :, 0:128] = pltpu.bitcast(blk[120:128], U32)
                toks += st_qk(0, range(f1, nj))
                st_softmax(0, zdyn)
                toks += st_qk(1, range(js(1)))
                toks += st_pvm(0)
                for va, (t0, t1) in zip(cfg["va_groups"], cfg["va_tok"]):
                    acc = [None] * len(va)
                    for kt in range(16):
                        lo = abuf[ns - 1, pl.ds(kt * 16, 8, stride=2), :]
                        hi = abuf[ns - 1, pl.ds(kt * 16 + 1, 8, stride=2), :]
                        tk = toks[t0 + kt * (t1 - t0) // 16]
                        lo, hi = lo + tk, hi + tk
                        for i, u in enumerate(va):
                            w = wq32[24 + kt, u * 3:u * 3 + 3]
                            pr = (pltpu.bitcast(w << 16, F32) * lo
                                  + pltpu.bitcast(w & jnp.uint32(0xFFFF0000), F32) * hi)
                            acc[i] = pr if acc[i] is None else acc[i] + pr
                    for i, u in enumerate(va):
                        late = []
                        for nt in range(3):
                            q = acc[i][nt]
                            q = q + pltpu.roll(q, 4, 0)
                            q = q + pltpu.roll(q, 2, 0)
                            late.append(q + pltpu.roll(q, 1, 0))
                        finish_q(u, late)
                return toks

            def block(bi):
                ua, ub = cfg["blocks"][bi]
                block_dma(ua, ub)
                toks = []
                if bi == 0:
                    toks += prologue()
                done = js(ua + 1)
                for t in range(ua, ub):
                    base = len(toks)
                    for u in cfg["ored_at"].get(t, ()):
                        st_ored(u)
                    if t + 1 < NU:
                        toks += st_qk(t + 1, range(done, nj))
                    g0 = len(toks)
                    if t == ua and bi > 0:
                        toks += st_pvm(t)
                    for u in cfg["oproj_at"].get(t, ()):
                        toks += st_oproj(*u) if isinstance(u, tuple) else st_oproj(u)
                    done = js(t + 2)
                    if t + 1 < ub:
                        gap = cfg["gap"]
                        done = max(-((len(toks) - g0 - gap) // 3), 0)
                    gap1 = cfg["gap1"]
                    d1 = min(max(-((len(toks) - g0 - gap1) // 3), 0), done)
                    if t + 2 < NU:
                        toks += st_qk(t + 2, range(d1))
                    if t + 1 < NU:
                        st_softmax(t + 1, zdyn, pin=t + 2 < NU and d1 < done)
                    if t + 2 < NU:
                        toks += st_qk(t + 2, range(d1, done))
                    if t + 1 < ub:
                        toks += st_pvm(t + 1)
                    st_pv(t, toks, [base + i for i in cfg["tok"][t]])
                    st_lsum(t)

            def tail(first_static):
                seen = set()
                for us in cfg["oproj_at"].values():
                    for u in us:
                        uu, ts = u if isinstance(u, tuple) else (u, (0, 1, 2))
                        seen |= {(uu, t) for t in ts}
                for u in range(NU - 1):
                    ts = tuple(t for t in range(3) if (u, t) not in seen)
                    if ts:
                        st_oproj(u, ts)
                extra = [[] for _ in range(D // 128)]
                st_olast(NU - 1, extra)
                mlp(first_static, extra, zdyn)

            for bi in range(len(cfg["blocks"])):
                block(bi)

            pl.when(first)(lambda: tail(True))
            pl.when(jnp.logical_not(first))(lambda: tail(False))
            return carry

        lax.fori_loop(0, 2, layer, 0)
        o_ref[...] = xs[0:1, :].astype(o_ref.dtype)

    return kernel


@jax.jit
def pallas_interleave_layers__sliding_block_cached__mixer_s_mlp__decode_kernel(
    A_x: jax.Array,
    A_k_cache: jax.Array,
    A_v_cache: jax.Array,
    A_wq: jax.Array,
    A_wo: jax.Array,
    B_x: jax.Array,
    B_w1: jax.Array,
    B_w2: jax.Array,
    B_w3: jax.Array,
    B_w4: jax.Array,
):
    b, sq, d = A_x.shape
    _, hkv, sk, dh = A_k_cache.shape
    assert (b, sq, d, hkv, dh) == (1, 1, D, H, DH)
    win = min(4096, max(256, sk // 4))
    assert win % 512 == 0 and sk % 128 == 0
    nj = win // 128

    kt = _tile_view(jnp.swapaxes(A_k_cache, 2, 3).reshape(H * DH, sk))
    vt = _head_view(jnp.swapaxes(A_v_cache, 2, 3).reshape(H * DH, sk))

    def buf(r, c):
        return pltpu.VMEM((r // 16, c // 128, 16, 128), BF16)

    def hbuf(h, c):
        return pltpu.VMEM((h, DH // 16, c // 128, 16, 128), BF16)

    bl = CFG["blocks"]
    ns = CFG.get("ns") or max(bl[i + 1][1] - bl[i][0] for i in range(len(bl) - 1))
    any_spec = pl.BlockSpec(memory_space=pl.ANY)
    out = pl.pallas_call(
        _make_kernel(sk, win, CFG),
        out_shape=jax.ShapeDtypeStruct((1, D), A_x.dtype),
        in_specs=[any_spec] * 7,
        out_specs=pl.BlockSpec(memory_space=pltpu.VMEM),
        scratch_shapes=[
            [buf(2 * DH, win)] * NU, [hbuf(2, win)] * NU, [hbuf(H - 8, D), hbuf(8, D)],
            [pltpu.VMEM((r // 16, 16, 128), BF16)
             for r in (FF,) * 4 + (CFG["w4_k"] * 128, FF - CFG["w4_k"] * 128)],
            pltpu.VMEM((H, DH // 16, max(len(CFG["jx"]), 1), 8, 128), F32),
            buf(D, H * DH), buf(D, FF),
            pltpu.VMEM((1, D), BF16),
            pltpu.VMEM((8, D), F32),
            pltpu.VMEM((H * DH // 128, 8, 128), F32),
            pltpu.VMEM((NU + 1, 8, 384), U32),
            pltpu.VMEM((2, 8, win // 4), F32),
            pltpu.VMEM((2, 8, win // 4), F32),
            pltpu.VMEM((1, 8, win // 4), F32),
            pltpu.VMEM((1, 8, win // 4), F32),
            pltpu.VMEM((8, 512), U32),
            pltpu.VMEM((ns, 2, 3, 8, 128), F32),
            pltpu.VMEM((ns, 8, 128), F32),
            pltpu.VMEM((ns, 384, 128), F32),
            pltpu.VMEM((NU, 8, 384), U32),
            pltpu.VMEM((3, D // 128, NU, 128), F32),
            pltpu.SemaphoreType.DMA((5,)),
        ],
        compiler_params=pltpu.CompilerParams(vmem_limit_bytes=int(CFG["vmem_mb"] * 1024 * 1024)),
        name="interleave_decode",
    )(A_x.reshape(1, D), kt, vt, _tile_view(A_wq), _head_view(A_wo),
      _tile_view(B_w3), _tile_view(B_w4))
    return out.reshape(b, sq, d)
```

```python
import jax
import jax.numpy as jnp
from jax import lax
import jax.experimental.pallas as pl
import jax.experimental.pallas.tpu as pltpu

F32 = jnp.float32
BF16 = jnp.bfloat16
U32 = jnp.uint32

D = 640
H = 32
DH = 192
FF = 1536
NU = H // 2
UT = 2 * DH // 16
EPS = 1e-5
NPIECE = 12

CFG = dict(
    blocks=((0, 4), (4, 8), (8, 12), (12, 15), (15, 16)),
    ns=7,
    jsplit=10, js_at={1: 13, 5: 19, 9: 19, 13: 16},
    gap=49, gap1=24,
    nm=4, nm_at={12: 5, 13: 5, 14: 5, 15: 0},
    va_groups=((6, 7, 8, 9), (10, 11, 12, 13, 14), (15,)), va_force=7,
    va_tok=((6, 43), (48, 94), (102, 112)),
    ored_at={4: (0,), 5: (1,), 6: (2,), 7: (3,), 8: (4,), 9: (5,), 10: (6,), 11: (7,),
             12: (8,), 13: (9,), 14: (10, 11), 15: (12, 13, 14)},
    oproj_at={4: ((0, (2,)),), 5: ((1, (2,)),), 6: ((2, (2,)),), 7: ((3, (2,)),),
              8: ((4, (0,)), (0, (0,))), 9: ((5, (0,)), (0, (1,))), 10: ((6, (0,)),), 11: ((7, (0,)),),
              12: ((8, (0,)),), 13: ((9, (0,)),),
              14: ((4, (1, 2)), (10, (0,)), (1, (0, 1)), (11, (0,))),
              15: ((2, (0, 1)), (3, (0, 1)), (5, (1, 2)), (6, (1, 2)), (7, (1, 2)), (8, (1, 2)), (9, (1, 2)),
                   (10, (1, 2)), (11, (1, 2)), 12, (13, (0, 1)))},
    jx=(1, 5, 9, 13, 17, 21, 25),
    vmem_mb=128,
    tok={
        0: [-26,-24,-22,-19,-17,-15,-13,-10,-8,-6,-3,-1,1,4,6,9,11,14,16,19,21,24,26,28,31,34,36,39,41,44,46,49,51,54,57,59,62,64,66,68,71,71,75,77,79,82,84,86],
        1: [-32,-29,-27,-25,-22,-20,-17,-15,-13,-10,-8,-5,-3,-1,2,4,7,9,11,14,16,18,21,23,26,28,30,33,35,37,40,42,44,47,49,51,54,56,58,60,62,65,67,69,71,73,76,78],
        2: [-28,-26,-23,-21,-18,-16,-14,-11,-9,-7,-4,-2,1,3,6,8,10,13,15,18,20,23,25,28,30,33,35,37,40,42,45,47,50,52,55,57,59,62,65,67,70,73,75,78,81,83,86,89],
        3: [-17,-15,-13,-10,-8,-6,-4,-2,0,2,5,7,9,11,14,16,19,22,24,27,29,32,34,37,39,42,44,47,49,52,55,57,60,62,65,67,70,72,74,77,79,81,84,86,88,90,93,95],
        4: [-27,-24,-22,-19,-17,-15,-12,-10,-7,-5,-4,-2,0,2,4,6,8,11,14,17,20,23,26,29,32,34,37,39,42,44,46,49,51,54,56,59,61,64,66,69,71,74,76,79,81,84,86,88],
        5: [-10,-8,-5,-2,0,3,5,8,10,13,15,18,18,20,25,28,30,33,35,38,40,43,45,48,50,53,56,58,61,64,66,69,71,74,76,78,80,82,84,87,89,91,94,97,99,102,105,108],
        6: [-15,-13,-11,-9,-7,-4,-2,0,2,5,8,10,13,16,19,21,24,27,29,31,34,36,39,41,43,44,49,51,54,56,59,61,61,66,69,71,73,76,78,81,83,86,88,91,93,96,98,101],
        7: [-10,-7,-5,-2,0,2,5,7,10,12,15,17,20,22,25,27,30,32,35,38,41,43,46,49,51,54,56,58,60,63,65,67,69,72,74,77,79,82,84,86,89,91,94,96,97,99,103,105],
        8: [-23,-21,-19,-17,-15,-14,-12,-10,-8,-6,-3,-1,1,3,5,7,10,12,15,17,20,23,25,28,31,33,36,39,41,44,47,49,52,54,57,59,62,64,66,69,71,74,76,79,81,84,87,89],
        9: [-8,-6,-4,-1,1,4,6,8,11,13,16,18,21,24,26,29,31,34,36,39,42,44,47,49,52,55,57,59,62,64,67,69,72,74,77,79,82,84,87,89,92,94,97,99,102,104,106,109],
        10: [-19,-16,-14,-11,-9,-7,-4,-2,1,3,6,8,10,13,15,18,20,23,25,28,30,33,35,38,40,43,45,48,50,53,56,58,61,63,66,68,70,73,75,78,80,83,85,88,90,93,95,98],
        11: [-19,-16,-14,-11,-8,-6,-3,0,2,5,7,9,12,14,17,19,21,24,26,29,32,34,37,39,42,45,47,50,53,56,58,61,64,66,69,71,73,76,78,81,83,85,88,90,92,94,97,99],
        12: [-29,-24,-21,-18,-17,-13,-11,-8,-6,-5,-4,-3,-1,2,2,4,10,12,15,20,23,25,28,31,33,35,38,40,45,46,47,50,52,55,57,60,63,66,68,71,74,76,78,80,83,85,87,89],
        13: [-21,-19,-17,-14,-10,-9,-7,-5,-2,0,3,5,7,10,12,12,17,19,21,24,25,27,29,31,33,36,39,42,45,47,50,53,55,57,60,62,64,67,69,73,75,77,80,82,84,86,89,91],
        14: [-38,-36,-34,-32,-30,-27,-25,-24,-22,-19,-16,-13,-11,-8,-5,-2,1,3,6,8,11,13,16,18,21,23,26,28,29,33,35,36,40,43,45,48,50,53,55,57,60,63,65,68,71,74,77,79],
        15: [-28,-26,-24,-22,-16,-16,-14,-12,-10,-10,-6,1,3,6,9,15,16,22,22,24,28,31,34,37,41,44,46,46,51,53,55,57,62,64,68,73,77,82,86,91,93,94,94,94,102,102,102,102],
    },
    w4_k=8, w4_nv=3, w4_pin=10, w4_tok=(14, 36), nq_mxu=6)


def _tile_view(a):
    r, c = a.shape
    a = a.reshape(r // 16, 2, 8, c // 128, 128)
    return jnp.swapaxes(a, 2, 3)


def _head_view(a):
    c = a.shape[1]
    a = a.reshape(H, 2, DH // 16, 8, c // 128, 128)
    return jnp.swapaxes(a, 3, 4)


def _as_bf16(w32):
    n = w32.shape[0]
    return pltpu.bitcast(w32.reshape(n * 8, 128), BF16)


def _lhs(top, fill=0.0):
    return jnp.concatenate([top, jnp.full(top.shape, fill, F32)], axis=0).astype(BF16)


def _ln_stats(x):
    m = jnp.mean(x, axis=-1, keepdims=True)
    m2 = jnp.mean(x * x, axis=-1, keepdims=True)
    v = jnp.maximum(m2 - m * m, 0.0)
    return m, lax.rsqrt(v + EPS)


def _round_bf16(x):
    return x.astype(BF16).astype(F32)


def _dot(a, b):
    return jnp.dot(a, b, preferred_element_type=F32)


def _make_kernel(sk, win, cfg):
    nj = win // 128
    j0 = (sk - win) // 128
    jq = nj // 4
    jx = list(cfg["jx"])
    assert nj == 32 and cfg["blocks"][-2][0] <= NU - 3 and cfg["blocks"][-1] == (NU - 1, NU)
    qscale = DH ** -0.5 * 1.4426950408889634

    def kernel(x_hbm, k_hbm, v_hbm, wq_hbm, wo_hbm, w3_hbm, w4_hbm, o_ref,
               kbuf, vbuf, wobuf, w4buf, vx, wqbuf, w3buf, xin,
               xs, qacc, qlhs, sx, sy, pbuf0, pbuf1, plhs, mbuf, lpart, abuf, olhs, gp,
               sems):
        pbuf = (pbuf0, pbuf1)
        ns = abuf.shape[0]


        def cps_w(hbm, buf, sem, lo=0, n=None):
            n = buf.shape[0] if n is None else n
            return [pltpu.make_async_copy(
                hbm.at[pl.ds(lo, n), e],
                buf.at[pl.ds(lo, n), :, pl.ds(e * 8, 8), :],
                sems.at[sem]) for e in range(2)]

        def cps_k(u, par):
            return [pltpu.make_async_copy(
                k_hbm.at[pl.ds(u * UT, UT), e, pl.ds(j0, nj)],
                kbuf[u].at[:, :, pl.ds(e * 8, 8), :],
                sems.at[par]) for e in range(2)]

        def cps_v(u, par):
            return [pltpu.make_async_copy(
                v_hbm.at[pl.ds(2 * u, 2), e, :, pl.ds(j0, nj)],
                vbuf[u].at[:, :, :, pl.ds(e * 8, 8), :],
                sems.at[2 + par]) for e in range(2)]

        def cps_wo(part):
            lo, n = ((0, H - 8), (H - 8, 8))[part]
            return [pltpu.make_async_copy(
                wo_hbm.at[pl.ds(lo, n), e], wobuf[part].at[:, :, :, pl.ds(e * 8, 8), :],
                sems.at[4]) for e in range(2)]

        cps_x_wq = lambda: cps_w(wq_hbm, wqbuf, 4) + [pltpu.make_async_copy(x_hbm, xin, sems.at[4])]
        cps_w3 = lambda: cps_w(w3_hbm, w3buf, 0)
        w4_k = cfg["w4_k"] * 128
        w4_parts = [(c, 0, FF) for c in range(D // 128 - 1)]
        w4_parts += [(D // 128 - 1, 0, w4_k), (D // 128 - 1, w4_k, FF - w4_k)]

        def cps_w4(i):
            c, lo, n = w4_parts[i]
            return [pltpu.make_async_copy(
                w4_hbm.at[pl.ds(lo // 16, n // 16), e, c],
                w4buf[i].at[:, pl.ds(e * 8, 8), :],
                sems.at[(2, 1, 3, 0, 4, 2)[i]]) for e in range(2)]

        def start(cps):
            for c in cps:
                c.start()

        def wait(cps):
            for c in cps:
                c.wait()

        start(cps_x_wq())
        start(cps_k(0, 0))
        start(cps_k(1, 1))
        start(cps_v(0, 0))
        start(cps_v(1, 1))

        k32 = [b.bitcast(U32) for b in kbuf]
        v32 = [b.bitcast(U32) for b in vbuf]
        wq32 = wqbuf.bitcast(U32)
        wo32p = [b.bitcast(U32) for b in wobuf]
        w332 = w3buf.bitcast(U32)
        w432p = [b.bitcast(U32) for b in w4buf]

        def wo32(h):
            return wo32p[0].at[h] if h < H - 8 else wo32p[1].at[h - (H - 8)]

        def w4_words(c, t0, n):
            i = c if t0 * 16 < w4_parts[c][2] else c + 1
            return w432p[i][pl.ds(t0 - w4_parts[i][1] // 16, n)]

        def js(u):
            return cfg["js_at"].get(u, cfg["jsplit"])

        def jms(u):
            return [nj - 1 - jq * (i % 4) - i // 4 for i in range(nmx(u))]

        def early_tiles(kb):
            return ((H * DH // 128,) * 3 + (3 * cfg["nq_mxu"], 0))[kb]

        def nmx(u):
            return cfg["nm_at"].get(u, cfg["nm"])

        def pack_q(q, u):
            q = q * qscale
            lane = lax.broadcasted_iota(jnp.int32, (8, 128), 1)
            sub = lax.broadcasted_iota(jnp.int32, (8, 128), 0)
            keep = (lane < DH - 128) == (sub % 2 == 0)
            q = jnp.concatenate(
                [q[:, 0:128], jnp.where(keep, q[:, 128:256], 0.0), q[:, 256:384]], axis=1)
            qlhs.at[u][:, 0:384] = pltpu.bitcast(_lhs(q), U32)

        def st_qk(u, js):
            sl = u % 2
            lhs = pltpu.bitcast(qlhs[u], BF16)
            toks = []
            for j in js:
                ra = 2 * (j // jq)
                cs = slice((j % jq) * 128, (j % jq + 1) * 128)
                for t in range(3):
                    w = _as_bf16(k32[u][pl.ds(t * 8, 8), j])
                    r = _dot(lhs[:, t * 128:(t + 1) * 128], w)
                    toks.append(r[8:16])
                    if t == 0:
                        sx[sl, ra:ra + 1, cs] = r[0:1]
                    elif t == 1:
                        sy[sl, ra:ra + 2, cs] = r[ra:ra + 2]
                    else:
                        sx[sl, ra + 1:ra + 2, cs] = r[0:1]
            return toks

        def st_softmax(u, zdyn, pin=False):
            sl = u % 2
            s = sx[sl] + sy[sl]
            m = s
            while m.shape[1] > 128:
                h = m.shape[1] // 2
                m = jnp.maximum(m[:, :h], m[:, h:])
            m = jnp.maximum(m, pltpu.roll(m, 2, 0))
            m = jnp.maximum(m, pltpu.roll(m, 4, 0))
            if pin:
                qlhs[NU + zdyn, :, 0:128] = pltpu.bitcast(m, U32)
            m = jnp.max(m, axis=1, keepdims=True)
            p = jnp.exp2(s - m)
            pbuf[sl][zdyn] = p
            for g in range((nmx(u) + 3) // 4):
                c = jq - 1 - g
                plhs[:, (2 * sl + g) * 128:(2 * sl + g + 1) * 128] = pltpu.bitcast(
                    _lhs(p[:, c * 128:(c + 1) * 128]), U32)

        def inv_l(l):
            l = jnp.sum(l, axis=1, keepdims=True)
            r0 = pl.reciprocal(l, approx=True)
            return jnp.broadcast_to(r0 * (2.0 - l * r0), (8, 128))

        def st_lsum(u):
            l = pbuf[u % 2][0, :, 0:128]
            for c in range(1, jq):
                l = l + pbuf[u % 2][0, :, c * 128:(c + 1) * 128]
            l = l + pltpu.roll(l, 2, 0)
            l = l + pltpu.roll(l, 4, 0)
            lpart[u % ns] = l

        def st_pvm(u):
            toks = []
            for j in jms(u):
                g = jq - 1 - j % jq
                pc = 2 * (u % 2) + g
                lhs = pltpu.bitcast(plhs[:, pc * 128:(pc + 1) * 128], BF16)
                ra = 2 * (j // jq)
                for t in range(3):
                    if t == 1:
                        w32 = jnp.concatenate(
                            [v32[u][0, 8:12, j], v32[u][1, 0:4, j]], axis=0)
                    else:
                        w32 = v32[u][t // 2, 2 * t:2 * t + 8, j]
                    r = _dot(lhs, _as_bf16(w32))
                    toks.append(r[8:16])
                    mbuf[u % ns, g, t, ra:ra + 2, :] = r[ra:ra + 2]
            return toks

        def st_expand(u):
            def body(dt, c):
                for hd in range(2):
                    for ix, j in enumerate(jx):
                        w = v32[u][hd, dt, j]
                        vx[2 * u + hd, dt, ix] = pltpu.bitcast(w << 16, F32)
                        vbuf[u][hd, dt, j] = pltpu.bitcast(w & jnp.uint32(0xFFFF0000), BF16)
                return c
            lax.fori_loop(0, UT // 2, body, 0)
            for j in jms(u):
                for t in range(3):
                    idx = [divmod(t * 8 + v, 12) for v in range(8)]
                    blk = jnp.concatenate([vbuf[u][hd, dt, j] for hd, dt in idx], axis=0)
                    blk = blk.astype(F32).T.astype(BF16)
                    for v, (hd, dt) in enumerate(idx):
                        vbuf[u][hd, dt, j] = blk[v * 16:(v + 1) * 16]

        def st_pv(u, toks, tok_map):
            nm, sl = nmx(u), u % ns
            for piece in range(NPIECE):
                hd, half = divmod(piece, NPIECE // 2)
                sub = len(tok_map) // NPIECE
                lo = hi = None
                for j in range(nj):
                    if j in jms(u):
                        continue
                    row = 2 * (j // jq) + hd
                    cs = slice((j % jq) * 128, (j % jq + 1) * 128)
                    pb = jnp.broadcast_to(pbuf[u % 2][0, row:row + 1, cs], (8, 128))
                    k = piece * sub + j * sub // nj
                    ti = tok_map[k] if j % (nj // sub) == 0 else -1
                    if j > 0 and tok_map[k - 1] == ti:
                        ti = -1
                    if toks and ti >= 0:
                        pb = pb + toks[min(ti, len(toks) - 1)]
                    w = v32[u][hd, pl.ds(half * 2, 2), j]
                    if j in jx:
                        a = vx[2 * u + hd, pl.ds(half * 2, 2), jx.index(j)] * pb
                        b = pltpu.bitcast(w, F32) * pb
                    else:
                        a = pltpu.bitcast(w << 16, F32) * pb
                        b = pltpu.bitcast(w & jnp.uint32(0xFFFF0000), F32) * pb
                    lo = a if lo is None else lo + a
                    hi = b if hi is None else hi + b
                for i in range(2):
                    base = (piece * 2 + i) * 16
                    abuf[sl, pl.ds(base, 8, stride=2), :] = lo[i]
                    abuf[sl, pl.ds(base + 1, 8, stride=2), :] = hi[i]

        def st_ored(u):
            nm, sl = nmx(u), u % ns
            ia = inv_l(lpart[sl])
            ib = pltpu.roll(ia, 1, 0)
            lane = lax.broadcasted_iota(jnp.int32, (8, 128), 1)
            for t in range(3):
                at = abuf[sl, t * 128:(t + 1) * 128, :].T
                o = at[0:8]
                for i in range(1, 16):
                    o = o + at[i * 8:(i + 1) * 8]
                if nm:
                    sub = lax.broadcasted_iota(jnp.int32, (8, 128), 0)
                    odd = (0, (lane >= DH - 128).astype(jnp.int32), 1)[t]
                    for g in range((nm + 3) // 4):
                        keep = (sub >= 8 - 2 * min(nm - 4 * g, 4)) & (sub % 2 == odd)
                        o = o + jnp.where(keep, mbuf[sl, g, t], 0.0)
                o = o + pltpu.roll(o, 4, 0)
                o = o + pltpu.roll(o, 2, 0)
                o = o + pltpu.roll(o, 1, 0)
                o = o * (ia, jnp.where(lane < DH - 128, ia, ib), ib)[t]
                olhs.at[u][:, t * 128:(t + 1) * 128] = pltpu.bitcast(_lhs(o), U32)

        def st_olast(u, out):
            sl = u % ns
            for hd in range(2):
                pa = [None, None]
                for dt in range(12):
                    base = (hd * 12 + dt) * 16
                    lo = jnp.sum(abuf[sl, pl.ds(base, 8, stride=2), :], axis=1, keepdims=True)
                    hi = jnp.sum(abuf[sl, pl.ds(base + 1, 8, stride=2), :], axis=1, keepdims=True)
                    w = wo32(2 * u + hd)[dt]
                    pr = (pltpu.bitcast(w << 16, F32) * lo
                          + pltpu.bitcast(w & jnp.uint32(0xFFFF0000), F32) * hi)
                    pa[dt % 2] = pr if pa[dt % 2] is None else pa[dt % 2] + pr
                inv = inv_l(jnp.broadcast_to(lpart[sl, hd:hd + 1, :], (8, 128)))
                tot = (pa[0] + pa[1]) * inv
                for n in range(D // 128):
                    out[n].append(tot[n])

        def st_oproj(u, ts=(0, 1, 2)):
            lhs = pltpu.bitcast(olhs[u], BF16)
            toks = []
            for t in ts:
                for n in range(D // 128):
                    if t == 1:
                        w32 = jnp.concatenate(
                            [wo32(2 * u)[8:12, n], wo32(2 * u + 1)[0:4, n]], axis=0)
                    else:
                        w32 = wo32(2 * u + t // 2)[2 * t:2 * t + 8, n]
                    r = _dot(lhs[:, t * 128:(t + 1) * 128], _as_bf16(w32))
                    toks.append(r[8:16])
                    gp[t, n, pl.ds(u, 1), :] = r[0:1]
            return toks

        def mlp(first, extra, zdyn):
            g = gp[0] + gp[1] + gp[2]
            g = g[:, 0:8] + g[:, 8:16]
            g = jnp.concatenate([sum(extra[n], g[n]) for n in range(D // 128)], axis=1)
            g = g + pltpu.roll(g, 4, 0)
            g = g + pltpu.roll(g, 2, 0)
            g = g + pltpu.roll(g, 1, 0)
            x1 = _round_bf16(xs[...] + g)
            lhs = _lhs(x1, 1.0)
            m1, r1 = _ln_stats(x1)
            y = (x1 - m1) * r1
            m2, r2 = _ln_stats(y)
            a = r1 * r2
            b = (m1 * r1 + m2) * r2
            if first:
                wait(cps_w3())
                start(cps_w4(3))
                start(cps_w4(4))
            hl, hs = [], []
            for n in range(FF // 128):
                r = _dot(lhs, _as_bf16(w332[:, n]))
                hn = jax.nn.gelu(r[0:8] * a - r[8:16] * b, approximate=True)
                hl.append(_lhs(hn))
                hs.append(hn)
            acc = x1 + y
            acc = [acc[:, c * 128:(c + 1) * 128] for c in range(D // 128)]

            def w4_dot(kt, c):
                return _dot(hl[kt], _as_bf16(w4_words(c, kt * 8, 8)))[0:8]

            if not first:
                nv, kpin, (t0, t1) = cfg["w4_nv"], cfg["w4_pin"], cfg["w4_tok"]
                toks = []
                for kt in range(nv, FF // 128):
                    if nv and kt == kpin:
                        for k in range(nv):
                            blk = jnp.broadcast_to(_round_bf16(hs[k][0:1]), (128, 128)).T
                            abuf[zdyn, k * 128:(k + 1) * 128, :] = blk
                            qlhs[NU + zdyn, :, 0:128] = pltpu.bitcast(blk[120:128], U32)
                        hl[kt] = pltpu.bitcast(qlhs[0, :, 0:128], BF16)
                    if nv and kt + 1 == kpin:
                        qlhs.at[0][:, 0:128] = pltpu.bitcast(hl[kpin], U32)
                    for c in range(D // 128):
                        r = _dot(hl[kt], _as_bf16(w4_words(c, kt * 8, 8)))
                        toks.append(r[8:16])
                        acc[c] = acc[c] + r[0:8]
                pa = None
                for dt in range(nv * 8):
                    tk = toks[t0 + dt * (t1 - t0) // (nv * 8)]
                    lo = abuf[0, pl.ds(dt * 16, 8, stride=2), :] + tk
                    hi = abuf[0, pl.ds(dt * 16 + 1, 8, stride=2), :] + tk
                    w = jnp.concatenate([w4_words(c, dt, 1) for c in range(D // 128)], axis=0)
                    pr = (pltpu.bitcast(w << 16, F32) * lo
                          + pltpu.bitcast(w & jnp.uint32(0xFFFF0000), F32) * hi)
                    pa = pr if pa is None else pa + pr
                for c in range(D // 128 if nv else 0):
                    pc = pa[c]
                    pc = pc + pltpu.roll(pc, 4, 0)
                    pc = pc + pltpu.roll(pc, 2, 0)
                    acc[c] = (pc + pltpu.roll(pc, 1, 0)) + acc[c]
                xs[...] = _round_bf16(jnp.concatenate(acc, axis=1))
                return
            for i, (c, lo, n) in enumerate(w4_parts):
                wait(cps_w4(i))
                if i == 0:
                    start(cps_w4(5))
                    for k, hn in enumerate(hs[cfg["w4_k"]:]):
                        abuf[k // 3, (k % 3) * 128:(k % 3 + 1) * 128, :] = jnp.broadcast_to(
                            _round_bf16(hn[0:1]), (128, 128)).T
                if lo == 0:
                    for kt in range(n // 128):
                        acc[c] = acc[c] + w4_dot(kt, c)
                else:
                    pas = [None] * 4
                    for dt in range(n // 16):
                        w = w4_words(c, lo // 16 + dt, 1)[0]
                        sl, r0 = dt // 24, dt % 24 * 16
                        pr = (pltpu.bitcast(w << 16, F32) * abuf[sl, pl.ds(r0, 8, stride=2), :]
                              + pltpu.bitcast(w & jnp.uint32(0xFFFF0000), F32)
                              * abuf[sl, pl.ds(r0 + 1, 8, stride=2), :])
                        pas[dt % 4] = pr if pas[dt % 4] is None else pas[dt % 4] + pr
                    pa = (pas[0] + pas[1]) + (pas[2] + pas[3])
                    pa = pa + pltpu.roll(pa, 4, 0)
                    pa = pa + pltpu.roll(pa, 2, 0)
                    acc[c] = acc[c] + (pa + pltpu.roll(pa, 1, 0))
                if lo + n == FF:
                    xc = _round_bf16(acc[c])
                    xs[:, c * 128:(c + 1) * 128] = xc
                    lhs = _lhs(xc)
                    for nt in range(early_tiles(c)):
                        r = _dot(lhs, _as_bf16(wq32[pl.ds(c * 8, 8), nt]))[0:4]
                        qacc[nt, 0:4, :] = r if c == 0 else qacc[nt, 0:4, :] + r

        gp[...] = jnp.zeros_like(gp)
        mbuf[...] = jnp.zeros_like(mbuf)
        wait(cps_x_wq())
        start(cps_wo(0))
        x0 = jnp.broadcast_to(xin[...].astype(F32), (8, D))
        sub0 = lax.broadcasted_iota(jnp.int32, (8, D), 0)
        lane0 = lax.broadcasted_iota(jnp.int32, (8, D), 1)
        for nkb, n0, n1 in ((4, 0, early_tiles(3)), (3, early_tiles(3), early_tiles(0))):
            lhs0 = _lhs(jnp.where(sub0 < 4, jnp.where(lane0 < nkb * 128, x0, 0.0), 1.0))

            def q0_body(nt, c, lhs0=lhs0):
                qacc[nt] = _dot(lhs0, _as_bf16(wq32[:, nt]))[0:8]
                return c
            lax.fori_loop(n0, n1, q0_body, 0)
        wait(cps_k(0, 0))
        start(cps_k(2, 0))
        wait(cps_k(1, 1))
        wait(cps_v(0, 0))
        xs[...] = x0

        def layer(li, carry):
            first = li == 0
            n_first = jnp.maximum(1 - li, 0)
            zdyn = li >> 4

            def block_dma(ua, ub):
                def last_wait(t):
                    if t == NU - 2:
                        wait(cps_k(NU - 1, (NU - 1) % 2))
                    else:
                        wait(cps_v(t + 1, (t + 1) % 2) if t + 1 < NU else cps_wo(1))

                def dma_ops(_, c):
                    for t in range(ua, ub):
                        if t + 3 < NU:
                            start(cps_k(t + 3, (t + 3) % 2))
                        if t + 2 < NU:
                            start(cps_v(t + 2, t % 2))
                        if t == NU - 2:
                            start(cps_w3())
                            start(cps_w4(0))
                        if t == NU - 1:
                            start(cps_w4(1))
                            wait(cps_v(t, t % 2))
                            start(cps_w4(2))
                        if t == 1:
                            wait(cps_wo(0))
                            start(cps_wo(1))
                        st_expand(t)
                        if t + 2 < NU - 1:
                            wait(cps_k(t + 2, t % 2))
                        if t < ub - 1:
                            last_wait(t)
                    return c

                lax.fori_loop(0, n_first, dma_ops, 0)
                pl.when(first)(lambda: last_wait(ub - 1))

            def prologue():
                x = xs[...]
                m, r = _ln_stats(x)
                nq = cfg["nq_mxu"]

                def finish_q(u, late):
                    qs = []
                    for nt in range(3):
                        qx = jnp.broadcast_to(qacc[u * 3 + nt, 0:1, :], (8, 128))
                        cs = jnp.broadcast_to(qacc[u * 3 + nt, 4:5, :], (8, 128))
                        qs.append((qx + late[nt] - cs * m) * r)
                    pack_q(jnp.concatenate(qs, axis=1), u)

                lhs = _lhs(x[:, D - 128:D])
                for u in range(nq):
                    finish_q(u, [_dot(lhs, _as_bf16(wq32[pl.ds(32, 8), u * 3 + nt]))[0:8]
                                 for nt in range(3)])
                f1 = cfg["va_force"]
                toks = st_qk(0, range(f1))
                for kb in range(2):
                    cs = slice((3 + kb) * 128, (4 + kb) * 128)
                    blk = jnp.broadcast_to(x[0:1, cs], (128, 128)).T
                    abuf[ns - 1 + zdyn, kb * 128:(kb + 1) * 128, :] = blk
                    qlhs[NU + zdyn, :, 0:128] = pltpu.bitcast(blk[120:128], U32)
                toks += st_qk(0, range(f1, nj))
                st_softmax(0, zdyn)
                toks += st_qk(1, range(js(1)))
                toks += st_pvm(0)
                for va, (t0, t1) in zip(cfg["va_groups"], cfg["va_tok"]):
                    acc = [None] * len(va)
                    for kt in range(16):
                        lo = abuf[ns - 1, pl.ds(kt * 16, 8, stride=2), :]
                        hi = abuf[ns - 1, pl.ds(kt * 16 + 1, 8, stride=2), :]
                        tk = toks[t0 + kt * (t1 - t0) // 16]
                        lo, hi = lo + tk, hi + tk
                        for i, u in enumerate(va):
                            w = wq32[24 + kt, u * 3:u * 3 + 3]
                            pr = (pltpu.bitcast(w << 16, F32) * lo
                                  + pltpu.bitcast(w & jnp.uint32(0xFFFF0000), F32) * hi)
                            acc[i] = pr if acc[i] is None else acc[i] + pr
                    for i, u in enumerate(va):
                        late = []
                        for nt in range(3):
                            q = acc[i][nt]
                            q = q + pltpu.roll(q, 4, 0)
                            q = q + pltpu.roll(q, 2, 0)
                            late.append(q + pltpu.roll(q, 1, 0))
                        finish_q(u, late)
                return toks

            def block(bi):
                ua, ub = cfg["blocks"][bi]
                block_dma(ua, ub)
                toks = []
                if bi == 0:
                    toks += prologue()
                done = js(ua + 1)
                for t in range(ua, ub):
                    base = len(toks)
                    for u in cfg["ored_at"].get(t, ()):
                        st_ored(u)
                    if t + 1 < NU:
                        toks += st_qk(t + 1, range(done, nj))
                    g0 = len(toks)
                    if t == ua and bi > 0:
                        toks += st_pvm(t)
                    for u in cfg["oproj_at"].get(t, ()):
                        toks += st_oproj(*u) if isinstance(u, tuple) else st_oproj(u)
                    done = js(t + 2)
                    if t + 1 < ub:
                        gap = cfg["gap"]
                        done = max(-((len(toks) - g0 - gap) // 3), 0)
                    gap1 = cfg["gap1"]
                    d1 = min(max(-((len(toks) - g0 - gap1) // 3), 0), done)
                    if t + 2 < NU:
                        toks += st_qk(t + 2, range(d1))
                    if t + 1 < NU:
                        st_softmax(t + 1, zdyn, pin=t + 2 < NU and d1 < done)
                    if t + 2 < NU:
                        toks += st_qk(t + 2, range(d1, done))
                    if t + 1 < ub:
                        toks += st_pvm(t + 1)
                    st_pv(t, toks, [base + i for i in cfg["tok"][t]])
                    st_lsum(t)

            def tail(first_static):
                seen = set()
                for us in cfg["oproj_at"].values():
                    for u in us:
                        uu, ts = u if isinstance(u, tuple) else (u, (0, 1, 2))
                        seen |= {(uu, t) for t in ts}
                for u in range(NU - 1):
                    ts = tuple(t for t in range(3) if (u, t) not in seen)
                    if ts:
                        st_oproj(u, ts)
                extra = [[] for _ in range(D // 128)]
                st_olast(NU - 1, extra)
                mlp(first_static, extra, zdyn)

            for bi in range(len(cfg["blocks"])):
                block(bi)

            pl.when(first)(lambda: tail(True))
            pl.when(jnp.logical_not(first))(lambda: tail(False))
            return carry

        lax.fori_loop(0, 2, layer, 0)
        o_ref[...] = xs[0:1, :].astype(o_ref.dtype)

    return kernel


@jax.jit
def pallas_interleave_layers__sliding_block_cached__mixer_s_mlp__decode_kernel(
    A_x: jax.Array,
    A_k_cache: jax.Array,
    A_v_cache: jax.Array,
    A_wq: jax.Array,
    A_wo: jax.Array,
    B_x: jax.Array,
    B_w1: jax.Array,
    B_w2: jax.Array,
    B_w3: jax.Array,
    B_w4: jax.Array,
):
    b, sq, d = A_x.shape
    _, hkv, sk, dh = A_k_cache.shape
    assert (b, sq, d, hkv, dh) == (1, 1, D, H, DH)
    win = min(4096, max(256, sk // 4))
    assert win % 512 == 0 and sk % 128 == 0
    nj = win // 128

    kt = _tile_view(jnp.swapaxes(A_k_cache, 2, 3).reshape(H * DH, sk))
    vt = _head_view(jnp.swapaxes(A_v_cache, 2, 3).reshape(H * DH, sk))

    def buf(r, c):
        return pltpu.VMEM((r // 16, c // 128, 16, 128), BF16)

    def hbuf(h, c):
        return pltpu.VMEM((h, DH // 16, c // 128, 16, 128), BF16)

    bl = CFG["blocks"]
    ns = CFG.get("ns") or max(bl[i + 1][1] - bl[i][0] for i in range(len(bl) - 1))
    any_spec = pl.BlockSpec(memory_space=pl.ANY)
    out = pl.pallas_call(
        _make_kernel(sk, win, CFG),
        out_shape=jax.ShapeDtypeStruct((1, D), A_x.dtype),
        in_specs=[any_spec] * 7,
        out_specs=pl.BlockSpec(memory_space=pltpu.VMEM),
        scratch_shapes=[
            [buf(2 * DH, win)] * NU, [hbuf(2, win)] * NU, [hbuf(H - 8, D), hbuf(8, D)],
            [pltpu.VMEM((r // 16, 16, 128), BF16)
             for r in (FF,) * 4 + (CFG["w4_k"] * 128, FF - CFG["w4_k"] * 128)],
            pltpu.VMEM((H, DH // 16, max(len(CFG["jx"]), 1), 8, 128), F32),
            buf(D, H * DH), buf(D, FF),
            pltpu.VMEM((1, D), BF16),
            pltpu.VMEM((8, D), F32),
            pltpu.VMEM((H * DH // 128, 8, 128), F32),
            pltpu.VMEM((NU + 1, 8, 384), U32),
            pltpu.VMEM((2, 8, win // 4), F32),
            pltpu.VMEM((2, 8, win // 4), F32),
            pltpu.VMEM((1, 8, win // 4), F32),
            pltpu.VMEM((1, 8, win // 4), F32),
            pltpu.VMEM((8, 512), U32),
            pltpu.VMEM((ns, 2, 3, 8, 128), F32),
            pltpu.VMEM((ns, 8, 128), F32),
            pltpu.VMEM((ns, 384, 128), F32),
            pltpu.VMEM((NU, 8, 384), U32),
            pltpu.VMEM((3, D // 128, NU, 128), F32),
            pltpu.SemaphoreType.DMA((5,)),
        ],
        compiler_params=pltpu.CompilerParams(vmem_limit_bytes=int(CFG["vmem_mb"] * 1024 * 1024)),
        name="interleave_decode",
    )(A_x.reshape(1, D), kt, vt, _tile_view(A_wq), _head_view(A_wo),
      _tile_view(B_w3), _tile_view(B_w4))
    return out.reshape(b, sq, d)
```
